```python
import jax
import jax.numpy as jnp

def _softmax(x, axis=-1):
    return jax.nn.softmax(x, axis=axis)
def _gelu(x):
    return jax.nn.gelu(x, approximate=True)
def _silu(x):
    return jax.nn.silu(x)
def _sigmoid(x):
    return jax.nn.sigmoid(x)
def _layernorm(x, axis=-1, eps=1e-5):
    m = jnp.mean(x, axis=axis, keepdims=True)
    v = jnp.var(x, axis=axis, keepdims=True)
    return (x - m) / jnp.sqrt(v + eps)
def _scatter_add(tgt, idx, src, axis=0):
    return tgt.at[idx].add(src)
def _segment_sum(src, seg, n):
    return jax.ops.segment_sum(src, seg, n)
class _Rng:
    def __init__(self, key):
        self._k = key
    def _next(self):
        self._k, sub = jax.random.split(self._k)
        return sub
    def normal(self, shape):
        return jax.random.normal(self._next(), shape, dtype=jnp.bfloat16)
    def randint(self, lo, hi, shape):
        return jax.random.randint(self._next(), shape, lo, hi, dtype=jnp.int32)
    def uniform(self, shape, lo=0.0, hi=1.0):
        return jax.random.uniform(self._next(), shape, jnp.bfloat16, lo, hi)
    def permutation(self, n):
        return jax.random.permutation(self._next(), n)


kernel_name = 'interleave_layers__sliding_block_cached__glu_gated_swiglu__decode'

def setup_inputs():
    _rng = _Rng(jax.random.key(int.from_bytes(__import__("os").urandom(4), "little")))
    _w = (lambda a: (lambda t: t.astype(jnp.bfloat16) if jnp.issubdtype(t.dtype, jnp.floating) else t)(jnp.asarray(a)))
    def _A_setup():
        B, Sq, D = 1, 1, 640
        Hq, Hkv, Sk, Dh = 32, 32, 32768, 192
        assert Hq % Hkv == 0, (Hq, Hkv)
        return {
            "x": _w((lambda *s: _rng.normal(s) * 0.05)(B, Sq, D)),
            "k_cache": _w((lambda *s: _rng.normal(s) * 0.05)(B, Hkv, Sk, Dh)),
            "v_cache": _w((lambda *s: _rng.normal(s) * 0.05)(B, Hkv, Sk, Dh)),
            "wq": _w((lambda *s: _rng.normal(s) * 0.05)(D, Hq * Dh) * (D ** -0.5)),
            "wo": _w((lambda *s: _rng.normal(s) * 0.05)(Hq * Dh, D) * ((Hq * Dh) ** -0.5)),
        }
    _A_in = _A_setup()

    def _B_setup():
        B, S, D, F = 1, 1, 640, 1536
        return {
            "x": _w((lambda *s: _rng.normal(s) * 0.05)(B, S, D)),
            "w1": _w((lambda *s: _rng.normal(s) * 0.05)(D, F) * (2.0 / D) ** 0.5),
            "w3": _w((lambda *s: _rng.normal(s) * 0.05)(D, F) * (2.0 / D) ** 0.5),
            "w2": _w((lambda *s: _rng.normal(s) * 0.05)(F, D) * (2.0 / F) ** 0.5),
        }
    _B_in = _B_setup()

    return {
        "A_x": _A_in["x"],
        "A_k_cache": _A_in["k_cache"],
        "A_v_cache": _A_in["v_cache"],
        "A_wq": _A_in["wq"],
        "A_wo": _A_in["wo"],
        "B_x": _B_in["x"],
        "B_w1": _B_in["w1"],
        "B_w3": _B_in["w3"],
        "B_w2": _B_in["w2"],
    }

def reference(A_x, A_k_cache, A_v_cache, A_wq, A_wo, B_x, B_w1, B_w3, B_w2):
    def _A_ref(x, k_cache, v_cache, wq, wo):
        B, Sq, D = x.shape
        Hq, Dh = 32, 192
        Hkv, Sk = k_cache.shape[1], k_cache.shape[2]
        W = min(4096, max(256, Sk // 4))
        rep = Hq // Hkv
        q = (lambda x, *d: x.transpose(*d))((x @ wq).reshape(B, Sq, Hq, Dh), 0, 2, 1, 3)
        k = jnp.repeat(k_cache[:, :, Sk - W:, :], rep, axis=1)
        v = jnp.repeat(v_cache[:, :, Sk - W:, :], rep, axis=1)
        scores = jnp.einsum("bhqd,bhkd->bhqk", q, k) * (Dh ** -0.5)
        p = _softmax(scores, axis=-1)
        o = jnp.einsum("bhqk,bhkd->bhqd", p, v)
        return (lambda x, *d: x.transpose(*d))(o, 0, 2, 1, 3).reshape(B, Sq, Hq * Dh) @ wo

    def _B_ref(x, w1, w3, w2):
        gate = jnp.einsum("bsd,df->bsf", x, w1)
        up = jnp.einsum("bsd,df->bsf", x, w3)
        h = _silu(gate) * up
        out = jnp.einsum("bsf,fd->bsd", h, w2)
        return out

    x = A_x
    x = x + _A_ref(_layernorm(x, axis=-1), A_k_cache, A_v_cache, A_wq, A_wo)
    x = x + _B_ref(_layernorm(x, axis=-1), B_w1, B_w3, B_w2)
    x = x + _A_ref(_layernorm(x, axis=-1), A_k_cache, A_v_cache, A_wq, A_wo)
    x = x + _B_ref(_layernorm(x, axis=-1), B_w1, B_w3, B_w2)
    return x
```

```python
import jax
import jax.numpy as jnp
from jax import lax
import jax.experimental.pallas as pl
import jax.experimental.pallas.tpu as pltpu

BF = jnp.bfloat16
F32 = jnp.float32
U32 = jnp.uint32

D = 640
H = 32
DH = 192
G = DH // 8
NP = H // 2
FF = 1536
EPS = 1e-5
NACC = 12


def _kernel(x_hbm, k_hbm, v_hbm, wq_hbm, wo_hbm, w1_hbm, w3_hbm, w2_hbm,
            o_ref,
            xb, kb, vb, wq, wo, w1, w3, w2,
            q_scr, part, p_scr, acc, o_scr,
            ksem, vsem, wsem, *, row0, nrows, scale):
    nblk = nrows // 8
    njp = nblk // 2

    def kcopy(m):
        return pltpu.make_async_copy(
            k_hbm.at[pl.ds(2 * m, 2), :, pl.ds(row0, nrows), :],
            kb.at[pl.ds(2 * m, 2)], ksem.at[m])

    def vcopy(m):
        return pltpu.make_async_copy(
            v_hbm.at[pl.ds(2 * m, 2), :, pl.ds(row0, nrows), :],
            vb.at[pl.ds(2 * m, 2)], vsem.at[m])

    c_x = pltpu.make_async_copy(x_hbm, xb, wsem.at[0])
    c_wq = pltpu.make_async_copy(wq_hbm, wq, wsem.at[1])
    c_wo = pltpu.make_async_copy(wo_hbm, wo, wsem.at[2])
    c_w1 = pltpu.make_async_copy(w1_hbm, w1, wsem.at[3])
    c_w3 = pltpu.make_async_copy(w3_hbm, w3, wsem.at[4])
    c_w2 = pltpu.make_async_copy(w2_hbm, w2, wsem.at[5])

    c_wq.start()
    c_x.start()
    kcopy(0).start()
    for m in range(NP):
        if m + 1 < NP:
            kcopy(m + 1).start()
        vcopy(m).start()
    c_wo.start()
    c_w1.start()
    c_w3.start()
    c_w2.start()

    ku = kb.bitcast(U32)
    vu = vb.bitcast(U32)

    lane = lax.broadcasted_iota(jnp.int32, (8, 128), 1)
    row = lax.broadcasted_iota(jnp.int32, (8, 128), 0)
    row_odd = (row & 1) == 1
    diag = ((lane >> 3) & 1) == (row & 1)
    lane_lo = lane < 64

    def layernorm(x):
        mu = jnp.mean(x, axis=-1, keepdims=True)
        xc = x - mu
        var = jnp.mean(xc * xc, axis=-1, keepdims=True)
        return xc / jnp.sqrt(var + EPS)

    def lhs_pattern(x0, x1):
        z = jnp.where(diag, jnp.where(row_odd, x1, x0), 0.0)
        return z.astype(BF)

    def scores(m, par):
        h = 2 * m + par
        xf = q_scr[3 * m + 2 * par]
        bh = q_scr[3 * m + 1]
        bh = jnp.where(lane_lo if par == 0 else ~lane_lo, bh, pltpu.roll(bh, 56, 1))
        pats = [lhs_pattern(xf, pltpu.roll(xf, 8, 1)),
                lhs_pattern(pltpu.roll(xf, 120, 1), xf),
                lhs_pattern(bh, pltpu.roll(bh, 8, 1))]
        gf = 8 * par
        gh = 16 * (1 - par)
        ev = [0, 2, 4, 6]
        od = [1, 3, 5, 7]
        groups = [[gf + 2 * i for i in range(8)],
                  [gf + 2 * i + 1 for i in range(8)],
                  [gh + b for b in (ev + od if par == 0 else od + ev)]]
        ops = []
        for jp in range(njp):
            for t in range(3):
                def op(jp=jp, t=t):
                    w = jnp.concatenate(
                        [ku[h, g, 8 * jp:8 * jp + 8, :] for g in groups[t]], axis=0)
                    r = jnp.dot(pats[t], pltpu.bitcast(w, BF),
                                preferred_element_type=F32)
                    u = jp % 4
                    part[par, t, 2 * jp:2 * jp + 2, :] = r[2 * u:2 * u + 2, :]
                ops.append(op)
        return ops

    def softmax(par):
        s = part[par, 0] + part[par, 1] + part[par, 2]
        mx = jnp.max(jnp.max(s, axis=0, keepdims=True), axis=1, keepdims=True)
        p = jnp.exp((s - mx) * scale)
        l = jnp.sum(jnp.sum(p, axis=0, keepdims=True), axis=1, keepdims=True)
        return p, jnp.broadcast_to(1.0 / l, (8, 128))

    def pv_ops(m, par, p):
        h = 2 * m + par
        a = {}
        ops = []
        for gb in range(G // NACC):
            for jp in range(njp):
                def op(gb=gb, jp=jp):
                    pb0 = jnp.broadcast_to(p[2 * jp:2 * jp + 1, :], (8, 128))
                    pb1 = jnp.broadcast_to(p[2 * jp + 1:2 * jp + 2, :], (8, 128))
                    for g in range(gb * NACC, (gb + 1) * NACC):
                        v = pltpu.bitcast(vu[h, g, 8 * jp:8 * jp + 8, :], BF).astype(F32)
                        t = v[:8] * pb0
                        a[g] = t if jp == 0 else a[g] + t
                        a[g] = a[g] + v[8:] * pb1
                        if jp == njp - 1:
                            r0 = DH * par + 8 * g
                            acc[r0:r0 + 8, :] = a[g]
                ops.append(op)
        return ops

    def finish(m, inv0, inv1):
        for c in range(3):
            t = acc[128 * c:128 * c + 128, :].T
            r = jnp.sum(t, axis=0, keepdims=True)
            inv = inv0 if c == 0 else (inv1 if c == 2 else jnp.where(lane_lo, inv0, inv1))
            o_scr[3 * m + c] = jnp.broadcast_to(r, (8, 128)) * inv

    def interleave(a, b):
        na, nb = len(a), len(b)
        ia = 0
        for ib in range(nb):
            while ia < na and ia * nb <= ib * na:
                a[ia]()
                ia += 1
            b[ib]()
        while ia < na:
            a[ia]()
            ia += 1

    def attention(x, first):
        y = jnp.broadcast_to(layernorm(x), (8, D)).astype(BF)
        if first:
            c_wq.wait()
        q = jnp.dot(y, wq[...], preferred_element_type=F32)
        for c in range(3 * NP):
            q_scr[c] = q[:, 128 * c:128 * c + 128]

        def qk_stage(m):
            ops0 = scores(m, 0)
            ops1 = scores(m, 1)
            out = {}
            def sm0():
                out[0] = softmax(0)
            def sm1():
                out[1] = softmax(1)
            return ops0 + [sm0] + ops1 + [sm1], out

        if first:
            kcopy(0).wait()
        ops, out = qk_stage(0)
        for op in ops:
            op()
        carry = (out[0][0], out[0][1], out[1][0], out[1][1])

        def step(m, carry, prev_inv, do_qk):
            p0, i0, p1, i1 = carry
            if first:
                if do_qk:
                    kcopy(m + 1).wait()
                vcopy(m).wait()
            if prev_inv is not None:
                finish(m - 1, *prev_inv)
            pv = pv_ops(m, 0, p0) + pv_ops(m, 1, p1)
            if do_qk:
                ops, out = qk_stage(m + 1)
                interleave(ops, pv)
                return (out[0][0], out[0][1], out[1][0], out[1][1]), (i0, i1)
            for op in pv:
                op()
            return None, (i0, i1)

        carry, inv = step(0, carry, None, True)

        def body(m, c):
            carry, inv = c
            return step(m, carry, inv, True)

        carry, inv = lax.fori_loop(1, NP - 1, body, (carry, inv))
        _, inv = step(NP - 1, carry, inv, False)
        finish(NP - 1, *inv)

        o = jnp.concatenate([o_scr[c] for c in range(3 * NP)], axis=1).astype(BF)
        if first:
            c_wo.wait()
        a = jnp.dot(o, wo[...], preferred_element_type=F32)[0:1]
        return (x + a.astype(BF).astype(F32)).astype(BF).astype(F32)

    def ffn(x, first):
        y = jnp.broadcast_to(layernorm(x), (8, D)).astype(BF)
        if first:
            c_w1.wait()
        g = jnp.dot(y, w1[...], preferred_element_type=F32)
        if first:
            c_w3.wait()
        u = jnp.dot(y, w3[...], preferred_element_type=F32)
        hh = (g * jax.nn.sigmoid(g) * u).astype(BF)
        if first:
            c_w2.wait()
        a = jnp.dot(hh, w2[...], preferred_element_type=F32)[0:1]
        return (x + a.astype(BF).astype(F32)).astype(BF).astype(F32)

    c_x.wait()
    x = xb[...].astype(F32)
    x = attention(x, True)
    x = ffn(x, True)
    x = attention(x, False)
    x = ffn(x, False)
    o_ref[...] = x.astype(o_ref.dtype)


@jax.jit
def pallas_interleave_layers__sliding_block_cached__glu_gated_swiglu__decode_kernel(
    A_x: jax.Array,
    A_k_cache: jax.Array,
    A_v_cache: jax.Array,
    A_wq: jax.Array,
    A_wo: jax.Array,
    B_x: jax.Array,
    B_w1: jax.Array,
    B_w3: jax.Array,
    B_w2: jax.Array,
):
    del B_x
    sk = A_k_cache.shape[2]
    win = min(4096, max(256, sk // 4))
    nb = sk // 128

    def tiles(c):
        return (c.reshape(H, nb, 128, G, 8).transpose(0, 3, 1, 4, 2)
                .reshape(H, G, nb * 8, 128))

    nrows = (win // 128) * 8
    row0 = nb * 8 - nrows
    kern = lambda *refs: _kernel(*refs, row0=row0, nrows=nrows, scale=DH ** -0.5)
    out = pl.pallas_call(
        kern,
        out_shape=jax.ShapeDtypeStruct((1, D), BF),
        in_specs=[pl.BlockSpec(memory_space=pl.ANY)] * 8,
        out_specs=pl.BlockSpec(memory_space=pltpu.VMEM),
        scratch_shapes=[
            pltpu.VMEM((1, D), BF),
            pltpu.VMEM((H, G, nrows, 128), BF),
            pltpu.VMEM((H, G, nrows, 128), BF),
            pltpu.VMEM((D, H * DH), BF),
            pltpu.VMEM((H * DH, D), BF),
            pltpu.VMEM((D, FF), BF),
            pltpu.VMEM((D, FF), BF),
            pltpu.VMEM((FF, D), BF),
            pltpu.VMEM((3 * NP, 8, 128), F32),
            pltpu.VMEM((2, 3, nrows // 8, 128), F32),
            pltpu.VMEM((2, nrows // 8, 128), F32),
            pltpu.VMEM((2 * DH, 128), F32),
            pltpu.VMEM((3 * NP, 8, 128), F32),
            pltpu.SemaphoreType.DMA((NP,)),
            pltpu.SemaphoreType.DMA((NP,)),
            pltpu.SemaphoreType.DMA((6,)),
        ],
        compiler_params=pltpu.CompilerParams(vmem_limit_bytes=124 * 1024 * 1024),
    )(A_x.reshape(1, D), tiles(A_k_cache), tiles(A_v_cache),
      A_wq, A_wo, B_w1, B_w3, B_w2)
    return out.reshape(1, 1, D)
```

```python
import math

import jax
import jax.numpy as jnp
from jax import lax
import jax.experimental.pallas as pl
import jax.experimental.pallas.tpu as pltpu

BF = jnp.bfloat16
F32 = jnp.float32
U32 = jnp.uint32

D = 640
H = 32
DH = 192
G = DH // 8
NP = H // 2
FF = 1536
EPS = 1e-5
NACC = 24
KD = D // 128
NEG = float(jnp.finfo(jnp.float32).min)


def _interleave(a, b):
    na, nb = len(a), len(b)
    ia = 0
    for ib in range(nb):
        while ia < na and ia * nb <= ib * na:
            a[ia]()
            ia += 1
        b[ib]()
    while ia < na:
        a[ia]()
        ia += 1


def _kernel(x_hbm, k_hbm, v_hbm, wq_hbm, wo_hbm, w1_hbm, w3_hbm, w2_hbm,
            o_ref,
            xb, kb, vb, wq, wo, w1, w3, w2,
            y_scr, qpart, q_scr, roll_scr, pat_scr, part, p_scr, ml_scr, ls_scr,
            mx_scr, accx, accy, zbuf, olhs, opart, out_scr,
            ksem, vsem, wsem, *, row0, nrows, scale):
    nblk = nrows // 8
    njp = nblk // 2
    c2 = scale * math.log2(math.e)

    def kcopy(m):
        return pltpu.make_async_copy(
            k_hbm.at[pl.ds(2 * m, 2), :, pl.ds(row0, nrows), :],
            kb.at[pl.ds(2 * m, 2)], ksem.at[m])

    def vcopy(m):
        return pltpu.make_async_copy(
            v_hbm.at[pl.ds(2 * m, 2), :, pl.ds(row0, nrows), :],
            vb.at[pl.ds(2 * m, 2)], vsem.at[m])

    c_x = pltpu.make_async_copy(x_hbm, xb, wsem.at[0])
    c_wq = [pltpu.make_async_copy(wq_hbm.at[:, pl.ds(128 * c, 128)], wq.at[c], wsem.at[1])
            for c in range(3 * NP)]
    c_wo = [pltpu.make_async_copy(wo_hbm.at[:, pl.ds(128 * n, 128)], wo.at[n], wsem.at[2])
            for n in range(KD)]
    c_w1 = pltpu.make_async_copy(w1_hbm, w1, wsem.at[3])
    c_w3 = pltpu.make_async_copy(w3_hbm, w3, wsem.at[4])
    c_w2 = pltpu.make_async_copy(w2_hbm, w2, wsem.at[5])

    kcopy(0).start()
    c_x.start()
    for c in c_wq:
        c.start()
    for c in c_wo:
        c.start()
    for m in range(NP):
        if m + 1 < NP:
            kcopy(m + 1).start()
        vcopy(m).start()
    c_w1.start()
    c_w3.start()
    c_w2.start()

    ku = kb.bitcast(U32)
    vu = vb.bitcast(U32)
    wqu = wq.bitcast(U32)
    wou = wo.bitcast(U32)

    lane = lax.broadcasted_iota(jnp.int32, (8, 128), 1)
    row = lax.broadcasted_iota(jnp.int32, (8, 128), 0)
    row_odd = (row & 1) == 1
    diag2 = ((lane >> 3) & 1) == (row & 1)
    diag8 = (lane & 7) == row
    lane_lo = lane < 64
    lane_bit = [((lane >> (3 + k)) & 1) == 1 for k in range(4)]

    def layernorm(x):
        mu = jnp.mean(x, axis=-1, keepdims=True)
        xc = x - mu
        var = jnp.mean(xc * xc, axis=-1, keepdims=True)
        return xc / jnp.sqrt(var + EPS)

    def pack8(z):
        return pltpu.bitcast(jnp.concatenate([z, z], axis=0).astype(BF), U32)

    def lhs(u):
        return pltpu.bitcast(u, BF)[:8]

    def tile_dot(l, w_u32):
        return jnp.dot(l, pltpu.bitcast(w_u32, BF), preferred_element_type=F32)

    def qproj_ops(m):
        ops = []
        for c in range(3):
            for k in range(KD):
                def op(c=c, k=k):
                    qpart[c * KD + k] = tile_dot(
                        lhs(y_scr[k]), wqu[3 * m + c, 64 * k:64 * k + 64, :])
                ops.append(op)
        return ops

    def oproj_ops(m):
        ops = []
        for c in range(3):
            for n in range(KD):
                def op(c=c, n=n):
                    r0 = pl.multiple_of((3 * m + c) * 64, 64)
                    opart[n * 3 + c] = tile_dot(
                        lhs(olhs[c]), wou[n, pl.ds(r0, 64), :])
                ops.append(op)
        return ops

    def qk_ops(m):
        ops = []
        ev = [0, 2, 4, 6]
        od = [1, 3, 5, 7]
        for par in range(2):
            gf = 8 * par
            gh = 16 * (1 - par)
            groups = [[gf + 2 * i for i in range(8)],
                      [gf + 2 * i + 1 for i in range(8)],
                      [gh + b for b in (ev + od if par == 0 else od + ev)]]
            for jp in range(njp):
                for t in range(3):
                    def op(par=par, jp=jp, t=t, groups=groups):
                        w = jnp.concatenate(
                            [ku[2 * m + par, g, 8 * jp:8 * jp + 8, :] for g in groups[t]],
                            axis=0)
                        r = tile_dot(lhs(pat_scr[3 * par + t]), w)
                        u = jp % 4
                        part[par, t, 2 * jp:2 * jp + 2, :] = r[2 * u:2 * u + 2, :]
                    ops.append(op)
        return ops

    def rolls():
        for i, (c, s) in enumerate(((0, 8), (0, 120), (1, 8), (1, 56), (1, 64),
                                    (2, 8), (2, 120))):
            roll_scr[i] = pltpu.roll(q_scr[c], s, 1)

    def xmax():
        for par in range(2):
            mx_scr[par] = jnp.broadcast_to(
                jnp.max(ml_scr[par], axis=1, keepdims=True), (8, 128))

    def xlane():
        for g in range(2 * G + 2):
            zbuf[g] = jnp.broadcast_to(
                jnp.sum(accy[g], axis=1, keepdims=True), (8, 128))

    def pv_ops(m):
        ops = []
        for par in range(2):
            a = {}
            for gb in range(G // NACC):
                for jp in range(njp):
                    def op(par=par, gb=gb, jp=jp, a=a):
                        pb0 = jnp.broadcast_to(p_scr[par, 2 * jp:2 * jp + 1, :], (8, 128))
                        pb1 = jnp.broadcast_to(p_scr[par, 2 * jp + 1:2 * jp + 2, :], (8, 128))
                        for g in range(gb * NACC, (gb + 1) * NACC):
                            v = pltpu.bitcast(
                                vu[2 * m + par, g, 8 * jp:8 * jp + 8, :], BF).astype(F32)
                            t = v[:8] * pb0
                            a[g] = t if jp == 0 else a[g] + t
                            a[g] = a[g] + v[8:] * pb1
                            if jp == njp - 1:
                                accx[G * par + g] = a[g]
                    ops.append(op)
        return ops

    def g_softmax():
        for par in range(2):
            s = part[par, 0] + part[par, 1] + part[par, 2]
            ml = jnp.maximum(jnp.max(s, axis=0, keepdims=True), NEG)
            p = jnp.exp2((s - ml) * c2)
            p_scr[par] = p
            ml_scr[par] = jnp.broadcast_to(ml, (8, 128))
            ls_scr[par] = (p[0:8] + p[8:16]) + (p[16:24] + p[24:32])

    def g_rescale():
        for par in range(2):
            w = jnp.exp2((ml_scr[par] - mx_scr[par]) * c2)
            for g in range(G):
                accy[G * par + g] = accx[G * par + g] * w
            accy[2 * G + par] = ls_scr[par] * w

    def g_olhs():
        inv = [1.0 / jnp.sum(zbuf[2 * G + par], axis=0, keepdims=True) for par in range(2)]
        inv = [jnp.broadcast_to(v, (8, 128)) for v in inv]
        for c in range(3):
            xs = [zbuf[16 * c + b] for b in range(16)]
            for k in range(4):
                xs = [jnp.where(lane_bit[k], xs[i + 1], xs[i]) for i in range(0, len(xs), 2)]
            iv = inv[0] if c == 0 else (inv[1] if c == 2 else jnp.where(lane_lo, inv[0], inv[1]))
            olhs[c] = pack8(jnp.where(diag8, xs[0] * iv, 0.0))

    def g_qsum():
        for c in range(3):
            xs = [qpart[c * KD + k] for k in range(KD)]
            q_scr[c] = ((xs[0] + xs[1]) + (xs[2] + xs[3])) + xs[4]

    def g_patterns():
        def pat(x0, x1):
            return pack8(jnp.where(diag2, jnp.where(row_odd, x1, x0), 0.0))
        a, b, c = q_scr[0], q_scr[1], q_scr[2]
        b8, b56, b64 = roll_scr[2], roll_scr[3], roll_scr[4]
        pat_scr[0] = pat(a, roll_scr[0])
        pat_scr[1] = pat(roll_scr[1], a)
        pat_scr[2] = pat(jnp.where(lane_lo, b, b56), jnp.where(lane_lo, b8, b64))
        pat_scr[3] = pat(c, roll_scr[5])
        pat_scr[4] = pat(roll_scr[6], c)
        pat_scr[5] = pat(jnp.where(lane_lo, b56, b), jnp.where(lane_lo, b64, b8))

    def g_out():
        for n in range(KD):
            out_scr[n] = (out_scr[n] + opart[3 * n]) + (opart[3 * n + 1] + opart[3 * n + 2])

    def run(ops):
        for op in ops:
            op()

    def layer(li, x):
        first = li == 0

        y = jnp.broadcast_to(layernorm(x), (8, D))
        for k in range(KD):
            y_scr[k] = pack8(y[:, 128 * k:128 * k + 128])
        zero = jnp.zeros((8, 128), F32)
        one = jnp.ones((8, 128), F32)
        for g in range(2 * G):
            accx[g] = zero
            zbuf[g] = zero
        for par in range(2):
            zbuf[2 * G + par] = one
            ml_scr[par] = zero
            mx_scr[par] = zero
            ls_scr[par] = one
        for i in range(3 * KD):
            opart[i] = zero
        for n in range(KD):
            out_scr[n] = zero

        @pl.when(first)
        def _():
            for c in c_wq:
                c.wait()
            kcopy(0).wait()
            for c in c_wo:
                c.wait()

        run(qproj_ops(0))
        g_qsum()
        rolls()
        run(qproj_ops(1))
        g_patterns()
        g_qsum()
        rolls()
        run(qproj_ops(2))
        run(qk_ops(0))

        def body(m, carry):
            g_rescale()
            g_softmax()
            g_olhs()
            g_patterns()
            g_qsum()
            g_out()

            @pl.when(first)
            def _():
                @pl.when(m + 1 < NP)
                def _():
                    kcopy(m + 1).wait()
                vcopy(m).wait()

            side = (qk_ops(jnp.minimum(m + 1, NP - 1))
                    + qproj_ops(jnp.minimum(m + 3, NP - 1))
                    + oproj_ops(jnp.maximum(m - 2, 0)))
            xmax()
            xlane()
            rolls()
            _interleave(side, pv_ops(m))
            return carry

        lax.fori_loop(0, NP, body, 0)

        g_rescale()
        g_olhs()
        g_out()
        run(oproj_ops(NP - 2))
        xlane()
        g_out()
        g_olhs()
        run(oproj_ops(NP - 1))
        g_out()
        a = jnp.concatenate(
            [jnp.sum(out_scr[n], axis=0, keepdims=True) for n in range(KD)], axis=1)
        x = (x + a.astype(BF).astype(F32)).astype(BF).astype(F32)

        y = jnp.broadcast_to(layernorm(x), (8, D)).astype(BF)

        @pl.when(first)
        def _():
            c_w1.wait()
            c_w3.wait()

        g = jnp.dot(y, w1[...], preferred_element_type=F32)
        u = jnp.dot(y, w3[...], preferred_element_type=F32)
        hh = (g * jax.nn.sigmoid(g) * u).astype(BF)

        @pl.when(first)
        def _():
            c_w2.wait()

        a = jnp.dot(hh, w2[...], preferred_element_type=F32)[0:1]
        return (x + a.astype(BF).astype(F32)).astype(BF).astype(F32)

    c_x.wait()
    x = lax.fori_loop(0, 2, layer, xb[...].astype(F32))
    o_ref[...] = x.astype(o_ref.dtype)


@jax.jit
def pallas_interleave_layers__sliding_block_cached__glu_gated_swiglu__decode_kernel(
    A_x: jax.Array,
    A_k_cache: jax.Array,
    A_v_cache: jax.Array,
    A_wq: jax.Array,
    A_wo: jax.Array,
    B_x: jax.Array,
    B_w1: jax.Array,
    B_w3: jax.Array,
    B_w2: jax.Array,
):
    del B_x
    sk = A_k_cache.shape[2]
    win = min(4096, max(256, sk // 4))
    nb = sk // 128

    def tiles(c):
        return (c.reshape(H, nb, 128, G, 8).transpose(0, 3, 1, 4, 2)
                .reshape(H, G, nb * 8, 128))

    nrows = (win // 128) * 8
    row0 = nb * 8 - nrows
    vreg = lambda n, dt=F32: pltpu.VMEM((n, 8, 128), dt)
    kern = lambda *refs: _kernel(*refs, row0=row0, nrows=nrows, scale=DH ** -0.5)
    out = pl.pallas_call(
        kern,
        out_shape=jax.ShapeDtypeStruct((1, D), BF),
        in_specs=[pl.BlockSpec(memory_space=pl.ANY)] * 8,
        out_specs=pl.BlockSpec(memory_space=pltpu.VMEM),
        scratch_shapes=[
            pltpu.VMEM((1, D), BF),
            pltpu.VMEM((H, G, nrows, 128), BF),
            pltpu.VMEM((H, G, nrows, 128), BF),
            pltpu.VMEM((3 * NP, D, 128), BF),
            pltpu.VMEM((KD, H * DH, 128), BF),
            pltpu.VMEM((D, FF), BF),
            pltpu.VMEM((D, FF), BF),
            pltpu.VMEM((FF, D), BF),
            vreg(KD, U32),
            vreg(3 * KD),
            vreg(3),
            vreg(7),
            vreg(6, U32),
            pltpu.VMEM((2, 3, nrows // 8, 128), F32),
            pltpu.VMEM((2, nrows // 8, 128), F32),
            vreg(2),
            vreg(2),
            vreg(2),
            vreg(2 * G),
            vreg(2 * G + 2),
            vreg(2 * G + 2),
            vreg(3, U32),
            vreg(3 * KD),
            vreg(KD),
            pltpu.SemaphoreType.DMA((NP,)),
            pltpu.SemaphoreType.DMA((NP,)),
            pltpu.SemaphoreType.DMA((6,)),
        ],
        compiler_params=pltpu.CompilerParams(vmem_limit_bytes=124 * 1024 * 1024),
    )(A_x.reshape(1, D), tiles(A_k_cache), tiles(A_v_cache),
      A_wq, A_wo, B_w1, B_w3, B_w2)
    return out.reshape(1, 1, D)
```

```python
import math

import jax
import jax.numpy as jnp
from jax import lax
import jax.experimental.pallas as pl
import jax.experimental.pallas.tpu as pltpu

BF = jnp.bfloat16
F32 = jnp.float32
U32 = jnp.uint32

D = 640
H = 32
DH = 192
G = DH // 8
G2 = DH // 16
NP = H // 2
FF = 1536
EPS = 1e-5
KD = D // 128
NEG = float(jnp.finfo(jnp.float32).min)
W2_CHUNKS = (768, 384, 256, 128)
NACC = 12
PMODE = 2
M32 = 1


def _interleave(a, b):
    na, nb = len(a), len(b)
    ia = 0
    for ib in range(nb):
        while ia < na and ia * nb <= ib * na:
            a[ia]()
            ia += 1
        b[ib]()
    while ia < na:
        a[ia]()
        ia += 1


def _kernel(x_hbm, k_hbm, v_hbm, wq_hbm, wo_hbm, w1_hbm, w3_hbm, w2_hbm,
            o_ref,
            xb, kb, vb, wq, wo, w1, w3, w2,
            y_scr, rs_scr, qpart, pat_scr, part, p_scr, ml_scr, ls_scr,
            mx_scr, accx, accy, zbuf, olhs, opart, out_scr, pb_scr,
            ksem, vsem, wsem, *, blk0, nblk, scale):
    njp = nblk // 2
    c2 = scale * math.log2(math.e)

    def kcopies(m):
        return [pltpu.make_async_copy(
            k_hbm.at[pl.ds(2 * m, 2), :, t, pl.ds(blk0, nblk)],
            kb.at[pl.ds(2 * m, 2), :, :, pl.ds(8 * t, 8), :], ksem.at[t, m])
            for t in range(2)]

    def vcopy(m):
        return pltpu.make_async_copy(
            v_hbm.at[pl.ds(2 * m, 2), :, pl.ds(8 * blk0, 8 * nblk), :],
            vb.at[pl.ds(2 * m, 2)], vsem.at[m])

    c_x = pltpu.make_async_copy(x_hbm, xb, wsem.at[0])
    c_wq = [pltpu.make_async_copy(wq_hbm.at[:, t], wq.at[:, :, pl.ds(8 * t, 8), :],
                                  wsem.at[1 + t]) for t in range(2)]
    c_wo = [pltpu.make_async_copy(wo_hbm.at[:, t], wo.at[:, :, pl.ds(8 * t, 8), :],
                                  wsem.at[3 + t]) for t in range(2)]
    def wcopies(src, dst, s0, r0=0, nr=None):
        nr = src.shape[0] if nr is None else nr
        return [pltpu.make_async_copy(src.at[pl.ds(r0, nr), t],
                                      dst.at[pl.ds(r0, nr), :, pl.ds(8 * t, 8), :],
                                      wsem.at[s0 + t]) for t in range(2)]

    c_w1 = wcopies(w1_hbm, w1, 5)
    c_w3 = wcopies(w3_hbm, w3, 7)
    w2_off = [sum(W2_CHUNKS[:i]) for i in range(len(W2_CHUNKS))]
    c_w2 = [wcopies(w2_hbm, w2, 9 + 2 * i, o // 16, n // 16)
            for i, (o, n) in enumerate(zip(w2_off, W2_CHUNKS))]

    for c in c_wq:
        c.start()
    c_x.start()
    for c in kcopies(0) + c_wo:
        c.start()
    for m in range(NP):
        if m + 1 < NP:
            for c in kcopies(m + 1):
                c.start()
        vcopy(m).start()
    for c in c_w1 + c_w3 + [c for cs in c_w2 for c in cs]:
        c.start()

    ku = kb.bitcast(U32)
    vu = vb.bitcast(U32)
    wqu = wq.bitcast(U32)
    wou = wo.bitcast(U32)

    lane = lax.broadcasted_iota(jnp.int32, (8, 128), 1)
    row = lax.broadcasted_iota(jnp.int32, (8, 128), 0)
    diag8 = (lane & 7) == row
    lane_lo = lane < 64
    lane_bit = [((lane >> (3 + k)) & 1) == 1 for k in range(4)]

    def center(x):
        xc = x - jnp.mean(x, axis=-1, keepdims=True)
        var = jnp.mean(xc * xc, axis=-1, keepdims=True)
        return xc, 1.0 / jnp.sqrt(var + EPS)

    def pack16(z0, z1):
        return pltpu.bitcast(jnp.concatenate([z0, z1], axis=0).astype(BF), U32)

    paced = [False]

    def tile_dot(l_u32, w_u32, rows=8):
        w = pltpu.bitcast(w_u32.reshape(64, 128), BF)
        if paced[0] and M32:
            l = pltpu.bitcast(jnp.concatenate([l_u32, l_u32], axis=0), BF)[:24]
            return jnp.dot(l, w, preferred_element_type=F32)[:rows]
        l = pltpu.bitcast(l_u32, BF)[:rows]
        return jnp.dot(l, w, preferred_element_type=F32)

    def qproj_ops(m):
        ops = []
        for c in range(3):
            for k in range(KD):
                def op(c=c, k=k):
                    qpart[c * KD + k] = tile_dot(y_scr[k], wqu[8 * k:8 * k + 8, 3 * m + c])
                ops.append(op)
        return ops

    def oproj_ops(m):
        ops = []
        for c in range(3):
            for n in range(KD):
                def op(c=c, n=n):
                    opart[n * 3 + c] = tile_dot(olhs[c], wou[pl.ds((3 * m + c) * 8, 8), n])
                ops.append(op)
        return ops

    def qk_ops(m, order="ABC"):
        he, ho = 2 * m, 2 * m + 1

        def op_a(j):
            r = tile_dot(pat_scr[0], ku[he, 0:8, j])
            part[0, 0, j:j + 1, :] = r[j % 8:j % 8 + 1, :]

        def op_c(j):
            r = tile_dot(pat_scr[2], ku[ho, 4:12, j])
            part[1, 0, j:j + 1, :] = r[j % 8:j % 8 + 1, :]

        def op_b(j):
            w = jnp.concatenate([ku[he, 8:12, j], ku[ho, 0:4, j]], axis=0)
            r = tile_dot(pat_scr[1], w, 16)
            part[0, 1, j:j + 1, :] = r[j % 8:j % 8 + 1, :]
            part[1, 1, j:j + 1, :] = r[8 + j % 8:8 + j % 8 + 1, :]

        fn = dict(A=op_a, B=op_b, C=op_c)
        return [(lambda f=fn[t], j=j: f(j)) for j in range(nblk) for t in order]

    def xmax():
        for par in range(2):
            mx_scr[par] = jnp.broadcast_to(
                jnp.max(ml_scr[par], axis=1, keepdims=True), (8, 128))

    def xlane():
        for g in range(2 * G + 2):
            zbuf[g] = jnp.broadcast_to(
                jnp.sum(accy[g], axis=1, keepdims=True), (8, 128))

    def pv_ops(m):
        ops = []
        for par in range(2):
            a = {}
            for gb in range(G // NACC):
                for jp in range(njp):
                    def op(par=par, gb=gb, jp=jp, a=a):
                        if PMODE == 0 or gb == 0:
                            pb0 = jnp.broadcast_to(p_scr[par, 2 * jp:2 * jp + 1, :], (8, 128))
                            pb1 = jnp.broadcast_to(p_scr[par, 2 * jp + 1:2 * jp + 2, :], (8, 128))
                            if PMODE == 2:
                                pb_scr[32 * par + 2 * jp] = pb0
                                pb_scr[32 * par + 2 * jp + 1] = pb1
                        else:
                            pb0 = pb_scr[32 * par + 2 * jp]
                            pb1 = pb_scr[32 * par + 2 * jp + 1]
                        for g in range(gb * NACC, (gb + 1) * NACC):
                            v = pltpu.bitcast(
                                vu[2 * m + par, g, 8 * jp:8 * jp + 8, :], BF).astype(F32)
                            t = v[:8] * pb0
                            a[g] = t if jp == 0 else a[g] + t
                            a[g] = a[g] + v[8:] * pb1
                            if jp == njp - 1:
                                accx[G * par + g] = a[g]
                    ops.append(op)
        return ops

    def g_softmax():
        for par in range(2):
            s = part[par, 0] + part[par, 1]
            ml = jnp.maximum(jnp.max(s, axis=0, keepdims=True), NEG)
            p = jnp.exp2((s - ml) * c2)
            p_scr[par] = p
            ml_scr[par] = jnp.broadcast_to(ml, (8, 128))
            ls_scr[par] = (p[0:8] + p[8:16]) + (p[16:24] + p[24:32])

    def g_rescale():
        for par in range(2):
            w = jnp.exp2((ml_scr[par] - mx_scr[par]) * c2)
            for g in range(G):
                accy[G * par + g] = accx[G * par + g] * w
            accy[2 * G + par] = ls_scr[par] * w

    def g_olhs():
        inv = [1.0 / jnp.sum(zbuf[2 * G + par], axis=0, keepdims=True) for par in range(2)]
        inv = [jnp.broadcast_to(v, (8, 128)) for v in inv]
        for c in range(3):
            xs = [zbuf[16 * c + b] for b in range(16)]
            for k in range(4):
                xs = [jnp.where(lane_bit[k], xs[i + 1], xs[i]) for i in range(0, len(xs), 2)]
            iv = inv[0] if c == 0 else (inv[1] if c == 2 else jnp.where(lane_lo, inv[0], inv[1]))
            z = jnp.where(diag8, xs[0] * iv, 0.0)
            olhs[c] = pack16(z, z)

    def g_query():
        rs = rs_scr[...]
        for c in range(3):
            xs = [qpart[c * KD + k] for k in range(KD)]
            q = (((xs[0] + xs[1]) + (xs[2] + xs[3])) + xs[4]) * rs
            if c == 1:
                pat_scr[c] = pack16(jnp.where(lane_lo, q, 0.0), jnp.where(lane_lo, 0.0, q))
            else:
                pat_scr[c] = pack16(q, q)

    def g_out():
        for n in range(KD):
            out_scr[n] = (out_scr[n] + opart[3 * n]) + (opart[3 * n + 1] + opart[3 * n + 2])

    def run(ops):
        for op in ops:
            op()

    def reset_pipeline():
        zero = jnp.zeros((8, 128), F32)
        one = jnp.ones((8, 128), F32)
        for g in range(2 * G):
            accx[g] = zero
            zbuf[g] = zero
        for par in range(2):
            zbuf[2 * G + par] = one
            ml_scr[par] = zero
            mx_scr[par] = zero
            ls_scr[par] = one
        for i in range(3 * KD):
            opart[i] = zero
        for n in range(KD):
            out_scr[n] = zero

    def residual(x, a):
        return (x + a.astype(BF).astype(F32)).astype(BF).astype(F32)

    def matvec(l, wu, r0, nr):
        cols = []
        for c in range(wu.shape[1]):
            w = pltpu.bitcast(wu[r0:r0 + nr, c].reshape(8 * nr, 128), BF)
            cols.append(jnp.dot(l, w, preferred_element_type=F32))
        return jnp.concatenate(cols, axis=1)

    def wait_all(cs):
        for c in cs:
            c.wait()

    def ffn(x, first):
        xc, rs = center(x)
        y = jnp.broadcast_to(xc, (8, D)).astype(BF)
        if first:
            reset_pipeline()
            wait_all(c_w1)
        g = matvec(y, w1.bitcast(U32), 0, D // 16) * rs
        if first:
            wait_all(c_w3)
        u = matvec(y, w3.bitcast(U32), 0, D // 16) * rs
        hh = (g * jax.nn.sigmoid(g) * u).astype(BF)
        w2u = w2.bitcast(U32)
        if first:
            a = None
            for cs, o, n in zip(c_w2, w2_off, W2_CHUNKS):
                wait_all(cs)
                t = matvec(hh[:, o:o + n], w2u, o // 16, n // 16)[0:1]
                a = t if a is None else a + t
        else:
            a = matvec(hh, w2u, 0, FF // 16)[0:1]
        return residual(x, a)

    def layer(li, x):
        first = li == 0

        xc, rs = center(x)
        y = jnp.broadcast_to(xc, (8, D))
        for k in range(KD):
            yk = y[:, 128 * k:128 * k + 128]
            y_scr[k] = pack16(yk, yk)
        rs_scr[...] = jnp.broadcast_to(rs, (8, 128))
        run(qproj_ops(0))
        g_query()
        run(qproj_ops(1))
        run(qk_ops(0))

        def body(m, carry):
            g_rescale()
            g_softmax()
            g_olhs()
            g_query()
            g_out()

            @pl.when(first)
            def _():
                @pl.when(m + 1 < NP)
                def _():
                    for c in kcopies(m + 1):
                        c.wait()
                vcopy(m).wait()

            side = (qk_ops(jnp.minimum(m + 1, NP - 1))
                    + qproj_ops(jnp.minimum(m + 2, NP - 1))
                    + oproj_ops(jnp.maximum(m - 2, 0)))
            xmax()
            xlane()
            paced[0] = True
            _interleave(side, pv_ops(m))
            paced[0] = False
            return carry

        lax.fori_loop(0, NP, body, 0)

        g_rescale()
        g_olhs()
        g_out()
        run(oproj_ops(NP - 2))
        xlane()
        g_out()
        g_olhs()
        run(oproj_ops(NP - 1))
        g_out()
        a = jnp.concatenate(
            [jnp.sum(out_scr[n], axis=0, keepdims=True) for n in range(KD)], axis=1)
        x = residual(x, a)
        return lax.cond(first, lambda x: ffn(x, True), lambda x: ffn(x, False), x)

    reset_pipeline()
    c_x.wait()
    for c in c_wq + kcopies(0) + c_wo:
        c.wait()
    x = lax.fori_loop(0, 2, layer, xb[...].astype(F32))
    o_ref[...] = x.astype(o_ref.dtype)


@jax.jit
def pallas_interleave_layers__sliding_block_cached__glu_gated_swiglu__decode_kernel(
    A_x: jax.Array,
    A_k_cache: jax.Array,
    A_v_cache: jax.Array,
    A_wq: jax.Array,
    A_wo: jax.Array,
    B_x: jax.Array,
    B_w1: jax.Array,
    B_w3: jax.Array,
    B_w2: jax.Array,
):
    del B_x
    sk = A_k_cache.shape[2]
    win = min(4096, max(256, sk // 4))
    nb = sk // 128
    nblk = win // 128

    def cache_tiles(c):
        return c.reshape(H, nb, 128, G, 8).transpose(0, 3, 1, 4, 2)

    def weight_tiles(w):
        r, c = w.shape
        return w.reshape(r // 16, 2, 8, c // 128, 128).transpose(0, 1, 3, 2, 4)

    vreg = lambda n, dt=F32: pltpu.VMEM((n, 8, 128), dt)
    kern = lambda *refs: _kernel(*refs, blk0=nb - nblk, nblk=nblk, scale=DH ** -0.5)
    out = pl.pallas_call(
        kern,
        out_shape=jax.ShapeDtypeStruct((1, D), BF),
        in_specs=[pl.BlockSpec(memory_space=pl.ANY)] * 8,
        out_specs=pl.BlockSpec(memory_space=pltpu.VMEM),
        scratch_shapes=[
            pltpu.VMEM((1, D), BF),
            pltpu.VMEM((H, G2, nblk, 16, 128), BF),
            pltpu.VMEM((H, G, 8 * nblk, 128), BF),
            pltpu.VMEM((D // 16, 3 * NP, 16, 128), BF),
            pltpu.VMEM((H * DH // 16, KD, 16, 128), BF),
            pltpu.VMEM((D // 16, FF // 128, 16, 128), BF),
            pltpu.VMEM((D // 16, FF // 128, 16, 128), BF),
            pltpu.VMEM((FF // 16, KD, 16, 128), BF),
            vreg(KD, U32),
            pltpu.VMEM((8, 128), F32),
            vreg(3 * KD),
            vreg(3, U32),
            pltpu.VMEM((2, 2, nblk, 128), F32),
            pltpu.VMEM((2, nblk, 128), F32),
            vreg(2),
            vreg(2),
            vreg(2),
            vreg(2 * G),
            vreg(2 * G + 2),
            vreg(2 * G + 2),
            vreg(3, U32),
            vreg(3 * KD),
            vreg(KD),
            vreg(64),
            pltpu.SemaphoreType.DMA((2, NP)),
            pltpu.SemaphoreType.DMA((NP,)),
            pltpu.SemaphoreType.DMA((9 + 2 * len(W2_CHUNKS),)),
        ],
        compiler_params=pltpu.CompilerParams(vmem_limit_bytes=124 * 1024 * 1024, disable_semaphore_checks=bool(1)),
    )(A_x.reshape(1, D),
      cache_tiles(A_k_cache).reshape(H, G2, 2, nb, 8, 128),
      cache_tiles(A_v_cache).reshape(H, G, nb * 8, 128),
      weight_tiles(A_wq), weight_tiles(A_wo),
      weight_tiles(B_w1), weight_tiles(B_w3), weight_tiles(B_w2))
    return out.reshape(1, 1, D)
```

```python
import math

import jax
import jax.numpy as jnp
from jax import lax
import jax.experimental.pallas as pl
import jax.experimental.pallas.tpu as pltpu

BF = jnp.bfloat16
F32 = jnp.float32
U32 = jnp.uint32

D = 640
H = 32
DH = 192
G = DH // 8
G2 = DH // 16
NP = H // 2
FF = 1536
EPS = 1e-5
KD = D // 128
NZ = 2 * G + 2
NR = NZ + 2
NEG = float(jnp.finfo(jnp.float32).min)
W2_CHUNKS = (768, 384, 256, 128)
NACC = 8
UNPACED = 4
LAST_KT = 24
KORD = 1
JB = 2
RS0 = 2
EXM = 1
PBS = 2
SCOPES = 0


def _merge(a, b):
    out = []
    na, nb = len(a), len(b)
    ia = 0
    for ib in range(nb):
        while ia < na and ia * nb <= ib * na:
            out.append(a[ia])
            ia += 1
        out.append(b[ib])
    return out + a[ia:]


def _run(ops):
    for op in ops:
        op()


def _kernel(x_hbm, k_hbm, v_hbm, wq_hbm, wo_hbm, w1_hbm, w3_hbm, w2_hbm,
            o_ref,
            xb, kvb, wq, wo, w1, w3, w2,
            y_scr, rs_scr, qpart, pat_scr, part, p_scr, pb_scr, ml_scr, ls_scr,
            mx_scr, w_scr, accx, accy, zbuf, zbuf2, olhs, opart, obig, out_scr,
            kvsem, wsem, *, blk0, nblk, scale):
    c2 = scale * math.log2(math.e)

    def kv_copies(m):
        return [pltpu.make_async_copy(
            src.at[pl.ds(2 * m, 2), :, t, pl.ds(blk0, nblk)],
            kvb.at[m, i, :, :, :, pl.ds(8 * t, 8), :], kvsem.at[m])
            for i, src in enumerate((k_hbm, v_hbm)) for t in range(2)]

    def kv_wait(m):
        pltpu.make_async_copy(kvb.at[m], kvb.at[m], kvsem.at[m]).wait()

    def wcopies(src, dst, s, r0=0, nr=None):
        nr = src.shape[0] if nr is None else nr
        return [pltpu.make_async_copy(src.at[pl.ds(r0, nr), t],
                                      dst.at[pl.ds(r0, nr), :, pl.ds(8 * t, 8), :],
                                      wsem.at[s]) for t in range(2)]

    c_x = pltpu.make_async_copy(x_hbm, xb, wsem.at[0])
    c_wq = [pltpu.make_async_copy(wq_hbm.at[:, pl.ds(128 * c, 128)], wq.at[c], wsem.at[1])
            for c in range(3 * NP)]
    c_wo = wcopies(wo_hbm, wo, 2)
    c_w1 = wcopies(w1_hbm, w1, 3)
    c_w3 = wcopies(w3_hbm, w3, 4)
    w2_off = [sum(W2_CHUNKS[:i]) for i in range(len(W2_CHUNKS))]
    c_w2 = [wcopies(w2_hbm, w2, 5 + i, o // 16, n // 16)
            for i, (o, n) in enumerate(zip(w2_off, W2_CHUNKS))]

    for c in c_wo + [c_x] + c_wq:
        c.start()
    for m in range(NP):
        for c in kv_copies(m):
            c.start()
    for c in c_w1 + c_w3 + [c for cs in c_w2 for c in cs]:
        c.start()

    def wait_all(cs):
        for c in cs:
            c.wait()

    kvu = kvb.bitcast(U32)
    wqu = wq.bitcast(U32)
    wou = wo.bitcast(U32)

    lane = lax.broadcasted_iota(jnp.int32, (8, 128), 1)
    row = lax.broadcasted_iota(jnp.int32, (8, 128), 0)
    diag8 = (lane & 7) == row
    lane_lo = lane < 64
    lane_bit = [((lane >> (3 + k)) & 1) == 1 for k in range(4)]

    def center(x):
        xc = x - jnp.mean(x, axis=-1, keepdims=True)
        var = jnp.mean(xc * xc, axis=-1, keepdims=True)
        return xc, 1.0 / jnp.sqrt(var + EPS)

    def pack16(z0, z1):
        return pltpu.bitcast(jnp.concatenate([z0, z1], axis=0).astype(BF), U32)

    def tile_dot(l_u32, w_u32, rows, paced):
        w = pltpu.bitcast(w_u32.reshape(64, 128), BF)
        if paced:
            l = pltpu.bitcast(jnp.concatenate([l_u32, l_u32], axis=0), BF)[:24]
            return jnp.dot(l, w, preferred_element_type=F32)[:rows]
        l = pltpu.bitcast(l_u32, BF)[:rows]
        return jnp.dot(l, w, preferred_element_type=F32)

    def qproj_ops(m):
        def op(paced, c, k):
            qpart[c * KD + k] = tile_dot(
                y_scr[k], wqu[3 * m + c, 64 * k:64 * k + 64, :], 8, paced)
        return [(lambda p, c=c, k=k: op(p, c, k)) for c in range(3) for k in range(KD)]

    def oproj_ops(kt, slot, dst, d0):
        def op(paced, n):
            dst[d0 + n] = tile_dot(olhs[slot], wou[pl.ds(kt * 8, 8), n], 8, paced)
        return [(lambda p, n=n: op(p, n)) for n in range(KD)]

    def qk_ops(m):
        def op_a(paced, j):
            r = tile_dot(pat_scr[0], kvu[m, 0, 0, 0:8, j], 8, paced)
            part[0, 0, j:j + 1, :] = r[j % 8:j % 8 + 1, :]

        def op_c(paced, j):
            r = tile_dot(pat_scr[2], kvu[m, 0, 1, 4:12, j], 8, paced)
            part[1, 0, j:j + 1, :] = r[j % 8:j % 8 + 1, :]

        def op_b(paced, j):
            w = jnp.concatenate([kvu[m, 0, 0, 8:12, j], kvu[m, 0, 1, 0:4, j]], axis=0)
            r = tile_dot(pat_scr[1], w, 16, paced)
            part[0, 1, j:j + 1, :] = r[j % 8:j % 8 + 1, :]
            part[1, 1, j:j + 1, :] = r[8 + j % 8:8 + j % 8 + 1, :]

        if KORD == 0:
            return [(lambda p, f=f, j=j: f(p, j)) for j in range(nblk) for f in (op_a, op_b, op_c)]
        if KORD == 1:
            return [(lambda p, f=f, j=j: f(p, j)) for f in (op_a, op_b, op_c) for j in range(nblk)]
        return [(lambda p, f=f, j=j: f(p, j)) for j0 in range(0, nblk, 4) for f in (op_a, op_b, op_c) for j in range(j0, j0 + 4)]

    def bind(ops, paced):
        n = len(ops) - UNPACED if paced else 0
        return [(lambda op=op, p=(i < n): op(p)) for i, op in enumerate(ops)]

    def xmax():
        for par in range(2):
            mx_scr[par] = jnp.broadcast_to(
                jnp.max(ml_scr[par], axis=1, keepdims=True), (8, 128))

    def lane_sum(v):
        return jnp.broadcast_to(jnp.sum(v, axis=1, keepdims=True), (8, 128))

    def xlane(base, dst):
        for g in range(NZ):
            dst[g] = lane_sum(accy[base + g])

    def rescale_ops(base):
        def op(par, g):
            if g < G:
                accy[base + (G * par + g)] = accx[G * par + g] * w_scr[par]
            else:
                accy[base + (2 * G + par)] = w_scr[2 + par]
        return [(lambda par=par, g=g: op(par, g)) for par in range(2) for g in range(G + 1)]

    def pv_ops(m, extra):
        ng = NACC // 2
        acc = {}

        def spread(par, q):
            p = p_scr[par, 8 * q:8 * q + 8, :]
            for r in range(8):
                pb_scr[pl.ds(8 * (nblk * par + 8 * q) + r, 8, stride=8), :] = p

        def get_pb(par, gb, j):
            i = nblk * par + j
            if PBS or gb > 0:
                return pb_scr[8 * i:8 * i + 8, :]
            pb = jnp.broadcast_to(p_scr[par, j:j + 1, :], (8, 128))
            pb_scr[8 * i:8 * i + 8, :] = pb
            return pb

        def op(par, gb, j0):
            pbs = [get_pb(par, gb, j) for j in range(j0, j0 + JB)]
            for g2 in range(gb * ng, (gb + 1) * ng):
                for j in range(j0, j0 + JB):
                    v = pltpu.bitcast(kvu[m, 1, par, g2, j], BF).astype(F32)
                    for t in range(2):
                        g = G * par + 2 * g2 + t
                        tv = v[8 * t:8 * t + 8] * pbs[j - j0]
                        acc[g] = tv if j == 0 else acc[g] + tv
                        if j == nblk - 1:
                            accx[g] = acc[g]

        ops = [(lambda par=par, gb=gb, j=j: op(par, gb, j))
               for par in range(2) for gb in range(G2 // ng) for j in range(0, nblk, JB)]
        nstep = nblk // JB
        nhead = len(ops) // 2
        sp = [[(lambda par=par, q=q: spread(par, q)) for q in range(nblk // 8)]
              for par in range(2)] if PBS else [[], []]
        if PBS == 2:
            sp[0] = sp[0][1:]
        ex0 = extra[:NACC]
        ex1 = extra[NACC:G + 1]
        ex2 = extra[G + 1:]
        lead = 1 if PBS == 1 else 0
        first = sp[0][:lead] + _merge(sp[0][lead:], ops[:nstep * 3 // 4]) + ops[nstep * 3 // 4:nstep - 1]
        first = first[:lead + RS0] + _merge(ex0 + (ex1 if EXM == 0 else []) + (ex2 if EXM == 0 else []), first[lead + RS0:])
        if EXM == 0:
            rest = _merge(sp[1], ops[nstep - 1:nhead]) + ops[nhead:]
        else:
            second = _merge(ex1, ops[nstep - 1:min(2 * nstep - 1, nhead)]) + ops[min(2 * nstep - 1, nhead):nhead]
            rest = _merge(sp[1], second) + _merge(ex2, ops[nhead:nhead + nstep - 1]) + ops[nhead + nstep - 1:]
        return first + rest

    def g_softmax():
        for par in range(2):
            s = part[par, 0] + part[par, 1]
            ml = jnp.maximum(jnp.max(s, axis=0, keepdims=True), NEG)
            p = jnp.exp2((s - ml) * c2)
            p_scr[par] = p
            if PBS == 2 and par == 0:
                for r in range(8):
                    pb_scr[pl.ds(r, 8, stride=8), :] = p[0:8]
            ml_scr[par] = jnp.broadcast_to(ml, (8, 128))
            ls_scr[par] = (p[0:8] + p[8:16]) + (p[16:24] + p[24:32])

    def g_weight():
        for par in range(2):
            w = jnp.exp2((ml_scr[par] - mx_scr[par]) * c2)
            w_scr[par] = w
            w_scr[2 + par] = ls_scr[par] * w

    def o_rows(z):
        inv = [1.0 / jnp.sum(z[2 * G + par], axis=0, keepdims=True) for par in range(2)]
        inv = [jnp.broadcast_to(v, (8, 128)) for v in inv]
        out = []
        for c in range(3):
            xs = [z[16 * c + b] for b in range(16)]
            for k in range(4):
                xs = [jnp.where(lane_bit[k], xs[i + 1], xs[i]) for i in range(0, len(xs), 2)]
            iv = inv[0] if c == 0 else (inv[1] if c == 2 else jnp.where(lane_lo, inv[0], inv[1]))
            out.append(jnp.where(diag8, xs[0] * iv, 0.0))
        return out

    def g_olhs(slot0):
        for c, z in enumerate(o_rows(zbuf)):
            olhs[slot0 + c] = pack16(z, z)

    def g_query():
        rs = rs_scr[0]
        for c in range(3):
            xs = [qpart[c * KD + k] for k in range(KD)]
            q = (((xs[0] + xs[1]) + (xs[2] + xs[3])) + xs[4]) * rs
            if c == 1:
                pat_scr[c] = pack16(jnp.where(lane_lo, q, 0.0), jnp.where(lane_lo, 0.0, q))
            else:
                pat_scr[c] = pack16(q, q)

    def g_out():
        for n in range(KD):
            out_scr[n] = out_scr[n] + opart[n]

    def reset_pipeline():
        zero = jnp.zeros((8, 128), F32)
        one = jnp.ones((8, 128), F32)
        for g in range(2 * G):
            accx[g] = zero
            accy[g] = zero
            zbuf[g] = zero
        for par in range(2):
            accy[2 * G + par] = one
            zbuf[2 * G + par] = one
            ml_scr[par] = zero
            mx_scr[par] = zero
            ls_scr[par] = one
        for c in range(3):
            olhs[6 + c] = jnp.zeros((8, 128), U32)
        for n in range(KD):
            opart[n] = zero
            out_scr[n] = zero

    def residual(x, a):
        return (x + a.astype(BF).astype(F32)).astype(BF).astype(F32)

    def matvec(l, wu, r0, nr):
        cols = []
        for c in range(wu.shape[1]):
            w = pltpu.bitcast(wu[r0:r0 + nr, c].reshape(8 * nr, 128), BF)
            cols.append(jnp.dot(l, w, preferred_element_type=F32))
        return cols

    def ffn(x, first):
        xc, rs = center(x)
        y = jnp.broadcast_to(xc, (8, D)).astype(BF)
        if first:
            reset_pipeline()
            wait_all(c_w1)
        g = jnp.concatenate(matvec(y, w1.bitcast(U32), 0, D // 16), axis=1) * rs
        if first:
            wait_all(c_w3)
        u = jnp.concatenate(matvec(y, w3.bitcast(U32), 0, D // 16), axis=1) * rs
        hh = (g * jax.nn.sigmoid(g) * u).astype(BF)
        w2u = w2.bitcast(U32)
        if first:
            a = None
            for cs, o, n in zip(c_w2, w2_off, W2_CHUNKS):
                wait_all(cs)
                t = jnp.concatenate(matvec(hh[:, o:o + n], w2u, o // 16, n // 16), axis=1)[0:1]
                a = t if a is None else a + t
        else:
            a = jnp.concatenate(matvec(hh, w2u, 0, FF // 16), axis=1)[0:1]
        return residual(x, a)

    def barrier(li):
        @pl.when(li > 2)
        def _():
            kv_wait(0)

    def layer(li, x):
        first = li == 0

        xc, rs = center(x)
        y = jnp.broadcast_to(xc, (8, D))
        for k in range(KD):
            yk = y[:, 128 * k:128 * k + 128]
            y_scr[k] = pack16(yk, yk)
        rs_scr[0] = jnp.broadcast_to(rs, (8, 128))
        _run(bind(qproj_ops(0), False))
        g_query()
        _run(bind(qproj_ops(1) + qk_ops(0), False))

        def body(m, carry):
            g_weight()
            g_softmax()
            g_olhs(3 * m)
            g_query()
            g_out()

            @pl.when(first)
            def _():
                kv_wait(m + 1)

            side = (qk_ops(m + 1) + qproj_ops(jnp.minimum(m + 2, NP - 1))
                    + oproj_ops(jnp.maximum(m - 3, 0), m + 6, opart, 0))
            base = m * NR
            xmax()
            xlane(base, zbuf)
            _run(_merge(bind(side, True), pv_ops(m, rescale_ops(base + NR))))
            return carry

        if SCOPES:
            with jax.named_scope("loop"):
                lax.fori_loop(0, NP - 1, body, 0)
        else:
            lax.fori_loop(0, NP - 1, body, 0)

        m = NP - 1
        kt0 = NP - 4
        g_weight()
        _run(rescale_ops((m + 1) * NR))
        g_softmax()
        g_olhs(3 * m)
        g_out()
        barrier(li)
        side = [op for i in range(LAST_KT)
                for op in oproj_ops(kt0 + i, kt0 + i + 9, obig, KD * i)]
        xmax()
        xlane(m * NR, zbuf)
        xlane((m + 1) * NR, zbuf2)
        _run(_merge(bind(side, True), pv_ops(m, [])))
        barrier(li)

        g_weight()
        z = [lane_sum(accx[G * par + g] * w_scr[par]) for par in range(2) for g in range(G)]
        z += [lane_sum(w_scr[2 + par]) for par in range(2)]
        kt1 = kt0 + LAST_KT
        rows = [pltpu.bitcast(olhs[kt + 9], BF)[:8] for kt in range(kt1, 3 * (NP - 3))]
        rows += [r.astype(BF) for zz in (zbuf, zbuf2) for r in o_rows(zz)]
        a0 = matvec(jnp.concatenate(rows, axis=1), wou, 8 * kt1, 8 * len(rows))
        rows = [r.astype(BF) for r in o_rows(z)]
        a1 = matvec(jnp.concatenate(rows, axis=1), wou, 8 * (3 * NP - 3), 24)
        cols = []
        for n in range(KD):
            xs = [out_scr[n]] + [obig[KD * i + n] for i in range(LAST_KT)]
            while len(xs) > 1:
                xs = [xs[i] + xs[i + 1] for i in range(0, len(xs) - 1, 2)] + xs[len(xs) & ~1:]
            cols.append(jnp.sum((xs[0] + a0[n]) + a1[n], axis=0, keepdims=True))
        x = residual(x, jnp.concatenate(cols, axis=1))
        if SCOPES:
            with jax.named_scope("ffn"):
                return lax.cond(first, lambda x: ffn(x, True), lambda x: ffn(x, False), x)
        return lax.cond(first, lambda x: ffn(x, True), lambda x: ffn(x, False), x)

    reset_pipeline()
    wait_all([c_x] + c_wq + c_wo)
    kv_wait(0)
    x = lax.fori_loop(0, 2, layer, xb[...].astype(F32))
    o_ref[...] = x.astype(o_ref.dtype)


@jax.jit
def pallas_interleave_layers__sliding_block_cached__glu_gated_swiglu__decode_kernel(
    A_x: jax.Array,
    A_k_cache: jax.Array,
    A_v_cache: jax.Array,
    A_wq: jax.Array,
    A_wo: jax.Array,
    B_x: jax.Array,
    B_w1: jax.Array,
    B_w3: jax.Array,
    B_w2: jax.Array,
):
    del B_x
    sk = A_k_cache.shape[2]
    win = min(4096, max(256, sk // 4))
    nb = sk // 128
    nblk = win // 128

    def cache_tiles(c):
        return c.reshape(H, nb, 128, G2, 2, 8).transpose(0, 3, 4, 1, 5, 2)

    def weight_tiles(w):
        r, c = w.shape
        return w.reshape(r // 16, 2, 8, c // 128, 128).transpose(0, 1, 3, 2, 4)

    vreg = lambda n, dt=F32: pltpu.VMEM((-(-n // 4) * 4, 8, 128), dt)
    kern = lambda *refs: _kernel(*refs, blk0=nb - nblk, nblk=nblk, scale=DH ** -0.5)
    out = pl.pallas_call(
        kern,
        out_shape=jax.ShapeDtypeStruct((1, D), BF),
        in_specs=[pl.BlockSpec(memory_space=pl.ANY)] * 8,
        out_specs=pl.BlockSpec(memory_space=pltpu.VMEM),
        scratch_shapes=[
            pltpu.VMEM((1, D), BF),
            pltpu.VMEM((NP, 2, 2, G2, nblk, 16, 128), BF),
            pltpu.VMEM((3 * NP, D, 128), BF),
            pltpu.VMEM((H * DH // 16, KD, 16, 128), BF),
            pltpu.VMEM((D // 16, FF // 128, 16, 128), BF),
            pltpu.VMEM((D // 16, FF // 128, 16, 128), BF),
            pltpu.VMEM((FF // 16, KD, 16, 128), BF),
            vreg(KD, U32),
            vreg(1),
            vreg(3 * KD),
            vreg(3, U32),
            pltpu.VMEM((2, 2, nblk, 128), F32),
            pltpu.VMEM((2, nblk, 128), F32),
            pltpu.VMEM((2 * nblk * 8, 128), F32),
            vreg(2),
            vreg(2),
            vreg(2),
            vreg(4),
            vreg(2 * G),
            vreg(NR * (NP + 1)),
            vreg(NZ),
            vreg(NZ),
            vreg(3 * NP, U32),
            vreg(KD),
            vreg(KD * LAST_KT),
            vreg(KD),
            pltpu.SemaphoreType.DMA((NP,)),
            pltpu.SemaphoreType.DMA((5 + len(W2_CHUNKS),)),
        ],
        compiler_params=pltpu.CompilerParams(
            vmem_limit_bytes=124 * 1024 * 1024, disable_semaphore_checks=True),
    )(A_x.reshape(1, D), cache_tiles(A_k_cache), cache_tiles(A_v_cache),
      A_wq, weight_tiles(A_wo),
      weight_tiles(B_w1), weight_tiles(B_w3), weight_tiles(B_w2))
    return out.reshape(1, 1, D)
```

```python
import math

import jax
import jax.numpy as jnp
from jax import lax
import jax.experimental.pallas as pl
import jax.experimental.pallas.tpu as pltpu

BF = jnp.bfloat16
F32 = jnp.float32
U32 = jnp.uint32

D = 640
H = 32
DH = 192
G = DH // 8
G2 = DH // 16
NP = H // 2
FF = 1536
EPS = 1e-5
KD = D // 128
NZ = 2 * G + 2
NR = NZ + 2
NEG = float(jnp.finfo(jnp.float32).min)
W2_CHUNKS = (768, 384, 256, 128)
NACC = 8
UNPACED = 200
LAST_KT = 24
KORD = 1
JB = 2
RS0 = 0
SPL = 1
RSL = 1
OPK = 1
XF = 1
XFIRST = 1
ORD = 4
LEAD = 32
TAIL = 2
PBS = 2
SCOPES = 0


def _merge(a, b):
    out = []
    na, nb = len(a), len(b)
    ia = 0
    for ib in range(nb):
        while ia < na and ia * nb <= ib * na:
            out.append(a[ia])
            ia += 1
        out.append(b[ib])
    return out + a[ia:]


def _run(ops):
    for op in ops:
        op()


def _kernel(x_hbm, k_hbm, v_hbm, wq_hbm, wo_hbm, w1_hbm, w3_hbm, w2_hbm,
            o_ref,
            xb, kvb, wq, wo, w1, w3, w2,
            y_scr, rs_scr, qpart, pat_scr, part, p_scr, pb_scr, ml_scr, ls_scr,
            mx_scr, w_scr, accx, accy, zbuf, olhs, opart, out_scr, vx,
            kvsem, wsem, *, blk0, nblk, scale):
    c2 = scale * math.log2(math.e)

    def kv_copies(m):
        return [pltpu.make_async_copy(
            src.at[pl.ds(2 * m, 2), :, t, pl.ds(blk0, nblk)],
            kvb.at[m, i, :, :, :, pl.ds(8 * t, 8), :], kvsem.at[m])
            for i, src in enumerate((k_hbm, v_hbm)) for t in range(2)]

    def kv_wait(m):
        pltpu.make_async_copy(kvb.at[m], kvb.at[m], kvsem.at[m]).wait()

    def wcopies(src, dst, s, r0=0, nr=None):
        nr = src.shape[0] if nr is None else nr
        return [pltpu.make_async_copy(src.at[pl.ds(r0, nr), t],
                                      dst.at[pl.ds(r0, nr), :, pl.ds(8 * t, 8), :],
                                      wsem.at[s]) for t in range(2)]

    c_x = pltpu.make_async_copy(x_hbm, xb, wsem.at[0])
    c_wq = [pltpu.make_async_copy(wq_hbm.at[:, pl.ds(128 * c, 128)], wq.at[c], wsem.at[1])
            for c in range(3 * NP)]
    c_wo = wcopies(wo_hbm, wo, 2)
    c_w1 = wcopies(w1_hbm, w1, 3)
    c_w3 = wcopies(w3_hbm, w3, 4)
    w2_off = [sum(W2_CHUNKS[:i]) for i in range(len(W2_CHUNKS))]
    c_w2 = [wcopies(w2_hbm, w2, 5 + i, o // 16, n // 16)
            for i, (o, n) in enumerate(zip(w2_off, W2_CHUNKS))]

    for c in c_wo + [c_x] + c_wq:
        c.start()
    for m in range(NP):
        for c in kv_copies(m):
            c.start()
    for c in c_w1 + c_w3 + [c for cs in c_w2 for c in cs]:
        c.start()

    def wait_all(cs):
        for c in cs:
            c.wait()

    kvu = kvb.bitcast(U32)
    wqu = wq.bitcast(U32)
    wou = wo.bitcast(U32)

    lane = lax.broadcasted_iota(jnp.int32, (8, 128), 1)
    row = lax.broadcasted_iota(jnp.int32, (8, 128), 0)
    diag8 = (lane & 7) == row
    lane_lo = lane < 64
    lane_bit = [((lane >> (3 + k)) & 1) == 1 for k in range(4)]

    def center(x):
        xc = x - jnp.mean(x, axis=-1, keepdims=True)
        var = jnp.mean(xc * xc, axis=-1, keepdims=True)
        return xc, 1.0 / jnp.sqrt(var + EPS)

    def pack16(z0, z1):
        return pltpu.bitcast(jnp.concatenate([z0, z1], axis=0).astype(BF), U32)

    def tile_dot(l_u32, w_u32, rows, paced):
        w = pltpu.bitcast(w_u32.reshape(64, 128), BF)
        if paced:
            l = pltpu.bitcast(jnp.concatenate([l_u32, l_u32], axis=0), BF)[:24]
            return jnp.dot(l, w, preferred_element_type=F32)[:rows]
        l = pltpu.bitcast(l_u32, BF)[:rows]
        return jnp.dot(l, w, preferred_element_type=F32)

    def qproj_ops(m):
        def op(paced, c, k):
            qpart[c * KD + k] = tile_dot(
                y_scr[k], wqu[3 * m + c, 64 * k:64 * k + 64, :], 8, paced)
        return [(lambda p, c=c, k=k: op(p, c, k)) for c in range(3) for k in range(KD)]

    def oproj_ops(kt, slot, dst, d0):
        def op(paced, n):
            dst[d0 + n] = tile_dot(olhs[slot], wou[pl.ds(kt * 8, 8), n], 8, paced)
        return [(lambda p, n=n: op(p, n)) for n in range(KD)]

    def qk_ops(m):
        def op_a(paced, j):
            r = tile_dot(pat_scr[0], kvu[m, 0, 0, 0:8, j], 8, paced)
            part[0, 0, j:j + 1, :] = r[j % 8:j % 8 + 1, :]

        def op_c(paced, j):
            r = tile_dot(pat_scr[2], kvu[m, 0, 1, 4:12, j], 8, paced)
            part[1, 0, j:j + 1, :] = r[j % 8:j % 8 + 1, :]

        def op_b(paced, j):
            w = jnp.concatenate([kvu[m, 0, 0, 8:12, j], kvu[m, 0, 1, 0:4, j]], axis=0)
            r = tile_dot(pat_scr[1], w, 16, paced)
            part[0, 1, j:j + 1, :] = r[j % 8:j % 8 + 1, :]
            part[1, 1, j:j + 1, :] = r[8 + j % 8:8 + j % 8 + 1, :]

        if KORD == 0:
            return [(lambda p, f=f, j=j: f(p, j)) for j in range(nblk) for f in (op_a, op_b, op_c)]
        if KORD == 1:
            return [(lambda p, f=f, j=j: f(p, j)) for f in (op_a, op_b, op_c) for j in range(nblk)]
        return [(lambda p, f=f, j=j: f(p, j)) for j0 in range(0, nblk, 4) for f in (op_a, op_b, op_c) for j in range(j0, j0 + 4)]

    def bind(ops, paced):
        n = len(ops) - UNPACED if paced else 0
        return [(lambda op=op, p=(i < n): op(p)) for i, op in enumerate(ops)]

    def emit(pv, side, xl):
        if ORD == 0:
            _run(pv)
            _run(xl + side if XFIRST else side + xl)
            return
        rounds = [(lambda c=side[i:i + ORD]: _run(c)) for i in range(0, len(side), ORD)]
        lead = len(pv) * LEAD // 100
        nr = len(rounds) - TAIL
        _run(pv[:lead] + xl + _merge(rounds[:nr], pv[lead:]) + rounds[nr:])

    def xmax():
        for par in range(2):
            mx_scr[par] = jnp.broadcast_to(
                jnp.max(ml_scr[par], axis=1, keepdims=True), (8, 128))

    def lane_sum(v):
        return jnp.broadcast_to(jnp.sum(v, axis=1, keepdims=True), (8, 128))

    def xlane(base, dst, d0=0):
        for g in range(NZ):
            dst[d0 + g] = lane_sum(accy[base + g])

    wide = {}
    for par in range(2):
        for g2 in range(3, G2, 4):
            for j in range(0, nblk, 2):
                if XF:
                    wide[(par, g2, j)] = len(wide)

    def widen(m):
        for (par, g2, j), e in wide.items():
            v = pltpu.bitcast(kvu[m, 1, par, g2, j], BF).astype(F32)
            kvu[m, 1, par, g2, j] = pltpu.bitcast(v[:8], U32)
            vx[m, e] = v[8:]

    def v_rows(m, par, g2, j):
        u = kvu[m, 1, par, g2, j]
        if (par, g2, j) in wide:
            return pltpu.bitcast(u, F32), vx[m, wide[(par, g2, j)]]
        v = pltpu.bitcast(u, BF).astype(F32)
        return v[:8], v[8:]

    def rescale_ops(base):
        def op(par, g):
            if g < G:
                accy[base + (G * par + g)] = accx[G * par + g] * w_scr[par]
            else:
                accy[base + (2 * G + par)] = w_scr[2 + par]
        return [(lambda par=par, g=g: op(par, g)) for par in range(2) for g in range(G + 1)]

    def pv_ops(m, extra):
        ng = NACC // 2
        acc = {}

        def spread(par, q, r):
            pb_scr[pl.ds(8 * (nblk * par + 8 * q) + r, 8, stride=8), :] = (
                p_scr[par, 8 * q:8 * q + 8, :])

        def get_pb(par, gb, j):
            i = nblk * par + j
            if PBS or gb > 0:
                return pb_scr[8 * i:8 * i + 8, :]
            pb = jnp.broadcast_to(p_scr[par, j:j + 1, :], (8, 128))
            pb_scr[8 * i:8 * i + 8, :] = pb
            return pb

        def op(par, gb, j0):
            pbs = [get_pb(par, gb, j) for j in range(j0, j0 + JB)]
            for g2 in range(gb * ng, (gb + 1) * ng):
                for j in range(j0, j0 + JB):
                    v = v_rows(m, par, g2, j)
                    for t in range(2):
                        g = G * par + 2 * g2 + t
                        tv = v[t] * pbs[j - j0]
                        acc[g] = tv if j == 0 else acc[g] + tv
                        if j == nblk - 1:
                            accx[g] = acc[g]

        ops = [(lambda par=par, gb=gb, j=j: op(par, gb, j))
               for par in range(2) for gb in range(G2 // ng) for j in range(0, nblk, JB)]
        nstep = nblk // JB
        nb_acc = len(ops) // nstep
        todo = []
        for par in range(2):
            for q in range(nblk // 8):
                if par == 0 and q == 0:
                    continue
                dl = par * (len(ops) // 2) + (8 * q) // JB - SPL
                todo += [(dl, (lambda par=par, q=q, r=r: spread(par, q, r))) for r in range(8)]
        for i, ex in enumerate(extra):
            par, g = divmod(i, G + 1)
            blk = par * (nb_acc // 2) + min(g, G - 1) // NACC
            todo.append(((blk + 1) * nstep - 1 - RSL, ex))
        todo.sort(key=lambda t: t[0])
        out = []
        k = 0
        for i, op_ in enumerate(ops):
            need = 0
            for n, (dl, _) in enumerate(todo[k:]):
                need = max(need, -(-(n + 1) // max(dl - i + 1, 1)))
            if i < RS0:
                need = sum(1 for dl, _ in todo[k:] if dl <= i)
            for _, f in todo[k:k + need]:
                out.append(f)
            k += min(need, len(todo) - k)
            out.append(op_)
        assert k == len(todo)
        return out

    def g_softmax():
        for par in range(2):
            s = part[par, 0] + part[par, 1]
            ml = jnp.maximum(jnp.max(s, axis=0, keepdims=True), NEG)
            p = jnp.exp2((s - ml) * c2)
            p_scr[par] = p
            if PBS == 2 and par == 0:
                for r in range(8):
                    pb_scr[pl.ds(r, 8, stride=8), :] = p[0:8]
            ml_scr[par] = jnp.broadcast_to(ml, (8, 128))
            ls_scr[par] = (p[0:8] + p[8:16]) + (p[16:24] + p[24:32])

    def g_weight():
        for par in range(2):
            w = jnp.exp2((ml_scr[par] - mx_scr[par]) * c2)
            w_scr[par] = w
            w_scr[2 + par] = ls_scr[par] * w

    def o_rows(zz, z0=0):
        z = [zz[z0 + g] for g in range(NZ)]
        inv = [1.0 / jnp.sum(z[2 * G + par], axis=0, keepdims=True) for par in range(2)]
        inv = [jnp.broadcast_to(v, (8, 128)) for v in inv]
        out = []
        for c in range(3):
            xs = [z[16 * c + b] for b in range(16)]
            for k in range(4):
                xs = [jnp.where(lane_bit[k], xs[i + 1], xs[i]) for i in range(0, len(xs), 2)]
            iv = inv[0] if c == 0 else (inv[1] if c == 2 else jnp.where(lane_lo, inv[0], inv[1]))
            out.append(jnp.where(diag8, xs[0] * iv, 0.0))
        return out

    def g_olhs(slot0):
        for c, z in enumerate(o_rows(zbuf)):
            olhs[slot0 + c] = pack16(z, z)

    def g_query():
        rs = rs_scr[0]
        for c in range(3):
            xs = [qpart[c * KD + k] for k in range(KD)]
            q = (((xs[0] + xs[1]) + (xs[2] + xs[3])) + xs[4]) * rs
            if c == 1:
                pat_scr[c] = pack16(jnp.where(lane_lo, q, 0.0), jnp.where(lane_lo, 0.0, q))
            else:
                pat_scr[c] = pack16(q, q)

    def g_out():
        for n in range(KD):
            t = out_scr[n]
            for i in range(OPK):
                t = t + opart[KD * i + n]
            out_scr[n] = t

    def reset_pipeline():
        zero = jnp.zeros((8, 128), F32)
        one = jnp.ones((8, 128), F32)
        for g in range(2 * G):
            accx[g] = zero
            accy[g] = zero
            zbuf[g] = zero
        for par in range(2):
            accy[2 * G + par] = one
            zbuf[2 * G + par] = one
            ml_scr[par] = zero
            mx_scr[par] = zero
            ls_scr[par] = one
        for c in range(9):
            olhs[c] = jnp.zeros((8, 128), U32)
        for n in range(KD * OPK):
            opart[n] = zero
        for n in range(KD):
            out_scr[n] = zero

    def residual(x, a):
        return (x + a.astype(BF).astype(F32)).astype(BF).astype(F32)

    def matvec(l, wu, r0, nr):
        cols = []
        for c in range(wu.shape[1]):
            w = pltpu.bitcast(wu[r0:r0 + nr, c].reshape(8 * nr, 128), BF)
            cols.append(jnp.dot(l, w, preferred_element_type=F32))
        return cols

    def ffn(x, first):
        xc, rs = center(x)
        y = jnp.broadcast_to(xc, (8, D)).astype(BF)
        if first:
            reset_pipeline()
            wait_all(c_w1)
        g = jnp.concatenate(matvec(y, w1.bitcast(U32), 0, D // 16), axis=1) * rs
        if first:
            wait_all(c_w3)
        u = jnp.concatenate(matvec(y, w3.bitcast(U32), 0, D // 16), axis=1) * rs
        hh = (g * jax.nn.sigmoid(g) * u).astype(BF)
        w2u = w2.bitcast(U32)
        if first:
            a = None
            for cs, o, n in zip(c_w2, w2_off, W2_CHUNKS):
                wait_all(cs)
                t = jnp.concatenate(matvec(hh[:, o:o + n], w2u, o // 16, n // 16), axis=1)[0:1]
                a = t if a is None else a + t
        else:
            a = jnp.concatenate(matvec(hh, w2u, 0, FF // 16), axis=1)[0:1]
        return residual(x, a)

    def barrier(li):
        @pl.when(li > 2)
        def _():
            reset_pipeline()

    def layer(li, x):
        first = li == 0

        xc, rs = center(x)
        y = jnp.broadcast_to(xc, (8, D))
        for k in range(KD):
            yk = y[:, 128 * k:128 * k + 128]
            y_scr[k] = pack16(yk, yk)
        rs_scr[0] = jnp.broadcast_to(rs, (8, 128))
        _run(bind(qproj_ops(0), False))
        g_query()
        _run(bind(qproj_ops(1) + qk_ops(0), False))

        def body(m, carry):
            g_weight()
            g_softmax()
            g_olhs(3 * m)
            g_query()
            g_out()

            @pl.when(first)
            def _():
                kv_wait(m + 1)
                widen(m + 1)

            side = (qk_ops(m + 1) + qproj_ops(jnp.minimum(m + 2, NP - 1))
                    + [op for i in range(OPK)
                       for op in oproj_ops(jnp.maximum(OPK * (m - 3) + i, 0),
                                           OPK * (m - 3) + i + 9, opart, KD * i)])
            base = m * NR
            emit(pv_ops(m, rescale_ops(base + NR)), bind(side, True),
                 [xmax, lambda: xlane(base, zbuf)])
            return carry

        if SCOPES:
            with jax.named_scope("loop"):
                lax.fori_loop(0, NP - 1, body, 0)
        else:
            lax.fori_loop(0, NP - 1, body, 0)

        m = NP - 1
        kt0 = OPK * (NP - 4)
        g_weight()
        s_acc, s_z, s_o = NR, 2 * NR, 3 * NR
        _run(rescale_ops(s_acc))
        g_softmax()
        g_olhs(3 * m)
        g_out()
        barrier(li)
        side = [op for i in range(LAST_KT)
                for op in oproj_ops(kt0 + i, kt0 + i + 9, accy, s_o + KD * i)]
        emit(pv_ops(m, []), bind(side, True),
             [xmax, lambda: xlane(m * NR, zbuf), lambda: xlane(s_acc, accy, s_z)])
        barrier(li)

        g_weight()
        z = [lane_sum(accx[G * par + g] * w_scr[par]) for par in range(2) for g in range(G)]
        z += [lane_sum(w_scr[2 + par]) for par in range(2)]
        kt1 = kt0 + LAST_KT
        rows = [pltpu.bitcast(olhs[kt + 9], BF)[:8] for kt in range(kt1, 3 * (NP - 3))]
        rows += [r.astype(BF) for r in o_rows(zbuf) + o_rows(accy, s_z)]
        a0 = matvec(jnp.concatenate(rows, axis=1), wou, 8 * kt1, 8 * len(rows))
        rows = [r.astype(BF) for r in o_rows(z)]
        a1 = matvec(jnp.concatenate(rows, axis=1), wou, 8 * (3 * NP - 3), 24)
        cols = []
        for n in range(KD):
            xs = [out_scr[n]] + [accy[s_o + KD * i + n] for i in range(LAST_KT)]
            while len(xs) > 1:
                xs = [xs[i] + xs[i + 1] for i in range(0, len(xs) - 1, 2)] + xs[len(xs) & ~1:]
            cols.append(jnp.sum((xs[0] + a0[n]) + a1[n], axis=0, keepdims=True))
        x = residual(x, jnp.concatenate(cols, axis=1))
        if SCOPES:
            with jax.named_scope("ffn"):
                return lax.cond(first, lambda x: ffn(x, True), lambda x: ffn(x, False), x)
        return lax.cond(first, lambda x: ffn(x, True), lambda x: ffn(x, False), x)

    reset_pipeline()
    wait_all([c_x] + c_wq + c_wo)
    kv_wait(0)
    widen(0)
    x = lax.fori_loop(0, 2, layer, xb[...].astype(F32))
    o_ref[...] = x.astype(o_ref.dtype)


@jax.jit
def pallas_interleave_layers__sliding_block_cached__glu_gated_swiglu__decode_kernel(
    A_x: jax.Array,
    A_k_cache: jax.Array,
    A_v_cache: jax.Array,
    A_wq: jax.Array,
    A_wo: jax.Array,
    B_x: jax.Array,
    B_w1: jax.Array,
    B_w3: jax.Array,
    B_w2: jax.Array,
):
    del B_x
    sk = A_k_cache.shape[2]
    win = min(4096, max(256, sk // 4))
    nb = sk // 128
    nblk = win // 128

    def cache_tiles(c):
        return c.reshape(H, nb, 128, G2, 2, 8).transpose(0, 3, 4, 1, 5, 2)

    def weight_tiles(w):
        r, c = w.shape
        return w.reshape(r // 16, 2, 8, c // 128, 128).transpose(0, 1, 3, 2, 4)

    vreg = lambda n, dt=F32: pltpu.VMEM((-(-n // 4) * 4, 8, 128), dt)
    kern = lambda *refs: _kernel(*refs, blk0=nb - nblk, nblk=nblk, scale=DH ** -0.5)
    out = pl.pallas_call(
        kern,
        out_shape=jax.ShapeDtypeStruct((1, D), BF),
        in_specs=[pl.BlockSpec(memory_space=pl.ANY)] * 8,
        out_specs=pl.BlockSpec(memory_space=pltpu.VMEM),
        scratch_shapes=[
            pltpu.VMEM((1, D), BF),
            pltpu.VMEM((NP, 2, 2, G2, nblk, 16, 128), BF),
            pltpu.VMEM((3 * NP, D, 128), BF),
            pltpu.VMEM((H * DH // 16, KD, 16, 128), BF),
            pltpu.VMEM((D // 16, FF // 128, 16, 128), BF),
            pltpu.VMEM((D // 16, FF // 128, 16, 128), BF),
            pltpu.VMEM((FF // 16, KD, 16, 128), BF),
            vreg(KD, U32),
            vreg(1),
            vreg(3 * KD),
            vreg(3, U32),
            pltpu.VMEM((2, 2, nblk, 128), F32),
            pltpu.VMEM((2, nblk, 128), F32),
            pltpu.VMEM((2 * nblk * 8, 128), F32),
            vreg(2),
            vreg(2),
            vreg(2),
            vreg(4),
            vreg(2 * G),
            vreg(NR * NP),
            vreg(NZ),
            vreg(3 * NP, U32),
            vreg(KD * OPK),
            vreg(KD),
            pltpu.VMEM((NP, 3 * nblk, 8, 128), F32),
            pltpu.SemaphoreType.DMA((NP,)),
            pltpu.SemaphoreType.DMA((5 + len(W2_CHUNKS),)),
        ],
        compiler_params=pltpu.CompilerParams(
            vmem_limit_bytes=128 * 1024 * 1024, disable_semaphore_checks=True),
    )(A_x.reshape(1, D), cache_tiles(A_k_cache), cache_tiles(A_v_cache),
      A_wq, weight_tiles(A_wo),
      weight_tiles(B_w1), weight_tiles(B_w3), weight_tiles(B_w2))
    return out.reshape(1, 1, D)
```

```python
import math

import jax
import jax.numpy as jnp
from jax import lax
import jax.experimental.pallas as pl
import jax.experimental.pallas.tpu as pltpu

BF = jnp.bfloat16
F32 = jnp.float32
U32 = jnp.uint32

D = 640
H = 32
DH = 192
G = DH // 8
G2 = DH // 16
NP = H // 2
FF = 1536
EPS = 1e-5
KD = D // 128
NZ = 2 * G + 2
NR = NZ + 2
NEG = float(jnp.finfo(jnp.float32).min)
W2_CHUNKS = (768, 384, 256, 128)
NACC = 8
UNPACED = 4
LAST_KT = 24
KORD = 1
JB = 2
RS0 = 0
SPL = 1
RSL = 1
OPK = 1
XF = 1
XFIRST = 1
ORD = 4
LEAD = 10
TAIL = 2
OPAT = 44
PEND = 2000
OLP = 1
SM0 = 22
RATE = 32
PSA = 1060
PSB = 2000
NPRE = 4
KT14 = 10
AEND = 4
NLAG = 1
CF = 4
PBS = 2
SCOPES = 0


def _merge(a, b):
    out = []
    na, nb = len(a), len(b)
    ia = 0
    for ib in range(nb):
        while ia < na and ia * nb <= ib * na:
            out.append(a[ia])
            ia += 1
        out.append(b[ib])
    return out + a[ia:]


def _run(ops):
    for op in ops:
        op()


def _kernel(x_hbm, k_hbm, v_hbm, wq_hbm, wo_hbm, w1_hbm, w3_hbm, w2_hbm,
            o_ref,
            xb, kvb, wq, wo, w1, w3, w2,
            y_scr, rs_scr, qpart, pat_scr, part, p_scr, pb_scr, pb0,
            accx, obig, olhs, opart, out_scr, vx,
            kvsem, wsem, *, blk0, nblk, scale):
    c2 = scale * math.log2(math.e)

    def kv_copies(m):
        return [pltpu.make_async_copy(
            src.at[pl.ds(2 * m, 2), :, t, pl.ds(blk0, nblk)],
            kvb.at[m, i, :, :, :, pl.ds(8 * t, 8), :], kvsem.at[m])
            for i, src in enumerate((k_hbm, v_hbm)) for t in range(2)]

    def kv_wait(m):
        pltpu.make_async_copy(kvb.at[m], kvb.at[m], kvsem.at[m]).wait()

    def wcopies(src, dst, s, r0=0, nr=None):
        nr = src.shape[0] if nr is None else nr
        return [pltpu.make_async_copy(src.at[pl.ds(r0, nr), t],
                                      dst.at[pl.ds(r0, nr), :, pl.ds(8 * t, 8), :],
                                      wsem.at[s]) for t in range(2)]

    c_x = pltpu.make_async_copy(x_hbm, xb, wsem.at[0])
    c_wq = [pltpu.make_async_copy(wq_hbm.at[:, pl.ds(128 * c, 128)], wq.at[c], wsem.at[1])
            for c in range(3 * NP)]
    c_wo = wcopies(wo_hbm, wo, 2)
    c_w1 = wcopies(w1_hbm, w1, 3)
    c_w3 = wcopies(w3_hbm, w3, 4)
    w2_off = [sum(W2_CHUNKS[:i]) for i in range(len(W2_CHUNKS))]
    c_w2 = [wcopies(w2_hbm, w2, 5 + i, o // 16, n // 16)
            for i, (o, n) in enumerate(zip(w2_off, W2_CHUNKS))]

    for c in c_wo + [c_x] + c_wq:
        c.start()
    for m in range(NP):
        for c in kv_copies(m):
            c.start()
    for c in c_w1 + c_w3 + [c for cs in c_w2 for c in cs]:
        c.start()

    def wait_all(cs):
        for c in cs:
            c.wait()

    kvu = kvb.bitcast(U32)
    wqu = wq.bitcast(U32)
    wou = wo.bitcast(U32)

    lane = lax.broadcasted_iota(jnp.int32, (8, 128), 1)
    row = lax.broadcasted_iota(jnp.int32, (8, 128), 0)
    diag8 = (lane & 7) == row
    lane_lo = lane < 64
    lane_bit = [((lane >> (3 + k)) & 1) == 1 for k in range(4)]

    def center(x):
        xc = x - jnp.mean(x, axis=-1, keepdims=True)
        var = jnp.mean(xc * xc, axis=-1, keepdims=True)
        return xc, 1.0 / jnp.sqrt(var + EPS)

    def pack16(z0, z1):
        return pltpu.bitcast(jnp.concatenate([z0, z1], axis=0).astype(BF), U32)

    def tile_dot(l_u32, w_u32, rows, paced):
        w = pltpu.bitcast(w_u32.reshape(64, 128), BF)
        if paced:
            l = pltpu.bitcast(jnp.concatenate([l_u32, l_u32], axis=0), BF)[:24]
            return jnp.dot(l, w, preferred_element_type=F32)[:rows]
        l = pltpu.bitcast(l_u32, BF)[:rows]
        return jnp.dot(l, w, preferred_element_type=F32)

    def qproj_ops(m):
        def op(paced, c, k):
            qpart[c * KD + k] = tile_dot(
                y_scr[k], wqu[3 * m + c, 64 * k:64 * k + 64, :], 8, paced)
        return [(lambda p, c=c, k=k: op(p, c, k)) for c in range(3) for k in range(KD)]

    def oproj_ops(kt, slot, dst, d0):
        def op(paced, n):
            dst[d0 + n] = tile_dot(olhs[slot], wou[pl.ds(kt * 8, 8), n], 8, paced)
        return [(lambda p, n=n: op(p, n)) for n in range(KD)]

    def qk_ops(m):
        def op_a(paced, j):
            r = tile_dot(pat_scr[0], kvu[m, 0, 0, 0:8, j], 8, paced)
            part[0, 0, j:j + 1, :] = r[j % 8:j % 8 + 1, :]

        def op_c(paced, j):
            r = tile_dot(pat_scr[2], kvu[m, 0, 1, 4:12, j], 8, paced)
            part[1, 0, j:j + 1, :] = r[j % 8:j % 8 + 1, :]

        def op_b(paced, j):
            w = jnp.concatenate([kvu[m, 0, 0, 8:12, j], kvu[m, 0, 1, 0:4, j]], axis=0)
            r = tile_dot(pat_scr[1], w, 16, paced)
            part[0, 1, j:j + 1, :] = r[j % 8:j % 8 + 1, :]
            part[1, 1, j:j + 1, :] = r[8 + j % 8:8 + j % 8 + 1, :]

        return [[(lambda p, f=f, j=j: f(p, j)) for j in range(nblk)] for f in (op_a, op_b, op_c)]

    def bind(ops, paced):
        n = len(ops) - UNPACED if paced else 0
        return [(lambda op=op, p=(i < n): op(p)) for i, op in enumerate(ops)]

    def lane_sum(v):
        return jnp.broadcast_to(jnp.sum(v, axis=1, keepdims=True), (8, 128))

    wide = {}
    for par in range(2):
        for g2 in range(3, G2, 4):
            for j in range(0, nblk, 2):
                if XF:
                    wide[(par, g2, j)] = len(wide)

    def widen(m):
        for (par, g2, j), e in wide.items():
            v = pltpu.bitcast(kvu[m, 1, par, g2, j], BF).astype(F32)
            kvu[m, 1, par, g2, j] = pltpu.bitcast(v[:8], U32)
            vx[m, e] = v[8:]

    def v_rows(m, par, g2, j):
        u = kvu[m, 1, par, g2, j]
        if (par, g2, j) in wide:
            return pltpu.bitcast(u, F32), vx[m, wide[(par, g2, j)]]
        v = pltpu.bitcast(u, BF).astype(F32)
        return v[:8], v[8:]

    def pv_ops(m, ph):
        wbase = NR * ph
        ng = NACC // 2
        acc = {}

        def spread(par, q, r):
            pb_scr[pl.ds(8 * (nblk * par + 8 * q) + r, 8, stride=8), :] = (
                p_scr[ph, par, 8 * q:8 * q + 8, :])

        def get_pb(par, gb, j):
            i = nblk * par + j
            if i < 8:
                return pb0[ph, 8 * i:8 * i + 8, :]
            if PBS or gb > 0:
                return pb_scr[8 * i:8 * i + 8, :]
            pb = jnp.broadcast_to(p_scr[par, j:j + 1, :], (8, 128))
            pb_scr[8 * i:8 * i + 8, :] = pb
            return pb

        def op(par, gb, j0):
            pbs = [get_pb(par, gb, j) for j in range(j0, j0 + JB)]
            for g2 in range(gb * ng, (gb + 1) * ng):
                for j in range(j0, j0 + JB):
                    v = v_rows(m, par, g2, j)
                    for t in range(2):
                        g = G * par + 2 * g2 + t
                        tv = v[t] * pbs[j - j0]
                        acc[g] = tv if j == 0 else acc[g] + tv
                        if j == nblk - 1:
                            accx[wbase + g] = acc[g]

        ops = [(lambda par=par, gb=gb, j=j: op(par, gb, j))
               for par in range(2) for gb in range(G2 // ng) for j in range(0, nblk, JB)]
        wts = [sum(4 if (par, g2, j) in wide else 6
                   for g2 in range(gb * ng, (gb + 1) * ng) for j in range(j0, j0 + JB))
               for par in range(2) for gb in range(G2 // ng) for j0 in range(0, nblk, JB)]
        nstep = nblk // JB
        nb_acc = len(ops) // nstep
        todo = []
        for par in range(2):
            for q in range(nblk // 8):
                if par == 0 and q == 0:
                    continue
                dl = par * (len(ops) // 2) + (8 * q) // JB - SPL
                todo += [(dl, (lambda par=par, q=q, r=r: spread(par, q, r))) for r in range(8)]
        def lsum(par):
            p = p_scr[ph, par]
            accx[wbase + (2 * G + par)] = (p[0:8] + p[8:16]) + (p[16:24] + p[24:32])

        todo += [(len(ops) // 2, (lambda par=par: lsum(par))) for par in range(2)]
        todo.sort(key=lambda t: t[0])
        out = []
        k = 0
        for i, op_ in enumerate(ops):
            need = 0
            for n, (dl, _) in enumerate(todo[k:]):
                need = max(need, -(-(n + 1) // max(dl - i + 1, 1)))
            if i < RS0:
                need = sum(1 for dl, _ in todo[k:] if dl <= i)
            for _, f in todo[k:k + need]:
                out.append((0, f))
            k += min(need, len(todo) - k)
            out.append((wts[i], op_))
        assert k == len(todo)
        return out

    toks = []

    def fence(dst, slot, zero_i):
        for i, t in enumerate(toks):
            dst[slot + i + zero_i] = t
        toks.clear()

    def g_softmax(ph, par):
        s = part[par, 0] + part[par, 1]
        mx = jnp.max(jnp.max(s, axis=0, keepdims=True), axis=1, keepdims=True)
        p = jnp.exp2((s - mx) * c2)
        p_scr[ph, par] = p
        if par == 0:
            for r in range(8):
                pb0[ph, pl.ds(r, 8, stride=8), :] = p[0:8]
        toks.append(pltpu.bitcast(p[24:32], U32))

    def o_rows(base):
        z = [lane_sum(accx[base + g]) for g in range(NZ)]
        inv = [1.0 / jnp.sum(z[2 * G + par], axis=0, keepdims=True) for par in range(2)]
        inv = [jnp.broadcast_to(v, (8, 128)) for v in inv]
        out = []
        for c in range(3):
            xs = [z[16 * c + b] for b in range(16)]
            for k in range(4):
                xs = [jnp.where(lane_bit[k], xs[i + 1], xs[i]) for i in range(0, len(xs), 2)]
            iv = inv[0] if c == 0 else (inv[1] if c == 2 else jnp.where(lane_lo, inv[0], inv[1]))
            out.append(jnp.where(diag8, xs[0] * iv, 0.0))
        return out

    def g_olhs(slot0, base):
        for c, z in enumerate(o_rows(base)):
            olhs[slot0 + c] = pack16(z, z)

    def g_query(c):
        xs = [qpart[c * KD + k] for k in range(KD)]
        q = (((xs[0] + xs[1]) + (xs[2] + xs[3])) + xs[4]) * rs_scr[0]
        if c == 1:
            u = pack16(jnp.where(lane_lo, q, 0.0), jnp.where(lane_lo, 0.0, q))
        else:
            u = pack16(q, q)
        pat_scr[c] = u
        if c > 0:
            toks.append(u)

    def g_out(ph):
        for n in range(KD):
            out_scr[n] = out_scr[n] + opart[8 * ph + n]

    def reset_pipeline():
        zero = jnp.zeros((8, 128), F32)
        one = jnp.ones((8, 128), F32)
        for g in range(2 * G):
            accx[NR + g] = zero
        for par in range(2):
            accx[NR + 2 * G + par] = one
        for n in range(KD):
            opart[8 + n] = zero
        for n in range(KD):
            out_scr[n] = zero

    def residual(x, a):
        return (x + a.astype(BF).astype(F32)).astype(BF).astype(F32)

    def matvec(l, wu, r0, nr):
        cols = []
        for c in range(wu.shape[1]):
            w = pltpu.bitcast(wu[r0:r0 + nr, c].reshape(8 * nr, 128), BF)
            cols.append(jnp.dot(l, w, preferred_element_type=F32))
        return cols

    def ffn(x, first):
        xc, rs = center(x)
        y = jnp.broadcast_to(xc, (8, D)).astype(BF)
        if first:
            reset_pipeline()
            wait_all(c_w1)
        g = jnp.concatenate(matvec(y, w1.bitcast(U32), 0, D // 16), axis=1) * rs
        if first:
            wait_all(c_w3)
        u = jnp.concatenate(matvec(y, w3.bitcast(U32), 0, D // 16), axis=1) * rs
        hh = (g * jax.nn.sigmoid(g) * u).astype(BF)
        w2u = w2.bitcast(U32)
        if first:
            a = None
            for cs, o, n in zip(c_w2, w2_off, W2_CHUNKS):
                wait_all(cs)
                t = jnp.concatenate(matvec(hh[:, o:o + n], w2u, o // 16, n // 16), axis=1)[0:1]
                a = t if a is None else a + t
        else:
            a = jnp.concatenate(matvec(hh, w2u, 0, FF // 16), axis=1)[0:1]
        return residual(x, a)

    def barrier(li):
        @pl.when(li > 2)
        def _():
            reset_pipeline()

    def layer(li, x):
        first = li == 0

        xc, rs = center(x)
        y = jnp.broadcast_to(xc, (8, D))
        for k in range(KD):
            yk = y[:, 128 * k:128 * k + 128]
            y_scr[k] = pack16(yk, yk)
        rs_scr[0] = jnp.broadcast_to(rs, (8, 128))
        _run(bind(qproj_ops(0), False))
        for c in range(3):
            g_query(c)
        qa, qb, qc = qk_ops(0)
        _run(bind(qproj_ops(1) + qa + qb + qc, False))
        g_softmax(0, 0)
        g_softmax(0, 1)
        for c in range(3):
            g_query(c)
        _run(bind(qk_ops(1)[0], False))
        toks.clear()
        zero_i = li >> 4

        def emit(pv, items):
            k = 0
            done = 0
            for pos, f in items:
                while k < len(pv) and done + pv[k][0] / 2 <= 4 * pos:
                    done += pv[k][0]
                    pv[k][1]()
                    k += 1
                f()
            for _, g in pv[k:]:
                g()

        def timeline(seq):
            items = []
            n = 0
            ntile = sum(not isinstance(e, tuple) for e in seq)
            for e in seq:
                if isinstance(e, tuple):
                    items.append((0, e[1]))
                else:
                    r = n // 4
                    r1 = (ntile - 1) // 4 - NLAG
                    pos = LEAD + RATE * min(r, r1)
                    if r > r1:
                        pos += (PSA - pos) * (r - r1) / NLAG
                    items.append((pos, (lambda e=e, p=(n < ntile - UNPACED): e(p))))
                    n += 1
            return items

        def arrive(m):
            @pl.when(first)
            def _():
                kv_wait(m)
                widen(m)

        def block(m, ph):
            arrive(m + 2)
            qp = qproj_ops(m + 2)
            _, qb, qc = qk_ops(m + 1)
            qa = qk_ops(m + 2)[0]
            op = oproj_ops(jnp.maximum(m - 1, 0), m + 2, opart, 8 * ph)
            seq = ([("now", lambda: g_out(1 - ph)), ("now", lambda: g_olhs(3 * m, NR * (1 - ph)))]
                   + qc[:CF] + qp[:KD] + [("now", lambda: g_query(0))] + qc[CF:] + qb
                   + [("now", lambda: g_softmax(1 - ph, 0)), ("now", lambda: g_softmax(1 - ph, 1))]
                   + qp[KD:] + [("now", lambda: g_query(1)), ("now", lambda: g_query(2))]
                   + op + qa[:32 - AEND] + [("now", lambda: fence(pat_scr, 4, zero_i))]
                   + qa[32 - AEND:])
            emit(pv_ops(m, ph), timeline(seq))

        def body(t, carry):
            block(2 * t, 0)
            block(2 * t + 1, 1)
            return carry

        if SCOPES:
            with jax.named_scope("loop"):
                lax.fori_loop(0, NP // 2 - 1, body, 0)
        else:
            lax.fori_loop(0, NP // 2 - 1, body, 0)


        def big(kts, i0):
            return [op for i, kt in enumerate(kts)
                    for op in oproj_ops(kt, kt + 3, obig, KD * (i0 + i))]

        m = NP - 2
        kts = list(range(NP - 3, 3 * (NP - 1)))
        barrier(li)
        _, qb, qc = qk_ops(m + 1)
        seq = ([("now", lambda: g_out(1)), ("now", lambda: g_olhs(3 * (NP - 2), NR))]
               + qc + qb
               + [("now", lambda: g_softmax(1, 0)), ("now", lambda: g_softmax(1, 1))]
               + big(kts[:KT14 - 2], 0) + big(kts[-6:-5], KT14 - 2)
               + [("now", lambda: fence(olhs, 3 * NP, zero_i))] + big(kts[KT14 - 2:KT14 - 1], KT14 - 1))
        kts = kts[:KT14 - 2] + kts[-6:-5] + kts[KT14 - 2:-6] + kts[-5:]
        emit(pv_ops(m, 0), timeline(seq))
        barrier(li)
        m = NP - 1
        seq = [("now", lambda: g_olhs(3 * (NP - 1), 0))] + big(kts[KT14:], KT14)
        emit(pv_ops(m, 1), timeline(seq))
        barrier(li)

        rows = [r.astype(BF) for r in o_rows(NR)]
        a1 = matvec(jnp.concatenate(rows, axis=1), wou, 8 * (3 * NP - 3), 24)
        cols = []
        for n in range(KD):
            xs = [out_scr[n]] + [obig[KD * i + n] for i in range(len(kts))]
            while len(xs) > 1:
                xs = [xs[i] + xs[i + 1] for i in range(0, len(xs) - 1, 2)] + xs[len(xs) & ~1:]
            cols.append(jnp.sum(xs[0] + a1[n], axis=0, keepdims=True))
        x = residual(x, jnp.concatenate(cols, axis=1))
        if SCOPES:
            with jax.named_scope("ffn"):
                return lax.cond(first, lambda x: ffn(x, True), lambda x: ffn(x, False), x)
        return lax.cond(first, lambda x: ffn(x, True), lambda x: ffn(x, False), x)

    reset_pipeline()
    wait_all([c_x] + c_wq + c_wo)
    for m in range(2):
        kv_wait(m)
        widen(m)
    x = lax.fori_loop(0, 2, layer, xb[...].astype(F32))
    o_ref[...] = x.astype(o_ref.dtype)


@jax.jit
def pallas_interleave_layers__sliding_block_cached__glu_gated_swiglu__decode_kernel(
    A_x: jax.Array,
    A_k_cache: jax.Array,
    A_v_cache: jax.Array,
    A_wq: jax.Array,
    A_wo: jax.Array,
    B_x: jax.Array,
    B_w1: jax.Array,
    B_w3: jax.Array,
    B_w2: jax.Array,
):
    del B_x
    sk = A_k_cache.shape[2]
    win = min(4096, max(256, sk // 4))
    nb = sk // 128
    nblk = win // 128

    def cache_tiles(c):
        return c.reshape(H, nb, 128, G2, 2, 8).transpose(0, 3, 4, 1, 5, 2)

    def weight_tiles(w):
        r, c = w.shape
        return w.reshape(r // 16, 2, 8, c // 128, 128).transpose(0, 1, 3, 2, 4)

    vreg = lambda n, dt=F32: pltpu.VMEM((-(-n // 4) * 4, 8, 128), dt)
    kern = lambda *refs: _kernel(*refs, blk0=nb - nblk, nblk=nblk, scale=DH ** -0.5)
    out = pl.pallas_call(
        kern,
        out_shape=jax.ShapeDtypeStruct((1, D), BF),
        in_specs=[pl.BlockSpec(memory_space=pl.ANY)] * 8,
        out_specs=pl.BlockSpec(memory_space=pltpu.VMEM),
        scratch_shapes=[
            pltpu.VMEM((1, D), BF),
            pltpu.VMEM((NP, 2, 2, G2, nblk, 16, 128), BF),
            pltpu.VMEM((3 * NP, D, 128), BF),
            pltpu.VMEM((H * DH // 16, KD, 16, 128), BF),
            pltpu.VMEM((D // 16, FF // 128, 16, 128), BF),
            pltpu.VMEM((D // 16, FF // 128, 16, 128), BF),
            pltpu.VMEM((FF // 16, KD, 16, 128), BF),
            vreg(KD, U32),
            vreg(1),
            vreg(3 * KD),
            vreg(8, U32),
            pltpu.VMEM((2, 2, nblk, 128), F32),
            pltpu.VMEM((2, 2, nblk, 128), F32),
            pltpu.VMEM((2 * nblk * 8, 128), F32),
            pltpu.VMEM((2, 64, 128), F32),
            vreg(NR * 2),
            vreg(KD * 2 * NP),
            vreg(3 * NP + 4, U32),
            vreg(16),
            vreg(KD),
            pltpu.VMEM((NP, 3 * nblk, 8, 128), F32),
            pltpu.SemaphoreType.DMA((NP,)),
            pltpu.SemaphoreType.DMA((5 + len(W2_CHUNKS),)),
        ],
        compiler_params=pltpu.CompilerParams(
            vmem_limit_bytes=128 * 1024 * 1024, disable_semaphore_checks=True),
    )(A_x.reshape(1, D), cache_tiles(A_k_cache), cache_tiles(A_v_cache),
      A_wq, weight_tiles(A_wo),
      weight_tiles(B_w1), weight_tiles(B_w3), weight_tiles(B_w2))
    return out.reshape(1, 1, D)
```

```python
import math

import jax
import jax.numpy as jnp
from jax import lax
import jax.experimental.pallas as pl
import jax.experimental.pallas.tpu as pltpu

BF = jnp.bfloat16
F32 = jnp.float32
U32 = jnp.uint32

D = 640
H = 32
DH = 192
G = DH // 8
G2 = DH // 16
NP = H // 2
FF = 1536
EPS = 1e-5
KD = D // 128
NZ = 2 * G + 2
NR = NZ + 2
W2_CHUNKS = (768, 384, 256, 128)

NG = 4
JB = 2
NW = 144
UNPACED = 4
LEAD = 10
RATE = 32
TAILC = 44
AEND = 4
CF = 4
OPM = 3
KT14 = 10
KT15 = 22
SCOPES = 0


def _run(ops):
    for op in ops:
        op()


def _kernel(x_hbm, k_hbm, v_hbm, wq_hbm, wo_hbm, w1_hbm, w3_hbm, w2_hbm,
            o_ref,
            xb, kvb, wq, wo, w1, w3, w2,
            y_scr, rs_scr, qpart, pat_scr, part, p_scr, pb_scr, pb0,
            accx, obig, olhs, opart, out_scr, vx,
            kvsem, wsem, *, blk0, nblk, scale):
    c2 = scale * math.log2(math.e)

    def kv_copies(m):
        return [pltpu.make_async_copy(
            src.at[pl.ds(2 * m, 2), :, t, pl.ds(blk0, nblk)],
            kvb.at[m, i, :, :, :, pl.ds(8 * t, 8), :], kvsem.at[m])
            for i, src in enumerate((k_hbm, v_hbm)) for t in range(2)]

    def kv_wait(m):
        pltpu.make_async_copy(kvb.at[m], kvb.at[m], kvsem.at[m]).wait()

    def wcopies(src, dst, s, r0=0, nr=None):
        nr = src.shape[0] if nr is None else nr
        return [pltpu.make_async_copy(src.at[pl.ds(r0, nr), t],
                                      dst.at[pl.ds(r0, nr), :, pl.ds(8 * t, 8), :],
                                      wsem.at[s]) for t in range(2)]

    c_x = pltpu.make_async_copy(x_hbm, xb, wsem.at[0])
    c_wq = [pltpu.make_async_copy(wq_hbm.at[:, pl.ds(128 * c, 128)], wq.at[c], wsem.at[1])
            for c in range(3 * NP)]
    c_wo = wcopies(wo_hbm, wo, 2)
    c_w1 = wcopies(w1_hbm, w1, 3)
    c_w3 = wcopies(w3_hbm, w3, 4)
    w2_off = [sum(W2_CHUNKS[:i]) for i in range(len(W2_CHUNKS))]
    c_w2 = [wcopies(w2_hbm, w2, 5 + i, o // 16, n // 16)
            for i, (o, n) in enumerate(zip(w2_off, W2_CHUNKS))]

    for c in c_wo + [c_x] + c_wq:
        c.start()
    for m in range(NP):
        for c in kv_copies(m):
            c.start()
    for c in c_w1 + c_w3 + [c for cs in c_w2 for c in cs]:
        c.start()

    def wait_all(cs):
        for c in cs:
            c.wait()

    kvu = kvb.bitcast(U32)
    wqu = wq.bitcast(U32)
    wou = wo.bitcast(U32)

    lane = lax.broadcasted_iota(jnp.int32, (8, 128), 1)
    row = lax.broadcasted_iota(jnp.int32, (8, 128), 0)
    diag8 = (lane & 7) == row
    lane_lo = lane < 64
    lane_bit = [((lane >> (3 + k)) & 1) == 1 for k in range(4)]

    def center(x):
        xc = x - jnp.mean(x, axis=-1, keepdims=True)
        var = jnp.mean(xc * xc, axis=-1, keepdims=True)
        return xc, 1.0 / jnp.sqrt(var + EPS)

    def pack16(z0, z1):
        return pltpu.bitcast(jnp.concatenate([z0, z1], axis=0).astype(BF), U32)

    def tile_dot(l_u32, w_u32, rows, paced):
        w = pltpu.bitcast(w_u32.reshape(64, 128), BF)
        if paced:
            l = pltpu.bitcast(jnp.concatenate([l_u32, l_u32], axis=0), BF)[:24]
            return jnp.dot(l, w, preferred_element_type=F32)[:rows]
        l = pltpu.bitcast(l_u32, BF)[:rows]
        return jnp.dot(l, w, preferred_element_type=F32)

    def qproj_ops(m):
        def op(paced, c, k):
            qpart[c * KD + k] = tile_dot(
                y_scr[k], wqu[3 * m + c, 64 * k:64 * k + 64, :], 8, paced)
        return [(lambda p, c=c, k=k: op(p, c, k)) for c in range(3) for k in range(KD)]

    def oproj_ops(kt, slot, dst, d0):
        def op(paced, n):
            dst[d0 + n] = tile_dot(olhs[slot], wou[pl.ds(kt * 8, 8), n], 8, paced)
        return [(lambda p, n=n: op(p, n)) for n in range(KD)]

    def qk_ops(m):
        def op_a(paced, j):
            r = tile_dot(pat_scr[0], kvu[m, 0, 0, 0:8, j], 8, paced)
            part[0, 0, j:j + 1, :] = r[j % 8:j % 8 + 1, :]

        def op_c(paced, j):
            r = tile_dot(pat_scr[2], kvu[m, 0, 1, 4:12, j], 8, paced)
            part[1, 0, j:j + 1, :] = r[j % 8:j % 8 + 1, :]

        def op_b(paced, j):
            w = jnp.concatenate([kvu[m, 0, 0, 8:12, j], kvu[m, 0, 1, 0:4, j]], axis=0)
            r = tile_dot(pat_scr[1], w, 16, paced)
            part[0, 1, j:j + 1, :] = r[j % 8:j % 8 + 1, :]
            part[1, 1, j:j + 1, :] = r[8 + j % 8:8 + j % 8 + 1, :]

        return [[(lambda p, f=f, j=j: f(p, j)) for j in range(nblk)] for f in (op_a, op_b, op_c)]

    def plain(ops):
        for op in ops:
            op(False)

    steps = [(par, gb, j0) for par in range(2) for gb in range(G2 // NG)
             for j0 in range(0, nblk, JB)]

    def step_blocks(par, gb, j0):
        return [(par, g2, j) for g2 in range(gb * NG, (gb + 1) * NG) for j in range(j0, j0 + JB)]

    order = [b for s in steps for b in step_blocks(*s)]
    wide = {}
    for i, b in enumerate(order):
        if (i + 1) * NW // len(order) > i * NW // len(order):
            wide[b] = len(wide)

    def widen(m):
        for (par, g2, j), e in wide.items():
            v = pltpu.bitcast(kvu[m, 1, par, g2, j], BF).astype(F32)
            kvu[m, 1, par, g2, j] = pltpu.bitcast(v[:8], U32)
            vx[m, e] = v[8:]

    def v_block(m, par, g2, j):
        u = kvu[m, 1, par, g2, j]
        if (par, g2, j) in wide:
            return jnp.concatenate([pltpu.bitcast(u, F32), vx[m, wide[(par, g2, j)]]], axis=0)
        return pltpu.bitcast(u, BF).astype(F32)

    def pv_ops(m, ph):
        acc = {}

        def spread(par, q, r):
            pb_scr[pl.ds(8 * (nblk * par + 8 * q) + r, 8, stride=8), :] = (
                p_scr[ph, par, 8 * q:8 * q + 8, :])

        def lsum(par):
            p = p_scr[ph, par]
            accx[ph, 8 * (2 * G + par):8 * (2 * G + par) + 8, :] = (
                (p[0:8] + p[8:16]) + (p[16:24] + p[24:32]))

        def step(par, gb, j0):
            pbs = {}
            for j in range(j0, j0 + JB):
                i = nblk * par + j
                pb = pb0[ph, 8 * i:8 * i + 8, :] if i < 8 else pb_scr[8 * i:8 * i + 8, :]
                pbs[j] = jnp.concatenate([pb, pb], axis=0)
            for _, g2, j in step_blocks(par, gb, j0):
                tv = v_block(m, par, g2, j) * pbs[j]
                acc[g2] = tv if j == 0 else acc[g2] + tv
                if j == nblk - 1:
                    r0 = DH * par + 16 * g2
                    accx[ph, r0:r0 + 16, :] = acc[g2]

        todo = []
        for par in range(2):
            for q in range(nblk // 8):
                if par or q:
                    dl = par * (len(steps) // 2) + (8 * q) // JB - 1
                    todo += [(dl, (lambda par=par, q=q, r=r: spread(par, q, r))) for r in range(8)]
        todo += [(len(steps) // 2, (lambda par=par: lsum(par))) for par in range(2)]
        todo.sort(key=lambda t: t[0])
        out = []
        k = 0
        for i, s in enumerate(steps):
            need = 0
            for n, (dl, _) in enumerate(todo[k:]):
                need = max(need, -(-(n + 1) // max(dl - i + 1, 1)))
            out += [(0, f) for _, f in todo[k:k + need]]
            k = min(k + need, len(todo))
            out.append((sum(4 if b in wide else 6 for b in step_blocks(*s)),
                        (lambda s=s: step(*s))))
        assert k == len(todo)
        return out

    toks = []

    def fence(dst, slot, zero_i):
        for i, t in enumerate(toks):
            dst[slot + i + zero_i] = t
        toks.clear()

    def g_softmax(ph, par):
        s = part[par, 0] + part[par, 1]
        mx = jnp.max(jnp.max(s, axis=0, keepdims=True), axis=1, keepdims=True)
        p = jnp.exp2((s - mx) * c2)
        p_scr[ph, par] = p
        if par == 0:
            for r in range(8):
                pb0[ph, pl.ds(r, 8, stride=8), :] = p[0:8]
        toks.append(pltpu.bitcast(p[24:32], U32))

    def o_rows(ph):
        z = [jnp.broadcast_to(jnp.sum(accx[ph, 8 * g:8 * g + 8, :], axis=1, keepdims=True), (8, 128))
             for g in range(NZ)]
        inv = [1.0 / jnp.sum(z[2 * G + par], axis=0, keepdims=True) for par in range(2)]
        inv = [jnp.broadcast_to(v, (8, 128)) for v in inv]
        out = []
        for c in range(3):
            xs = z[16 * c:16 * c + 16]
            for k in range(4):
                xs = [jnp.where(lane_bit[k], xs[i + 1], xs[i]) for i in range(0, len(xs), 2)]
            iv = inv[0] if c == 0 else (inv[1] if c == 2 else jnp.where(lane_lo, inv[0], inv[1]))
            out.append(jnp.where(diag8, xs[0] * iv, 0.0))
        return out

    def g_olhs(slot0, ph):
        for c, z in enumerate(o_rows(ph)):
            olhs[slot0 + c] = pack16(z, z)

    def g_query(c):
        xs = [qpart[c * KD + k] for k in range(KD)]
        q = (((xs[0] + xs[1]) + (xs[2] + xs[3])) + xs[4]) * rs_scr[0]
        if c == 1:
            u = pack16(jnp.where(lane_lo, q, 0.0), jnp.where(lane_lo, 0.0, q))
        else:
            u = pack16(q, q)
        pat_scr[c] = u
        if c > 0:
            toks.append(u)

    def g_out(ph):
        for n in range(KD):
            out_scr[n] = out_scr[n] + opart[8 * ph + n]

    def reset_pipeline():
        zero = jnp.zeros((8, 128), F32)
        accx[1, 0:16 * G, :] = jnp.zeros((16 * G, 128), F32)
        accx[1, 16 * G:16 * G + 16, :] = jnp.ones((16, 128), F32)
        for n in range(KD):
            opart[n] = zero
            opart[8 + n] = zero
            out_scr[n] = zero

    def residual(x, a):
        return (x + a.astype(BF).astype(F32)).astype(BF).astype(F32)

    def matvec(l, wu, r0, nr):
        cols = []
        for c in range(wu.shape[1]):
            w = pltpu.bitcast(wu[r0:r0 + nr, c].reshape(8 * nr, 128), BF)
            cols.append(jnp.dot(l, w, preferred_element_type=F32))
        return cols

    def ffn(x, first):
        xc, rs = center(x)
        y = jnp.broadcast_to(xc, (8, D)).astype(BF)
        if first:
            reset_pipeline()
            wait_all(c_w1)
        g = jnp.concatenate(matvec(y, w1.bitcast(U32), 0, D // 16), axis=1) * rs
        if first:
            wait_all(c_w3)
        u = jnp.concatenate(matvec(y, w3.bitcast(U32), 0, D // 16), axis=1) * rs
        hh = (g * jax.nn.sigmoid(g) * u).astype(BF)
        w2u = w2.bitcast(U32)
        if first:
            a = None
            for cs, o, n in zip(c_w2, w2_off, W2_CHUNKS):
                wait_all(cs)
                t = jnp.concatenate(matvec(hh[:, o:o + n], w2u, o // 16, n // 16), axis=1)[0:1]
                a = t if a is None else a + t
        else:
            a = jnp.concatenate(matvec(hh, w2u, 0, FF // 16), axis=1)[0:1]
        return residual(x, a)

    def emit(pv, seq):
        ntile = sum(not isinstance(e, tuple) for e in seq)
        total = sum(w for w, _ in pv) / 4
        k = done = n = 0
        for e in seq:
            if isinstance(e, tuple):
                e[1]()
                continue
            pos = LEAD + RATE * (n // 4) if n // 4 < (ntile - 1) // 4 else total - TAILC
            while k < len(pv) and done + pv[k][0] / 2 <= 4 * pos:
                done += pv[k][0]
                pv[k][1]()
                k += 1
            e(n < ntile - UNPACED)
            n += 1
        for _, g in pv[k:]:
            g()

    def layer(li, x):
        first = li == 0
        zero_i = li >> 4

        def barrier():
            @pl.when(li > 2)
            def _():
                reset_pipeline()

        xc, rs = center(x)
        y = jnp.broadcast_to(xc, (8, D))
        for k in range(KD):
            yk = y[:, 128 * k:128 * k + 128]
            y_scr[k] = pack16(yk, yk)
        rs_scr[0] = jnp.broadcast_to(rs, (8, 128))
        plain(qproj_ops(0))
        for c in range(3):
            g_query(c)
        qa, qb, qc = qk_ops(0)
        plain(qproj_ops(1) + qa + qb + qc)
        g_softmax(0, 0)
        g_softmax(0, 1)
        for c in range(3):
            g_query(c)
        plain(qk_ops(1)[0])
        toks.clear()

        nop = [bin(OPM & 1).count("1"), bin(OPM).count("1")]

        def block(t, ph):
            m = 2 * t + ph

            @pl.when(first)
            def _():
                kv_wait(m + 2)
                widen(m + 2)

            qp = qproj_ops(m + 2)
            _, qb, qc = qk_ops(m + 1)
            qa = qk_ops(m + 2)[0]
            pre, op = [], []
            if OPM >> (1 - ph) & 1:
                pre = [("now", lambda: g_out(1 - ph))]
            if OPM >> ph & 1:
                kt = nop[1] * t + (nop[0] if ph else 0) - (OPM & 1)
                op = oproj_ops(jnp.maximum(kt, 0), kt + 3, opart, 8 * ph)

            def olhs_stage():
                g_olhs(3 * m, 1 - ph)
                if not op:
                    toks.append(olhs[3 * m + 2])

            seq = (pre + [("now", olhs_stage)]
                   + qc[:CF] + qp[:KD] + [("now", lambda: g_query(0))] + qc[CF:] + qb
                   + [("now", lambda: g_softmax(1 - ph, 0)), ("now", lambda: g_softmax(1 - ph, 1))]
                   + qp[KD:] + [("now", lambda: g_query(1)), ("now", lambda: g_query(2))]
                   + op + qa[:32 - AEND] + [("now", lambda: fence(pat_scr, 3, zero_i))]
                   + qa[32 - AEND:])
            emit(pv_ops(m, ph), seq)

        def body(t, carry):
            block(t, 0)
            block(t, 1)
            return carry

        if SCOPES:
            with jax.named_scope("loop"):
                lax.fori_loop(0, NP // 2 - 1, body, 0)
        else:
            lax.fori_loop(0, NP // 2 - 1, body, 0)

        def big(kts, i0):
            return [op for i, kt in enumerate(kts)
                    for op in oproj_ops(kt, kt + 3, obig, KD * (i0 + i))]

        kt0 = nop[1] * (NP // 2 - 1) - (OPM & 1)
        old = list(range(kt0, 3 * (NP - 3)))
        barrier()
        _, qb, qc = qk_ops(NP - 1)
        k14 = old[:KT14 - 4] + list(range(3 * (NP - 3), 3 * (NP - 2)))
        seq = (([("now", lambda: g_out(1))] if OPM & 2 else [])
               + [("now", lambda: g_olhs(3 * (NP - 2), 1))] + qc + qb
               + [("now", lambda: g_softmax(1, 0)), ("now", lambda: g_softmax(1, 1))]
               + big(k14, 0) + [("now", lambda: fence(olhs, 3 * NP, zero_i))]
               + big(old[KT14 - 4:KT14 - 3], KT14 - 1))
        emit(pv_ops(NP - 2, 0), seq)
        old = old[KT14 - 3:]
        barrier()
        k15 = old[:KT15 - 4] + list(range(3 * (NP - 2), 3 * (NP - 1))) + old[KT15 - 4:KT15 - 3]
        emit(pv_ops(NP - 1, 1), [("now", lambda: g_olhs(3 * (NP - 1), 0))] + big(k15, KT14))
        old = old[KT15 - 3:]
        barrier()

        rows = [r.astype(BF) for r in o_rows(1)]
        a = [[out_scr[n]] + [obig[KD * i + n] for i in range(KT14 + len(k15))] for n in range(KD)]
        if old:
            l = jnp.concatenate([pltpu.bitcast(olhs[kt + 3], BF)[:8] for kt in old], axis=1)
            for n, t in enumerate(matvec(l, wou, 8 * old[0], 8 * len(old))):
                a[n].append(t)
        last = matvec(jnp.concatenate(rows, axis=1), wou, 8 * (3 * NP - 3), 24)
        cols = []
        for n in range(KD):
            xs = a[n]
            while len(xs) > 1:
                xs = [xs[i] + xs[i + 1] for i in range(0, len(xs) - 1, 2)] + xs[len(xs) & ~1:]
            cols.append(jnp.sum(xs[0] + last[n], axis=0, keepdims=True))
        x = residual(x, jnp.concatenate(cols, axis=1))
        if SCOPES:
            with jax.named_scope("ffn"):
                return lax.cond(first, lambda x: ffn(x, True), lambda x: ffn(x, False), x)
        return lax.cond(first, lambda x: ffn(x, True), lambda x: ffn(x, False), x)

    reset_pipeline()
    wait_all([c_x] + c_wq + c_wo)
    for m in range(2):
        kv_wait(m)
        widen(m)
    x = lax.fori_loop(0, 2, layer, xb[...].astype(F32))
    o_ref[...] = x.astype(o_ref.dtype)


@jax.jit
def pallas_interleave_layers__sliding_block_cached__glu_gated_swiglu__decode_kernel(
    A_x: jax.Array,
    A_k_cache: jax.Array,
    A_v_cache: jax.Array,
    A_wq: jax.Array,
    A_wo: jax.Array,
    B_x: jax.Array,
    B_w1: jax.Array,
    B_w3: jax.Array,
    B_w2: jax.Array,
):
    del B_x
    sk = A_k_cache.shape[2]
    win = min(4096, max(256, sk // 4))
    nb = sk // 128
    nblk = win // 128

    def cache_tiles(c):
        return c.reshape(H, nb, 128, G2, 2, 8).transpose(0, 3, 4, 1, 5, 2)

    def weight_tiles(w):
        r, c = w.shape
        return w.reshape(r // 16, 2, 8, c // 128, 128).transpose(0, 1, 3, 2, 4)

    vreg = lambda n, dt=F32: pltpu.VMEM((-(-n // 4) * 4, 8, 128), dt)
    kern = lambda *refs: _kernel(*refs, blk0=nb - nblk, nblk=nblk, scale=DH ** -0.5)
    out = pl.pallas_call(
        kern,
        out_shape=jax.ShapeDtypeStruct((1, D), BF),
        in_specs=[pl.BlockSpec(memory_space=pl.ANY)] * 8,
        out_specs=pl.BlockSpec(memory_space=pltpu.VMEM),
        scratch_shapes=[
            pltpu.VMEM((1, D), BF),
            pltpu.VMEM((NP, 2, 2, G2, nblk, 16, 128), BF),
            pltpu.VMEM((3 * NP, D, 128), BF),
            pltpu.VMEM((H * DH // 16, KD, 16, 128), BF),
            pltpu.VMEM((D // 16, FF // 128, 16, 128), BF),
            pltpu.VMEM((D // 16, FF // 128, 16, 128), BF),
            pltpu.VMEM((FF // 16, KD, 16, 128), BF),
            vreg(KD, U32),
            vreg(1),
            vreg(3 * KD),
            vreg(8, U32),
            pltpu.VMEM((2, 2, nblk, 128), F32),
            pltpu.VMEM((2, 2, nblk, 128), F32),
            pltpu.VMEM((2 * nblk * 8, 128), F32),
            pltpu.VMEM((2, 64, 128), F32),
            pltpu.VMEM((2, 8 * NR, 128), F32),
            vreg(KD * (KT14 + KT15)),
            vreg(3 * NP + 4, U32),
            vreg(16),
            vreg(KD),
            pltpu.VMEM((NP, max(-(-NW // 4) * 4, 4), 8, 128), F32),
            pltpu.SemaphoreType.DMA((NP,)),
            pltpu.SemaphoreType.DMA((5 + len(W2_CHUNKS),)),
        ],
        compiler_params=pltpu.CompilerParams(
            vmem_limit_bytes=128 * 1024 * 1024, disable_semaphore_checks=True),
    )(A_x.reshape(1, D), cache_tiles(A_k_cache), cache_tiles(A_v_cache),
      A_wq, weight_tiles(A_wo),
      weight_tiles(B_w1), weight_tiles(B_w3), weight_tiles(B_w2))
    return out.reshape(1, 1, D)
```

```python
import math

import jax
import jax.numpy as jnp
from jax import lax
import jax.experimental.pallas as pl
import jax.experimental.pallas.tpu as pltpu

BF = jnp.bfloat16
F32 = jnp.float32
U32 = jnp.uint32

D = 640
H = 32
DH = 192
G = DH // 8
G2 = DH // 16
NP = H // 2
FF = 1536
EPS = 1e-5
KD = D // 128
NZ = 2 * G + 2
NR = NZ + 2
W2_CHUNKS = (768, 384, 256, 128)

NG = 4
JB = 2
NW = 144
UNPACED = 4
LEAD = 10
RATE = 32
TAILC = 44
AEND = 4
CF = 4
OPM = 3
KT14 = 10
KT15 = 22
KM = 3
FCH = 1
FPRE = 6
FSTEP = 3
SCOPES = 0


def _run(ops):
    for op in ops:
        op()


def _kernel(x_hbm, k_hbm, v_hbm, wq_hbm, wo_hbm, w1_hbm, w3_hbm, w2_hbm,
            o_ref,
            xb, kvb, wq, wo, w1, w3, w2,
            y_scr, rs_scr, qpart, pat_scr, part, p_scr, pb_scr, pb0,
            accx, obig, olhs, opart, out_scr, vx,
            kvsem, wsem, *, blk0, nblk, scale):
    c2 = scale * math.log2(math.e)

    def kv_copies(m):
        return [pltpu.make_async_copy(
            src.at[pl.ds(2 * m, 2), :, t, pl.ds(blk0, nblk)],
            kvb.at[m, i, :, :, :, pl.ds(8 * t, 8), :], kvsem.at[m])
            for i, src in enumerate((k_hbm, v_hbm)) for t in range(2)]

    def kv_wait(m):
        pltpu.make_async_copy(kvb.at[m], kvb.at[m], kvsem.at[m]).wait()

    def wcopies(src, dst, s, r0=0, nr=None):
        nr = src.shape[0] if nr is None else nr
        return [pltpu.make_async_copy(src.at[pl.ds(r0, nr), t],
                                      dst.at[pl.ds(r0, nr), :, pl.ds(8 * t, 8), :],
                                      wsem.at[s]) for t in range(2)]

    c_x = pltpu.make_async_copy(x_hbm, xb, wsem.at[0])
    c_wq = [pltpu.make_async_copy(wq_hbm.at[:, pl.ds(128 * c, 128)], wq.at[c], wsem.at[1])
            for c in range(3 * NP)]
    c_wo = wcopies(wo_hbm, wo, 2)
    c_w1 = wcopies(w1_hbm, w1, 3)
    c_w3 = wcopies(w3_hbm, w3, 4)
    w2_off = [sum(W2_CHUNKS[:i]) for i in range(len(W2_CHUNKS))]
    c_w2 = [wcopies(w2_hbm, w2, 5 + i, o // 16, n // 16)
            for i, (o, n) in enumerate(zip(w2_off, W2_CHUNKS))]

    for c in c_wo + [c_x] + c_wq:
        c.start()
    for m in range(NP):
        for c in kv_copies(m):
            c.start()
    for c in c_w1 + c_w3 + [c for cs in c_w2 for c in cs]:
        c.start()

    def wait_all(cs):
        for c in cs:
            c.wait()

    kvu = kvb.bitcast(U32)
    wqu = wq.bitcast(U32)
    wou = wo.bitcast(U32)

    lane = lax.broadcasted_iota(jnp.int32, (8, 128), 1)
    row = lax.broadcasted_iota(jnp.int32, (8, 128), 0)
    diag8 = (lane & 7) == row
    lane_lo = lane < 64
    lane_bit = [((lane >> (3 + k)) & 1) == 1 for k in range(4)]

    def center(x):
        xc = x - jnp.mean(x, axis=-1, keepdims=True)
        var = jnp.mean(xc * xc, axis=-1, keepdims=True)
        return xc, 1.0 / jnp.sqrt(var + EPS)

    def pack16(z0, z1):
        return pltpu.bitcast(jnp.concatenate([z0, z1], axis=0).astype(BF), U32)

    def tile_dot(l_u32, w_u32, rows, paced):
        w = pltpu.bitcast(w_u32.reshape(64, 128), BF)
        if paced:
            l = pltpu.bitcast(jnp.concatenate([l_u32, l_u32], axis=0), BF)[:24]
            return jnp.dot(l, w, preferred_element_type=F32)[:rows]
        l = pltpu.bitcast(l_u32, BF)[:rows]
        return jnp.dot(l, w, preferred_element_type=F32)

    def qproj_ops(m):
        def op(paced, c, k):
            qpart[c * KD + k] = tile_dot(
                y_scr[k], wqu[3 * m + c, 64 * k:64 * k + 64, :], 8, paced)
        return [(lambda p, c=c, k=k: op(p, c, k)) for c in range(3) for k in range(KD)]

    def oproj_ops(kt, slot, dst, d0):
        def op(paced, n):
            dst[d0 + n] = tile_dot(olhs[slot], wou[pl.ds(kt * 8, 8), n], 8, paced)
        return [(lambda p, n=n: op(p, n)) for n in range(KD)]

    def qk_ops(m):
        def op_a(paced, j):
            r = tile_dot(pat_scr[0], kvu[m, 0, 0, 0:8, j], 8, paced)
            part[0, 0, j:j + 1, :] = r[j % 8:j % 8 + 1, :]

        def op_c(paced, j):
            r = tile_dot(pat_scr[2], kvu[m, 0, 1, 4:12, j], 8, paced)
            part[1, 0, j:j + 1, :] = r[j % 8:j % 8 + 1, :]

        def op_b(paced, j):
            w = jnp.concatenate([kvu[m, 0, 0, 8:12, j], kvu[m, 0, 1, 0:4, j]], axis=0)
            r = tile_dot(pat_scr[1], w, 16, paced)
            part[0, 1, j:j + 1, :] = r[j % 8:j % 8 + 1, :]
            part[1, 1, j:j + 1, :] = r[8 + j % 8:8 + j % 8 + 1, :]

        return [[(lambda p, f=f, j=j: f(p, j)) for j in range(nblk)] for f in (op_a, op_b, op_c)]

    def plain(ops):
        for op in ops:
            op(False)

    steps = [(par, gb, j0) for par in range(2) for gb in range(G2 // NG)
             for j0 in range(0, nblk, JB)]

    def step_blocks(par, gb, j0):
        return [(par, g2, j) for g2 in range(gb * NG, (gb + 1) * NG) for j in range(j0, j0 + JB)]

    order = [b for s in steps for b in step_blocks(*s)]
    wide = {}
    for i, b in enumerate(order):
        if (i + 1) * NW // len(order) > i * NW // len(order):
            wide[b] = len(wide)

    def widen(m):
        for (par, g2, j), e in wide.items():
            v = pltpu.bitcast(kvu[m, 1, par, g2, j], BF).astype(F32)
            kvu[m, 1, par, g2, j] = pltpu.bitcast(v[:8], U32)
            vx[m, e] = v[8:]

    def v_block(m, par, g2, j):
        u = kvu[m, 1, par, g2, j]
        if (par, g2, j) in wide:
            return jnp.concatenate([pltpu.bitcast(u, F32), vx[m, wide[(par, g2, j)]]], axis=0)
        return pltpu.bitcast(u, BF).astype(F32)

    def pv_ops(m, ph):
        acc = {}

        def spread(par, q, r):
            pb_scr[pl.ds(8 * (nblk * par + 8 * q) + r, 8, stride=8), :] = (
                p_scr[ph, par, 8 * q:8 * q + 8, :])

        def lsum(par):
            p = p_scr[ph, par]
            accx[ph, 8 * (2 * G + par):8 * (2 * G + par) + 8, :] = (
                (p[0:8] + p[8:16]) + (p[16:24] + p[24:32]))

        def step(par, gb, j0):
            pbs = {}
            for j in range(j0, j0 + JB):
                i = nblk * par + j
                pb = pb0[ph, 8 * i:8 * i + 8, :] if i < 8 else pb_scr[8 * i:8 * i + 8, :]
                pbs[j] = jnp.concatenate([pb, pb], axis=0)
            for _, g2, j in step_blocks(par, gb, j0):
                tv = v_block(m, par, g2, j) * pbs[j]
                acc[g2] = tv if j == 0 else acc[g2] + tv
                if j == nblk - 1:
                    r0 = DH * par + 16 * g2
                    accx[ph, r0:r0 + 16, :] = acc[g2]

        todo = []
        for par in range(2):
            for q in range(nblk // 8):
                if par or q:
                    dl = par * (len(steps) // 2) + (8 * q) // JB - 1
                    todo += [(dl, (lambda par=par, q=q, r=r: spread(par, q, r))) for r in range(8)]
        todo += [(len(steps) // 2, (lambda par=par: lsum(par))) for par in range(2)]
        todo.sort(key=lambda t: t[0])
        out = []
        k = 0
        for i, s in enumerate(steps):
            need = 0
            for n, (dl, _) in enumerate(todo[k:]):
                need = max(need, -(-(n + 1) // max(dl - i + 1, 1)))
            out += [(0, f) for _, f in todo[k:k + need]]
            k = min(k + need, len(todo))
            out.append((sum(4 if b in wide else 6 for b in step_blocks(*s)),
                        (lambda s=s: step(*s))))
        assert k == len(todo)
        return out

    toks = []

    def fence(dst, slot, zero_i):
        for i, t in enumerate(toks):
            dst[slot + i + zero_i] = t
        toks.clear()

    def g_softmax(ph, par):
        s = part[par, 0] + part[par, 1]
        mx = jnp.max(jnp.max(s, axis=0, keepdims=True), axis=1, keepdims=True)
        p = jnp.exp2((s - mx) * c2)
        p_scr[ph, par] = p
        if par == 0:
            for r in range(8):
                pb0[ph, pl.ds(r, 8, stride=8), :] = p[0:8]
        toks.append(pltpu.bitcast(p[24:32], U32))

    def o_rows(ph):
        z = [jnp.broadcast_to(jnp.sum(accx[ph, 8 * g:8 * g + 8, :], axis=1, keepdims=True), (8, 128))
             for g in range(NZ)]
        inv = [1.0 / jnp.sum(z[2 * G + par], axis=0, keepdims=True) for par in range(2)]
        inv = [jnp.broadcast_to(v, (8, 128)) for v in inv]
        out = []
        for c in range(3):
            xs = z[16 * c:16 * c + 16]
            for k in range(4):
                xs = [jnp.where(lane_bit[k], xs[i + 1], xs[i]) for i in range(0, len(xs), 2)]
            iv = inv[0] if c == 0 else (inv[1] if c == 2 else jnp.where(lane_lo, inv[0], inv[1]))
            out.append(jnp.where(diag8, xs[0] * iv, 0.0))
        return out

    def g_olhs(slot0, ph):
        for c, z in enumerate(o_rows(ph)):
            olhs[slot0 + c] = pack16(z, z)

    def g_query(c):
        xs = [qpart[c * KD + k] for k in range(KD)]
        q = (((xs[0] + xs[1]) + (xs[2] + xs[3])) + xs[4]) * rs_scr[0]
        if c == 1:
            u = pack16(jnp.where(lane_lo, q, 0.0), jnp.where(lane_lo, 0.0, q))
        else:
            u = pack16(q, q)
        pat_scr[c] = u
        if c > 0:
            toks.append(u)

    def g_out(ph):
        for n in range(KD):
            out_scr[n] = out_scr[n] + opart[8 * ph + n]

    def reset_pipeline():
        zero = jnp.zeros((8, 128), F32)
        accx[1, 0:16 * G, :] = jnp.zeros((16 * G, 128), F32)
        accx[1, 16 * G:16 * G + 16, :] = jnp.ones((16, 128), F32)
        for n in range(KD):
            opart[n] = zero
            opart[8 + n] = zero
            out_scr[n] = zero

    def residual(x, a):
        return (x + a.astype(BF).astype(F32)).astype(BF).astype(F32)

    def matvec(l, wu, r0, nr):
        cols = []
        for c in range(wu.shape[1]):
            w = pltpu.bitcast(wu[r0:r0 + nr, c].reshape(8 * nr, 128), BF)
            cols.append(jnp.dot(l, w, preferred_element_type=F32))
        return cols

    def ffn(x, first):
        xc, rs = center(x)
        y = jnp.broadcast_to(xc, (8, D)).astype(BF)
        if first:
            reset_pipeline()
            wait_all(c_w1)
        g = jnp.concatenate(matvec(y, w1.bitcast(U32), 0, D // 16), axis=1) * rs
        if first:
            wait_all(c_w3)
        u = jnp.concatenate(matvec(y, w3.bitcast(U32), 0, D // 16), axis=1) * rs
        hh = (g * jax.nn.sigmoid(g) * u).astype(BF)
        w2u = w2.bitcast(U32)
        if first:
            a = None
            for cs, o, n in zip(c_w2, w2_off, W2_CHUNKS):
                wait_all(cs)
                t = jnp.concatenate(matvec(hh[:, o:o + n], w2u, o // 16, n // 16), axis=1)[0:1]
                a = t if a is None else a + t
        else:
            a = jnp.concatenate(matvec(hh, w2u, 0, FF // 16), axis=1)[0:1]
        return residual(x, a)

    def ffn2(x):
        w1u, w3u, w2u = w1.bitcast(U32), w3.bitcast(U32), w2.bitcast(U32)
        mu = jnp.mean(x, axis=-1, keepdims=True)
        xc = x - mu
        rs = 1.0 / jnp.sqrt(jnp.mean(xc * xc, axis=-1, keepdims=True) + EPS)
        xb8 = jnp.broadcast_to(x, (8, D))
        rowk = lax.broadcasted_iota(jnp.int32, (8, 128 * KM), 0)
        y = jnp.where(rowk == 0, xb8[:, :128 * KM], jnp.where(rowk == 1, 1.0, 0.0)).astype(BF)
        coef = jnp.where(row == 0, 1.0, -mu)
        dl = lane - row
        yb = [jnp.broadcast_to(
            jnp.sum(jnp.where(dl == 8 * b, xb8[:, 128 * k:128 * k + 128], 0.0), axis=1, keepdims=True),
            (8, 128)) - mu for k in range(KM, KD) for b in range(16)]
        yb = jnp.concatenate(yb, axis=0)
        NC = FF // 128
        mx = {}

        def mxu_col(c):
            mx[c] = [jnp.dot(y, pltpu.bitcast(wu[0:8 * KM, c].reshape(64 * KM, 128), BF),
                             preferred_element_type=F32) * coef for wu in (w1u, w3u)]

        def h_col(c):
            gu = []
            for i, wu in enumerate((w1u, w3u)):
                acc = None
                for r in range(8 * KM, 8 * KD):
                    v = pltpu.bitcast(wu[r, c], BF).astype(F32)
                    o = 16 * (r - 8 * KM)
                    if FCH == 1:
                        for t in range(2):
                            tv = v[8 * t:8 * t + 8] * yb[o + 8 * t:o + 8 * t + 8]
                            acc = tv if acc is None else acc + tv
                    else:
                        tv = v * yb[o:o + 16]
                        acc = tv if acc is None else acc + tv
                if FCH != 1:
                    acc = acc[:8] + acc[8:]
                gu.append(jnp.sum(acc + mx[c][i], axis=0, keepdims=True) * rs)
            g, u = gu
            return jnp.broadcast_to(g * jax.nn.sigmoid(g) * u, (8, 128)).astype(BF)

        out = [None] * KD
        nxt = 0
        for c in range(NC):
            while nxt < NC and nxt < FPRE + c * FSTEP / 4:
                mxu_col(nxt)
                nxt += 1
            h = h_col(c)
            for n in range(KD):
                t = jnp.dot(h, pltpu.bitcast(w2u[8 * c:8 * c + 8, n].reshape(64, 128), BF),
                            preferred_element_type=F32)[0:1]
                out[n] = t if out[n] is None else out[n] + t
        return residual(x, jnp.concatenate(out, axis=1))

    def emit(pv, seq):
        ntile = sum(not isinstance(e, tuple) for e in seq)
        total = sum(w for w, _ in pv) / 4
        k = done = n = 0
        for e in seq:
            if isinstance(e, tuple):
                e[1]()
                continue
            pos = LEAD + RATE * (n // 4) if n // 4 < (ntile - 1) // 4 else total - TAILC
            while k < len(pv) and done + pv[k][0] / 2 <= 4 * pos:
                done += pv[k][0]
                pv[k][1]()
                k += 1
            e(n < ntile - UNPACED)
            n += 1
        for _, g in pv[k:]:
            g()

    def layer(li, x):
        first = li == 0
        zero_i = li >> 4

        def barrier():
            @pl.when(li > 2)
            def _():
                reset_pipeline()

        xc, rs = center(x)
        y = jnp.broadcast_to(xc, (8, D))
        for k in range(KD):
            yk = y[:, 128 * k:128 * k + 128]
            y_scr[k] = pack16(yk, yk)
        rs_scr[0] = jnp.broadcast_to(rs, (8, 128))
        plain(qproj_ops(0))
        for c in range(3):
            g_query(c)
        qa, qb, qc = qk_ops(0)
        plain(qproj_ops(1) + qa + qb + qc)
        g_softmax(0, 0)
        g_softmax(0, 1)
        for c in range(3):
            g_query(c)
        plain(qk_ops(1)[0])
        toks.clear()

        nop = [bin(OPM & 1).count("1"), bin(OPM).count("1")]

        def block(t, ph):
            m = 2 * t + ph

            @pl.when(first)
            def _():
                kv_wait(m + 2)
                widen(m + 2)

            qp = qproj_ops(m + 2)
            _, qb, qc = qk_ops(m + 1)
            qa = qk_ops(m + 2)[0]
            pre, op = [], []
            if OPM >> (1 - ph) & 1:
                pre = [("now", lambda: g_out(1 - ph))]
            if OPM >> ph & 1:
                kt = nop[1] * t + (nop[0] if ph else 0) - (OPM & 1)
                op = oproj_ops(jnp.maximum(kt, 0), kt + 3, opart, 8 * ph)

            def olhs_stage():
                g_olhs(3 * m, 1 - ph)
                if not op:
                    toks.append(olhs[3 * m + 2])

            seq = (pre + [("now", olhs_stage)]
                   + qc[:CF] + qp[:KD] + [("now", lambda: g_query(0))] + qc[CF:] + qb
                   + [("now", lambda: g_softmax(1 - ph, 0)), ("now", lambda: g_softmax(1 - ph, 1))]
                   + qp[KD:] + [("now", lambda: g_query(1)), ("now", lambda: g_query(2))]
                   + op + qa[:32 - AEND] + [("now", lambda: fence(pat_scr, 3, zero_i))]
                   + qa[32 - AEND:])
            emit(pv_ops(m, ph), seq)

        def body(t, carry):
            block(t, 0)
            block(t, 1)
            return carry

        if SCOPES:
            with jax.named_scope("loop"):
                lax.fori_loop(0, NP // 2 - 1, body, 0)
        else:
            lax.fori_loop(0, NP // 2 - 1, body, 0)

        def big(kts, i0):
            return [op for i, kt in enumerate(kts)
                    for op in oproj_ops(kt, kt + 3, obig, KD * (i0 + i))]

        kt0 = nop[1] * (NP // 2 - 1) - (OPM & 1)
        old = list(range(kt0, 3 * (NP - 3)))
        barrier()
        _, qb, qc = qk_ops(NP - 1)
        k14 = old[:KT14 - 4] + list(range(3 * (NP - 3), 3 * (NP - 2)))
        seq = (([("now", lambda: g_out(1))] if OPM & 2 else [])
               + [("now", lambda: g_olhs(3 * (NP - 2), 1))] + qc + qb
               + [("now", lambda: g_softmax(1, 0)), ("now", lambda: g_softmax(1, 1))]
               + big(k14, 0) + [("now", lambda: fence(olhs, 3 * NP, zero_i))]
               + big(old[KT14 - 4:KT14 - 3], KT14 - 1))
        emit(pv_ops(NP - 2, 0), seq)
        old = old[KT14 - 3:]
        barrier()
        k15 = old[:KT15 - 4] + list(range(3 * (NP - 2), 3 * (NP - 1))) + old[KT15 - 4:KT15 - 3]
        emit(pv_ops(NP - 1, 1), [("now", lambda: g_olhs(3 * (NP - 1), 0))] + big(k15, KT14))
        old = old[KT15 - 3:]
        barrier()

        rows = [r.astype(BF) for r in o_rows(1)]
        a = [[out_scr[n]] + [obig[KD * i + n] for i in range(KT14 + len(k15))] for n in range(KD)]
        if old:
            l = jnp.concatenate([pltpu.bitcast(olhs[kt + 3], BF)[:8] for kt in old], axis=1)
            for n, t in enumerate(matvec(l, wou, 8 * old[0], 8 * len(old))):
                a[n].append(t)
        last = matvec(jnp.concatenate(rows, axis=1), wou, 8 * (3 * NP - 3), 24)
        cols = []
        for n in range(KD):
            xs = a[n]
            while len(xs) > 1:
                xs = [xs[i] + xs[i + 1] for i in range(0, len(xs) - 1, 2)] + xs[len(xs) & ~1:]
            cols.append(jnp.sum(xs[0] + last[n], axis=0, keepdims=True))
        x = residual(x, jnp.concatenate(cols, axis=1))
        if SCOPES:
            with jax.named_scope("ffn"):
                return lax.cond(first, lambda x: ffn(x, True), (ffn2 if KM < KD else lambda x: ffn(x, False)), x)
        return lax.cond(first, lambda x: ffn(x, True), (ffn2 if KM < KD else lambda x: ffn(x, False)), x)

    reset_pipeline()
    wait_all([c_x] + c_wq + c_wo)
    for m in range(2):
        kv_wait(m)
        widen(m)
    x = lax.fori_loop(0, 2, layer, xb[...].astype(F32))
    o_ref[...] = x.astype(o_ref.dtype)


@jax.jit
def pallas_interleave_layers__sliding_block_cached__glu_gated_swiglu__decode_kernel(
    A_x: jax.Array,
    A_k_cache: jax.Array,
    A_v_cache: jax.Array,
    A_wq: jax.Array,
    A_wo: jax.Array,
    B_x: jax.Array,
    B_w1: jax.Array,
    B_w3: jax.Array,
    B_w2: jax.Array,
):
    del B_x
    sk = A_k_cache.shape[2]
    win = min(4096, max(256, sk // 4))
    nb = sk // 128
    nblk = win // 128

    def cache_tiles(c):
        return c.reshape(H, nb, 128, G2, 2, 8).transpose(0, 3, 4, 1, 5, 2)

    def weight_tiles(w):
        r, c = w.shape
        return w.reshape(r // 16, 2, 8, c // 128, 128).transpose(0, 1, 3, 2, 4)

    vreg = lambda n, dt=F32: pltpu.VMEM((-(-n // 4) * 4, 8, 128), dt)
    kern = lambda *refs: _kernel(*refs, blk0=nb - nblk, nblk=nblk, scale=DH ** -0.5)
    out = pl.pallas_call(
        kern,
        out_shape=jax.ShapeDtypeStruct((1, D), BF),
        in_specs=[pl.BlockSpec(memory_space=pl.ANY)] * 8,
        out_specs=pl.BlockSpec(memory_space=pltpu.VMEM),
        scratch_shapes=[
            pltpu.VMEM((1, D), BF),
            pltpu.VMEM((NP, 2, 2, G2, nblk, 16, 128), BF),
            pltpu.VMEM((3 * NP, D, 128), BF),
            pltpu.VMEM((H * DH // 16, KD, 16, 128), BF),
            pltpu.VMEM((D // 16, FF // 128, 16, 128), BF),
            pltpu.VMEM((D // 16, FF // 128, 16, 128), BF),
            pltpu.VMEM((FF // 16, KD, 16, 128), BF),
            vreg(KD, U32),
            vreg(1),
            vreg(3 * KD),
            vreg(8, U32),
            pltpu.VMEM((2, 2, nblk, 128), F32),
            pltpu.VMEM((2, 2, nblk, 128), F32),
            pltpu.VMEM((2 * nblk * 8, 128), F32),
            pltpu.VMEM((2, 64, 128), F32),
            pltpu.VMEM((2, 8 * NR, 128), F32),
            vreg(KD * (KT14 + KT15)),
            vreg(3 * NP + 4, U32),
            vreg(16),
            vreg(KD),
            pltpu.VMEM((NP, max(-(-NW // 4) * 4, 4), 8, 128), F32),
            pltpu.SemaphoreType.DMA((NP,)),
            pltpu.SemaphoreType.DMA((5 + len(W2_CHUNKS),)),
        ],
        compiler_params=pltpu.CompilerParams(
            vmem_limit_bytes=128 * 1024 * 1024, disable_semaphore_checks=True),
    )(A_x.reshape(1, D), cache_tiles(A_k_cache), cache_tiles(A_v_cache),
      A_wq, weight_tiles(A_wo),
      weight_tiles(B_w1), weight_tiles(B_w3), weight_tiles(B_w2))
    return out.reshape(1, 1, D)
```

```python
import math

import jax
import jax.numpy as jnp
from jax import lax
import jax.experimental.pallas as pl
import jax.experimental.pallas.tpu as pltpu

BF = jnp.bfloat16
F32 = jnp.float32
U32 = jnp.uint32

D = 640
H = 32
DH = 192
G = DH // 8
G2 = DH // 16
NP = H // 2
FF = 1536
EPS = 1e-5
KD = D // 128
NZ = 2 * G + 2
NR = NZ + 2
W2_CHUNKS = (768, 384, 256, 128)

NG = 4
JB = 2
NW = 136
UNPACED = 4
LEAD = 10
RATE = 32
TAILC = 44
AEND = 4
CF = 4
OPM = 3
KT14 = 10
KT15 = 22
KM = 3
FCH = 1
FPRE = 6
FSTEP = 3
PVA = 32
PVB = 6
PGRP = 2
PF0 = 0
PFS = 4
PCH = 1
PFB = 1.5
PQH = 4
PTK = 4
SCOPES = 0


def _run(ops):
    for op in ops:
        op()


def _kernel(x_hbm, k_hbm, v_hbm, wq_hbm, wo_hbm, w1_hbm, w3_hbm, w2_hbm,
            o_ref,
            xb, kvb, wq, wo, w1, w3, w2,
            y_scr, rs_scr, qpart, pat_scr, part_a, part, p_scr, pb_scr, pb0,
            accx, obig, olhs, opart, out_scr, vx,
            kvsem, wsem, *, blk0, nblk, scale):
    c2 = scale * math.log2(math.e)

    def kv_copies(m):
        return [pltpu.make_async_copy(
            src.at[pl.ds(2 * m, 2), :, t, pl.ds(blk0, nblk)],
            kvb.at[m, i, :, :, :, pl.ds(8 * t, 8), :], kvsem.at[m])
            for i, src in enumerate((k_hbm, v_hbm)) for t in range(2)]

    def kv_wait(m):
        pltpu.make_async_copy(kvb.at[m], kvb.at[m], kvsem.at[m]).wait()

    def wcopies(src, dst, s, r0=0, nr=None):
        nr = src.shape[0] if nr is None else nr
        return [pltpu.make_async_copy(src.at[pl.ds(r0, nr), t],
                                      dst.at[pl.ds(r0, nr), :, pl.ds(8 * t, 8), :],
                                      wsem.at[s]) for t in range(2)]

    c_x = pltpu.make_async_copy(x_hbm, xb, wsem.at[0])
    c_wq = [pltpu.make_async_copy(wq_hbm.at[:, pl.ds(128 * c, 128)], wq.at[c], wsem.at[1])
            for c in range(3 * NP)]
    c_wo = wcopies(wo_hbm, wo, 2)
    c_w1 = wcopies(w1_hbm, w1, 3)
    c_w3 = wcopies(w3_hbm, w3, 4)
    w2_off = [sum(W2_CHUNKS[:i]) for i in range(len(W2_CHUNKS))]
    c_w2 = [wcopies(w2_hbm, w2, 5 + i, o // 16, n // 16)
            for i, (o, n) in enumerate(zip(w2_off, W2_CHUNKS))]

    for c in c_wo + [c_x] + c_wq:
        c.start()
    for m in range(NP):
        for c in kv_copies(m):
            c.start()
    for c in c_w1 + c_w3 + [c for cs in c_w2 for c in cs]:
        c.start()

    def wait_all(cs):
        for c in cs:
            c.wait()

    kvu = kvb.bitcast(U32)
    wqu = wq.bitcast(U32)
    wou = wo.bitcast(U32)

    lane = lax.broadcasted_iota(jnp.int32, (8, 128), 1)
    row = lax.broadcasted_iota(jnp.int32, (8, 128), 0)
    diag8 = (lane & 7) == row
    lane_lo = lane < 64
    lane_bit = [((lane >> (3 + k)) & 1) == 1 for k in range(4)]

    def center(x):
        xc = x - jnp.mean(x, axis=-1, keepdims=True)
        var = jnp.mean(xc * xc, axis=-1, keepdims=True)
        return xc, 1.0 / jnp.sqrt(var + EPS)

    def pack16(z0, z1):
        return pltpu.bitcast(jnp.concatenate([z0, z1], axis=0).astype(BF), U32)

    def tile_dot(l_u32, w_u32, rows, paced):
        w = pltpu.bitcast(w_u32.reshape(64, 128), BF)
        if paced:
            l = pltpu.bitcast(jnp.concatenate([l_u32, l_u32], axis=0), BF)[:24]
            return jnp.dot(l, w, preferred_element_type=F32)[:rows]
        l = pltpu.bitcast(l_u32, BF)[:rows]
        return jnp.dot(l, w, preferred_element_type=F32)

    def qproj_ops(m):
        def op(paced, c, k):
            qpart[c * KD + k] = tile_dot(
                y_scr[k], wqu[3 * m + c, 64 * k:64 * k + 64, :], 8, paced)
        return [(lambda p, c=c, k=k: op(p, c, k)) for c in range(3) for k in range(KD)]

    def oproj_ops(kt, slot, dst, d0):
        def op(paced, n):
            dst[d0 + n] = tile_dot(olhs[slot], wou[pl.ds(kt * 8, 8), n], 8, paced)
        return [(lambda p, n=n: op(p, n)) for n in range(KD)]

    nq = nblk // 8

    def put_row(par, t, j, r):
        if par == 0 and t == 0:
            part_a[j // 8, j % 8:j % 8 + 1, :] = r
        else:
            part[(2 * par + t) * nq + j // 8, j % 8:j % 8 + 1, :] = r

    def qk_ops(m):
        def op_a(paced, j):
            r = tile_dot(pat_scr[0], kvu[m, 0, 0, 0:8, j], 8, paced)
            put_row(0, 0, j, r[j % 8:j % 8 + 1, :])

        def op_c(paced, j):
            r = tile_dot(pat_scr[2], kvu[m, 0, 1, 4:12, j], 8, paced)
            put_row(1, 0, j, r[j % 8:j % 8 + 1, :])

        def op_b(paced, j):
            w = jnp.concatenate([kvu[m, 0, 0, 8:12, j], kvu[m, 0, 1, 0:4, j]], axis=0)
            r = tile_dot(pat_scr[1], w, 16, paced)
            put_row(0, 1, j, r[j % 8:j % 8 + 1, :])
            put_row(1, 1, j, r[8 + j % 8:8 + j % 8 + 1, :])

        return [[(lambda p, f=f, j=j: f(p, j)) for j in range(nblk)] for f in (op_a, op_b, op_c)]

    def plain(ops):
        for op in ops:
            op(False)

    steps = [(par, gb, j0) for par in range(2) for gb in range(G2 // NG)
             for j0 in range(0, nblk, JB)]

    def step_blocks(par, gb, j0):
        return [(par, g2, j) for g2 in range(gb * NG, (gb + 1) * NG) for j in range(j0, j0 + JB)]

    order = [b for s in steps for b in step_blocks(*s)]
    wide = {}
    for i, b in enumerate(order):
        if (i + 1) * NW // len(order) > i * NW // len(order):
            wide[b] = len(wide)

    def widen(m):
        for (par, g2, j), e in wide.items():
            v = pltpu.bitcast(kvu[m, 1, par, g2, j], BF).astype(F32)
            kvu[m, 1, par, g2, j] = pltpu.bitcast(v[:8], U32)
            vx[m, e] = v[8:]

    def v_block(m, par, g2, j):
        u = kvu[m, 1, par, g2, j]
        if (par, g2, j) in wide:
            return jnp.concatenate([pltpu.bitcast(u, F32), vx[m, wide[(par, g2, j)]]], axis=0)
        return pltpu.bitcast(u, BF).astype(F32)

    def pv_ops(m, ph):
        acc = {}

        def spread(par, q, r):
            pb_scr[pl.ds(8 * (nblk * par + 8 * q) + r, 8, stride=8), :] = (
                p_scr[ph, par, 8 * q:8 * q + 8, :])

        def lsum(par):
            p = p_scr[ph, par]
            accx[ph, 8 * (2 * G + par):8 * (2 * G + par) + 8, :] = (
                (p[0:8] + p[8:16]) + (p[16:24] + p[24:32]))

        def step(par, gb, j0):
            pbs = {}
            for j in range(j0, j0 + JB):
                i = nblk * par + j
                pb = pb0[ph, 8 * i:8 * i + 8, :] if i < 8 else pb_scr[8 * i:8 * i + 8, :]
                pbs[j] = jnp.concatenate([pb, pb], axis=0)
            for _, g2, j in step_blocks(par, gb, j0):
                tv = v_block(m, par, g2, j) * pbs[j]
                acc[g2] = tv if j == 0 else acc[g2] + tv
                if j == nblk - 1:
                    r0 = DH * par + 16 * g2
                    accx[ph, r0:r0 + 16, :] = acc[g2]

        todo = []
        for par in range(2):
            for q in range(nblk // 8):
                if par or q:
                    dl = par * (len(steps) // 2) + (8 * q) // JB - 1
                    todo += [(dl, (lambda par=par, q=q, r=r: spread(par, q, r))) for r in range(8)]
        todo += [(len(steps) // 2, (lambda par=par: lsum(par))) for par in range(2)]
        todo.sort(key=lambda t: t[0])
        out = []
        k = 0
        for i, s in enumerate(steps):
            need = 0
            for n, (dl, _) in enumerate(todo[k:]):
                need = max(need, -(-(n + 1) // max(dl - i + 1, 1)))
            out += [(0, f) for _, f in todo[k:k + need]]
            k = min(k + need, len(todo))
            out.append((sum(4 if b in wide else 6 for b in step_blocks(*s)),
                        (lambda s=s: step(*s))))
        assert k == len(todo)
        return out

    toks = []

    def fence(dst, slot, zero_i):
        for i, t in enumerate(toks):
            dst[slot + i + zero_i] = t
        toks.clear()

    def g_softmax(ph, par):
        a = 2 * par * nq
        s0 = part[a:a + nq] if par else part_a[0:nq]
        s = (s0 + part[a + nq:a + 2 * nq]).reshape(nblk, 128)
        mx = jnp.max(jnp.max(s, axis=0, keepdims=True), axis=1, keepdims=True)
        cs = rs_scr[0]
        p = jnp.exp2((s - mx) * jnp.concatenate([cs] * (nblk // 8), axis=0))
        p_scr[ph, par] = p
        if par == 0:
            for r in range(8):
                pb0[ph, pl.ds(r, 8, stride=8), :] = p[0:8]
        toks.append(pltpu.bitcast(p[24:32], U32))

    def o_rows(ph):
        z = [jnp.broadcast_to(jnp.sum(accx[ph, 8 * g:8 * g + 8, :], axis=1, keepdims=True), (8, 128))
             for g in range(NZ)]
        inv = [1.0 / jnp.sum(z[2 * G + par], axis=0, keepdims=True) for par in range(2)]
        inv = [jnp.broadcast_to(v, (8, 128)) for v in inv]
        out = []
        for c in range(3):
            xs = z[16 * c:16 * c + 16]
            for k in range(4):
                xs = [jnp.where(lane_bit[k], xs[i + 1], xs[i]) for i in range(0, len(xs), 2)]
            iv = inv[0] if c == 0 else (inv[1] if c == 2 else jnp.where(lane_lo, inv[0], inv[1]))
            out.append(jnp.where(diag8, xs[0] * iv, 0.0))
        return out

    def g_olhs(slot0, ph):
        for c, z in enumerate(o_rows(ph)):
            olhs[slot0 + c] = pack16(z, z)

    def set_pat(c, q):
        if c == 1:
            u = pack16(jnp.where(lane_lo, q, 0.0), jnp.where(lane_lo, 0.0, q))
        else:
            u = pack16(q, q)
        pat_scr[c] = u
        if c > 0:
            toks.append(u)

    def g_query(c):
        xs = [qpart[c * KD + k] for k in range(KD)]
        set_pat(c, ((xs[0] + xs[1]) + (xs[2] + xs[3])) + xs[4])

    def g_out(ph):
        for n in range(KD):
            out_scr[n] = out_scr[n] + opart[8 * ph + n]

    def reset_pipeline():
        zero = jnp.zeros((8, 128), F32)
        accx[1, 0:16 * G, :] = jnp.zeros((16 * G, 128), F32)
        accx[1, 16 * G:16 * G + 16, :] = jnp.ones((16, 128), F32)
        for n in range(KD):
            opart[n] = zero
            opart[8 + n] = zero
            out_scr[n] = zero

    def residual(x, a):
        return (x + a.astype(BF).astype(F32)).astype(BF).astype(F32)

    def matvec(l, wu, r0, nr):
        cols = []
        for c in range(wu.shape[1]):
            w = pltpu.bitcast(wu[r0:r0 + nr, c].reshape(8 * nr, 128), BF)
            cols.append(jnp.dot(l, w, preferred_element_type=F32))
        return cols

    def ffn(x, first):
        xc, rs = center(x)
        y = jnp.broadcast_to(xc, (8, D)).astype(BF)
        if first:
            reset_pipeline()
            wait_all(c_w1)
        g = jnp.concatenate(matvec(y, w1.bitcast(U32), 0, D // 16), axis=1) * rs
        if first:
            wait_all(c_w3)
        u = jnp.concatenate(matvec(y, w3.bitcast(U32), 0, D // 16), axis=1) * rs
        hh = (g * jax.nn.sigmoid(g) * u).astype(BF)
        w2u = w2.bitcast(U32)
        if first:
            a = None
            for cs, o, n in zip(c_w2, w2_off, W2_CHUNKS):
                wait_all(cs)
                t = jnp.concatenate(matvec(hh[:, o:o + n], w2u, o // 16, n // 16), axis=1)[0:1]
                a = t if a is None else a + t
        else:
            a = jnp.concatenate(matvec(hh, w2u, 0, FF // 16), axis=1)[0:1]
        return residual(x, a)

    def ffn2(x):
        w1u, w3u, w2u = w1.bitcast(U32), w3.bitcast(U32), w2.bitcast(U32)
        mu = jnp.mean(x, axis=-1, keepdims=True)
        xc = x - mu
        rs = 1.0 / jnp.sqrt(jnp.mean(xc * xc, axis=-1, keepdims=True) + EPS)
        xb8 = jnp.broadcast_to(x, (8, D))
        rowk = lax.broadcasted_iota(jnp.int32, (8, 128 * KM), 0)
        y = jnp.where(rowk == 0, xb8[:, :128 * KM], jnp.where(rowk == 1, 1.0, 0.0)).astype(BF)
        coef = jnp.where(row == 0, 1.0, -mu)
        dl = lane - row
        yb = [jnp.broadcast_to(
            jnp.sum(jnp.where(dl == 8 * b, xb8[:, 128 * k:128 * k + 128], 0.0), axis=1, keepdims=True),
            (8, 128)) - mu for k in range(KM, KD) for b in range(16)]
        yb = jnp.concatenate(yb, axis=0)
        NC = FF // 128
        mx = {}

        def mxu_col(c):
            mx[c] = [jnp.dot(y, pltpu.bitcast(wu[0:8 * KM, c].reshape(64 * KM, 128), BF),
                             preferred_element_type=F32) * coef for wu in (w1u, w3u)]

        def h_col(c):
            gu = []
            for i, wu in enumerate((w1u, w3u)):
                acc = None
                for r in range(8 * KM, 8 * KD):
                    v = pltpu.bitcast(wu[r, c], BF).astype(F32)
                    o = 16 * (r - 8 * KM)
                    if FCH == 1:
                        for t in range(2):
                            tv = v[8 * t:8 * t + 8] * yb[o + 8 * t:o + 8 * t + 8]
                            acc = tv if acc is None else acc + tv
                    else:
                        tv = v * yb[o:o + 16]
                        acc = tv if acc is None else acc + tv
                if FCH != 1:
                    acc = acc[:8] + acc[8:]
                gu.append(jnp.sum(acc + mx[c][i], axis=0, keepdims=True) * rs)
            g, u = gu
            return jnp.broadcast_to(g * jax.nn.sigmoid(g) * u, (8, 128)).astype(BF)

        out = [None] * KD
        nxt = 0
        for c in range(NC):
            while nxt < NC and nxt < FPRE + c * FSTEP / 4:
                mxu_col(nxt)
                nxt += 1
            h = h_col(c)
            for n in range(KD):
                t = jnp.dot(h, pltpu.bitcast(w2u[8 * c:8 * c + 8, n].reshape(64, 128), BF),
                            preferred_element_type=F32)[0:1]
                out[n] = t if out[n] is None else out[n] + t
        return residual(x, jnp.concatenate(out, axis=1))

    def emit(pv, seq):
        ntile = sum(not isinstance(e, tuple) for e in seq)
        total = sum(w for w, _ in pv) / 4
        k = done = n = 0
        for e in seq:
            if isinstance(e, tuple):
                e[1]()
                continue
            pos = LEAD + RATE * (n // 4) if n // 4 < (ntile - 1) // 4 else total - TAILC
            while k < len(pv) and done + pv[k][0] / 2 <= 4 * pos:
                done += pv[k][0]
                pv[k][1]()
                k += 1
            e(n < ntile - UNPACED)
            n += 1
        for _, g in pv[k:]:
            g()

    def layer(li, x):
        first = li == 0
        zero_i = li >> 4

        def barrier():
            @pl.when(li > 2)
            def _():
                reset_pipeline()

        mu = jnp.mean(x, axis=-1, keepdims=True)
        xc = x - mu
        rs = 1.0 / jnp.sqrt(jnp.mean(xc * xc, axis=-1, keepdims=True) + EPS)
        y = jnp.broadcast_to(xc, (8, D))
        for k in range(KD):
            yk = y[:, 128 * k:128 * k + 128]
            y_scr[k] = pack16(yk, yk)
        rs_scr[0] = jnp.broadcast_to(rs * c2, (8, 128))
        rowd = lax.broadcasted_iota(jnp.int32, (8, D), 0)
        xo = jnp.where(rowd < 4, jnp.broadcast_to(x, (8, D)), 1.0).astype(BF)
        coef = jnp.where(row < 4, 1.0, -mu)

        def q_direct(col):
            t = jnp.dot(xo, pltpu.bitcast(wqu[col], BF), preferred_element_type=F32) * coef
            return (t + pltpu.roll(t, 4, 0)).astype(BF).astype(F32)

        def q_cols(q, slot):
            dl = lane - row
            for b in range(16):
                part[slot + b] = jnp.broadcast_to(
                    jnp.sum(jnp.where(dl == 8 * b, q, 0.0), axis=1, keepdims=True), (8, 128))

        def vpu_a(m, slot, js):
            acc = {}
            for g2 in range(8):
                qc = jnp.concatenate([part[slot + 2 * g2 + t + zero_i] for t in range(2)], axis=0)
                for j in js:
                    tv = pltpu.bitcast(kvu[m, 0, 0, g2, j], BF).astype(F32) * qc
                    acc[j] = tv if g2 == 0 else acc[j] + tv
            for j in js:
                put_row(0, 0, j, jnp.sum(acc[j], axis=0, keepdims=True))

        def mix(mx, m, slot, nv, f0, fs, hook=None):
            k = 0
            for gi in range(-(-nv // PGRP)):
                n = min(len(mx), int(f0 + fs * gi))
                plain(mx[k:n])
                k = max(k, n)
                if hook is not None and gi == hook[0]:
                    hook[1]()
                vpu_a(m, slot, range(gi * PGRP, min(nv, (gi + 1) * PGRP)))
            plain(mx[k:])

        q0 = [q_direct(c) for c in range(3)]
        q10 = q_direct(3)
        s0, s1 = 4 * nq, 4 * nq + 16
        q_cols(q0[0], s0)
        set_pat(1, q0[1])
        set_pat(2, q0[2])
        qa, qb, qc = qk_ops(0)
        if PVA < nblk:
            set_pat(0, q0[0])
        mix(qa[PVA:] + qb + qc, 0, s0, PVA, PF0, PFS,
            (PQH, lambda: q_cols(q10, s1)) if PVB else None)
        g_softmax(0, 0)
        g_softmax(0, 1)
        plain(qproj_ops(1)[KD:])
        g_query(1)
        g_query(2)
        set_pat(0, q10)
        plain(qk_ops(1)[0][PVB:])
        for i in range(0, PVB, PGRP):
            part[0] = qpart[min(KD + PTK + int(i * PFB), 3 * KD - 1)]
            vpu_a(1, s1, range(i, min(PVB, i + PGRP)))
        toks.clear()

        nop = [bin(OPM & 1).count("1"), bin(OPM).count("1")]

        def block(t, ph):
            m = 2 * t + ph

            @pl.when(first)
            def _():
                kv_wait(m + 2)
                widen(m + 2)

            qp = qproj_ops(m + 2)
            _, qb, qc = qk_ops(m + 1)
            qa = qk_ops(m + 2)[0]
            pre, op = [], []
            if OPM >> (1 - ph) & 1:
                pre = [("now", lambda: g_out(1 - ph))]
            if OPM >> ph & 1:
                kt = nop[1] * t + (nop[0] if ph else 0) - (OPM & 1)
                op = oproj_ops(jnp.maximum(kt, 0), kt + 3, opart, 8 * ph)

            def olhs_stage():
                g_olhs(3 * m, 1 - ph)
                if not op:
                    toks.append(olhs[3 * m + 2])

            seq = (pre + [("now", olhs_stage)]
                   + qc[:CF] + qp[:KD] + [("now", lambda: g_query(0))] + qc[CF:] + qb
                   + [("now", lambda: g_softmax(1 - ph, 0)), ("now", lambda: g_softmax(1 - ph, 1))]
                   + qp[KD:] + [("now", lambda: g_query(1)), ("now", lambda: g_query(2))]
                   + op + qa[:32 - AEND] + [("now", lambda: fence(pat_scr, 3, zero_i))]
                   + qa[32 - AEND:])
            emit(pv_ops(m, ph), seq)

        def body(t, carry):
            block(t, 0)
            block(t, 1)
            return carry

        if SCOPES:
            with jax.named_scope("loop"):
                lax.fori_loop(0, NP // 2 - 1, body, 0)
        else:
            lax.fori_loop(0, NP // 2 - 1, body, 0)

        def big(kts, i0):
            return [op for i, kt in enumerate(kts)
                    for op in oproj_ops(kt, kt + 3, obig, KD * (i0 + i))]

        kt0 = nop[1] * (NP // 2 - 1) - (OPM & 1)
        old = list(range(kt0, 3 * (NP - 3)))
        barrier()
        _, qb, qc = qk_ops(NP - 1)
        k14 = old[:KT14 - 4] + list(range(3 * (NP - 3), 3 * (NP - 2)))
        seq = (([("now", lambda: g_out(1))] if OPM & 2 else [])
               + [("now", lambda: g_olhs(3 * (NP - 2), 1))] + qc + qb
               + [("now", lambda: g_softmax(1, 0)), ("now", lambda: g_softmax(1, 1))]
               + big(k14, 0) + [("now", lambda: fence(olhs, 3 * NP, zero_i))]
               + big(old[KT14 - 4:KT14 - 3], KT14 - 1))
        emit(pv_ops(NP - 2, 0), seq)
        old = old[KT14 - 3:]
        barrier()
        k15 = old[:KT15 - 4] + list(range(3 * (NP - 2), 3 * (NP - 1))) + old[KT15 - 4:KT15 - 3]
        emit(pv_ops(NP - 1, 1), [("now", lambda: g_olhs(3 * (NP - 1), 0))] + big(k15, KT14))
        old = old[KT15 - 3:]
        barrier()

        rows = [r.astype(BF) for r in o_rows(1)]
        a = [[out_scr[n]] + [obig[KD * i + n] for i in range(KT14 + len(k15))] for n in range(KD)]
        if old:
            l = jnp.concatenate([pltpu.bitcast(olhs[kt + 3], BF)[:8] for kt in old], axis=1)
            for n, t in enumerate(matvec(l, wou, 8 * old[0], 8 * len(old))):
                a[n].append(t)
        last = matvec(jnp.concatenate(rows, axis=1), wou, 8 * (3 * NP - 3), 24)
        cols = []
        for n in range(KD):
            xs = a[n]
            while len(xs) > 1:
                xs = [xs[i] + xs[i + 1] for i in range(0, len(xs) - 1, 2)] + xs[len(xs) & ~1:]
            cols.append(jnp.sum(xs[0] + last[n], axis=0, keepdims=True))
        x = residual(x, jnp.concatenate(cols, axis=1))
        if SCOPES:
            with jax.named_scope("ffn"):
                return lax.cond(first, lambda x: ffn(x, True), (ffn2 if KM < KD else lambda x: ffn(x, False)), x)
        return lax.cond(first, lambda x: ffn(x, True), (ffn2 if KM < KD else lambda x: ffn(x, False)), x)

    reset_pipeline()
    wait_all([c_x] + c_wq + c_wo)
    for m in range(2):
        kv_wait(m)
        widen(m)
    x = lax.fori_loop(0, 2, layer, xb[...].astype(F32))
    o_ref[...] = x.astype(o_ref.dtype)


@jax.jit
def pallas_interleave_layers__sliding_block_cached__glu_gated_swiglu__decode_kernel(
    A_x: jax.Array,
    A_k_cache: jax.Array,
    A_v_cache: jax.Array,
    A_wq: jax.Array,
    A_wo: jax.Array,
    B_x: jax.Array,
    B_w1: jax.Array,
    B_w3: jax.Array,
    B_w2: jax.Array,
):
    del B_x
    sk = A_k_cache.shape[2]
    win = min(4096, max(256, sk // 4))
    nb = sk // 128
    nblk = win // 128

    def cache_tiles(c):
        return c.reshape(H, nb, 128, G2, 2, 8).transpose(0, 3, 4, 1, 5, 2)

    def weight_tiles(w):
        r, c = w.shape
        return w.reshape(r // 16, 2, 8, c // 128, 128).transpose(0, 1, 3, 2, 4)

    vreg = lambda n, dt=F32: pltpu.VMEM((-(-n // 4) * 4, 8, 128), dt)
    kern = lambda *refs: _kernel(*refs, blk0=nb - nblk, nblk=nblk, scale=DH ** -0.5)
    out = pl.pallas_call(
        kern,
        out_shape=jax.ShapeDtypeStruct((1, D), BF),
        in_specs=[pl.BlockSpec(memory_space=pl.ANY)] * 8,
        out_specs=pl.BlockSpec(memory_space=pltpu.VMEM),
        scratch_shapes=[
            pltpu.VMEM((1, D), BF),
            pltpu.VMEM((NP, 2, 2, G2, nblk, 16, 128), BF),
            pltpu.VMEM((3 * NP, D, 128), BF),
            pltpu.VMEM((H * DH // 16, KD, 16, 128), BF),
            pltpu.VMEM((D // 16, FF // 128, 16, 128), BF),
            pltpu.VMEM((D // 16, FF // 128, 16, 128), BF),
            pltpu.VMEM((FF // 16, KD, 16, 128), BF),
            vreg(KD, U32),
            vreg(1),
            vreg(3 * KD),
            vreg(8, U32),
            vreg(nblk // 8),
            vreg(nblk // 2 + 32),
            pltpu.VMEM((2, 2, nblk, 128), F32),
            pltpu.VMEM((2 * nblk * 8, 128), F32),
            pltpu.VMEM((2, 64, 128), F32),
            pltpu.VMEM((2, 8 * NR, 128), F32),
            vreg(KD * (KT14 + KT15)),
            vreg(3 * NP + 4, U32),
            vreg(16),
            vreg(KD),
            pltpu.VMEM((NP, max(-(-NW // 4) * 4, 4), 8, 128), F32),
            pltpu.SemaphoreType.DMA((NP,)),
            pltpu.SemaphoreType.DMA((5 + len(W2_CHUNKS),)),
        ],
        compiler_params=pltpu.CompilerParams(
            vmem_limit_bytes=128 * 1024 * 1024, disable_semaphore_checks=True),
    )(A_x.reshape(1, D), cache_tiles(A_k_cache), cache_tiles(A_v_cache),
      A_wq, weight_tiles(A_wo),
      weight_tiles(B_w1), weight_tiles(B_w3), weight_tiles(B_w2))
    return out.reshape(1, 1, D)
```

```python
import math

import jax
import jax.numpy as jnp
from jax import lax
import jax.experimental.pallas as pl
import jax.experimental.pallas.tpu as pltpu

BF = jnp.bfloat16
F32 = jnp.float32
U32 = jnp.uint32

D = 640
H = 32
DH = 192
G = DH // 8
G2 = DH // 16
NP = H // 2
FF = 1536
EPS = 1e-5
KD = D // 128
NZ = 2 * G + 2
NR = NZ + 2
W2_CHUNKS = (768, 384, 256, 96, 32)

NG = 4
JB = 2
NW = 136
UNPACED = 4
LEAD = 10
RATE = 32
TAILC = 44
AEND = 4
CF = 4
OPM = 3
KT14 = 10
KT15 = 22
KM = 3
FCH = 2
FPRE = 6
FSTEP = 3
PVA = 32
PVB = 6
PGRP = 2
PF0 = 0
PFS = 4
PCH = 1
PFB = 1.5
PQH = 4
PTK = 4
NVC = 2
FLINK = 0
FTANH = 1
SCOPES = 0


def _run(ops):
    for op in ops:
        op()


def _kernel(x_hbm, k_hbm, v_hbm, wq_hbm, wo_hbm, w1_hbm, w3_hbm, w2_hbm,
            o_ref,
            xb, kvb, wq, wo, w1, w3, w2,
            y_scr, rs_scr, qpart, pat_scr, part_a, part, p_scr, pb_scr, pb0,
            accx, obig, olhs, opart, out_scr, vx,
            kvsem, wsem, *, blk0, nblk, scale):
    c2 = scale * math.log2(math.e)

    def kv_copies(m):
        return [pltpu.make_async_copy(
            src.at[pl.ds(2 * m, 2), :, t, pl.ds(blk0, nblk)],
            kvb.at[m, i, :, :, :, pl.ds(8 * t, 8), :], kvsem.at[m])
            for i, src in enumerate((k_hbm, v_hbm)) for t in range(2)]

    def kv_wait(m):
        pltpu.make_async_copy(kvb.at[m], kvb.at[m], kvsem.at[m]).wait()

    def wcopies(src, dst, s, r0=0, nr=None):
        nr = src.shape[0] if nr is None else nr
        return [pltpu.make_async_copy(src.at[pl.ds(r0, nr), t],
                                      dst.at[pl.ds(r0, nr), :, pl.ds(8 * t, 8), :],
                                      wsem.at[s]) for t in range(2)]

    c_x = pltpu.make_async_copy(x_hbm, xb, wsem.at[0])
    c_wq = [pltpu.make_async_copy(wq_hbm.at[:, pl.ds(128 * c, 128)], wq.at[c], wsem.at[1])
            for c in range(3 * NP)]
    c_wo = wcopies(wo_hbm, wo, 2)
    c_w1 = wcopies(w1_hbm, w1, 3)
    c_w3 = wcopies(w3_hbm, w3, 4)
    w2_off = [sum(W2_CHUNKS[:i]) for i in range(len(W2_CHUNKS))]
    c_w2 = [wcopies(w2_hbm, w2, 5 + i, o // 16, n // 16)
            for i, (o, n) in enumerate(zip(w2_off, W2_CHUNKS))]

    for c in c_wo + [c_x] + c_wq:
        c.start()
    for m in range(NP):
        for c in kv_copies(m):
            c.start()
    for c in c_w1 + c_w3 + [c for cs in c_w2 for c in cs]:
        c.start()

    def wait_all(cs):
        for c in cs:
            c.wait()

    kvu = kvb.bitcast(U32)
    wqu = wq.bitcast(U32)
    wou = wo.bitcast(U32)

    lane = lax.broadcasted_iota(jnp.int32, (8, 128), 1)
    row = lax.broadcasted_iota(jnp.int32, (8, 128), 0)
    diag8 = (lane & 7) == row
    lane_lo = lane < 64
    lane_bit = [((lane >> (3 + k)) & 1) == 1 for k in range(4)]

    def center(x):
        xc = x - jnp.mean(x, axis=-1, keepdims=True)
        var = jnp.mean(xc * xc, axis=-1, keepdims=True)
        return xc, 1.0 / jnp.sqrt(var + EPS)

    def pack16(z0, z1):
        return pltpu.bitcast(jnp.concatenate([z0, z1], axis=0).astype(BF), U32)

    def tile_dot(l_u32, w_u32, rows, paced):
        w = pltpu.bitcast(w_u32.reshape(64, 128), BF)
        if paced:
            l = pltpu.bitcast(jnp.concatenate([l_u32, l_u32], axis=0), BF)[:24]
            return jnp.dot(l, w, preferred_element_type=F32)[:rows]
        l = pltpu.bitcast(l_u32, BF)[:rows]
        return jnp.dot(l, w, preferred_element_type=F32)

    def qproj_ops(m):
        def op(paced, c, k):
            qpart[c * KD + k] = tile_dot(
                y_scr[k], wqu[3 * m + c, 64 * k:64 * k + 64, :], 8, paced)
        return [(lambda p, c=c, k=k: op(p, c, k)) for c in range(3) for k in range(KD)]

    def oproj_ops(kt, slot, dst, d0):
        def op(paced, n):
            dst[d0 + n] = tile_dot(olhs[slot], wou[pl.ds(kt * 8, 8), n], 8, paced)
        return [(lambda p, n=n: op(p, n)) for n in range(KD)]

    nq = nblk // 8

    def put_row(par, t, j, r):
        if par == 0 and t == 0:
            part_a[j // 8, j % 8:j % 8 + 1, :] = r
        else:
            part[(2 * par + t) * nq + j // 8, j % 8:j % 8 + 1, :] = r

    def qk_ops(m):
        def op_a(paced, j):
            r = tile_dot(pat_scr[0], kvu[m, 0, 0, 0:8, j], 8, paced)
            put_row(0, 0, j, r[j % 8:j % 8 + 1, :])

        def op_c(paced, j):
            r = tile_dot(pat_scr[2], kvu[m, 0, 1, 4:12, j], 8, paced)
            put_row(1, 0, j, r[j % 8:j % 8 + 1, :])

        def op_b(paced, j):
            w = jnp.concatenate([kvu[m, 0, 0, 8:12, j], kvu[m, 0, 1, 0:4, j]], axis=0)
            r = tile_dot(pat_scr[1], w, 16, paced)
            put_row(0, 1, j, r[j % 8:j % 8 + 1, :])
            put_row(1, 1, j, r[8 + j % 8:8 + j % 8 + 1, :])

        return [[(lambda p, f=f, j=j: f(p, j)) for j in range(nblk)] for f in (op_a, op_b, op_c)]

    def plain(ops):
        for op in ops:
            op(False)

    steps = [(par, gb, j0) for par in range(2) for gb in range(G2 // NG)
             for j0 in range(0, nblk, JB)]

    def step_blocks(par, gb, j0):
        return [(par, g2, j) for g2 in range(gb * NG, (gb + 1) * NG) for j in range(j0, j0 + JB)]

    order = [b for s in steps for b in step_blocks(*s)]
    wide = {}
    for i, b in enumerate(order):
        if (i + 1) * NW // len(order) > i * NW // len(order):
            wide[b] = len(wide)

    def widen(m):
        for (par, g2, j), e in wide.items():
            v = pltpu.bitcast(kvu[m, 1, par, g2, j], BF).astype(F32)
            kvu[m, 1, par, g2, j] = pltpu.bitcast(v[:8], U32)
            vx[m, e] = v[8:]

    def v_block(m, par, g2, j):
        u = kvu[m, 1, par, g2, j]
        if (par, g2, j) in wide:
            return jnp.concatenate([pltpu.bitcast(u, F32), vx[m, wide[(par, g2, j)]]], axis=0)
        return pltpu.bitcast(u, BF).astype(F32)

    def pv_ops(m, ph):
        acc = {}

        def spread(par, q, r):
            pb_scr[pl.ds(8 * (nblk * par + 8 * q) + r, 8, stride=8), :] = (
                p_scr[ph, par, 8 * q:8 * q + 8, :])

        def lsum(par):
            p = p_scr[ph, par]
            accx[ph, 8 * (2 * G + par):8 * (2 * G + par) + 8, :] = (
                (p[0:8] + p[8:16]) + (p[16:24] + p[24:32]))

        def step(par, gb, j0):
            pbs = {}
            for j in range(j0, j0 + JB):
                i = nblk * par + j
                pb = pb0[ph, 8 * i:8 * i + 8, :] if i < 8 else pb_scr[8 * i:8 * i + 8, :]
                pbs[j] = jnp.concatenate([pb, pb], axis=0)
            for _, g2, j in step_blocks(par, gb, j0):
                tv = v_block(m, par, g2, j) * pbs[j]
                acc[g2] = tv if j == 0 else acc[g2] + tv
                if j == nblk - 1:
                    r0 = DH * par + 16 * g2
                    accx[ph, r0:r0 + 16, :] = acc[g2]

        todo = []
        for par in range(2):
            for q in range(nblk // 8):
                if par or q:
                    dl = par * (len(steps) // 2) + (8 * q) // JB - 1
                    todo += [(dl, (lambda par=par, q=q, r=r: spread(par, q, r))) for r in range(8)]
        todo += [(len(steps) // 2, (lambda par=par: lsum(par))) for par in range(2)]
        todo.sort(key=lambda t: t[0])
        out = []
        k = 0
        for i, s in enumerate(steps):
            need = 0
            for n, (dl, _) in enumerate(todo[k:]):
                need = max(need, -(-(n + 1) // max(dl - i + 1, 1)))
            out += [(0, f) for _, f in todo[k:k + need]]
            k = min(k + need, len(todo))
            out.append((sum(4 if b in wide else 6 for b in step_blocks(*s)),
                        (lambda s=s: step(*s))))
        assert k == len(todo)
        return out

    toks = []

    def fence(dst, slot, zero_i):
        for i, t in enumerate(toks):
            dst[slot + i + zero_i] = t
        toks.clear()

    def g_softmax(ph, par):
        a = 2 * par * nq
        s0 = part[a:a + nq] if par else part_a[0:nq]
        s = (s0 + part[a + nq:a + 2 * nq]).reshape(nblk, 128)
        mx = jnp.max(jnp.max(s, axis=0, keepdims=True), axis=1, keepdims=True)
        cs = rs_scr[0]
        p = jnp.exp2((s - mx) * jnp.concatenate([cs] * (nblk // 8), axis=0))
        p_scr[ph, par] = p
        if par == 0:
            for r in range(8):
                pb0[ph, pl.ds(r, 8, stride=8), :] = p[0:8]
        toks.append(pltpu.bitcast(p[24:32], U32))

    def o_rows(ph):
        z = [jnp.broadcast_to(jnp.sum(accx[ph, 8 * g:8 * g + 8, :], axis=1, keepdims=True), (8, 128))
             for g in range(NZ)]
        inv = [1.0 / jnp.sum(z[2 * G + par], axis=0, keepdims=True) for par in range(2)]
        inv = [jnp.broadcast_to(v, (8, 128)) for v in inv]
        out = []
        for c in range(3):
            xs = z[16 * c:16 * c + 16]
            for k in range(4):
                xs = [jnp.where(lane_bit[k], xs[i + 1], xs[i]) for i in range(0, len(xs), 2)]
            iv = inv[0] if c == 0 else (inv[1] if c == 2 else jnp.where(lane_lo, inv[0], inv[1]))
            out.append(jnp.where(diag8, xs[0] * iv, 0.0))
        return out

    def g_olhs(slot0, ph):
        for c, z in enumerate(o_rows(ph)):
            olhs[slot0 + c] = pack16(z, z)

    def set_pat(c, q):
        if c == 1:
            u = pack16(jnp.where(lane_lo, q, 0.0), jnp.where(lane_lo, 0.0, q))
        else:
            u = pack16(q, q)
        pat_scr[c] = u
        if c > 0:
            toks.append(u)

    def g_query(c):
        xs = [qpart[c * KD + k] for k in range(KD)]
        set_pat(c, ((xs[0] + xs[1]) + (xs[2] + xs[3])) + xs[4])

    def g_out(ph):
        for n in range(KD):
            out_scr[n] = out_scr[n] + opart[8 * ph + n]

    def reset_pipeline():
        zero = jnp.zeros((8, 128), F32)
        accx[1, 0:16 * G, :] = jnp.zeros((16 * G, 128), F32)
        accx[1, 16 * G:16 * G + 16, :] = jnp.ones((16, 128), F32)
        for n in range(KD):
            opart[n] = zero
            opart[8 + n] = zero
            out_scr[n] = zero

    def residual(x, a):
        return (x + a.astype(BF).astype(F32)).astype(BF).astype(F32)

    def matvec(l, wu, r0, nr):
        cols = []
        for c in range(wu.shape[1]):
            w = pltpu.bitcast(wu[r0:r0 + nr, c].reshape(8 * nr, 128), BF)
            cols.append(jnp.dot(l, w, preferred_element_type=F32))
        return cols

    def ffn(x, first):
        xc, rs = center(x)
        y = jnp.broadcast_to(xc, (8, D)).astype(BF)
        if first:
            reset_pipeline()
            wait_all(c_w1)
        g = jnp.concatenate(matvec(y, w1.bitcast(U32), 0, D // 16), axis=1) * rs
        if first:
            wait_all(c_w3)
        u = jnp.concatenate(matvec(y, w3.bitcast(U32), 0, D // 16), axis=1) * rs
        hh = (g * jax.nn.sigmoid(g) * u).astype(BF)
        w2u = w2.bitcast(U32)
        if first:
            o_v = w2_off[-NVC]
            hf = hh[:, o_v:].astype(F32)
            dl = lane - row
            hb = [jnp.broadcast_to(
                jnp.sum(jnp.where(dl == (8 * b) % 128, hf[:, 128 * (b // 16):128 * (b // 16) + 128], 0.0),
                        axis=1, keepdims=True), (8, 128)) for b in range((FF - o_v) // 8)]
            a = None
            acc = [None] * KD
            for cs, o, n in zip(c_w2, w2_off, W2_CHUNKS):
                if SCOPES:
                    with jax.named_scope("w2wait"):
                        wait_all(cs)
                else:
                    wait_all(cs)
                if o < o_v:
                    t = jnp.concatenate(matvec(hh[:, o:o + n], w2u, o // 16, n // 16), axis=1)[0:1]
                    a = t if a is None else a + t
                else:
                    for r in range(o // 16, (o + n) // 16):
                        b = 2 * (r - o_v // 16)
                        for c in range(KD):
                            v = pltpu.bitcast(w2u[r, c], BF).astype(F32)
                            tv = v[:8] * hb[b] + v[8:] * hb[b + 1]
                            acc[c] = tv if acc[c] is None else acc[c] + tv
            a = a + jnp.concatenate([jnp.sum(t, axis=0, keepdims=True) for t in acc], axis=1)
        else:
            a = jnp.concatenate(matvec(hh, w2u, 0, FF // 16), axis=1)[0:1]
        return residual(x, a)

    def ffn2(x, zero_i):
        w1u, w3u, w2u = w1.bitcast(U32), w3.bitcast(U32), w2.bitcast(U32)
        mu = jnp.mean(x, axis=-1, keepdims=True)
        xc = x - mu
        rs = 1.0 / jnp.sqrt(jnp.mean(xc * xc, axis=-1, keepdims=True) + EPS)
        xb8 = jnp.broadcast_to(x, (8, D))
        rowk = lax.broadcasted_iota(jnp.int32, (8, 128 * KM), 0)
        y = jnp.where(rowk == 0, xb8[:, :128 * KM], jnp.where(rowk == 1, 1.0, 0.0)).astype(BF)
        coef = jnp.where(row == 0, 1.0, -mu)
        dl = lane - row
        yb = [jnp.broadcast_to(
            jnp.sum(jnp.where(dl == 8 * b, xb8[:, 128 * k:128 * k + 128], 0.0), axis=1, keepdims=True),
            (8, 128)) - mu for k in range(KM, KD) for b in range(16)]
        yb = jnp.concatenate(yb, axis=0)
        NC = FF // 128
        mx = {}
        done = {}
        never = lane < zero_i

        def mxu_col(c):
            mx[c] = [jnp.dot(y, pltpu.bitcast(wu[0:8 * KM, c].reshape(64 * KM, 128), BF),
                             preferred_element_type=F32) * coef for wu in (w1u, w3u)]

        def h_col(c):
            gu = []
            for i, wu in enumerate((w1u, w3u)):
                acc = None
                for r in range(8 * KM, 8 * KD):
                    v = pltpu.bitcast(wu[r, c], BF).astype(F32)
                    o = 16 * (r - 8 * KM)
                    if FCH == 1:
                        for t in range(2):
                            tv = v[8 * t:8 * t + 8] * yb[o + 8 * t:o + 8 * t + 8]
                            if acc is None and FLINK and (c - FLINK, i) in done:
                                tv = jnp.where(never, done[c - FLINK, i], tv)
                            acc = tv if acc is None else acc + tv
                    else:
                        tv = v * yb[o:o + 16]
                        if acc is None and FLINK and (c - FLINK, i) in done:
                            tv = jnp.where(jnp.concatenate([never, never], axis=0), done[c - FLINK, i], tv)
                        acc = tv if acc is None else acc + tv
                done[c, i] = acc
                if FCH != 1:
                    acc = acc[:8] + acc[8:]
                gu.append(jnp.sum(acc + mx[c][i], axis=0, keepdims=True) * rs)
            g, u = gu
            if FTANH:
                hg = 0.5 * g
                return jnp.broadcast_to((hg * jnp.tanh(hg) + hg) * u, (8, 128)).astype(BF)
            return jnp.broadcast_to(g * jax.nn.sigmoid(g) * u, (8, 128)).astype(BF)

        out = [None] * KD
        nxt = 0
        for c in range(NC):
            while nxt < NC and nxt < FPRE + c * FSTEP / 4:
                mxu_col(nxt)
                nxt += 1
            h = h_col(c)
            for n in range(KD):
                t = jnp.dot(h, pltpu.bitcast(w2u[8 * c:8 * c + 8, n].reshape(64, 128), BF),
                            preferred_element_type=F32)[0:1]
                out[n] = t if out[n] is None else out[n] + t
        return residual(x, jnp.concatenate(out, axis=1))

    def emit(pv, seq):
        ntile = sum(not isinstance(e, tuple) for e in seq)
        total = sum(w for w, _ in pv) / 4
        k = done = n = 0
        for e in seq:
            if isinstance(e, tuple):
                e[1]()
                continue
            pos = LEAD + RATE * (n // 4) if n // 4 < (ntile - 1) // 4 else total - TAILC
            while k < len(pv) and done + pv[k][0] / 2 <= 4 * pos:
                done += pv[k][0]
                pv[k][1]()
                k += 1
            e(n < ntile - UNPACED)
            n += 1
        for _, g in pv[k:]:
            g()

    def layer(li, x):
        first = li == 0
        zero_i = li >> 4

        def barrier():
            @pl.when(li > 2)
            def _():
                reset_pipeline()

        mu = jnp.mean(x, axis=-1, keepdims=True)
        xc = x - mu
        rs = 1.0 / jnp.sqrt(jnp.mean(xc * xc, axis=-1, keepdims=True) + EPS)
        y = jnp.broadcast_to(xc, (8, D))
        for k in range(KD):
            yk = y[:, 128 * k:128 * k + 128]
            y_scr[k] = pack16(yk, yk)
        rs_scr[0] = jnp.broadcast_to(rs * c2, (8, 128))
        rowd = lax.broadcasted_iota(jnp.int32, (8, D), 0)
        xo = jnp.where(rowd < 4, jnp.broadcast_to(x, (8, D)), 1.0).astype(BF)
        coef = jnp.where(row < 4, 1.0, -mu)

        def q_direct(col):
            t = jnp.dot(xo, pltpu.bitcast(wqu[col], BF), preferred_element_type=F32) * coef
            return (t + pltpu.roll(t, 4, 0)).astype(BF).astype(F32)

        def q_cols(q, slot):
            dl = lane - row
            for b in range(16):
                part[slot + b] = jnp.broadcast_to(
                    jnp.sum(jnp.where(dl == 8 * b, q, 0.0), axis=1, keepdims=True), (8, 128))

        def vpu_a(m, slot, js):
            acc = {}
            for g2 in range(8):
                qc = jnp.concatenate([part[slot + 2 * g2 + t + zero_i] for t in range(2)], axis=0)
                for j in js:
                    tv = pltpu.bitcast(kvu[m, 0, 0, g2, j], BF).astype(F32) * qc
                    acc[j] = tv if g2 == 0 else acc[j] + tv
            for j in js:
                put_row(0, 0, j, jnp.sum(acc[j], axis=0, keepdims=True))

        def mix(mx, m, slot, nv, f0, fs, hook=None):
            k = 0
            for gi in range(-(-nv // PGRP)):
                n = min(len(mx), int(f0 + fs * gi))
                plain(mx[k:n])
                k = max(k, n)
                if hook is not None and gi == hook[0]:
                    hook[1]()
                vpu_a(m, slot, range(gi * PGRP, min(nv, (gi + 1) * PGRP)))
            plain(mx[k:])

        q0 = [q_direct(c) for c in range(3)]
        q10 = q_direct(3)
        s0, s1 = 4 * nq, 4 * nq + 16
        q_cols(q0[0], s0)
        set_pat(1, q0[1])
        set_pat(2, q0[2])
        qa, qb, qc = qk_ops(0)
        if PVA < nblk:
            set_pat(0, q0[0])
        mix(qa[PVA:] + qb + qc, 0, s0, PVA, PF0, PFS,
            (PQH, lambda: q_cols(q10, s1)) if PVB else None)
        g_softmax(0, 0)
        g_softmax(0, 1)
        plain(qproj_ops(1)[KD:])
        g_query(1)
        g_query(2)
        set_pat(0, q10)
        plain(qk_ops(1)[0][PVB:])
        for i in range(0, PVB, PGRP):
            part[0] = qpart[min(KD + PTK + int(i * PFB), 3 * KD - 1)]
            vpu_a(1, s1, range(i, min(PVB, i + PGRP)))
        toks.clear()

        nop = [bin(OPM & 1).count("1"), bin(OPM).count("1")]

        def block(t, ph):
            m = 2 * t + ph

            @pl.when(first)
            def _():
                kv_wait(m + 2)
                widen(m + 2)

            qp = qproj_ops(m + 2)
            _, qb, qc = qk_ops(m + 1)
            qa = qk_ops(m + 2)[0]
            pre, op = [], []
            if OPM >> (1 - ph) & 1:
                pre = [("now", lambda: g_out(1 - ph))]
            if OPM >> ph & 1:
                kt = nop[1] * t + (nop[0] if ph else 0) - (OPM & 1)
                op = oproj_ops(jnp.maximum(kt, 0), kt + 3, opart, 8 * ph)

            def olhs_stage():
                g_olhs(3 * m, 1 - ph)
                if not op:
                    toks.append(olhs[3 * m + 2])

            seq = (pre + [("now", olhs_stage)]
                   + qc[:CF] + qp[:KD] + [("now", lambda: g_query(0))] + qc[CF:] + qb
                   + [("now", lambda: g_softmax(1 - ph, 0)), ("now", lambda: g_softmax(1 - ph, 1))]
                   + qp[KD:] + [("now", lambda: g_query(1)), ("now", lambda: g_query(2))]
                   + op + qa[:32 - AEND] + [("now", lambda: fence(pat_scr, 3, zero_i))]
                   + qa[32 - AEND:])
            emit(pv_ops(m, ph), seq)

        def body(t, carry):
            block(t, 0)
            block(t, 1)
            return carry

        if SCOPES:
            with jax.named_scope("loop"):
                lax.fori_loop(0, NP // 2 - 1, body, 0)
        else:
            lax.fori_loop(0, NP // 2 - 1, body, 0)

        def big(kts, i0):
            return [op for i, kt in enumerate(kts)
                    for op in oproj_ops(kt, kt + 3, obig, KD * (i0 + i))]

        kt0 = nop[1] * (NP // 2 - 1) - (OPM & 1)
        old = list(range(kt0, 3 * (NP - 3)))
        barrier()
        _, qb, qc = qk_ops(NP - 1)
        k14 = old[:KT14 - 4] + list(range(3 * (NP - 3), 3 * (NP - 2)))
        seq = (([("now", lambda: g_out(1))] if OPM & 2 else [])
               + [("now", lambda: g_olhs(3 * (NP - 2), 1))] + qc + qb
               + [("now", lambda: g_softmax(1, 0)), ("now", lambda: g_softmax(1, 1))]
               + big(k14, 0) + [("now", lambda: fence(olhs, 3 * NP, zero_i))]
               + big(old[KT14 - 4:KT14 - 3], KT14 - 1))
        emit(pv_ops(NP - 2, 0), seq)
        old = old[KT14 - 3:]
        barrier()
        k15 = old[:KT15 - 4] + list(range(3 * (NP - 2), 3 * (NP - 1))) + old[KT15 - 4:KT15 - 3]
        emit(pv_ops(NP - 1, 1), [("now", lambda: g_olhs(3 * (NP - 1), 0))] + big(k15, KT14))
        old = old[KT15 - 3:]

        def epilogue(x):
            def lsum(g):
                return jnp.broadcast_to(
                    jnp.sum(accx[1, 8 * g:8 * g + 8, :], axis=1, keepdims=True), (8, 128))

            inv = [1.0 / jnp.sum(lsum(2 * G + par), axis=0, keepdims=True) for par in range(2)]
            last = [None] * KD
            for par in range(2):
                acc = [None] * KD
                for g2 in range(G2):
                    g = G * par + 2 * g2
                    z = jnp.concatenate([lsum(g), lsum(g + 1)], axis=0)
                    for n in range(KD):
                        tv = pltpu.bitcast(wou[(NP - 1) * G + G2 * par + g2, n], BF).astype(F32) * z
                        acc[n] = tv if g2 == 0 else acc[n] + tv
                for n in range(KD):
                    t = (acc[n][:8] + acc[n][8:]) * inv[par]
                    last[n] = t if par == 0 else last[n] + t
            a = [[out_scr[n]] + [obig[KD * i + n] for i in range(KT14 + len(k15))] for n in range(KD)]
            if old:
                l = jnp.concatenate([pltpu.bitcast(olhs[kt + 3], BF)[:8] for kt in old], axis=1)
                for n, t in enumerate(matvec(l, wou, 8 * old[0], 8 * len(old))):
                    a[n].append(t)
            cols = []
            for n in range(KD):
                xs = a[n]
                while len(xs) > 1:
                    xs = [xs[i] + xs[i + 1] for i in range(0, len(xs) - 1, 2)] + xs[len(xs) & ~1:]
                cols.append(jnp.sum(xs[0] + last[n], axis=0, keepdims=True))
            return residual(x, jnp.concatenate(cols, axis=1))
        if SCOPES:
            with jax.named_scope("ffn"):
                return lax.cond(first, lambda x: ffn(epilogue(x), True), lambda x: ffn2(epilogue(x), zero_i), x)
        return lax.cond(first, lambda x: ffn(epilogue(x), True), lambda x: ffn2(epilogue(x), zero_i), x)

    reset_pipeline()
    wait_all([c_x] + c_wq + c_wo)
    for m in range(2):
        kv_wait(m)
        widen(m)
    x = lax.fori_loop(0, 2, layer, xb[...].astype(F32))
    o_ref[...] = x.astype(o_ref.dtype)


@jax.jit
def pallas_interleave_layers__sliding_block_cached__glu_gated_swiglu__decode_kernel(
    A_x: jax.Array,
    A_k_cache: jax.Array,
    A_v_cache: jax.Array,
    A_wq: jax.Array,
    A_wo: jax.Array,
    B_x: jax.Array,
    B_w1: jax.Array,
    B_w3: jax.Array,
    B_w2: jax.Array,
):
    del B_x
    sk = A_k_cache.shape[2]
    win = min(4096, max(256, sk // 4))
    nb = sk // 128
    nblk = win // 128

    def cache_tiles(c):
        return c.reshape(H, nb, 128, G2, 2, 8).transpose(0, 3, 4, 1, 5, 2)

    def weight_tiles(w):
        r, c = w.shape
        return w.reshape(r // 16, 2, 8, c // 128, 128).transpose(0, 1, 3, 2, 4)

    vreg = lambda n, dt=F32: pltpu.VMEM((-(-n // 4) * 4, 8, 128), dt)
    kern = lambda *refs: _kernel(*refs, blk0=nb - nblk, nblk=nblk, scale=DH ** -0.5)
    out = pl.pallas_call(
        kern,
        out_shape=jax.ShapeDtypeStruct((1, D), BF),
        in_specs=[pl.BlockSpec(memory_space=pl.ANY)] * 8,
        out_specs=pl.BlockSpec(memory_space=pltpu.VMEM),
        scratch_shapes=[
            pltpu.VMEM((1, D), BF),
            pltpu.VMEM((NP, 2, 2, G2, nblk, 16, 128), BF),
            pltpu.VMEM((3 * NP, D, 128), BF),
            pltpu.VMEM((H * DH // 16, KD, 16, 128), BF),
            pltpu.VMEM((D // 16, FF // 128, 16, 128), BF),
            pltpu.VMEM((D // 16, FF // 128, 16, 128), BF),
            pltpu.VMEM((FF // 16, KD, 16, 128), BF),
            vreg(KD, U32),
            vreg(1),
            vreg(3 * KD),
            vreg(8, U32),
            vreg(nblk // 8),
            vreg(nblk // 2 + 32),
            pltpu.VMEM((2, 2, nblk, 128), F32),
            pltpu.VMEM((2 * nblk * 8, 128), F32),
            pltpu.VMEM((2, 64, 128), F32),
            pltpu.VMEM((2, 8 * NR, 128), F32),
            vreg(KD * (KT14 + KT15)),
            vreg(3 * NP + 4, U32),
            vreg(16),
            vreg(KD),
            pltpu.VMEM((NP, max(-(-NW // 4) * 4, 4), 8, 128), F32),
            pltpu.SemaphoreType.DMA((NP,)),
            pltpu.SemaphoreType.DMA((5 + len(W2_CHUNKS),)),
        ],
        compiler_params=pltpu.CompilerParams(
            vmem_limit_bytes=128 * 1024 * 1024, disable_semaphore_checks=True),
    )(A_x.reshape(1, D), cache_tiles(A_k_cache), cache_tiles(A_v_cache),
      A_wq, weight_tiles(A_wo),
      weight_tiles(B_w1), weight_tiles(B_w3), weight_tiles(B_w2))
    return out.reshape(1, 1, D)
```

```python
import math

import jax
import jax.numpy as jnp
from jax import lax
import jax.experimental.pallas as pl
import jax.experimental.pallas.tpu as pltpu

BF = jnp.bfloat16
F32 = jnp.float32
U32 = jnp.uint32

D = 640
H = 32
DH = 192
G = DH // 8
G2 = DH // 16
NP = H // 2
FF = 1536
EPS = 1e-5
KD = D // 128
NC = FF // 128
NZ = 2 * G + 2
NR = NZ + 2
W2_CHUNKS = (768, 384, 256, 128)

NG = 4
JB = 2
NW = 72
UNPACED = 8
LEAD = 16
RATE = 32.5
TAILC = 30
AEND = 4
CF = 8
KT14 = 10
PVB = 6
KM = 3
FPRE = 6
FSTEP = 3


def _kernel(x_hbm, k_hbm, v_hbm, wq_hbm, wo_hbm, w1_hbm, w3_hbm, w2_hbm,
            o_ref,
            xb, kvb, wq, wo, w1, w3, w2,
            y_scr, rs_scr, qpart, pat_scr, part_a, part, p_scr, pb_scr, pb0,
            accx, olhs, opart, out_scr, vx,
            kvsem, wsem, *, blk0, nblk, scale):
    c2 = scale * math.log2(math.e)
    nq = nblk // 8
    SP = 4 * nq

    def kv_copies(m):
        return [pltpu.make_async_copy(
            src.at[pl.ds(2 * m, 2), :, t, pl.ds(blk0, nblk)],
            kvb.at[m, i, :, :, :, pl.ds(8 * t, 8), :], kvsem.at[m])
            for i, src in enumerate((k_hbm, v_hbm)) for t in range(2)]

    def kv_wait(m):
        pltpu.make_async_copy(kvb.at[m], kvb.at[m], kvsem.at[m]).wait()

    def wcopies(src, dst, s, r0=0, nr=None):
        nr = src.shape[0] if nr is None else nr
        return [pltpu.make_async_copy(src.at[pl.ds(r0, nr), t],
                                      dst.at[pl.ds(r0, nr), :, pl.ds(8 * t, 8), :],
                                      wsem.at[s]) for t in range(2)]

    c_x = pltpu.make_async_copy(x_hbm, xb, wsem.at[0])
    c_wq = [pltpu.make_async_copy(wq_hbm.at[:, pl.ds(128 * c, 128)], wq.at[c], wsem.at[1])
            for c in range(3 * NP)]
    c_wo = wcopies(wo_hbm, wo, 2)
    c_w1 = wcopies(w1_hbm, w1, 3)
    c_w3 = wcopies(w3_hbm, w3, 4)
    w2_off = [sum(W2_CHUNKS[:i]) for i in range(len(W2_CHUNKS))]
    c_w2 = [wcopies(w2_hbm, w2, 5 + i, o // 16, n // 16)
            for i, (o, n) in enumerate(zip(w2_off, W2_CHUNKS))]

    for c in c_wo + [c_x] + c_wq:
        c.start()
    for m in range(NP):
        for c in kv_copies(m):
            c.start()
    for c in c_w1 + c_w3 + [c for cs in c_w2 for c in cs]:
        c.start()

    def wait_all(cs):
        for c in cs:
            c.wait()

    kvu = kvb.bitcast(U32)
    wqu = wq.bitcast(U32)
    wou = wo.bitcast(U32)
    w1u, w3u, w2u = w1.bitcast(U32), w3.bitcast(U32), w2.bitcast(U32)
    y_u, pat_u, olhs_u = y_scr.bitcast(U32), pat_scr.bitcast(U32), olhs.bitcast(U32)

    def f32_rows(u):
        return pltpu.bitcast(u, BF).astype(F32)

    lane = lax.broadcasted_iota(jnp.int32, (8, 128), 1)
    row = lax.broadcasted_iota(jnp.int32, (8, 128), 0)
    diag_i = ((lane & 7) == row).astype(jnp.int32) * 64
    bit_i = [(lane << (3 - k)) & 64 for k in range(4)]
    uid = [0]

    def lane_sum(v):
        return jnp.broadcast_to(jnp.sum(v, axis=1, keepdims=True), (8, 128))

    def columns(v8):
        uid[0] += 1
        off = 256 * uid[0]
        dl = lane - row + off
        return [lane_sum(jnp.where(dl == off + 8 * b, v8[:, 128 * k:128 * k + 128], 0.0))
                for k in range(v8.shape[1] // 128) for b in range(16)]

    def moments(x):
        mu = jnp.mean(x, axis=-1, keepdims=True)
        xc = x - mu
        return mu, xc, 1.0 / jnp.sqrt(jnp.mean(xc * xc, axis=-1, keepdims=True) + EPS)

    def residual(x, a):
        return (x + a.astype(BF).astype(F32)).astype(BF).astype(F32)

    def matvec(l, wu, r0, nr):
        return [jnp.dot(l, pltpu.bitcast(wu[r0:r0 + nr, c].reshape(8 * nr, 128), BF),
                        preferred_element_type=F32) for c in range(wu.shape[1])]

    def tile_dot(l_u32, w_u32, rows, paced):
        w = pltpu.bitcast(w_u32.reshape(64, 128), BF)
        if paced:
            l = pltpu.bitcast(jnp.concatenate([l_u32, l_u32], axis=0), BF)[:24]
            return jnp.dot(l, w, preferred_element_type=F32)[:rows]
        l = pltpu.bitcast(l_u32, BF)[:rows]
        return jnp.dot(l, w, preferred_element_type=F32)

    def qproj_ops(m):
        def op(paced, c, k):
            qpart[c * KD + k] = tile_dot(
                y_u[k], wqu[3 * m + c, 64 * k:64 * k + 64, :], 8, paced)
        return [(lambda p, c=c, k=k: op(p, c, k)) for c in range(3) for k in range(KD)]

    def oproj_ops(kt, slot, dst, d0):
        def op(paced, n):
            dst[d0 + n] = tile_dot(olhs_u[slot], wou[pl.ds(kt * 8, 8), n], 8, paced)
        return [(lambda p, n=n: op(p, n)) for n in range(KD)]

    def qk_ops(m):
        def op_a(paced, j):
            r = tile_dot(pat_u[0], kvu[m, 0, 0, 0:8, j], 8, paced)
            part_a[j // 8, j % 8:j % 8 + 1, :] = r[j % 8:j % 8 + 1, :]

        def op_c(paced, j):
            r = tile_dot(pat_u[2], kvu[m, 0, 1, 4:12, j], 8, paced)
            part[2 * nq + j // 8, j % 8:j % 8 + 1, :] = r[j % 8:j % 8 + 1, :]

        def op_b(paced, j):
            w = jnp.concatenate([kvu[m, 0, 0, 8:12, j], kvu[m, 0, 1, 0:4, j]], axis=0)
            r = tile_dot(pat_u[1], w, 16, paced)
            part[nq + j // 8, j % 8:j % 8 + 1, :] = r[j % 8:j % 8 + 1, :]
            part[3 * nq + j // 8, j % 8:j % 8 + 1, :] = r[8 + j % 8:8 + j % 8 + 1, :]

        return [[(lambda p, f=f, j=j: f(p, j)) for j in range(nblk)] for f in (op_a, op_b, op_c)]

    def plain(ops):
        for op in ops:
            op(False)

    steps = [(par, gb, j0) for par in range(2) for gb in range(G2 // NG)
             for j0 in range(0, nblk, JB)]

    def units(par, gb, j0):
        return [(par, g2, j0) for g2 in range(gb * NG, (gb + 1) * NG)]

    order = [u for s in steps for u in units(*s)]
    wide = {}
    for i, u in enumerate(order):
        if (i + 1) * NW // len(order) > i * NW // len(order):
            wide[u] = len(wide)

    def widen(m):
        for (par, g2, j), e in wide.items():
            v = f32_rows(kvu[m, 1, par, g2, j:j + JB])
            kvu[m, 1, par, g2, j:j + JB] = pltpu.bitcast(v[:, :8], U32)
            vx[m, e] = v[:, 8:]

    def v_unit(m, par, g2, j):
        u = kvu[m, 1, par, g2, j:j + JB]
        if (par, g2, j) in wide:
            return jnp.concatenate([pltpu.bitcast(u, F32), vx[m, wide[(par, g2, j)]]], axis=1)
        return f32_rows(u)

    def pv_ops(m, ph):
        acc = {}

        def spread(par, q, r):
            pb_scr[pl.ds(64 * q + r, 8, stride=8), :] = p_scr[ph, par, 8 * q:8 * q + 8, :]

        def psum(par):
            p = p_scr[ph, par]
            accx[ph, 8 * (2 * G + par):8 * (2 * G + par) + 8, :] = (
                (p[0:8] + p[8:16]) + (p[16:24] + p[24:32]))

        def step(par, gb, j0):
            if par == 0 and j0 < 8:
                pb = pb0[ph, 8 * j0:8 * (j0 + JB), :]
            else:
                pb = pb_scr[8 * j0:8 * (j0 + JB), :]
            pb = pb.reshape(JB, 8, 128)
            pb = jnp.concatenate([pb, pb], axis=1)
            for _, g2, _ in units(par, gb, j0):
                tv = jnp.sum(v_unit(m, par, g2, j0) * pb, axis=0)
                acc[g2] = tv if j0 == 0 else acc[g2] + tv
                if j0 == nblk - JB:
                    r0 = DH * par + 16 * g2
                    accx[ph, r0:r0 + 16, :] = acc[g2]

        half = len(steps) // 2
        spq = 8 // JB
        side = {}
        for q in range(nq):
            for r in range(8):
                if q:
                    side.setdefault((spq * (8 * (q - 1) + r)) // 9, []).append(
                        lambda q=q, r=r: spread(0, q, r))
                side.setdefault(half - nblk // JB + spq * (q + 1) + 1 + r, []).append(
                    lambda q=q, r=r: spread(1, q, r))
        for par in range(2):
            side.setdefault(half // 2 + par, []).append(lambda par=par: psum(par))
        out = []
        for i, s in enumerate(steps):
            out += [(0, f) for f in side.get(i, [])]
            out.append((JB * sum(4 if u in wide else 6 for u in units(*s)),
                        (lambda s=s: step(*s))))
        return out

    toks = []

    def fence(dst, slot, zero_i):
        for i, t in enumerate(toks):
            dst[slot + i + zero_i] = t
        toks.clear()

    def g_softmax(ph, par):
        s0 = part[2 * nq:3 * nq] if par else part_a[0:nq]
        s = (s0 + part[(2 * par + 1) * nq:(2 * par + 2) * nq]).reshape(nblk, 128)
        mx = jnp.max(jnp.max(s, axis=0, keepdims=True), axis=1, keepdims=True)
        p = jnp.exp2((s - mx) * jnp.concatenate([rs_scr[0]] * nq, axis=0))
        p_scr[ph, par] = p
        if par == 0:
            for r in range(8):
                pb0[ph, pl.ds(r, 8, stride=8), :] = p[0:8]
        toks.append(pltpu.bitcast(p[nblk - 8:nblk], U32))

    def recip(d):
        r = pl.reciprocal(d, approx=True)
        return r * (2.0 - d * r)

    def g_olhs(slot0, ph):
        z = [lane_sum(accx[ph, 8 * g:8 * g + 8, :]) for g in range(NZ)]
        inv = [jnp.broadcast_to(recip(jnp.sum(z[2 * G + par], axis=0, keepdims=True)), (8, 128))
               for par in range(2)]
        uid[0] += 1
        bit = [b > uid[0] for b in bit_i]
        for c in range(3):
            xs = z[16 * c:16 * c + 16]
            for k in range(4):
                xs = [jnp.where(bit[k], xs[i + 1], xs[i]) for i in range(0, len(xs), 2)]
            iv = inv[0] if c == 0 else (inv[1] if c == 2 else jnp.where(bit[3], inv[1], inv[0]))
            olhs[slot0 + c, 0:8, :] = jnp.where(diag_i > uid[0], xs[0] * iv, 0.0).astype(BF)

    def set_pat(c, q):
        if c == 1:
            hi = bit_i[3] > uid[0]
            pat_scr[c, 0:8, :] = jnp.where(hi, 0.0, q).astype(BF)
            pat_scr[c, 8:16, :] = jnp.where(hi, q, 0.0).astype(BF)
        else:
            pat_scr[c, 0:8, :] = q.astype(BF)
        if c > 0:
            toks.append(pltpu.bitcast(q, U32))

    def g_query(c):
        xs = [qpart[c * KD + k] for k in range(KD)]
        set_pat(c, ((xs[0] + xs[1]) + (xs[2] + xs[3])) + xs[4])

    def g_out(ph):
        for n in range(KD):
            out_scr[n] = out_scr[n] + opart[8 * ph + n]

    def reset_pipeline():
        accx[1, 0:16 * G, :] = jnp.zeros((16 * G, 128), F32)
        accx[1, 16 * G:16 * G + 16, :] = jnp.ones((16, 128), F32)
        for n in range(KD):
            opart[8 + n] = jnp.zeros((8, 128), F32)
            out_scr[n] = jnp.zeros((8, 128), F32)

    def emit(pv, seq):
        ntile = sum(not isinstance(e, tuple) for e in seq)
        total = sum(w for w, _ in pv) / 4
        k = done = n = 0
        for e in seq:
            if isinstance(e, tuple):
                e[0]()
                continue
            pos = LEAD + RATE * (n // 4) if n // 4 < (ntile - 1) // 4 else total - TAILC
            while k < len(pv) and done + pv[k][0] / 2 <= 4 * pos:
                done += pv[k][0]
                pv[k][1]()
                k += 1
            e(n < ntile - UNPACED)
            n += 1
        for _, g in pv[k:]:
            g()

    def ffn1(x):
        _, xc, rs = moments(x)
        y = jnp.broadcast_to(xc, (8, D)).astype(BF)
        reset_pipeline()
        wait_all(c_w1)
        g = jnp.concatenate(matvec(y, w1u, 0, D // 16), axis=1) * rs
        wait_all(c_w3)
        u = jnp.concatenate(matvec(y, w3u, 0, D // 16), axis=1) * rs
        hh = (g * jax.nn.sigmoid(g) * u).astype(BF)
        hb = columns(hh[:, w2_off[-1]:].astype(F32))
        a = None
        for cs, o, n in list(zip(c_w2, w2_off, W2_CHUNKS))[:-1]:
            wait_all(cs)
            t = jnp.concatenate(matvec(hh[:, o:o + n], w2u, o // 16, n // 16), axis=1)[0:1]
            a = t if a is None else a + t
        wait_all(c_w2[-1])
        acc = [None] * KD
        for r in range(W2_CHUNKS[-1] // 16):
            for c in range(KD):
                v = f32_rows(w2u[w2_off[-1] // 16 + r, c])
                tv = v[:8] * hb[2 * r] + v[8:] * hb[2 * r + 1]
                acc[c] = tv if r == 0 else acc[c] + tv
        a = a + jnp.concatenate([jnp.sum(t, axis=0, keepdims=True) for t in acc], axis=1)
        return residual(x, a)

    def ffn2(x):
        mu, _, rs = moments(x)
        x8 = jnp.broadcast_to(x, (8, D))
        rowk = lax.broadcasted_iota(jnp.int32, (8, 128 * KM), 0)
        y = jnp.where(rowk == 0, x8[:, :128 * KM], jnp.where(rowk == 1, 1.0, 0.0)).astype(BF)
        coef = jnp.where(row == 0, 1.0, -mu)
        yb = jnp.concatenate([c - mu for c in columns(x8[:, 128 * KM:])], axis=0)
        mx = {}
        out = [None] * KD
        for c in range(NC):
            while len(mx) < min(NC, FPRE + c * FSTEP / 4):
                cc = len(mx)
                mx[cc] = [jnp.dot(y, pltpu.bitcast(wu[0:8 * KM, cc].reshape(64 * KM, 128), BF),
                                  preferred_element_type=F32) * coef for wu in (w1u, w3u)]
            gu = []
            for i, wu in enumerate((w1u, w3u)):
                acc = None
                for r in range(8 * (KD - KM)):
                    tv = f32_rows(wu[8 * KM + r, c]) * yb[16 * r:16 * r + 16]
                    acc = tv if r == 0 else acc + tv
                gu.append(jnp.sum((acc[:8] + acc[8:]) + mx[c][i], axis=0, keepdims=True) * rs)
            hg = 0.5 * gu[0]
            h = jnp.broadcast_to((hg * jnp.tanh(hg) + hg) * gu[1], (8, 128)).astype(BF)
            for n in range(KD):
                t = jnp.dot(h, pltpu.bitcast(w2u[8 * c:8 * c + 8, n].reshape(64, 128), BF),
                            preferred_element_type=F32)[0:1]
                out[n] = t if c == 0 else out[n] + t
        return residual(x, jnp.concatenate(out, axis=1))

    def layer(li, x):
        first = li == 0
        zero_i = li >> 4

        def barrier():
            @pl.when(li > 2)
            def _():
                reset_pipeline()

        mu, xc, rs = moments(x)
        y = jnp.broadcast_to(xc, (8, D))
        for k in range(KD):
            y_scr[k, 0:8, :] = y[:, 128 * k:128 * k + 128].astype(BF)
        rs_scr[0] = jnp.broadcast_to(rs * c2, (8, 128))
        rowd = lax.broadcasted_iota(jnp.int32, (8, D), 0)
        xo = jnp.where(rowd < 4, jnp.broadcast_to(x, (8, D)), 1.0).astype(BF)
        coef = jnp.where(row < 4, 1.0, -mu)

        def q_direct(col):
            t = jnp.dot(xo, pltpu.bitcast(wqu[col], BF), preferred_element_type=F32) * coef
            return (t + pltpu.roll(t, 4, 0)).astype(BF).astype(F32)

        def q_cols(q, slot):
            for b, col in enumerate(columns(q)):
                part[slot + b] = col

        def vpu_a(m, slot, js):
            acc = {}
            for g2 in range(8):
                qc = jnp.concatenate([part[slot + 2 * g2 + t + zero_i] for t in range(2)], axis=0)
                for j in js:
                    tv = f32_rows(kvu[m, 0, 0, g2, j]) * qc
                    acc[j] = tv if g2 == 0 else acc[j] + tv
            for j in js:
                part_a[j // 8, j % 8:j % 8 + 1, :] = jnp.sum(acc[j], axis=0, keepdims=True)

        q0 = [q_direct(c) for c in range(4)]
        q_cols(q0[0], SP)
        set_pat(1, q0[1])
        set_pat(2, q0[2])
        _, qb, qc = qk_ops(0)
        for i in range(nblk // 2):
            if i == 4:
                q_cols(q0[3], SP + 16)
            vpu_a(0, SP, (2 * i, 2 * i + 1))
            plain((qb + qc)[4 * i:4 * i + 4])
        g_softmax(0, 0)
        g_softmax(0, 1)
        plain(qproj_ops(1)[KD:])
        g_query(1)
        g_query(2)
        set_pat(0, q0[3])
        plain(qk_ops(1)[0][PVB:])
        for i in range(0, PVB, 2):
            part[0] = qpart[min(KD + 4 + 3 * i // 2, 3 * KD - 1)]
            vpu_a(1, SP + 16, (i, i + 1))
        toks.clear()

        def block(m, ph):
            @pl.when(first)
            def _():
                kv_wait(m + 2)
                widen(m + 2)

            qp = qproj_ops(m + 2)
            _, qb, qc = qk_ops(m + 1)
            qa = qk_ops(m + 2)[0]
            op = oproj_ops(jnp.maximum(m - 1, 0), m + 2, opart, 8 * ph)
            seq = ([(lambda: g_out(1 - ph),), (lambda: g_olhs(3 * m, 1 - ph),)]
                   + qc[:CF] + qp[:KD] + [(lambda: g_query(0),)] + qc[CF:] + qb
                   + [(lambda: g_softmax(1 - ph, 0),), (lambda: g_softmax(1 - ph, 1),)]
                   + qp[KD:] + [(lambda: g_query(1),), (lambda: g_query(2),)]
                   + op + qa[:nblk - AEND] + [(lambda: fence(pat_u, 3, zero_i),)]
                   + qa[nblk - AEND:])
            emit(pv_ops(m, ph), seq)

        def body(t, carry):
            block(2 * t, 0)
            block(2 * t + 1, 1)
            return carry

        lax.fori_loop(0, NP // 2 - 1, body, 0)

        def big(kts, i0):
            return [op for i, kt in enumerate(kts)
                    for op in oproj_ops(kt, kt + 3, part, SP + KD * (i0 + i))]

        old = list(range(NP - 3, 3 * (NP - 3)))
        barrier()
        _, qb, qc = qk_ops(NP - 1)
        seq = ([(lambda: g_out(1),), (lambda: g_olhs(3 * (NP - 2), 1),)] + qc + qb
               + [(lambda: g_softmax(1, 0),), (lambda: g_softmax(1, 1),)]
               + big(old[:KT14 - 4] + list(range(3 * (NP - 3), 3 * (NP - 2))), 0)
               + [(lambda: fence(olhs_u, 3 * NP, zero_i),)]
               + big(old[KT14 - 4:KT14 - 3], KT14 - 1))
        emit(pv_ops(NP - 2, 0), seq)
        barrier()
        k15 = old[KT14 - 3:-1] + list(range(3 * (NP - 2), 3 * (NP - 1))) + old[-1:]
        emit(pv_ops(NP - 1, 1), [(lambda: g_olhs(3 * (NP - 1), 0),)] + big(k15, KT14))

        def epilogue(x):
            def lsum(g):
                return lane_sum(accx[1, 8 * g:8 * g + 8, :])

            inv = [recip(jnp.sum(lsum(2 * G + par), axis=0, keepdims=True)) for par in range(2)]
            last = [None] * KD
            for par in range(2):
                acc = [None] * KD
                for g2 in range(G2):
                    g = G * par + 2 * g2
                    z = jnp.concatenate([lsum(g), lsum(g + 1)], axis=0)
                    for n in range(KD):
                        tv = f32_rows(wou[(NP - 1) * G + G2 * par + g2, n]) * z
                        acc[n] = tv if g2 == 0 else acc[n] + tv
                for n in range(KD):
                    t = (acc[n][:8] + acc[n][8:]) * inv[par]
                    last[n] = t if par == 0 else last[n] + t
            cols = []
            for n in range(KD):
                t = out_scr[n]
                for i in range(2 * NP):
                    t = t + part[SP + KD * i + n]
                cols.append(jnp.sum(t + last[n], axis=0, keepdims=True))
            return residual(x, jnp.concatenate(cols, axis=1))

        return lax.cond(first, lambda x: ffn1(epilogue(x)), lambda x: ffn2(epilogue(x)), x)

    for r in (y_u, pat_u, olhs_u):
        r[...] = jnp.zeros(r.shape, U32)
    reset_pipeline()
    wait_all([c_x] + c_wq + c_wo)
    for m in range(2):
        kv_wait(m)
        widen(m)
    x = lax.fori_loop(0, 2, layer, xb[...].astype(F32))
    o_ref[...] = x.astype(o_ref.dtype)


@jax.jit
def pallas_interleave_layers__sliding_block_cached__glu_gated_swiglu__decode_kernel(
    A_x: jax.Array,
    A_k_cache: jax.Array,
    A_v_cache: jax.Array,
    A_wq: jax.Array,
    A_wo: jax.Array,
    B_x: jax.Array,
    B_w1: jax.Array,
    B_w3: jax.Array,
    B_w2: jax.Array,
):
    del B_x
    sk = A_k_cache.shape[2]
    win = min(4096, max(256, sk // 4))
    nb = sk // 128
    nblk = win // 128

    def cache_tiles(c):
        return c.reshape(H, nb, 128, G2, 2, 8).transpose(0, 3, 4, 1, 5, 2)

    def weight_tiles(w):
        r, c = w.shape
        return w.reshape(r // 16, 2, 8, c // 128, 128).transpose(0, 1, 3, 2, 4)

    vreg = lambda n: pltpu.VMEM((-(-n // 4) * 4, 8, 128), F32)
    lhs = lambda n: pltpu.VMEM((-(-n // 4) * 4, 16, 128), BF)
    kern = lambda *refs: _kernel(*refs, blk0=nb - nblk, nblk=nblk, scale=DH ** -0.5)
    out = pl.pallas_call(
        kern,
        out_shape=jax.ShapeDtypeStruct((1, D), BF),
        in_specs=[pl.BlockSpec(memory_space=pl.ANY)] * 8,
        out_specs=pl.BlockSpec(memory_space=pltpu.VMEM),
        scratch_shapes=[
            pltpu.VMEM((1, D), BF),
            pltpu.VMEM((NP, 2, 2, G2, nblk, 16, 128), BF),
            pltpu.VMEM((3 * NP, D, 128), BF),
            pltpu.VMEM((H * DH // 16, KD, 16, 128), BF),
            pltpu.VMEM((D // 16, NC, 16, 128), BF),
            pltpu.VMEM((D // 16, NC, 16, 128), BF),
            pltpu.VMEM((FF // 16, KD, 16, 128), BF),
            lhs(KD),
            vreg(1),
            vreg(3 * KD),
            lhs(8),
            vreg(nblk // 8),
            vreg(nblk // 2 + 2 * NP * KD),
            pltpu.VMEM((2, 2, nblk, 128), F32),
            pltpu.VMEM((nblk * 8, 128), F32),
            pltpu.VMEM((2, 64, 128), F32),
            pltpu.VMEM((2, 8 * NR, 128), F32),
            lhs(3 * NP + 4),
            vreg(16),
            vreg(KD),
            pltpu.VMEM((NP, NW, JB, 8, 128), F32),
            pltpu.SemaphoreType.DMA((NP,)),
            pltpu.SemaphoreType.DMA((5 + len(W2_CHUNKS),)),
        ],
        compiler_params=pltpu.CompilerParams(
            vmem_limit_bytes=128 * 1024 * 1024, disable_semaphore_checks=True),
    )(A_x.reshape(1, D), cache_tiles(A_k_cache), cache_tiles(A_v_cache),
      A_wq, weight_tiles(A_wo),
      weight_tiles(B_w1), weight_tiles(B_w3), weight_tiles(B_w2))
    return out.reshape(1, 1, D)
```

```python
import math

import jax
import jax.numpy as jnp
from jax import lax
import jax.experimental.pallas as pl
import jax.experimental.pallas.tpu as pltpu

BF = jnp.bfloat16
F32 = jnp.float32
U32 = jnp.uint32

D = 640
H = 32
DH = 192
G = DH // 8
G2 = DH // 16
NP = H // 2
FF = 1536
EPS = 1e-5
KD = D // 128
NC = FF // 128
NZ = 2 * G + 2
NR = NZ + 2
W2_CHUNKS = (768, 384, 256, 128)

NA = 8
VT = 0
NW = 72
UNPACED = 8
LEAD = 16
RATE = 32.5
TAILC = 30
AEND = 4
CF = 8
KT14 = 10
PVB = 6
KM = 3
FPRE = 6
FSTEP = 3
NST = 17
SC = 9
QB = 4
KVW = 4


def _kernel(x_hbm, k_hbm, v_hbm, wq_hbm, wo_hbm, w1_hbm, w3_hbm, w2_hbm,
            o_ref,
            xb, kvb, wq, wo, w1, w3, w2,
            y_scr, rs_scr, qpart, pat_scr, part_a, part, p_scr, pb_scr, pb0,
            accx, olhs, opart, out_scr, vx, stage,
            kvsem, wsem, ssem, *, blk0, nblk, scale):
    c2 = scale * math.log2(math.e)
    nq = nblk // 8
    SP = 4 * nq

    def kv_copy(m, i):
        return pltpu.make_async_copy(
            (k_hbm, v_hbm)[i].at[pl.ds(2 * m, 2), :, :, pl.ds(blk0 // 2, nblk // 2)],
            kvb.at[m, i], kvsem.at[i, m])

    def wcopies(src, dst, s, r0=0, nr=None):
        nr = src.shape[0] if nr is None else nr
        return [pltpu.make_async_copy(src.at[pl.ds(r0, nr), t],
                                      dst.at[pl.ds(r0, nr), :, pl.ds(8 * t, 8), :],
                                      wsem.at[s]) for t in range(2)]

    c_x = pltpu.make_async_copy(x_hbm, xb, ssem.at[2])
    QA = 3 * NP - QB
    c_wq = [pltpu.make_async_copy(wq_hbm.at[:, pl.ds(128 * c, 128)], wq.at[c],
                                  wsem.at[1 if c < QA else 0]) for c in range(3 * NP)]
    R0 = H * G2 - NST * SC
    c_wo = wcopies(wo_hbm, wo, 2, 0, R0)

    def to_stage(k):
        return pltpu.make_async_copy(wo_hbm.at[pl.ds(R0 + SC * k, SC)], stage.at[k & 1],
                                     ssem.at[0])

    def from_stage(k):
        return [pltpu.make_async_copy(
            stage.at[k & 1, :, t, n], wo.at[pl.ds(R0 + SC * k, SC), n, pl.ds(8 * t, 8), :],
            ssem.at[1]) for t in range(2) for n in range(KD)]

    def stage_step(k, lo=2, hi=None):
        hi = k if hi is None else hi

        def guard(cond_static_true, cond, f):
            if cond_static_true:
                f()
            else:
                pl.when(cond)(f)

        if hi >= 2:
            guard(lo >= 2 and hi <= NST + 1, jnp.logical_and(k >= 2, k <= NST + 1),
                  lambda: wait_all(from_stage(k - 2)))

        def forward():
            to_stage(k - 1).wait()
            for c in from_stage(k - 1):
                c.start()

        if hi >= 1:
            guard(lo >= 1 and hi <= NST, jnp.logical_and(k >= 1, k <= NST), forward)
        guard(hi < NST, k < NST, lambda: to_stage(k).start())

    c_w1 = wcopies(w1_hbm, w1, 3)
    c_w3 = wcopies(w3_hbm, w3, 4)
    w2_off = [sum(W2_CHUNKS[:i]) for i in range(len(W2_CHUNKS))]
    c_w2 = [wcopies(w2_hbm, w2, 5 + i, o // 16, n // 16)
            for i, (o, n) in enumerate(zip(w2_off, W2_CHUNKS))]

    def wait_all(cs):
        for c in cs:
            c.wait()

    c_wq[0].start()
    stage_step(0, 0)
    for c in c_wo + [c_x] + c_wq[1:]:
        c.start()

    def start_ffn_weights():
        for c in c_w1 + c_w3 + [c for cs in c_w2 for c in cs]:
            c.start()

    kvu = kvb.bitcast(U32)
    wqu = wq.bitcast(U32)
    wou = wo.bitcast(U32)
    w1u, w3u, w2u = w1.bitcast(U32), w3.bitcast(U32), w2.bitcast(U32)
    y_u, pat_u, olhs_u = y_scr.bitcast(U32), pat_scr.bitcast(U32), olhs.bitcast(U32)

    def f32_rows(u):
        return pltpu.bitcast(u, BF).astype(F32)

    lane = lax.broadcasted_iota(jnp.int32, (8, 128), 1)
    row = lax.broadcasted_iota(jnp.int32, (8, 128), 0)
    diag_i = ((lane & 7) == row).astype(jnp.int32) * 64
    bit_i = [(lane << (3 - k)) & 64 for k in range(4)]
    uid = [0]

    def lane_sum(v):
        return jnp.broadcast_to(jnp.sum(v, axis=1, keepdims=True), (8, 128))

    def columns(v8):
        uid[0] += 1
        off = 256 * uid[0]
        dl = lane - row + off
        return [lane_sum(jnp.where(dl == off + 8 * b, v8[:, 128 * k:128 * k + 128], 0.0))
                for k in range(v8.shape[1] // 128) for b in range(16)]

    def moments(x):
        mu = jnp.mean(x, axis=-1, keepdims=True)
        xc = x - mu
        return mu, xc, 1.0 / jnp.sqrt(jnp.mean(xc * xc, axis=-1, keepdims=True) + EPS)

    def residual(x, a):
        return (x + a.astype(BF).astype(F32)).astype(BF).astype(F32)

    def matvec(l, wu, r0, nr):
        return [jnp.dot(l, pltpu.bitcast(wu[r0:r0 + nr, c].reshape(8 * nr, 128), BF),
                        preferred_element_type=F32) for c in range(wu.shape[1])]

    def tile_dot(l_u32, w_u32, rows, paced):
        w = pltpu.bitcast(w_u32.reshape(64, 128), BF)
        if paced:
            l = pltpu.bitcast(jnp.concatenate([l_u32, l_u32], axis=0), BF)[:24]
            return jnp.dot(l, w, preferred_element_type=F32)[:rows]
        l = pltpu.bitcast(l_u32, BF)[:rows]
        return jnp.dot(l, w, preferred_element_type=F32)

    def qproj_ops(m):
        def op(paced, c, k):
            qpart[c * KD + k] = tile_dot(
                y_u[k], wqu[3 * m + c, 64 * k:64 * k + 64, :], 8, paced)
        return [(lambda p, c=c, k=k: op(p, c, k)) for c in range(3) for k in range(KD)]

    def oproj_ops(kt, slot, dst, d0):
        def op(paced, n):
            dst[d0 + n] = tile_dot(olhs_u[slot], wou[pl.ds(kt * 8, 8), n], 8, paced)
        return [(lambda p, n=n: op(p, n)) for n in range(KD)]

    def pair_rows(m):
        def body(i, c):
            par, g2 = i // G2, i % G2
            a, b = kvu[m, 0, par, g2, 0], kvu[m, 0, par, g2, 1]
            kvu[m, 0, par, g2, 0] = jnp.concatenate([a[:, :4], b[:, :4]], axis=1)
            kvu[m, 0, par, g2, 1] = jnp.concatenate([a[:, 4:], b[:, 4:]], axis=1)
            return c
        lax.fori_loop(0, 2 * G2, body, 0)

    def k_blocks(m, par, g0, g1, j):
        return kvu[m, 0, par, g0:g1, j & 1, j >> 1]

    jord = [8 * (i // 8) + 2 * (i % 4) + (i % 8) // 4 for i in range(nblk)]

    def qk_ops(m):
        def op_a(paced, j):
            r = tile_dot(pat_u[0], k_blocks(m, 0, 0, 8, j), 8, paced)
            part_a[j // 8, j % 8:j % 8 + 1, :] = r[j % 8:j % 8 + 1, :]

        def op_c(paced, j):
            r = tile_dot(pat_u[2], k_blocks(m, 1, 4, 12, j), 8, paced)
            part[2 * nq + j // 8, j % 8:j % 8 + 1, :] = r[j % 8:j % 8 + 1, :]

        def op_b(paced, j):
            w = jnp.concatenate([k_blocks(m, 0, 8, 12, j), k_blocks(m, 1, 0, 4, j)], axis=0)
            r = tile_dot(pat_u[1], w, 16, paced)
            part[nq + j // 8, j % 8:j % 8 + 1, :] = r[j % 8:j % 8 + 1, :]
            part[3 * nq + j // 8, j % 8:j % 8 + 1, :] = r[8 + j % 8:8 + j % 8 + 1, :]

        return [[(lambda p, f=f, j=j: f(p, j)) for j in jord] for f in (op_a, op_b, op_c)]

    def plain(ops):
        for op in ops:
            op(False)

    steps = [(par, gb, j0) for par in range(2) for gb in range(G // NA)
             for j0 in range(0, nblk, 4)]

    def units(par, gb, j0):
        return [(par, g, j0) for g in range(gb * NA, (gb + 1) * NA)]

    order = [u for s in steps for u in units(*s)]
    wide = {}
    for i, u in enumerate(order):
        if (i + 1) * NW // len(order) > i * NW // len(order):
            wide[u] = len(wide)

    def widen(m):
        for (par, g, j), e in wide.items():
            v = f32_rows(kvu[m, 1, par, g // 2, g % 2, j // 2:j // 2 + 2])
            kvu[m, 1, par, g // 2, g % 2, j // 2:j // 2 + 2] = pltpu.bitcast(v[:, :8], U32)
            vx[m, e] = v[:, 8:]

    def v_unit(m, par, g, j):
        u = kvu[m, 1, par, g // 2, g % 2, j // 2:j // 2 + 2]
        if (par, g, j) in wide:
            return jnp.concatenate([pltpu.bitcast(u, F32), vx[m, wide[(par, g, j)]]], axis=1)
        return f32_rows(u)

    def pv_ops(m, ph):
        acc = {}

        def spread(par, q, r):
            pb_scr[pl.ds(64 * q + r, 8, stride=8), :] = p_scr[ph, par, 8 * q:8 * q + 8, :]

        def psum(par):
            p = p_scr[ph, par]
            accx[ph, 8 * (2 * G + par):8 * (2 * G + par) + 8, :] = (
                (p[0:8] + p[8:16]) + (p[16:24] + p[24:32]))

        pbv = {}

        def piece(par, gb, j0, k):
            if k == 0:
                if par == 0 and j0 < 8:
                    pb = pb0[ph, 8 * j0:8 * j0 + 32, :]
                else:
                    pb = pb_scr[8 * j0:8 * j0 + 32, :]
                pbv[0] = pb.reshape(4, 8, 128)
            for _, g, _ in units(par, gb, j0)[4 * k:4 * k + 4]:
                tv = v_unit(m, par, g, j0).reshape(4, 8, 128) * pbv[0]
                if VT:
                    tv = tv[0:2] + tv[2:4]
                tv = jnp.sum(tv, axis=0)
                acc[g] = tv if j0 == 0 else acc[g] + tv
                if j0 == nblk - 4:
                    r0 = DH * par + 8 * g
                    accx[ph, r0:r0 + 8, :] = acc[g]

        pieces = [s + (k,) for s in steps for k in range(NA // 4)]
        half = len(pieces) // 2
        spq = 2 * (NA // 4)
        side = {}
        for q in range(nq):
            for r in range(8):
                if q:
                    side.setdefault((spq * (8 * (q - 1) + r)) // 9, []).append(
                        lambda q=q, r=r: spread(0, q, r))
                side.setdefault(half - nq * spq + spq * (q + 1) + (r * (3 * spq - 1)) // 8, []).append(
                    lambda q=q, r=r: spread(1, q, r))
        for par in range(2):
            side.setdefault(half // 2 + par, []).append(lambda par=par: psum(par))
        out = []
        for i, s in enumerate(pieces):
            out += [(0, f) for f in side.get(i, [])]
            out.append((2 * sum(4 if u in wide else 6 for u in units(*s[:3])[4 * s[3]:4 * s[3] + 4]),
                        (lambda s=s: piece(*s))))
        return out

    toks = []

    def fence(dst, slot, zero_i):
        for i, t in enumerate(toks):
            dst[slot + i + zero_i] = t
        toks.clear()

    def g_softmax(ph, par):
        s0 = part[2 * nq:3 * nq] if par else part_a[0:nq]
        s = (s0 + part[(2 * par + 1) * nq:(2 * par + 2) * nq]).reshape(nblk, 128)
        mx = jnp.max(jnp.max(s, axis=0, keepdims=True), axis=1, keepdims=True)
        p = jnp.exp2((s - mx) * jnp.concatenate([rs_scr[0]] * nq, axis=0))
        p_scr[ph, par] = p
        if par == 0:
            for r in range(8):
                pb0[ph, pl.ds(r, 8, stride=8), :] = p[0:8]
        toks.append(pltpu.bitcast(p[nblk - 8:nblk], U32))

    def recip(d):
        r = pl.reciprocal(d, approx=True)
        return r * (2.0 - d * r)

    def g_olhs(slot0, ph):
        z = [lane_sum(accx[ph, 8 * g:8 * g + 8, :]) for g in range(NZ)]
        inv = [jnp.broadcast_to(recip(jnp.sum(z[2 * G + par], axis=0, keepdims=True)), (8, 128))
               for par in range(2)]
        uid[0] += 1
        bit = [b > uid[0] for b in bit_i]
        for c in range(3):
            xs = z[16 * c:16 * c + 16]
            for k in range(4):
                xs = [jnp.where(bit[k], xs[i + 1], xs[i]) for i in range(0, len(xs), 2)]
            iv = inv[0] if c == 0 else (inv[1] if c == 2 else jnp.where(bit[3], inv[1], inv[0]))
            olhs[slot0 + c, 0:8, :] = jnp.where(diag_i > uid[0], xs[0] * iv, 0.0).astype(BF)

    def set_pat(c, q):
        if c == 1:
            hi = bit_i[3] > uid[0]
            pat_scr[c, 0:8, :] = jnp.where(hi, 0.0, q).astype(BF)
            pat_scr[c, 8:16, :] = jnp.where(hi, q, 0.0).astype(BF)
        else:
            pat_scr[c, 0:8, :] = q.astype(BF)
        if c > 0:
            toks.append(pltpu.bitcast(q, U32))

    def g_query(c):
        xs = [qpart[c * KD + k] for k in range(KD)]
        set_pat(c, ((xs[0] + xs[1]) + (xs[2] + xs[3])) + xs[4])

    def g_out(ph):
        for n in range(KD):
            out_scr[n] = out_scr[n] + opart[8 * ph + n]

    def reset_pipeline():
        accx[1, 0:16 * G, :] = jnp.zeros((16 * G, 128), F32)
        accx[1, 16 * G:16 * G + 16, :] = jnp.ones((16, 128), F32)
        for n in range(KD):
            opart[8 + n] = jnp.zeros((8, 128), F32)
            out_scr[n] = jnp.zeros((8, 128), F32)

    def emit(pv, seq):
        ntile = sum(not isinstance(e, tuple) for e in seq)
        total = sum(w for w, _ in pv) / 4
        k = done = n = 0
        for e in seq:
            if isinstance(e, tuple):
                e[0]()
                continue
            pos = LEAD + RATE * (n // 4) if n // 4 < (ntile - 1) // 4 else total - TAILC
            while k < len(pv) and done + pv[k][0] / 2 <= 4 * pos:
                done += pv[k][0]
                pv[k][1]()
                k += 1
            e(n < ntile - UNPACED)
            n += 1
        for _, g in pv[k:]:
            g()

    def ffn1(x):
        _, xc, rs = moments(x)
        y = jnp.broadcast_to(xc, (8, D)).astype(BF)
        reset_pipeline()
        wait_all(c_w1)
        g = jnp.concatenate(matvec(y, w1u, 0, D // 16), axis=1) * rs
        wait_all(c_w3)
        u = jnp.concatenate(matvec(y, w3u, 0, D // 16), axis=1) * rs
        hh = (g * jax.nn.sigmoid(g) * u).astype(BF)
        hb = columns(hh[:, w2_off[-1]:].astype(F32))
        a = None
        for cs, o, n in list(zip(c_w2, w2_off, W2_CHUNKS))[:-1]:
            wait_all(cs)
            t = jnp.concatenate(matvec(hh[:, o:o + n], w2u, o // 16, n // 16), axis=1)[0:1]
            a = t if a is None else a + t
        wait_all(c_w2[-1])
        acc = [None] * KD
        for r in range(W2_CHUNKS[-1] // 16):
            for c in range(KD):
                v = f32_rows(w2u[w2_off[-1] // 16 + r, c])
                tv = v[:8] * hb[2 * r] + v[8:] * hb[2 * r + 1]
                acc[c] = tv if r == 0 else acc[c] + tv
        a = a + jnp.concatenate([jnp.sum(t, axis=0, keepdims=True) for t in acc], axis=1)
        return residual(x, a)

    def ffn2(x):
        mu, _, rs = moments(x)
        x8 = jnp.broadcast_to(x, (8, D))
        rowk = lax.broadcasted_iota(jnp.int32, (8, 128 * KM), 0)
        y = jnp.where(rowk == 0, x8[:, :128 * KM], jnp.where(rowk == 1, 1.0, 0.0)).astype(BF)
        coef = jnp.where(row == 0, 1.0, -mu)
        yb = jnp.concatenate([c - mu for c in columns(x8[:, 128 * KM:])], axis=0)
        mx = {}
        out = [None] * KD
        for c in range(NC):
            while len(mx) < min(NC, FPRE + c * FSTEP / 4):
                cc = len(mx)
                mx[cc] = [jnp.dot(y, pltpu.bitcast(wu[0:8 * KM, cc].reshape(64 * KM, 128), BF),
                                  preferred_element_type=F32) * coef for wu in (w1u, w3u)]
            gu = []
            for i, wu in enumerate((w1u, w3u)):
                acc = None
                for r in range(8 * (KD - KM)):
                    tv = f32_rows(wu[8 * KM + r, c]) * yb[16 * r:16 * r + 16]
                    acc = tv if r == 0 else acc + tv
                gu.append(jnp.sum((acc[:8] + acc[8:]) + mx[c][i], axis=0, keepdims=True) * rs)
            hg = 0.5 * gu[0]
            h = jnp.broadcast_to((hg * jnp.tanh(hg) + hg) * gu[1], (8, 128)).astype(BF)
            for n in range(KD):
                t = jnp.dot(h, pltpu.bitcast(w2u[8 * c:8 * c + 8, n].reshape(64, 128), BF),
                            preferred_element_type=F32)[0:1]
                out[n] = t if c == 0 else out[n] + t
        return residual(x, jnp.concatenate(out, axis=1))

    def layer(li, x):
        first = li == 0
        zero_i = li >> 4

        def barrier():
            @pl.when(li > 2)
            def _():
                reset_pipeline()

        mu, xc, rs = moments(x)
        y = jnp.broadcast_to(xc, (8, D))
        for k in range(KD):
            y_scr[k, 0:8, :] = y[:, 128 * k:128 * k + 128].astype(BF)
        rs_scr[0] = jnp.broadcast_to(rs * c2, (8, 128))
        rowd = lax.broadcasted_iota(jnp.int32, (8, D), 0)
        xo = jnp.where(rowd < 4, jnp.broadcast_to(x, (8, D)), 1.0).astype(BF)
        coef = jnp.where(row < 4, 1.0, -mu)

        def q_direct(col):
            t = jnp.dot(xo, pltpu.bitcast(wqu[col], BF), preferred_element_type=F32) * coef
            return (t + pltpu.roll(t, 4, 0)).astype(BF).astype(F32)

        def q_cols(q, slot):
            for b, col in enumerate(columns(q)):
                part[slot + b] = col

        def vpu_a(m, slot, js):
            acc = {}
            for g2 in range(8):
                qc = jnp.concatenate([part[slot + 2 * g2 + t + zero_i] for t in range(2)], axis=0)
                for j in js:
                    tv = f32_rows(kvu[m, 0, 0, g2, j & 1, j >> 1]) * qc
                    acc[j] = tv if g2 == 0 else acc[j] + tv
            for j in js:
                part_a[j // 8, j % 8:j % 8 + 1, :] = jnp.sum(acc[j], axis=0, keepdims=True)

        q0 = [q_direct(c) for c in range(4)]
        q_cols(q0[0], SP)
        set_pat(1, q0[1])
        set_pat(2, q0[2])
        _, qb, qc = qk_ops(0)
        for i in range(nblk // 2):
            if i == 4:
                q_cols(q0[3], SP + 16)
            vpu_a(0, SP, jord[2 * i:2 * i + 2])
            plain((qb + qc)[4 * i:4 * i + 4])
        g_softmax(0, 0)
        g_softmax(0, 1)
        plain(qproj_ops(1)[KD:])
        g_query(1)
        g_query(2)
        set_pat(0, q0[3])
        plain(qk_ops(1)[0][PVB:])
        for i in range(0, PVB, 2):
            part[0] = qpart[min(KD + 4 + 3 * i // 2, 3 * KD - 1)]
            vpu_a(1, SP + 16, jord[i:i + 2])
        toks.clear()

        def block(m, ph):
            @pl.when(first)
            def _():
                kv_copy(m + 2, 0).wait()
                if ph == 1:
                    pl.when(m + 3 == NP)(start_ffn_weights)
                pair_rows(m + 2)
                kv_copy(m + 2, 1).wait()
                stage_step(m + 5, 5, NP + 2)

                @pl.when(m + 2 + KVW < NP)
                def _():
                    for i in range(2):
                        kv_copy(m + 2 + KVW, i).start()

                widen(m + 2)

            qp = qproj_ops(m + 2)
            _, qb, qc = qk_ops(m + 1)
            qa = qk_ops(m + 2)[0]
            op = oproj_ops(jnp.maximum(m - 1, 0), m + 2, opart, 8 * ph)
            seq = ([(lambda: g_out(1 - ph),), (lambda: g_olhs(3 * m, 1 - ph),)]
                   + qc[:CF] + qp[:KD] + [(lambda: g_query(0),)] + qc[CF:] + qb
                   + [(lambda: g_softmax(1 - ph, 0),), (lambda: g_softmax(1 - ph, 1),)]
                   + qp[KD:] + [(lambda: g_query(1),), (lambda: g_query(2),)]
                   + op + qa[:nblk - AEND] + [(lambda: fence(pat_u, 3, zero_i),)]
                   + qa[nblk - AEND:])
            emit(pv_ops(m, ph), seq)

        def body(t, carry):
            block(2 * t, 0)
            block(2 * t + 1, 1)
            return carry

        lax.fori_loop(0, NP // 2 - 1, body, 0)

        def big(kts, i0):
            return [op for i, kt in enumerate(kts)
                    for op in oproj_ops(kt, kt + 3, part, SP + KD * (i0 + i))]

        old = list(range(NP - 3, 3 * (NP - 3)))
        barrier()
        _, qb, qc = qk_ops(NP - 1)
        seq = ([(lambda: g_out(1),), (lambda: g_olhs(3 * (NP - 2), 1),)] + qc + qb
               + [(lambda: g_softmax(1, 0),), (lambda: g_softmax(1, 1),)]
               + big(old[:KT14 - 4] + list(range(3 * (NP - 3), 3 * (NP - 2))), 0)
               + [(lambda: fence(olhs_u, 3 * NP, zero_i),)]
               + big(old[KT14 - 4:KT14 - 3], KT14 - 1))
        emit(pv_ops(NP - 2, 0), seq)
        barrier()
        k15 = old[KT14 - 3:-1] + list(range(3 * (NP - 2), 3 * (NP - 1))) + old[-1:]
        emit(pv_ops(NP - 1, 1), [(lambda: g_olhs(3 * (NP - 1), 0),)] + big(k15, KT14))

        def epilogue(x):
            def lsum(g):
                return lane_sum(accx[1, 8 * g:8 * g + 8, :])

            inv = [recip(jnp.sum(lsum(2 * G + par), axis=0, keepdims=True)) for par in range(2)]
            last = [None] * KD
            for par in range(2):
                acc = [None] * KD
                for g2 in range(G2):
                    g = G * par + 2 * g2
                    z = jnp.concatenate([lsum(g), lsum(g + 1)], axis=0)
                    for n in range(KD):
                        tv = f32_rows(wou[(NP - 1) * G + G2 * par + g2, n]) * z
                        acc[n] = tv if g2 == 0 else acc[n] + tv
                for n in range(KD):
                    t = (acc[n][:8] + acc[n][8:]) * inv[par]
                    last[n] = t if par == 0 else last[n] + t
            cols = []
            for n in range(KD):
                t = out_scr[n]
                for i in range(2 * NP):
                    t = t + part[SP + KD * i + n]
                cols.append(jnp.sum(t + last[n], axis=0, keepdims=True))
            return residual(x, jnp.concatenate(cols, axis=1))

        return lax.cond(first, lambda x: ffn1(epilogue(x)), lambda x: ffn2(epilogue(x)), x)

    for r in (y_u, pat_u, olhs_u):
        r[...] = jnp.zeros(r.shape, U32)
    reset_pipeline()
    wait_all(c_wo)
    stage_step(1, 1)
    wait_all(c_wq[:QA])
    for m in range(KVW + 2):
        for i in range(2):
            kv_copy(m, i).start()
    stage_step(2)
    for m in range(2):
        kv_copy(m, 0).wait()
        pair_rows(m)
        kv_copy(m, 1).wait()
        stage_step(3 + m)
        widen(m)
    wait_all([c_x] + c_wq[QA:])
    x = lax.fori_loop(0, 2, layer, xb[...].astype(F32))
    o_ref[...] = x.astype(o_ref.dtype)


@jax.jit
def pallas_interleave_layers__sliding_block_cached__glu_gated_swiglu__decode_kernel(
    A_x: jax.Array,
    A_k_cache: jax.Array,
    A_v_cache: jax.Array,
    A_wq: jax.Array,
    A_wo: jax.Array,
    B_x: jax.Array,
    B_w1: jax.Array,
    B_w3: jax.Array,
    B_w2: jax.Array,
):
    del B_x
    sk = A_k_cache.shape[2]
    win = min(4096, max(256, sk // 4))
    nb = sk // 128
    nblk = win // 128

    def cache_tiles(c):
        return (c.reshape(H, nb, 128, G2, 2, 8).transpose(0, 3, 4, 1, 5, 2)
                .reshape(H, G2, 2, nb // 2, 16, 128))

    def weight_tiles(w):
        r, c = w.shape
        return w.reshape(r // 16, 2, 8, c // 128, 128).transpose(0, 1, 3, 2, 4)

    vreg = lambda n: pltpu.VMEM((-(-n // 4) * 4, 8, 128), F32)
    lhs = lambda n: pltpu.VMEM((-(-n // 4) * 4, 16, 128), BF)
    kern = lambda *refs: _kernel(*refs, blk0=nb - nblk, nblk=nblk, scale=DH ** -0.5)
    out = pl.pallas_call(
        kern,
        out_shape=jax.ShapeDtypeStruct((1, D), BF),
        in_specs=[pl.BlockSpec(memory_space=pl.ANY)] * 8,
        out_specs=pl.BlockSpec(memory_space=pltpu.VMEM),
        scratch_shapes=[
            pltpu.VMEM((1, D), BF),
            pltpu.VMEM((NP, 2, 2, G2, 2, nblk // 2, 16, 128), BF),
            pltpu.VMEM((3 * NP, D, 128), BF),
            pltpu.VMEM((H * DH // 16, KD, 16, 128), BF),
            pltpu.VMEM((D // 16, NC, 16, 128), BF),
            pltpu.VMEM((D // 16, NC, 16, 128), BF),
            pltpu.VMEM((FF // 16, KD, 16, 128), BF),
            lhs(KD),
            vreg(1),
            vreg(3 * KD),
            lhs(8),
            vreg(nblk // 8),
            vreg(nblk // 2 + 2 * NP * KD),
            pltpu.VMEM((2, 2, nblk, 128), F32),
            pltpu.VMEM((nblk * 8, 128), F32),
            pltpu.VMEM((2, 64, 128), F32),
            pltpu.VMEM((2, 8 * NR, 128), F32),
            lhs(3 * NP + 4),
            vreg(16),
            vreg(KD),
            pltpu.VMEM((NP, NW, 2, 8, 128), F32),
            pltpu.SMEM((2, SC, 2, KD, 8, 128), BF),
            pltpu.SemaphoreType.DMA((2, NP)),
            pltpu.SemaphoreType.DMA((5 + len(W2_CHUNKS),)),
            pltpu.SemaphoreType.DMA((3,)),
        ],
        compiler_params=pltpu.CompilerParams(
            vmem_limit_bytes=128 * 1024 * 1024, disable_semaphore_checks=True),
    )(A_x.reshape(1, D), cache_tiles(A_k_cache), cache_tiles(A_v_cache),
      A_wq, weight_tiles(A_wo),
      weight_tiles(B_w1), weight_tiles(B_w3), weight_tiles(B_w2))
    return out.reshape(1, 1, D)
```

```python
import math

import jax
import jax.numpy as jnp
from jax import lax
import jax.experimental.pallas as pl
import jax.experimental.pallas.tpu as pltpu

BF = jnp.bfloat16
F32 = jnp.float32
U32 = jnp.uint32

D = 640
H = 32
DH = 192
G = DH // 8
G2 = DH // 16
NP = H // 2
FF = 1536
EPS = 1e-5
KD = D // 128
NC = FF // 128
NZ = 2 * G + 2
NR = NZ + 2
W2_CHUNKS = (768, 384, 256, 128)

NA = 8
VT = 0
NW = 72
UNPACED = 8
LEAD = 16
RATE = 32.5
TAILC = 30
AEND = 4
CF = 8
KT14 = 10
PVB = 6
KM = 3
FPRE = 6
FSTEP = 3
NST = 17
SC = 10
QB = 4
KVW = 4
Q0 = 16


def _kernel(x_hbm, k_hbm, v_hbm, wq_hbm, wo_hbm, w1_hbm, w3_hbm, w2_hbm,
            o_ref,
            xb, kvb, wq, wo, w1, w3, w2,
            y_scr, rs_scr, qpart, pat_scr, part_a, part, p_scr, pb_scr, pb0,
            accx, olhs, opart, out_scr, vx, stage,
            kvsem, wsem, ssem, *, blk0, nblk, scale):
    c2 = scale * math.log2(math.e)
    nq = nblk // 8
    SP = 4 * nq

    def kv_copy(m, i):
        return pltpu.make_async_copy(
            (k_hbm, v_hbm)[i].at[pl.ds(2 * m, 2), :, :, pl.ds(blk0 // 2, nblk // 2)],
            kvb.at[m, i], kvsem.at[i, m])

    def wcopies(src, dst, s, r0=0, nr=None):
        nr = src.shape[0] if nr is None else nr
        return [pltpu.make_async_copy(src.at[pl.ds(r0, nr), t],
                                      dst.at[pl.ds(r0, nr), :, pl.ds(8 * t, 8), :],
                                      wsem.at[s]) for t in range(2)]

    c_x = pltpu.make_async_copy(x_hbm, xb, ssem.at[2])
    QA = 3 * NP - QB
    c_wq = [pltpu.make_async_copy(wq_hbm.at[:, pl.ds(128 * c, 128)], wq.at[c],
                                  wsem.at[1 if c < QA else 0]) for c in range(3 * NP)]
    R0 = H * G2 - NST * SC
    c_wo = wcopies(wo_hbm, wo, 2, 0, R0)

    def to_stage(k):
        return pltpu.make_async_copy(wo_hbm.at[pl.ds(R0 + SC * k, SC)], stage.at[k & 1],
                                     ssem.at[0])

    def from_stage(k):
        return [pltpu.make_async_copy(
            stage.at[k & 1, :, t, n], wo.at[pl.ds(R0 + SC * k, SC), n, pl.ds(8 * t, 8), :],
            ssem.at[1]) for t in range(2) for n in range(KD)]

    def stage_step(k, lo=2, hi=None):
        hi = k if hi is None else hi

        def guard(cond_static_true, cond, f):
            if cond_static_true:
                f()
            else:
                pl.when(cond)(f)

        if hi >= 2:
            guard(lo >= 2 and hi <= NST + 1, jnp.logical_and(k >= 2, k <= NST + 1),
                  lambda: wait_all(from_stage(k - 2)))

        def forward():
            to_stage(k - 1).wait()
            for c in from_stage(k - 1):
                c.start()

        if hi >= 1:
            guard(lo >= 1 and hi <= NST, jnp.logical_and(k >= 1, k <= NST), forward)
        guard(hi < NST, k < NST, lambda: to_stage(k).start())

    c_w1 = wcopies(w1_hbm, w1, 3)
    c_w3 = wcopies(w3_hbm, w3, 4)
    w2_off = [sum(W2_CHUNKS[:i]) for i in range(len(W2_CHUNKS))]
    c_w2 = [wcopies(w2_hbm, w2, 5 + i, o // 16, n // 16)
            for i, (o, n) in enumerate(zip(w2_off, W2_CHUNKS))]

    def wait_all(cs):
        for c in cs:
            c.wait()

    c_wo[0].start()
    stage_step(0, 0)
    for c in c_wo[1:] + [c_x] + c_wq[:Q0]:
        c.start()

    def start_ffn_weights():
        for c in c_w1 + c_w3 + [c for cs in c_w2 for c in cs]:
            c.start()

    kvu = kvb.bitcast(U32)
    wqu = wq.bitcast(U32)
    wou = wo.bitcast(U32)
    w1u, w3u, w2u = w1.bitcast(U32), w3.bitcast(U32), w2.bitcast(U32)
    y_u, pat_u, olhs_u = y_scr.bitcast(U32), pat_scr.bitcast(U32), olhs.bitcast(U32)

    def f32_rows(u):
        return pltpu.bitcast(u, BF).astype(F32)

    lane = lax.broadcasted_iota(jnp.int32, (8, 128), 1)
    row = lax.broadcasted_iota(jnp.int32, (8, 128), 0)
    diag_i = ((lane & 7) == row).astype(jnp.int32) * 64
    bit_i = [(lane << (3 - k)) & 64 for k in range(4)]
    uid = [0]

    def lane_sum(v):
        return jnp.broadcast_to(jnp.sum(v, axis=1, keepdims=True), (8, 128))

    def columns(v8):
        uid[0] += 1
        off = 256 * uid[0]
        dl = lane - row + off
        return [lane_sum(jnp.where(dl == off + 8 * b, v8[:, 128 * k:128 * k + 128], 0.0))
                for k in range(v8.shape[1] // 128) for b in range(16)]

    def moments(x):
        mu = jnp.mean(x, axis=-1, keepdims=True)
        xc = x - mu
        return mu, xc, 1.0 / jnp.sqrt(jnp.mean(xc * xc, axis=-1, keepdims=True) + EPS)

    def residual(x, a):
        return (x + a.astype(BF).astype(F32)).astype(BF).astype(F32)

    def matvec(l, wu, r0, nr):
        return [jnp.dot(l, pltpu.bitcast(wu[r0:r0 + nr, c].reshape(8 * nr, 128), BF),
                        preferred_element_type=F32) for c in range(wu.shape[1])]

    def tile_dot(l_u32, w_u32, rows, paced):
        w = pltpu.bitcast(w_u32.reshape(64, 128), BF)
        if paced:
            l = pltpu.bitcast(jnp.concatenate([l_u32, l_u32], axis=0), BF)[:24]
            return jnp.dot(l, w, preferred_element_type=F32)[:rows]
        l = pltpu.bitcast(l_u32, BF)[:rows]
        return jnp.dot(l, w, preferred_element_type=F32)

    def qproj_ops(m):
        def op(paced, c, k):
            qpart[c * KD + k] = tile_dot(
                y_u[k], wqu[3 * m + c, 64 * k:64 * k + 64, :], 8, paced)
        return [(lambda p, c=c, k=k: op(p, c, k)) for c in range(3) for k in range(KD)]

    def oproj_ops(kt, slot, dst, d0):
        def op(paced, n):
            dst[d0 + n] = tile_dot(olhs_u[slot], wou[pl.ds(kt * 8, 8), n], 8, paced)
        return [(lambda p, n=n: op(p, n)) for n in range(KD)]

    def pair_rows(m):
        def body(i, c):
            par, g2 = i // G2, i % G2
            a, b = kvu[m, 0, par, g2, 0], kvu[m, 0, par, g2, 1]
            kvu[m, 0, par, g2, 0] = jnp.concatenate([a[:, :4], b[:, :4]], axis=1)
            kvu[m, 0, par, g2, 1] = jnp.concatenate([a[:, 4:], b[:, 4:]], axis=1)
            return c
        lax.fori_loop(0, 2 * G2, body, 0)

    def k_blocks(m, par, g0, g1, j):
        return kvu[m, 0, par, g0:g1, j & 1, j >> 1]

    jord = [8 * (i // 8) + 2 * (i % 4) + (i % 8) // 4 for i in range(nblk)]

    def qk_ops(m):
        def op_a(paced, j):
            r = tile_dot(pat_u[0], k_blocks(m, 0, 0, 8, j), 8, paced)
            part_a[j // 8, j % 8:j % 8 + 1, :] = r[j % 8:j % 8 + 1, :]

        def op_c(paced, j):
            r = tile_dot(pat_u[2], k_blocks(m, 1, 4, 12, j), 8, paced)
            part[2 * nq + j // 8, j % 8:j % 8 + 1, :] = r[j % 8:j % 8 + 1, :]

        def op_b(paced, j):
            w = jnp.concatenate([k_blocks(m, 0, 8, 12, j), k_blocks(m, 1, 0, 4, j)], axis=0)
            r = tile_dot(pat_u[1], w, 16, paced)
            part[nq + j // 8, j % 8:j % 8 + 1, :] = r[j % 8:j % 8 + 1, :]
            part[3 * nq + j // 8, j % 8:j % 8 + 1, :] = r[8 + j % 8:8 + j % 8 + 1, :]

        return [[(lambda p, f=f, j=j: f(p, j)) for j in jord] for f in (op_a, op_b, op_c)]

    def plain(ops):
        for op in ops:
            op(False)

    steps = [(par, gb, j0) for par in range(2) for gb in range(G // NA)
             for j0 in range(0, nblk, 4)]

    def units(par, gb, j0):
        return [(par, g, j0) for g in range(gb * NA, (gb + 1) * NA)]

    order = [u for s in steps for u in units(*s)]
    wide = {}
    for i, u in enumerate(order):
        if (i + 1) * NW // len(order) > i * NW // len(order):
            wide[u] = len(wide)

    def widen(m):
        for (par, g, j), e in wide.items():
            v = f32_rows(kvu[m, 1, par, g // 2, g % 2, j // 2:j // 2 + 2])
            kvu[m, 1, par, g // 2, g % 2, j // 2:j // 2 + 2] = pltpu.bitcast(v[:, :8], U32)
            vx[m, e] = v[:, 8:]

    def v_unit(m, par, g, j):
        u = kvu[m, 1, par, g // 2, g % 2, j // 2:j // 2 + 2]
        if (par, g, j) in wide:
            return jnp.concatenate([pltpu.bitcast(u, F32), vx[m, wide[(par, g, j)]]], axis=1)
        return f32_rows(u)

    def pv_ops(m, ph):
        acc = {}

        def spread(par, q, r):
            pb_scr[pl.ds(64 * q + r, 8, stride=8), :] = p_scr[ph, par, 8 * q:8 * q + 8, :]

        def psum(par):
            p = p_scr[ph, par]
            accx[ph, 8 * (2 * G + par):8 * (2 * G + par) + 8, :] = (
                (p[0:8] + p[8:16]) + (p[16:24] + p[24:32]))

        pbv = {}

        def piece(par, gb, j0, k):
            if k == 0:
                if par == 0 and j0 < 8:
                    pb = pb0[ph, 8 * j0:8 * j0 + 32, :]
                else:
                    pb = pb_scr[8 * j0:8 * j0 + 32, :]
                pbv[0] = pb.reshape(4, 8, 128)
            for _, g, _ in units(par, gb, j0)[4 * k:4 * k + 4]:
                tv = v_unit(m, par, g, j0).reshape(4, 8, 128) * pbv[0]
                if VT:
                    tv = tv[0:2] + tv[2:4]
                tv = jnp.sum(tv, axis=0)
                acc[g] = tv if j0 == 0 else acc[g] + tv
                if j0 == nblk - 4:
                    r0 = DH * par + 8 * g
                    accx[ph, r0:r0 + 8, :] = acc[g]

        pieces = [s + (k,) for s in steps for k in range(NA // 4)]
        half = len(pieces) // 2
        spq = 2 * (NA // 4)
        side = {}
        for q in range(nq):
            for r in range(8):
                if q:
                    side.setdefault((spq * (8 * (q - 1) + r)) // 9, []).append(
                        lambda q=q, r=r: spread(0, q, r))
                side.setdefault(half - nq * spq + spq * (q + 1) + (r * (3 * spq - 1)) // 8, []).append(
                    lambda q=q, r=r: spread(1, q, r))
        for par in range(2):
            side.setdefault(half // 2 + par, []).append(lambda par=par: psum(par))
        out = []
        for i, s in enumerate(pieces):
            out += [(0, f) for f in side.get(i, [])]
            out.append((2 * sum(4 if u in wide else 6 for u in units(*s[:3])[4 * s[3]:4 * s[3] + 4]),
                        (lambda s=s: piece(*s))))
        return out

    toks = []

    def fence(dst, slot, zero_i):
        for i, t in enumerate(toks):
            dst[slot + i + zero_i] = t
        toks.clear()

    def g_softmax(ph, par):
        s0 = part[2 * nq:3 * nq] if par else part_a[0:nq]
        s = (s0 + part[(2 * par + 1) * nq:(2 * par + 2) * nq]).reshape(nblk, 128)
        mx = jnp.max(jnp.max(s, axis=0, keepdims=True), axis=1, keepdims=True)
        p = jnp.exp2((s - mx) * jnp.concatenate([rs_scr[0]] * nq, axis=0))
        p_scr[ph, par] = p
        if par == 0:
            for r in range(8):
                pb0[ph, pl.ds(r, 8, stride=8), :] = p[0:8]
        toks.append(pltpu.bitcast(p[nblk - 8:nblk], U32))

    def recip(d):
        r = pl.reciprocal(d, approx=True)
        return r * (2.0 - d * r)

    def g_olhs(slot0, ph):
        z = [lane_sum(accx[ph, 8 * g:8 * g + 8, :]) for g in range(NZ)]
        inv = [jnp.broadcast_to(recip(jnp.sum(z[2 * G + par], axis=0, keepdims=True)), (8, 128))
               for par in range(2)]
        uid[0] += 1
        bit = [b > uid[0] for b in bit_i]
        for c in range(3):
            xs = z[16 * c:16 * c + 16]
            for k in range(4):
                xs = [jnp.where(bit[k], xs[i + 1], xs[i]) for i in range(0, len(xs), 2)]
            iv = inv[0] if c == 0 else (inv[1] if c == 2 else jnp.where(bit[3], inv[1], inv[0]))
            olhs[slot0 + c, 0:8, :] = jnp.where(diag_i > uid[0], xs[0] * iv, 0.0).astype(BF)

    def set_pat(c, q):
        if c == 1:
            hi = bit_i[3] > uid[0]
            pat_scr[c, 0:8, :] = jnp.where(hi, 0.0, q).astype(BF)
            pat_scr[c, 8:16, :] = jnp.where(hi, q, 0.0).astype(BF)
        else:
            pat_scr[c, 0:8, :] = q.astype(BF)
        if c > 0:
            toks.append(pltpu.bitcast(q, U32))

    def g_query(c):
        xs = [qpart[c * KD + k] for k in range(KD)]
        set_pat(c, ((xs[0] + xs[1]) + (xs[2] + xs[3])) + xs[4])

    def g_out(ph):
        for n in range(KD):
            out_scr[n] = out_scr[n] + opart[8 * ph + n]

    def reset_pipeline():
        accx[1, 0:16 * G, :] = jnp.zeros((16 * G, 128), F32)
        accx[1, 16 * G:16 * G + 16, :] = jnp.ones((16, 128), F32)
        for n in range(KD):
            opart[8 + n] = jnp.zeros((8, 128), F32)
            out_scr[n] = jnp.zeros((8, 128), F32)

    def emit(pv, seq):
        ntile = sum(not isinstance(e, tuple) for e in seq)
        total = sum(w for w, _ in pv) / 4
        k = done = n = 0
        for e in seq:
            if isinstance(e, tuple):
                e[0]()
                continue
            pos = LEAD + RATE * (n // 4) if n // 4 < (ntile - 1) // 4 else total - TAILC
            while k < len(pv) and done + pv[k][0] / 2 <= 4 * pos:
                done += pv[k][0]
                pv[k][1]()
                k += 1
            e(n < ntile - UNPACED)
            n += 1
        for _, g in pv[k:]:
            g()

    def ffn1(x):
        _, xc, rs = moments(x)
        y = jnp.broadcast_to(xc, (8, D)).astype(BF)
        reset_pipeline()
        wait_all(c_w1)
        g = jnp.concatenate(matvec(y, w1u, 0, D // 16), axis=1) * rs
        wait_all(c_w3)
        u = jnp.concatenate(matvec(y, w3u, 0, D // 16), axis=1) * rs
        hh = (g * jax.nn.sigmoid(g) * u).astype(BF)
        hb = columns(hh[:, w2_off[-1]:].astype(F32))
        a = None
        for cs, o, n in list(zip(c_w2, w2_off, W2_CHUNKS))[:-1]:
            wait_all(cs)
            t = jnp.concatenate(matvec(hh[:, o:o + n], w2u, o // 16, n // 16), axis=1)[0:1]
            a = t if a is None else a + t
        wait_all(c_w2[-1])
        acc = [None] * KD
        for r in range(W2_CHUNKS[-1] // 16):
            for c in range(KD):
                v = f32_rows(w2u[w2_off[-1] // 16 + r, c])
                tv = v[:8] * hb[2 * r] + v[8:] * hb[2 * r + 1]
                acc[c] = tv if r == 0 else acc[c] + tv
        a = a + jnp.concatenate([jnp.sum(t, axis=0, keepdims=True) for t in acc], axis=1)
        return residual(x, a)

    def ffn2(x):
        mu, _, rs = moments(x)
        x8 = jnp.broadcast_to(x, (8, D))
        rowk = lax.broadcasted_iota(jnp.int32, (8, 128 * KM), 0)
        y = jnp.where(rowk == 0, x8[:, :128 * KM], jnp.where(rowk == 1, 1.0, 0.0)).astype(BF)
        coef = jnp.where(row == 0, 1.0, -mu)
        yb = jnp.concatenate([c - mu for c in columns(x8[:, 128 * KM:])], axis=0)
        mx = {}
        out = [None] * KD
        for c in range(NC):
            while len(mx) < min(NC, FPRE + c * FSTEP / 4):
                cc = len(mx)
                mx[cc] = [jnp.dot(y, pltpu.bitcast(wu[0:8 * KM, cc].reshape(64 * KM, 128), BF),
                                  preferred_element_type=F32) * coef for wu in (w1u, w3u)]
            gu = []
            for i, wu in enumerate((w1u, w3u)):
                acc = None
                for r in range(8 * (KD - KM)):
                    tv = f32_rows(wu[8 * KM + r, c]) * yb[16 * r:16 * r + 16]
                    acc = tv if r == 0 else acc + tv
                gu.append(jnp.sum((acc[:8] + acc[8:]) + mx[c][i], axis=0, keepdims=True) * rs)
            hg = 0.5 * gu[0]
            h = jnp.broadcast_to((hg * jnp.tanh(hg) + hg) * gu[1], (8, 128)).astype(BF)
            for n in range(KD):
                t = jnp.dot(h, pltpu.bitcast(w2u[8 * c:8 * c + 8, n].reshape(64, 128), BF),
                            preferred_element_type=F32)[0:1]
                out[n] = t if c == 0 else out[n] + t
        return residual(x, jnp.concatenate(out, axis=1))

    def layer(li, x):
        first = li == 0
        zero_i = li >> 4

        def barrier():
            @pl.when(li > 2)
            def _():
                reset_pipeline()

        mu, xc, rs = moments(x)
        y = jnp.broadcast_to(xc, (8, D))
        for k in range(KD):
            y_scr[k, 0:8, :] = y[:, 128 * k:128 * k + 128].astype(BF)
        rs_scr[0] = jnp.broadcast_to(rs * c2, (8, 128))
        rowd = lax.broadcasted_iota(jnp.int32, (8, D), 0)
        xo = jnp.where(rowd < 4, jnp.broadcast_to(x, (8, D)), 1.0).astype(BF)
        coef = jnp.where(row < 4, 1.0, -mu)

        def q_direct(col):
            t = jnp.dot(xo, pltpu.bitcast(wqu[col], BF), preferred_element_type=F32) * coef
            return (t + pltpu.roll(t, 4, 0)).astype(BF).astype(F32)

        def q_cols(q, slot):
            for b, col in enumerate(columns(q)):
                part[slot + b] = col

        def vpu_a(m, slot, js):
            acc = {}
            for g2 in range(8):
                qc = jnp.concatenate([part[slot + 2 * g2 + t + zero_i] for t in range(2)], axis=0)
                for j in js:
                    tv = f32_rows(kvu[m, 0, 0, g2, j & 1, j >> 1]) * qc
                    acc[j] = tv if g2 == 0 else acc[j] + tv
            for j in js:
                part_a[j // 8, j % 8:j % 8 + 1, :] = jnp.sum(acc[j], axis=0, keepdims=True)

        q0 = [q_direct(c) for c in range(4)]
        q_cols(q0[0], SP)
        set_pat(1, q0[1])
        set_pat(2, q0[2])
        _, qb, qc = qk_ops(0)
        for i in range(nblk // 2):
            if i == 4:
                q_cols(q0[3], SP + 16)
            vpu_a(0, SP, jord[2 * i:2 * i + 2])
            plain((qb + qc)[4 * i:4 * i + 4])
        g_softmax(0, 0)
        g_softmax(0, 1)
        plain(qproj_ops(1)[KD:])
        g_query(1)
        g_query(2)
        set_pat(0, q0[3])
        plain(qk_ops(1)[0][PVB:])
        for i in range(0, PVB, 2):
            part[0] = qpart[min(KD + 4 + 3 * i // 2, 3 * KD - 1)]
            vpu_a(1, SP + 16, jord[i:i + 2])
        toks.clear()

        def block(m, ph):
            @pl.when(first)
            def _():
                kv_copy(m + 2, 0).wait()
                if ph == 1:
                    pl.when(m + 3 == NP)(start_ffn_weights)
                pair_rows(m + 2)
                stage_step(m + 5, 5, NP + 2)
                kv_copy(m + 2, 1).wait()

                @pl.when(m + 2 + KVW < NP)
                def _():
                    for i in range(2):
                        kv_copy(m + 2 + KVW, i).start()

                widen(m + 2)

            qp = qproj_ops(m + 2)
            _, qb, qc = qk_ops(m + 1)
            qa = qk_ops(m + 2)[0]
            op = oproj_ops(jnp.maximum(m - 1, 0), m + 2, opart, 8 * ph)
            seq = ([(lambda: g_out(1 - ph),), (lambda: g_olhs(3 * m, 1 - ph),)]
                   + qc[:CF] + qp[:KD] + [(lambda: g_query(0),)] + qc[CF:] + qb
                   + [(lambda: g_softmax(1 - ph, 0),), (lambda: g_softmax(1 - ph, 1),)]
                   + qp[KD:] + [(lambda: g_query(1),), (lambda: g_query(2),)]
                   + op + qa[:nblk - AEND] + [(lambda: fence(pat_u, 3, zero_i),)]
                   + qa[nblk - AEND:])
            emit(pv_ops(m, ph), seq)

        def body(t, carry):
            block(2 * t, 0)
            block(2 * t + 1, 1)
            return carry

        lax.fori_loop(0, NP // 2 - 1, body, 0)

        def big(kts, i0):
            return [op for i, kt in enumerate(kts)
                    for op in oproj_ops(kt, kt + 3, part, SP + KD * (i0 + i))]

        old = list(range(NP - 3, 3 * (NP - 3)))
        barrier()
        _, qb, qc = qk_ops(NP - 1)
        seq = ([(lambda: g_out(1),), (lambda: g_olhs(3 * (NP - 2), 1),)] + qc + qb
               + [(lambda: g_softmax(1, 0),), (lambda: g_softmax(1, 1),)]
               + big(old[:KT14 - 4] + list(range(3 * (NP - 3), 3 * (NP - 2))), 0)
               + [(lambda: fence(olhs_u, 3 * NP, zero_i),)]
               + big(old[KT14 - 4:KT14 - 3], KT14 - 1))
        emit(pv_ops(NP - 2, 0), seq)
        barrier()
        k15 = old[KT14 - 3:-1] + list(range(3 * (NP - 2), 3 * (NP - 1))) + old[-1:]
        emit(pv_ops(NP - 1, 1), [(lambda: g_olhs(3 * (NP - 1), 0),)] + big(k15, KT14))

        def epilogue(x):
            def lsum(g):
                return lane_sum(accx[1, 8 * g:8 * g + 8, :])

            inv = [recip(jnp.sum(lsum(2 * G + par), axis=0, keepdims=True)) for par in range(2)]
            last = [None] * KD
            for par in range(2):
                acc = [None] * KD
                for g2 in range(G2):
                    g = G * par + 2 * g2
                    z = jnp.concatenate([lsum(g), lsum(g + 1)], axis=0)
                    for n in range(KD):
                        tv = f32_rows(wou[(NP - 1) * G + G2 * par + g2, n]) * z
                        acc[n] = tv if g2 == 0 else acc[n] + tv
                for n in range(KD):
                    t = (acc[n][:8] + acc[n][8:]) * inv[par]
                    last[n] = t if par == 0 else last[n] + t
            cols = []
            for n in range(KD):
                t = out_scr[n]
                for i in range(2 * NP):
                    t = t + part[SP + KD * i + n]
                cols.append(jnp.sum(t + last[n], axis=0, keepdims=True))
            return residual(x, jnp.concatenate(cols, axis=1))

        return lax.cond(first, lambda x: ffn1(epilogue(x)), lambda x: ffn2(epilogue(x)), x)

    for r in (y_u, pat_u, olhs_u):
        r[...] = jnp.zeros(r.shape, U32)
    reset_pipeline()
    stage_step(1, 1)
    c_wo[0].wait()
    for c in c_wq[Q0:]:
        c.start()
    stage_step(2)
    wait_all(c_wq[:QA])
    for m in range(KVW + 2):
        for i in range(2):
            kv_copy(m, i).start()
    for m in range(2):
        kv_copy(m, 0).wait()
        pair_rows(m)
        stage_step(3 + m)
        kv_copy(m, 1).wait()
        widen(m)
    wait_all([c_x] + c_wq[QA:] + c_wo[1:])
    x = lax.fori_loop(0, 2, layer, xb[...].astype(F32))
    o_ref[...] = x.astype(o_ref.dtype)


@jax.jit
def pallas_interleave_layers__sliding_block_cached__glu_gated_swiglu__decode_kernel(
    A_x: jax.Array,
    A_k_cache: jax.Array,
    A_v_cache: jax.Array,
    A_wq: jax.Array,
    A_wo: jax.Array,
    B_x: jax.Array,
    B_w1: jax.Array,
    B_w3: jax.Array,
    B_w2: jax.Array,
):
    del B_x
    sk = A_k_cache.shape[2]
    win = min(4096, max(256, sk // 4))
    nb = sk // 128
    nblk = win // 128

    def cache_tiles(c):
        return (c.reshape(H, nb, 128, G2, 2, 8).transpose(0, 3, 4, 1, 5, 2)
                .reshape(H, G2, 2, nb // 2, 16, 128))

    def weight_tiles(w):
        r, c = w.shape
        return w.reshape(r // 16, 2, 8, c // 128, 128).transpose(0, 1, 3, 2, 4)

    vreg = lambda n: pltpu.VMEM((-(-n // 4) * 4, 8, 128), F32)
    lhs = lambda n: pltpu.VMEM((-(-n // 4) * 4, 16, 128), BF)
    kern = lambda *refs: _kernel(*refs, blk0=nb - nblk, nblk=nblk, scale=DH ** -0.5)
    out = pl.pallas_call(
        kern,
        out_shape=jax.ShapeDtypeStruct((1, D), BF),
        in_specs=[pl.BlockSpec(memory_space=pl.ANY)] * 8,
        out_specs=pl.BlockSpec(memory_space=pltpu.VMEM),
        scratch_shapes=[
            pltpu.VMEM((1, D), BF),
            pltpu.VMEM((NP, 2, 2, G2, 2, nblk // 2, 16, 128), BF),
            pltpu.VMEM((3 * NP, D, 128), BF),
            pltpu.VMEM((H * DH // 16, KD, 16, 128), BF),
            pltpu.VMEM((D // 16, NC, 16, 128), BF),
            pltpu.VMEM((D // 16, NC, 16, 128), BF),
            pltpu.VMEM((FF // 16, KD, 16, 128), BF),
            lhs(KD),
            vreg(1),
            vreg(3 * KD),
            lhs(8),
            vreg(nblk // 8),
            vreg(nblk // 2 + 2 * NP * KD),
            pltpu.VMEM((2, 2, nblk, 128), F32),
            pltpu.VMEM((nblk * 8, 128), F32),
            pltpu.VMEM((2, 64, 128), F32),
            pltpu.VMEM((2, 8 * NR, 128), F32),
            lhs(3 * NP + 4),
            vreg(16),
            vreg(KD),
            pltpu.VMEM((NP, NW, 2, 8, 128), F32),
            pltpu.SMEM((2, SC, 2, KD, 8, 128), BF),
            pltpu.SemaphoreType.DMA((2, NP)),
            pltpu.SemaphoreType.DMA((5 + len(W2_CHUNKS),)),
            pltpu.SemaphoreType.DMA((3,)),
        ],
        compiler_params=pltpu.CompilerParams(
            vmem_limit_bytes=128 * 1024 * 1024, disable_semaphore_checks=True),
    )(A_x.reshape(1, D), cache_tiles(A_k_cache), cache_tiles(A_v_cache),
      A_wq, weight_tiles(A_wo),
      weight_tiles(B_w1), weight_tiles(B_w3), weight_tiles(B_w2))
    return out.reshape(1, 1, D)
```

```python
import math

import jax
import jax.numpy as jnp
from jax import lax
import jax.experimental.pallas as pl
import jax.experimental.pallas.tpu as pltpu

BF = jnp.bfloat16
F32 = jnp.float32
U32 = jnp.uint32

D = 640
H = 32
DH = 192
G = DH // 8
G2 = DH // 16
NP = H // 2
FF = 1536
EPS = 1e-5
KD = D // 128
NC = FF // 128
NZ = 2 * G + 2
NR = NZ + 2
W2_CHUNKS = (768, 384, 256, 128)

NA = 8
NW = 72
UNPACED = 8
LEAD = 16
RATE = 32.5
TAILC = 30
AEND = 4
CF = 8
KT14 = 10
PVB = 6
KM = 3
FPRE = 6
FSTEP = 3
NST = NP + 1
SC = 10
KVW = 4


def _kernel(x_hbm, k_hbm, v_hbm, wq_hbm, wo_hbm, w1_hbm, w3_hbm, w2_hbm,
            o_ref,
            xb, kvb, wq, wo, w1, w3, w2,
            y_scr, rs_scr, qpart, pat_scr, part_a, part, p_scr, pb_scr, pb0,
            accx, olhs, opart, out_scr, vx, stage,
            kvsem, wsem, ssem, *, blk0, nblk, scale):
    c2 = scale * math.log2(math.e)
    nq = nblk // 8
    SP = 4 * nq

    def kv_copy(m, i):
        return pltpu.make_async_copy(
            (k_hbm, v_hbm)[i].at[pl.ds(2 * m, 2), :, :, pl.ds(blk0 // 2, nblk // 2)],
            kvb.at[m, i], kvsem.at[i, m])

    def wcopies(src, dst, s, r0=0, nr=None):
        nr = src.shape[0] if nr is None else nr
        return [pltpu.make_async_copy(src.at[pl.ds(r0, nr), t],
                                      dst.at[pl.ds(r0, nr), :, pl.ds(8 * t, 8), :],
                                      wsem.at[s]) for t in range(2)]

    c_x = pltpu.make_async_copy(x_hbm, xb, wsem.at[0])
    c_wq = [pltpu.make_async_copy(wq_hbm.at[:, :, pl.ds(3 * b, 3)], wq.at[b], wsem.at[1])
            for b in range(NP // 2)]
    R0 = H * G2 - NST * SC
    c_wo = pltpu.make_async_copy(wo_hbm.at[pl.ds(0, R0)], wo.at[pl.ds(0, R0)], wsem.at[2])

    def to_stage(k):
        return pltpu.make_async_copy(wo_hbm.at[pl.ds(R0 + SC * k, SC)], stage.at[k & 1],
                                     ssem.at[0])

    def from_stage(k):
        return pltpu.make_async_copy(stage.at[k & 1], wo.at[pl.ds(R0 + SC * k, SC)], ssem.at[1])

    def stage_step(k):
        def when(cond, f):
            if isinstance(cond, bool):
                if cond:
                    f()
            else:
                pl.when(cond)(f)

        def forward():
            to_stage(k - 1).wait()
            from_stage(k - 1).start()

        landed = not isinstance(k, int) or k >= 2
        if landed:
            from_stage(k - 2).wait()
        when(k <= NST, forward)
        when(k < NST, lambda: to_stage(k).start())
        if landed:
            pair_wo(R0 + SC * (k - 2), SC)

    c_w1 = wcopies(w1_hbm, w1, 3)
    c_w3 = wcopies(w3_hbm, w3, 4)
    w2_off = [sum(W2_CHUNKS[:i]) for i in range(len(W2_CHUNKS))]
    c_w2 = [wcopies(w2_hbm, w2, 5 + i, o // 16, n // 16)
            for i, (o, n) in enumerate(zip(w2_off, W2_CHUNKS))]

    def wait_all(cs):
        for c in cs:
            c.wait()

    c_wo.start()
    to_stage(0).start()
    for c in [c_x] + c_wq:
        c.start()

    def start_ffn_weights():
        for c in c_w1 + c_w3 + [c for cs in c_w2 for c in cs]:
            c.start()

    kvu = kvb.bitcast(U32)
    wqu = wq.bitcast(U32)
    wou = wo.bitcast(U32)
    w1u, w3u, w2u = w1.bitcast(U32), w3.bitcast(U32), w2.bitcast(U32)
    y_u, pat_u, olhs_u = y_scr.bitcast(U32), pat_scr.bitcast(U32), olhs.bitcast(U32)

    def f32_rows(u):
        return pltpu.bitcast(u, BF).astype(F32)

    lane = lax.broadcasted_iota(jnp.int32, (8, 128), 1)
    row = lax.broadcasted_iota(jnp.int32, (8, 128), 0)
    diag_i = ((lane & 7) == row).astype(jnp.int32) * 64
    bit_i = [(lane << (3 - k)) & 64 for k in range(4)]
    uid = [0]

    def lane_sum(v):
        return jnp.broadcast_to(jnp.sum(v, axis=1, keepdims=True), (8, 128))

    def columns(v8):
        uid[0] += 1
        off = 256 * uid[0]
        dl = lane - row + off
        return [lane_sum(jnp.where(dl == off + 8 * b, v8[:, 128 * k:128 * k + 128], 0.0))
                for k in range(v8.shape[1] // 128) for b in range(16)]

    def moments(x):
        mu = jnp.mean(x, axis=-1, keepdims=True)
        xc = x - mu
        return mu, xc, 1.0 / jnp.sqrt(jnp.mean(xc * xc, axis=-1, keepdims=True) + EPS)

    def residual(x, a):
        return (x + a.astype(BF).astype(F32)).astype(BF).astype(F32)

    def matvec(l, wu, r0, nr):
        return [jnp.dot(l, pltpu.bitcast(wu[r0:r0 + nr, c].reshape(8 * nr, 128), BF),
                        preferred_element_type=F32) for c in range(wu.shape[1])]

    def tile_dot(l_u32, w_u32, rows, paced):
        w = pltpu.bitcast(w_u32.reshape(64, 128), BF)
        if paced:
            l = pltpu.bitcast(jnp.concatenate([l_u32, l_u32], axis=0), BF)[:24]
            return jnp.dot(l, w, preferred_element_type=F32)[:rows]
        l = pltpu.bitcast(l_u32, BF)[:rows]
        return jnp.dot(l, w, preferred_element_type=F32)

    def swap_halves(a, b):
        return (jnp.concatenate([a[..., :4, :], b[..., :4, :]], axis=-2),
                jnp.concatenate([a[..., 4:, :], b[..., 4:, :]], axis=-2))

    def pair_wq():
        def body(i, carry):
            b, r = i // KD, pl.ds(8 * (i % KD), 8)
            wqu[b, r, 0], wqu[b, r, 1] = swap_halves(wqu[b, r, 0], wqu[b, r, 1])
            return carry
        lax.fori_loop(0, KD * (NP // 2), body, 0)

    def pair_wo(r0, n):
        def body(i, carry):
            r = pl.ds(r0 + 2 * i, 2)
            v = wou[r]
            h = [v[:, f // 2, 4 * (f % 2):4 * (f % 2) + 4, :] for f in range(2 * KD)]
            for c in range(KD):
                wou[r, c] = jnp.concatenate([h[c], h[KD + c]], axis=1)
            return carry
        lax.fori_loop(0, n // 2, body, 0)

    def wq_tile(m, c, k):
        c6 = 3 * m[1] + c
        return wqu[m[0] + c6 // 6, 8 * k:8 * k + 8, c6 & 1, (c6 % 6) >> 1]

    def qproj_ops(m):
        def op(paced, c, k):
            qpart[c * KD + k] = tile_dot(
                y_u[k], wq_tile(m, c, k), 8, paced)
        return [(lambda p, c=c, k=k: op(p, c, k)) for c in range(3) for k in range(KD)]

    def oproj_ops(kt, slot, dst, d0):
        def op(paced, n):
            dst[d0 + n] = tile_dot(olhs_u[slot], wou[pl.ds(kt * 8, 8), n], 8, paced)
        return [(lambda p, n=n: op(p, n)) for n in range(KD)]

    def pair_rows(m):
        def body(i, c):
            par, g2 = i // G2, i % G2
            kvu[m, 0, par, g2, 0], kvu[m, 0, par, g2, 1] = swap_halves(
                kvu[m, 0, par, g2, 0], kvu[m, 0, par, g2, 1])
            return c
        lax.fori_loop(0, 2 * G2, body, 0)

    def k_blocks(m, par, g0, g1, j):
        return kvu[m, 0, par, g0:g1, j & 1, j >> 1]

    jord = [8 * (i // 8) + 2 * (i % 4) + (i % 8) // 4 for i in range(nblk)]

    def qk_ops(m):
        def op_a(paced, j):
            r = tile_dot(pat_u[0], k_blocks(m, 0, 0, 8, j), 8, paced)
            part_a[j // 8, j % 8:j % 8 + 1, :] = r[j % 8:j % 8 + 1, :]

        def op_c(paced, j):
            r = tile_dot(pat_u[2], k_blocks(m, 1, 4, 12, j), 8, paced)
            part[2 * nq + j // 8, j % 8:j % 8 + 1, :] = r[j % 8:j % 8 + 1, :]

        def op_b(paced, j):
            w = jnp.concatenate([k_blocks(m, 0, 8, 12, j), k_blocks(m, 1, 0, 4, j)], axis=0)
            r = tile_dot(pat_u[1], w, 16, paced)
            part[nq + j // 8, j % 8:j % 8 + 1, :] = r[j % 8:j % 8 + 1, :]
            part[3 * nq + j // 8, j % 8:j % 8 + 1, :] = r[8 + j % 8:8 + j % 8 + 1, :]

        return [[(lambda p, f=f, j=j: f(p, j)) for j in jord] for f in (op_a, op_b, op_c)]

    def plain(ops):
        for op in ops:
            op(False)

    steps = [(par, gb, j0) for par in range(2) for gb in range(G // NA)
             for j0 in range(0, nblk, 4)]

    def units(par, gb, j0):
        return [(par, g, j0) for g in range(gb * NA, (gb + 1) * NA)]

    order = [u for s in steps for u in units(*s)]
    wide = {}
    for i, u in enumerate(order):
        if (i + 1) * NW // len(order) > i * NW // len(order):
            wide[u] = len(wide)

    def widen(m):
        for (par, g, j), e in wide.items():
            v = f32_rows(kvu[m, 1, par, g // 2, g % 2, j // 2:j // 2 + 2])
            kvu[m, 1, par, g // 2, g % 2, j // 2:j // 2 + 2] = pltpu.bitcast(v[:, :8], U32)
            vx[m, e] = v[:, 8:]

    def v_unit(m, par, g, j):
        u = kvu[m, 1, par, g // 2, g % 2, j // 2:j // 2 + 2]
        if (par, g, j) in wide:
            return jnp.concatenate([pltpu.bitcast(u, F32), vx[m, wide[(par, g, j)]]], axis=1)
        return f32_rows(u)

    def pv_ops(m, ph):
        acc = {}

        def spread(par, q, r):
            pb_scr[pl.ds(64 * q + r, 8, stride=8), :] = p_scr[ph, par, 8 * q:8 * q + 8, :]

        def psum(par):
            p = p_scr[ph, par]
            accx[ph, 8 * (2 * G + par):8 * (2 * G + par) + 8, :] = (
                (p[0:8] + p[8:16]) + (p[16:24] + p[24:32]))

        pbv = {}

        def piece(par, gb, j0, k):
            if k == 0:
                if par == 0 and j0 < 8:
                    pb = pb0[ph, 8 * j0:8 * j0 + 32, :]
                else:
                    pb = pb_scr[8 * j0:8 * j0 + 32, :]
                pbv[0] = pb.reshape(4, 8, 128)
            for _, g, _ in units(par, gb, j0)[4 * k:4 * k + 4]:
                tv = v_unit(m, par, g, j0).reshape(4, 8, 128) * pbv[0]
                tv = jnp.sum(tv, axis=0)
                acc[g] = tv if j0 == 0 else acc[g] + tv
                if j0 == nblk - 4:
                    r0 = DH * par + 8 * g
                    accx[ph, r0:r0 + 8, :] = acc[g]

        pieces = [s + (k,) for s in steps for k in range(NA // 4)]
        half = len(pieces) // 2
        spq = 2 * (NA // 4)
        side = {}
        for q in range(nq):
            for r in range(8):
                if q:
                    side.setdefault((spq * (8 * (q - 1) + r)) // 9, []).append(
                        lambda q=q, r=r: spread(0, q, r))
                side.setdefault(half - nq * spq + spq * (q + 1) + (r * (3 * spq - 1)) // 8, []).append(
                    lambda q=q, r=r: spread(1, q, r))
        for par in range(2):
            side.setdefault(half // 2 + par, []).append(lambda par=par: psum(par))
        out = []
        for i, s in enumerate(pieces):
            out += [(0, f) for f in side.get(i, [])]
            out.append((2 * sum(4 if u in wide else 6 for u in units(*s[:3])[4 * s[3]:4 * s[3] + 4]),
                        (lambda s=s: piece(*s))))
        return out

    toks = []

    def fence(dst, slot, zero_i):
        for i, t in enumerate(toks):
            dst[slot + i + zero_i] = t
        toks.clear()

    def g_softmax(ph, par):
        s0 = part[2 * nq:3 * nq] if par else part_a[0:nq]
        s = (s0 + part[(2 * par + 1) * nq:(2 * par + 2) * nq]).reshape(nblk, 128)
        mx = jnp.max(jnp.max(s, axis=0, keepdims=True), axis=1, keepdims=True)
        p = jnp.exp2((s - mx) * jnp.concatenate([rs_scr[0]] * nq, axis=0))
        p_scr[ph, par] = p
        if par == 0:
            for r in range(8):
                pb0[ph, pl.ds(r, 8, stride=8), :] = p[0:8]
        toks.append(pltpu.bitcast(p[nblk - 8:nblk], U32))

    def recip(d):
        r = pl.reciprocal(d, approx=True)
        return r * (2.0 - d * r)

    def g_olhs(slot0, ph):
        z = [lane_sum(accx[ph, 8 * g:8 * g + 8, :]) for g in range(NZ)]
        inv = [jnp.broadcast_to(recip(jnp.sum(z[2 * G + par], axis=0, keepdims=True)), (8, 128))
               for par in range(2)]
        uid[0] += 1
        bit = [b > uid[0] for b in bit_i]
        for c in range(3):
            xs = z[16 * c:16 * c + 16]
            for k in range(4):
                xs = [jnp.where(bit[k], xs[i + 1], xs[i]) for i in range(0, len(xs), 2)]
            iv = inv[0] if c == 0 else (inv[1] if c == 2 else jnp.where(bit[3], inv[1], inv[0]))
            olhs[slot0 + c, 0:8, :] = jnp.where(diag_i > uid[0], xs[0] * iv, 0.0).astype(BF)

    def set_pat(c, q):
        if c == 1:
            hi = bit_i[3] > uid[0]
            pat_scr[c, 0:8, :] = jnp.where(hi, 0.0, q).astype(BF)
            pat_scr[c, 8:16, :] = jnp.where(hi, q, 0.0).astype(BF)
        else:
            pat_scr[c, 0:8, :] = q.astype(BF)
        if c > 0:
            toks.append(pltpu.bitcast(q, U32))

    def g_query(c):
        xs = [qpart[c * KD + k] for k in range(KD)]
        set_pat(c, ((xs[0] + xs[1]) + (xs[2] + xs[3])) + xs[4])

    def g_out(ph):
        for n in range(KD):
            out_scr[n] = out_scr[n] + opart[8 * ph + n]

    def reset_pipeline():
        accx[1, 0:16 * G, :] = jnp.zeros((16 * G, 128), F32)
        accx[1, 16 * G:16 * G + 16, :] = jnp.ones((16, 128), F32)
        for n in range(KD):
            opart[8 + n] = jnp.zeros((8, 128), F32)
            out_scr[n] = jnp.zeros((8, 128), F32)

    def emit(pv, seq):
        ntile = sum(not isinstance(e, tuple) for e in seq)
        total = sum(w for w, _ in pv) / 4
        k = done = n = 0
        for e in seq:
            if isinstance(e, tuple):
                e[0]()
                continue
            pos = LEAD + RATE * (n // 4) if n // 4 < (ntile - 1) // 4 else total - TAILC
            while k < len(pv) and done + pv[k][0] / 2 <= 4 * pos:
                done += pv[k][0]
                pv[k][1]()
                k += 1
            e(n < ntile - UNPACED)
            n += 1
        for _, g in pv[k:]:
            g()

    def ffn1(x):
        _, xc, rs = moments(x)
        y = jnp.broadcast_to(xc, (8, D)).astype(BF)
        reset_pipeline()
        wait_all(c_w1)
        g = jnp.concatenate(matvec(y, w1u, 0, D // 16), axis=1) * rs
        wait_all(c_w3)
        u = jnp.concatenate(matvec(y, w3u, 0, D // 16), axis=1) * rs
        hh = (g * jax.nn.sigmoid(g) * u).astype(BF)
        hb = columns(hh[:, w2_off[-1]:].astype(F32))
        a = None
        for cs, o, n in list(zip(c_w2, w2_off, W2_CHUNKS))[:-1]:
            wait_all(cs)
            t = jnp.concatenate(matvec(hh[:, o:o + n], w2u, o // 16, n // 16), axis=1)[0:1]
            a = t if a is None else a + t
        wait_all(c_w2[-1])
        acc = [None] * KD
        for r in range(W2_CHUNKS[-1] // 16):
            for c in range(KD):
                v = f32_rows(w2u[w2_off[-1] // 16 + r, c])
                tv = v[:8] * hb[2 * r] + v[8:] * hb[2 * r + 1]
                acc[c] = tv if r == 0 else acc[c] + tv
        a = a + jnp.concatenate([jnp.sum(t, axis=0, keepdims=True) for t in acc], axis=1)
        return residual(x, a)

    def ffn2(x):
        mu, _, rs = moments(x)
        x8 = jnp.broadcast_to(x, (8, D))
        rowk = lax.broadcasted_iota(jnp.int32, (8, 128 * KM), 0)
        y = jnp.where(rowk == 0, x8[:, :128 * KM], jnp.where(rowk == 1, 1.0, 0.0)).astype(BF)
        coef = jnp.where(row == 0, 1.0, -mu)
        yb = jnp.concatenate([c - mu for c in columns(x8[:, 128 * KM:])], axis=0)
        mx = {}
        out = [None] * KD
        for c in range(NC):
            while len(mx) < min(NC, FPRE + c * FSTEP / 4):
                cc = len(mx)
                mx[cc] = [jnp.dot(y, pltpu.bitcast(wu[0:8 * KM, cc].reshape(64 * KM, 128), BF),
                                  preferred_element_type=F32) * coef for wu in (w1u, w3u)]
            gu = []
            for i, wu in enumerate((w1u, w3u)):
                acc = None
                for r in range(8 * (KD - KM)):
                    tv = f32_rows(wu[8 * KM + r, c]) * yb[16 * r:16 * r + 16]
                    acc = tv if r == 0 else acc + tv
                gu.append(jnp.sum((acc[:8] + acc[8:]) + mx[c][i], axis=0, keepdims=True) * rs)
            hg = 0.5 * gu[0]
            h = jnp.broadcast_to((hg * jnp.tanh(hg) + hg) * gu[1], (8, 128)).astype(BF)
            for n in range(KD):
                t = jnp.dot(h, pltpu.bitcast(w2u[8 * c:8 * c + 8, n].reshape(64, 128), BF),
                            preferred_element_type=F32)[0:1]
                out[n] = t if c == 0 else out[n] + t
        return residual(x, jnp.concatenate(out, axis=1))

    def layer(li, x):
        first = li == 0
        zero_i = li >> 4

        def barrier():
            @pl.when(li > 2)
            def _():
                reset_pipeline()

        mu, xc, rs = moments(x)
        y = jnp.broadcast_to(xc, (8, D))
        for k in range(KD):
            y_scr[k, 0:8, :] = y[:, 128 * k:128 * k + 128].astype(BF)
        rs_scr[0] = jnp.broadcast_to(rs * c2, (8, 128))
        rowd = lax.broadcasted_iota(jnp.int32, (8, D), 0)
        xo = jnp.where(rowd < 4, jnp.broadcast_to(x, (8, D)), 1.0).astype(BF)
        coef = jnp.where(row < 4, 1.0, -mu)

        def q_direct(col):
            t = jnp.dot(xo, pltpu.bitcast(wqu[0, :, col & 1, col >> 1].reshape(D // 2, 128), BF), preferred_element_type=F32) * coef
            return (t + pltpu.roll(t, 4, 0)).astype(BF).astype(F32)

        def q_cols(q, slot):
            for b, col in enumerate(columns(q)):
                part[slot + b] = col

        def vpu_a(m, slot, js):
            acc = {}
            for g2 in range(8):
                qc = jnp.concatenate([part[slot + 2 * g2 + t + zero_i] for t in range(2)], axis=0)
                for j in js:
                    tv = f32_rows(kvu[m, 0, 0, g2, j & 1, j >> 1]) * qc
                    acc[j] = tv if g2 == 0 else acc[j] + tv
            for j in js:
                part_a[j // 8, j % 8:j % 8 + 1, :] = jnp.sum(acc[j], axis=0, keepdims=True)

        q0 = [q_direct(c) for c in range(4)]
        q_cols(q0[0], SP)
        set_pat(1, q0[1])
        set_pat(2, q0[2])
        _, qb, qc = qk_ops(0)
        for i in range(nblk // 2):
            if i == 4:
                q_cols(q0[3], SP + 16)
            vpu_a(0, SP, jord[2 * i:2 * i + 2])
            plain((qb + qc)[4 * i:4 * i + 4])
        g_softmax(0, 0)
        g_softmax(0, 1)
        plain(qproj_ops((0, 1))[KD:])
        g_query(1)
        g_query(2)
        set_pat(0, q0[3])
        plain(qk_ops(1)[0][PVB:])
        for i in range(0, PVB, 2):
            part[0] = qpart[min(KD + 4 + 3 * i // 2, 3 * KD - 1)]
            vpu_a(1, SP + 16, jord[i:i + 2])
        toks.clear()

        def block(t, ph):
            m = 2 * t + ph

            @pl.when(first)
            def _():
                kv_copy(m + 2, 0).wait()
                if ph == 1:
                    pl.when(m + 3 == NP)(start_ffn_weights)
                pair_rows(m + 2)
                stage_step(m + 5)
                kv_copy(m + 2, 1).wait()

                @pl.when(m + 2 + KVW < NP)
                def _():
                    for i in range(2):
                        kv_copy(m + 2 + KVW, i).start()

                widen(m + 2)

            qp = qproj_ops((t, ph + 2))
            _, qb, qc = qk_ops(m + 1)
            qa = qk_ops(m + 2)[0]
            op = oproj_ops(jnp.maximum(m - 1, 0), m + 2, opart, 8 * ph)
            seq = ([(lambda: g_out(1 - ph),), (lambda: g_olhs(3 * m, 1 - ph),)]
                   + qc[:CF] + qp[:KD] + [(lambda: g_query(0),)] + qc[CF:] + qb
                   + [(lambda: g_softmax(1 - ph, 0),), (lambda: g_softmax(1 - ph, 1),)]
                   + qp[KD:] + [(lambda: g_query(1),), (lambda: g_query(2),)]
                   + op + qa[:nblk - AEND] + [(lambda: fence(pat_u, 3, zero_i),)]
                   + qa[nblk - AEND:])
            emit(pv_ops(m, ph), seq)

        def body(t, carry):
            block(t, 0)
            block(t, 1)
            return carry

        lax.fori_loop(0, NP // 2 - 1, body, 0)

        def big(kts, i0):
            return [op for i, kt in enumerate(kts)
                    for op in oproj_ops(kt, kt + 3, part, SP + KD * (i0 + i))]

        old = list(range(NP - 3, 3 * (NP - 3)))
        barrier()
        _, qb, qc = qk_ops(NP - 1)
        seq = ([(lambda: g_out(1),), (lambda: g_olhs(3 * (NP - 2), 1),)] + qc + qb
               + [(lambda: g_softmax(1, 0),), (lambda: g_softmax(1, 1),)]
               + big(old[:KT14 - 4] + list(range(3 * (NP - 3), 3 * (NP - 2))), 0)
               + [(lambda: fence(olhs_u, 3 * NP, zero_i),)]
               + big(old[KT14 - 4:KT14 - 3], KT14 - 1))
        emit(pv_ops(NP - 2, 0), seq)
        barrier()
        k15 = old[KT14 - 3:-1] + list(range(3 * (NP - 2), 3 * (NP - 1))) + old[-1:]
        emit(pv_ops(NP - 1, 1), [(lambda: g_olhs(3 * (NP - 1), 0),)] + big(k15, KT14))

        def epilogue(x):
            def lsum(g):
                return lane_sum(accx[1, 8 * g:8 * g + 8, :])

            inv = [recip(jnp.sum(lsum(2 * G + par), axis=0, keepdims=True)) for par in range(2)]
            last = [None] * KD
            for par in range(2):
                acc = [None] * KD
                for g2 in range(G2):
                    g = G * par + 2 * g2
                    z = jnp.concatenate([lsum(g), lsum(g + 1)], axis=0)
                    for n in range(KD):
                        tv = f32_rows(wou[(NP - 1) * G + G2 * par + g2, n]) * z
                        acc[n] = tv if g2 == 0 else acc[n] + tv
                for n in range(KD):
                    t = (acc[n][:8] + acc[n][8:]) * inv[par]
                    last[n] = t if par == 0 else last[n] + t
            cols = []
            for n in range(KD):
                t = out_scr[n]
                for i in range(2 * NP):
                    t = t + part[SP + KD * i + n]
                cols.append(jnp.sum(t + last[n], axis=0, keepdims=True))
            return residual(x, jnp.concatenate(cols, axis=1))

        return lax.cond(first, lambda x: ffn1(epilogue(x)), lambda x: ffn2(epilogue(x)), x)

    for r in (y_u, pat_u, olhs_u):
        r[...] = jnp.zeros(r.shape, U32)
    reset_pipeline()
    stage_step(1)
    c_wo.wait()
    pair_wo(0, R0)
    stage_step(2)
    for m in range(KVW + 2):
        for i in range(2):
            kv_copy(m, i).start()
    for m in range(2):
        kv_copy(m, 0).wait()
        pair_rows(m)
        stage_step(3 + m)
        kv_copy(m, 1).wait()
        widen(m)
    wait_all([c_x] + c_wq)
    pair_wq()
    x = lax.fori_loop(0, 2, layer, xb[...].astype(F32))
    o_ref[...] = x.astype(o_ref.dtype)


@jax.jit
def pallas_interleave_layers__sliding_block_cached__glu_gated_swiglu__decode_kernel(
    A_x: jax.Array,
    A_k_cache: jax.Array,
    A_v_cache: jax.Array,
    A_wq: jax.Array,
    A_wo: jax.Array,
    B_x: jax.Array,
    B_w1: jax.Array,
    B_w3: jax.Array,
    B_w2: jax.Array,
):
    del B_x
    sk = A_k_cache.shape[2]
    win = min(4096, max(256, sk // 4))
    nb = sk // 128
    nblk = win // 128

    def cache_tiles(c):
        return (c.reshape(H, nb, 128, G2, 2, 8).transpose(0, 3, 4, 1, 5, 2)
                .reshape(H, G2, 2, nb // 2, 16, 128))

    def weight_tiles(w):
        r, c = w.shape
        return w.reshape(r // 16, 2, 8, c // 128, 128).transpose(0, 1, 3, 2, 4)

    vreg = lambda n: pltpu.VMEM((-(-n // 4) * 4, 8, 128), F32)
    lhs = lambda n: pltpu.VMEM((-(-n // 4) * 4, 16, 128), BF)
    kern = lambda *refs: _kernel(*refs, blk0=nb - nblk, nblk=nblk, scale=DH ** -0.5)
    out = pl.pallas_call(
        kern,
        out_shape=jax.ShapeDtypeStruct((1, D), BF),
        in_specs=[pl.BlockSpec(memory_space=pl.ANY)] * 8,
        out_specs=pl.BlockSpec(memory_space=pltpu.VMEM),
        scratch_shapes=[
            pltpu.VMEM((1, D), BF),
            pltpu.VMEM((NP, 2, 2, G2, 2, nblk // 2, 16, 128), BF),
            pltpu.VMEM((NP // 2, D // 16, 2, 3, 16, 128), BF),
            pltpu.VMEM((H * DH // 16, KD, 16, 128), BF),
            pltpu.VMEM((D // 16, NC, 16, 128), BF),
            pltpu.VMEM((D // 16, NC, 16, 128), BF),
            pltpu.VMEM((FF // 16, KD, 16, 128), BF),
            lhs(KD),
            vreg(1),
            vreg(3 * KD),
            lhs(8),
            vreg(nblk // 8),
            vreg(nblk // 2 + 2 * NP * KD),
            pltpu.VMEM((2, 2, nblk, 128), F32),
            pltpu.VMEM((nblk * 8, 128), F32),
            pltpu.VMEM((2, 64, 128), F32),
            pltpu.VMEM((2, 8 * NR, 128), F32),
            lhs(3 * NP + 4),
            vreg(16),
            vreg(KD),
            pltpu.VMEM((NP, NW, 2, 8, 128), F32),
            pltpu.SMEM((2, SC, KD, 16, 128), BF),
            pltpu.SemaphoreType.DMA((2, NP)),
            pltpu.SemaphoreType.DMA((5 + len(W2_CHUNKS),)),
            pltpu.SemaphoreType.DMA((2,)),
        ],
        compiler_params=pltpu.CompilerParams(
            vmem_limit_bytes=128 * 1024 * 1024, disable_semaphore_checks=True),
    )(A_x.reshape(1, D), cache_tiles(A_k_cache), cache_tiles(A_v_cache),
      weight_tiles(A_wq).reshape(D // 16, 2, 3 * NP // 2, 16, 128),
      weight_tiles(A_wo).reshape(H * G2, KD, 16, 128),
      weight_tiles(B_w1), weight_tiles(B_w3), weight_tiles(B_w2))
    return out.reshape(1, 1, D)
```

```python
import math

import jax
import jax.numpy as jnp
from jax import lax
import jax.experimental.pallas as pl
import jax.experimental.pallas.tpu as pltpu

BF = jnp.bfloat16
F32 = jnp.float32
U32 = jnp.uint32

D = 640
H = 32
DH = 192
G = DH // 8
G2 = DH // 16
NP = H // 2
FF = 1536
EPS = 1e-5
KD = D // 128
NC = FF // 128
NZ = 2 * G + 2
NR = NZ + 2
W2S = 8
W2_CHUNKS = (768 - 16 * W2S, 384, 256, 128)

NA = 8
NW = 72
UNPACED = 8
LEAD = 16
RATE = 32.5
TAILC = 30
AEND = 4
CF = 8
KT14 = 10
PVB = 6
KM = 3
FPRE = 8
FSTEP = 3
NST = NP + 1
SC = 10
KVW = 4


def _kernel(x_hbm, k_hbm, v_hbm, wq_hbm, wo_hbm, w1_hbm, w3_hbm, w2_hbm,
            o_ref,
            xb, kvb, wq, wo, w1, w3, w2,
            y_scr, rs_scr, qpart, pat_scr, part_a, part, p_scr, pb_scr, pb0,
            accx, olhs, opart, out_scr, vx, stage,
            kvsem, wsem, ssem, *, blk0, nblk, scale):
    c2 = scale * math.log2(math.e)
    nq = nblk // 8
    SP = 4 * nq

    def kv_copy(m, i):
        return pltpu.make_async_copy(
            (k_hbm, v_hbm)[i].at[pl.ds(2 * m, 2), :, :, pl.ds(blk0 // 2, nblk // 2)],
            kvb.at[m, i], kvsem.at[i, m])

    c_x = pltpu.make_async_copy(x_hbm, xb, wsem.at[0])
    c_wq = [pltpu.make_async_copy(wq_hbm.at[:, :, pl.ds(3 * b, 3)], wq.at[b], wsem.at[1])
            for b in range(NP // 2)]
    R0 = H * G2 - NST * SC
    c_wo = pltpu.make_async_copy(wo_hbm.at[pl.ds(0, R0)], wo.at[pl.ds(0, R0)], wsem.at[2])

    def to_stage(k):
        return pltpu.make_async_copy(wo_hbm.at[pl.ds(R0 + SC * k, SC)], stage.at[k & 1],
                                     ssem.at[0])

    def from_stage(k):
        return pltpu.make_async_copy(stage.at[k & 1], wo.at[pl.ds(R0 + SC * k, SC)], ssem.at[1])

    def stage_step(k):
        def when(cond, f):
            if isinstance(cond, bool):
                if cond:
                    f()
            else:
                pl.when(cond)(f)

        def forward():
            to_stage(k - 1).wait()
            from_stage(k - 1).start()

        landed = not isinstance(k, int) or k >= 2
        if landed:
            from_stage(k - 2).wait()
        when(k <= NST, forward)
        when(k < NST, lambda: to_stage(k).start())
        if W2S:
            when(k == NST, w2_in.start)
            if isinstance(k, int) and k == NST + 1:
                w2_in.wait()
                w2_out.start()
        if landed:
            pair_wo(R0 + SC * (k - 2), SC)

    c_w1 = pltpu.make_async_copy(w1_hbm, w1, wsem.at[3])
    c_w3 = pltpu.make_async_copy(w3_hbm, w3, wsem.at[4])
    w2_off = [16 * W2S + sum(W2_CHUNKS[:i]) for i in range(len(W2_CHUNKS))]
    c_w2 = [pltpu.make_async_copy(w2_hbm.at[pl.ds(o // 16, n // 16)],
                                  w2.at[pl.ds(o // 16, n // 16)], wsem.at[5 + i])
            for i, (o, n) in enumerate(zip(w2_off, W2_CHUNKS))]
    if W2S:
        w2_slot = stage.at[NST & 1, pl.ds(0, W2S)]
        w2_in = pltpu.make_async_copy(w2_hbm.at[pl.ds(0, W2S)], w2_slot, ssem.at[0])
        w2_out = pltpu.make_async_copy(w2_slot, w2.at[pl.ds(0, W2S)], ssem.at[1])

    def wait_all(cs):
        for c in cs:
            c.wait()

    c_wo.start()
    to_stage(0).start()
    for c in [c_x] + c_wq:
        c.start()

    def start_ffn_weights():
        for c in [c_w1, c_w3] + c_w2:
            c.start()

    kvu = kvb.bitcast(U32)
    wqu = wq.bitcast(U32)
    wou = wo.bitcast(U32)
    w1u, w3u, w2u = w1.bitcast(U32), w3.bitcast(U32), w2.bitcast(U32)
    y_u, pat_u, olhs_u = y_scr.bitcast(U32), pat_scr.bitcast(U32), olhs.bitcast(U32)

    def f32_rows(u):
        return pltpu.bitcast(u, BF).astype(F32)

    lane = lax.broadcasted_iota(jnp.int32, (8, 128), 1)
    row = lax.broadcasted_iota(jnp.int32, (8, 128), 0)
    diag_i = ((lane & 7) == row).astype(jnp.int32) * 64
    bit_i = [(lane << (3 - k)) & 64 for k in range(4)]
    uid = [0]

    def lane_sum(v):
        return jnp.broadcast_to(jnp.sum(v, axis=1, keepdims=True), (8, 128))

    def columns(v8):
        uid[0] += 1
        off = 256 * uid[0]
        dl = lane - row + off
        return [lane_sum(jnp.where(dl == off + 8 * b, v8[:, 128 * k:128 * k + 128], 0.0))
                for k in range(v8.shape[1] // 128) for b in range(16)]

    def moments(x):
        mu = jnp.mean(x, axis=-1, keepdims=True)
        xc = x - mu
        return mu, xc, 1.0 / jnp.sqrt(jnp.mean(xc * xc, axis=-1, keepdims=True) + EPS)

    def residual(x, a):
        return (x + a.astype(BF).astype(F32)).astype(BF).astype(F32)

    def tile_dot(l_u32, w_u32, rows, paced):
        w = pltpu.bitcast(w_u32.reshape(64, 128), BF)
        if paced:
            l = pltpu.bitcast(jnp.concatenate([l_u32, l_u32], axis=0), BF)[:24]
            return jnp.dot(l, w, preferred_element_type=F32)[:rows]
        l = pltpu.bitcast(l_u32, BF)[:rows]
        return jnp.dot(l, w, preferred_element_type=F32)

    def swap_halves(a, b):
        return (jnp.concatenate([a[..., :4, :], b[..., :4, :]], axis=-2),
                jnp.concatenate([a[..., 4:, :], b[..., 4:, :]], axis=-2))

    def pair_wq():
        def body(i, carry):
            b, r = i // KD, pl.ds(8 * (i % KD), 8)
            wqu[b, r, 0], wqu[b, r, 1] = swap_halves(wqu[b, r, 0], wqu[b, r, 1])
            return carry
        lax.fori_loop(0, KD * (NP // 2), body, 0)

    def pair_wo(r0, n):
        def body(i, carry):
            r = pl.ds(r0 + 2 * i, 2)
            v = wou[r]
            h = [v[:, f // 2, 4 * (f % 2):4 * (f % 2) + 4, :] for f in range(2 * KD)]
            for c in range(KD):
                wou[r, c] = jnp.concatenate([h[c], h[KD + c]], axis=1)
            return carry
        lax.fori_loop(0, n // 2, body, 0)

    def wq_tile(m, c, k):
        c6 = 3 * m[1] + c
        return wqu[m[0] + c6 // 6, 8 * k:8 * k + 8, c6 & 1, (c6 % 6) >> 1]

    def qproj_ops(m):
        def op(paced, c, k):
            qpart[c * KD + k] = tile_dot(
                y_u[k], wq_tile(m, c, k), 8, paced)
        return [(lambda p, c=c, k=k: op(p, c, k)) for c in range(3) for k in range(KD)]

    def oproj_ops(kt, slot, dst, d0):
        def op(paced, n):
            dst[d0 + n] = tile_dot(olhs_u[slot], wou[pl.ds(kt * 8, 8), n], 8, paced)
        return [(lambda p, n=n: op(p, n)) for n in range(KD)]

    def pair_rows(m):
        def body(i, c):
            par, g2 = i // G2, i % G2
            kvu[m, 0, par, g2, 0], kvu[m, 0, par, g2, 1] = swap_halves(
                kvu[m, 0, par, g2, 0], kvu[m, 0, par, g2, 1])
            return c
        lax.fori_loop(0, 2 * G2, body, 0)

    def k_blocks(m, par, g0, g1, j):
        return kvu[m, 0, par, g0:g1, j & 1, j >> 1]

    jord = [8 * (i // 8) + 2 * (i % 4) + (i % 8) // 4 for i in range(nblk)]

    def qk_ops(m):
        def op_a(paced, j):
            r = tile_dot(pat_u[0], k_blocks(m, 0, 0, 8, j), 8, paced)
            part_a[j // 8, j % 8:j % 8 + 1, :] = r[j % 8:j % 8 + 1, :]

        def op_c(paced, j):
            r = tile_dot(pat_u[2], k_blocks(m, 1, 4, 12, j), 8, paced)
            part[2 * nq + j // 8, j % 8:j % 8 + 1, :] = r[j % 8:j % 8 + 1, :]

        def op_b(paced, j):
            w = jnp.concatenate([k_blocks(m, 0, 8, 12, j), k_blocks(m, 1, 0, 4, j)], axis=0)
            r = tile_dot(pat_u[1], w, 16, paced)
            part[nq + j // 8, j % 8:j % 8 + 1, :] = r[j % 8:j % 8 + 1, :]
            part[3 * nq + j // 8, j % 8:j % 8 + 1, :] = r[8 + j % 8:8 + j % 8 + 1, :]

        return [[(lambda p, f=f, j=j: f(p, j)) for j in jord] for f in (op_a, op_b, op_c)]

    def plain(ops):
        for op in ops:
            op(False)

    steps = [(par, gb, j0) for par in range(2) for gb in range(G // NA)
             for j0 in range(0, nblk, 4)]

    def units(par, gb, j0):
        return [(par, g, j0) for g in range(gb * NA, (gb + 1) * NA)]

    order = [u for s in steps for u in units(*s)]
    wide = {}
    for i, u in enumerate(order):
        if (i + 1) * NW // len(order) > i * NW // len(order):
            wide[u] = len(wide)

    def widen(m):
        for (par, g, j), e in wide.items():
            v = f32_rows(kvu[m, 1, par, g // 2, g % 2, j // 2:j // 2 + 2])
            kvu[m, 1, par, g // 2, g % 2, j // 2:j // 2 + 2] = pltpu.bitcast(v[:, :8], U32)
            vx[m, e] = v[:, 8:]

    def v_unit(m, par, g, j):
        u = kvu[m, 1, par, g // 2, g % 2, j // 2:j // 2 + 2]
        if (par, g, j) in wide:
            return jnp.concatenate([pltpu.bitcast(u, F32), vx[m, wide[(par, g, j)]]], axis=1)
        return f32_rows(u)

    def pv_ops(m, ph):
        acc = {}

        def spread(par, q, r):
            pb_scr[pl.ds(64 * q + r, 8, stride=8), :] = p_scr[ph, par, 8 * q:8 * q + 8, :]

        def psum(par):
            p = p_scr[ph, par]
            accx[ph, 8 * (2 * G + par):8 * (2 * G + par) + 8, :] = (
                (p[0:8] + p[8:16]) + (p[16:24] + p[24:32]))

        pbv = {}

        def piece(par, gb, j0, k):
            if k == 0:
                if par == 0 and j0 < 8:
                    pb = pb0[ph, 8 * j0:8 * j0 + 32, :]
                else:
                    pb = pb_scr[8 * j0:8 * j0 + 32, :]
                pbv[0] = pb.reshape(4, 8, 128)
            for _, g, _ in units(par, gb, j0)[4 * k:4 * k + 4]:
                tv = v_unit(m, par, g, j0).reshape(4, 8, 128) * pbv[0]
                tv = jnp.sum(tv, axis=0)
                acc[g] = tv if j0 == 0 else acc[g] + tv
                if j0 == nblk - 4:
                    r0 = DH * par + 8 * g
                    accx[ph, r0:r0 + 8, :] = acc[g]

        pieces = [s + (k,) for s in steps for k in range(NA // 4)]
        half = len(pieces) // 2
        spq = 2 * (NA // 4)
        side = {}
        for q in range(nq):
            for r in range(8):
                if q:
                    side.setdefault((spq * (8 * (q - 1) + r)) // 9, []).append(
                        lambda q=q, r=r: spread(0, q, r))
                side.setdefault(half - nq * spq + spq * (q + 1) + (r * (3 * spq - 1)) // 8, []).append(
                    lambda q=q, r=r: spread(1, q, r))
        for par in range(2):
            side.setdefault(half // 2 + par, []).append(lambda par=par: psum(par))
        out = []
        for i, s in enumerate(pieces):
            out += [(0, f) for f in side.get(i, [])]
            out.append((2 * sum(4 if u in wide else 6 for u in units(*s[:3])[4 * s[3]:4 * s[3] + 4]),
                        (lambda s=s: piece(*s))))
        return out

    toks = []

    def fence(dst, slot, zero_i):
        for i, t in enumerate(toks):
            dst[slot + i + zero_i] = t
        toks.clear()

    def g_softmax(ph, par):
        s0 = part[2 * nq:3 * nq] if par else part_a[0:nq]
        s = (s0 + part[(2 * par + 1) * nq:(2 * par + 2) * nq]).reshape(nblk, 128)
        mx = jnp.max(jnp.max(s, axis=0, keepdims=True), axis=1, keepdims=True)
        p = jnp.exp2((s - mx) * jnp.concatenate([rs_scr[0]] * nq, axis=0))
        p_scr[ph, par] = p
        if par == 0:
            for r in range(8):
                pb0[ph, pl.ds(r, 8, stride=8), :] = p[0:8]
        toks.append(pltpu.bitcast(p[nblk - 8:nblk], U32))

    def recip(d):
        r = pl.reciprocal(d, approx=True)
        return r * (2.0 - d * r)

    def g_olhs(slot0, ph):
        z = [lane_sum(accx[ph, 8 * g:8 * g + 8, :]) for g in range(NZ)]
        inv = [jnp.broadcast_to(recip(jnp.sum(z[2 * G + par], axis=0, keepdims=True)), (8, 128))
               for par in range(2)]
        uid[0] += 1
        bit = [b > uid[0] for b in bit_i]
        for c in range(3):
            xs = z[16 * c:16 * c + 16]
            for k in range(4):
                xs = [jnp.where(bit[k], xs[i + 1], xs[i]) for i in range(0, len(xs), 2)]
            iv = inv[0] if c == 0 else (inv[1] if c == 2 else jnp.where(bit[3], inv[1], inv[0]))
            olhs[slot0 + c, 0:8, :] = jnp.where(diag_i > uid[0], xs[0] * iv, 0.0).astype(BF)

    def set_pat(c, q):
        if c == 1:
            hi = bit_i[3] > uid[0]
            pat_scr[c, 0:8, :] = jnp.where(hi, 0.0, q).astype(BF)
            pat_scr[c, 8:16, :] = jnp.where(hi, q, 0.0).astype(BF)
        else:
            pat_scr[c, 0:8, :] = q.astype(BF)
        if c > 0:
            toks.append(pltpu.bitcast(q, U32))

    def g_query(c):
        xs = [qpart[c * KD + k] for k in range(KD)]
        set_pat(c, ((xs[0] + xs[1]) + (xs[2] + xs[3])) + xs[4])

    def g_out(ph):
        for n in range(KD):
            out_scr[n] = out_scr[n] + opart[8 * ph + n]

    def reset_pipeline():
        accx[1, 0:16 * G, :] = jnp.zeros((16 * G, 128), F32)
        accx[1, 16 * G:16 * G + 16, :] = jnp.ones((16, 128), F32)
        for n in range(KD):
            opart[8 + n] = jnp.zeros((8, 128), F32)
            out_scr[n] = jnp.zeros((8, 128), F32)

    def emit(pv, seq):
        ntile = sum(not isinstance(e, tuple) for e in seq)
        total = sum(w for w, _ in pv) / 4
        k = done = n = 0
        for e in seq:
            if isinstance(e, tuple):
                e[0]()
                continue
            pos = LEAD + RATE * (n // 4) if n // 4 < (ntile - 1) // 4 else total - TAILC
            while k < len(pv) and done + pv[k][0] / 2 <= 4 * pos:
                done += pv[k][0]
                pv[k][1]()
                k += 1
            e(n < ntile - UNPACED)
            n += 1
        for _, g in pv[k:]:
            g()

    def ffn1(x):
        _, xc, rs = moments(x)
        y = jnp.broadcast_to(xc, (8, D)).astype(BF)
        reset_pipeline()

        def up(wu):
            cols = []
            for cp in range(NC // 2):
                ev, od = swap_halves(wu[:, 0, cp], wu[:, 1, cp])
                wu[:, 0, cp], wu[:, 1, cp] = ev, od
                cols += [jnp.dot(y, pltpu.bitcast(w.reshape(D // 2, 128), BF),
                                 preferred_element_type=F32) for w in (ev, od)]
            return jnp.concatenate(cols, axis=1) * rs

        def w2_rows(r0, n):
            v = w2u[r0:r0 + n]
            h = [v[:, f // 2, 4 * (f % 2):4 * (f % 2) + 4, :] for f in range(2 * KD)]
            nat = [jnp.concatenate([h[c], h[KD + c]], axis=1) for c in range(KD)]
            for c in range(KD):
                w2u[r0:r0 + n, c] = nat[c]
            return v, nat

        def down(o, n):
            cols = [None] * KD
            for k in range(o // 128, (o + n) // 128):
                for c, w in enumerate(w2_rows(8 * k, 8)[1]):
                    t = jnp.dot(hh[:, 128 * k:128 * k + 128], pltpu.bitcast(w.reshape(64, 128), BF),
                                preferred_element_type=F32)[0:1]
                    cols[c] = t if cols[c] is None else cols[c] + t
            return jnp.concatenate(cols, axis=1)

        c_w1.wait()
        g = up(w1u)
        c_w3.wait()
        u = up(w3u)
        hh = (g * jax.nn.sigmoid(g) * u).astype(BF)
        hb = columns(hh[:, w2_off[-1]:].astype(F32))
        a = None
        parts = list(zip(c_w2, w2_off, W2_CHUNKS))[:-1]
        if W2S:
            parts.insert(1, (w2_out, 0, 16 * W2S))
        for c, o, n in parts:
            c.wait()
            a = down(o, n) if a is None else a + down(o, n)
        c_w2[-1].wait()
        acc = [None] * KD
        for r in range(W2_CHUNKS[-1] // 16):
            v = f32_rows(w2_rows(w2_off[-1] // 16 + r, 1)[0][0])
            for f in range(2 * KD):
                tv = v[f // 2, 8 * (f % 2):8 * (f % 2) + 8] * hb[2 * r + f // KD]
                acc[f % KD] = tv if acc[f % KD] is None else acc[f % KD] + tv
        a = a + jnp.concatenate([jnp.sum(t, axis=0, keepdims=True) for t in acc], axis=1)
        return residual(x, a)

    def ffn2(x):
        mu, _, rs = moments(x)
        x8 = jnp.broadcast_to(x, (8, D))
        rowk = lax.broadcasted_iota(jnp.int32, (8, 128 * KM), 0)
        y = jnp.where(rowk == 0, x8[:, :128 * KM], jnp.where(rowk == 1, 1.0, 0.0)).astype(BF)
        coef = jnp.where(row == 0, 1.0, -mu)
        yb = jnp.concatenate([c - mu for c in columns(x8[:, 128 * KM:])], axis=0)
        mx = {}
        out = [None] * KD
        for c in range(NC):
            while len(mx) < min(NC, FPRE + c * FSTEP / 4):
                cc = len(mx)
                mx[cc] = [jnp.dot(y, pltpu.bitcast(wu[0:8 * KM, cc & 1, cc >> 1].reshape(64 * KM, 128), BF),
                                  preferred_element_type=F32) * coef for wu in (w1u, w3u)]
            gu = []
            for i, wu in enumerate((w1u, w3u)):
                acc = None
                for r in range(8 * (KD - KM)):
                    tv = f32_rows(wu[8 * KM + r, c & 1, c >> 1]) * yb[16 * r:16 * r + 16]
                    acc = tv if r == 0 else acc + tv
                gu.append(jnp.sum((acc[:8] + acc[8:]) + mx[c][i], axis=0, keepdims=True) * rs)
            hg = 0.5 * gu[0]
            h = jnp.broadcast_to((hg * jnp.tanh(hg) + hg) * gu[1], (8, 128)).astype(BF)
            for n in range(KD):
                t = jnp.dot(h, pltpu.bitcast(w2u[8 * c:8 * c + 8, n].reshape(64, 128), BF),
                            preferred_element_type=F32)[0:1]
                out[n] = t if c == 0 else out[n] + t
        return residual(x, jnp.concatenate(out, axis=1))

    def layer(li, x):
        first = li == 0
        zero_i = li >> 4

        def barrier():
            @pl.when(li > 2)
            def _():
                reset_pipeline()

        mu, xc, rs = moments(x)
        y = jnp.broadcast_to(xc, (8, D))
        for k in range(KD):
            y_scr[k, 0:8, :] = y[:, 128 * k:128 * k + 128].astype(BF)
        rs_scr[0] = jnp.broadcast_to(rs * c2, (8, 128))
        rowd = lax.broadcasted_iota(jnp.int32, (8, D), 0)
        xo = jnp.where(rowd < 4, jnp.broadcast_to(x, (8, D)), 1.0).astype(BF)
        coef = jnp.where(row < 4, 1.0, -mu)

        def q_direct(col):
            t = jnp.dot(xo, pltpu.bitcast(wqu[0, :, col & 1, col >> 1].reshape(D // 2, 128), BF), preferred_element_type=F32) * coef
            return (t + pltpu.roll(t, 4, 0)).astype(BF).astype(F32)

        def q_cols(q, slot):
            for b, col in enumerate(columns(q)):
                part[slot + b] = col

        def vpu_a(m, slot, js):
            acc = {}
            for g2 in range(8):
                qc = jnp.concatenate([part[slot + 2 * g2 + t + zero_i] for t in range(2)], axis=0)
                for j in js:
                    tv = f32_rows(kvu[m, 0, 0, g2, j & 1, j >> 1]) * qc
                    acc[j] = tv if g2 == 0 else acc[j] + tv
            for j in js:
                part_a[j // 8, j % 8:j % 8 + 1, :] = jnp.sum(acc[j], axis=0, keepdims=True)

        q0 = [q_direct(c) for c in range(4)]
        q_cols(q0[0], SP)
        set_pat(1, q0[1])
        set_pat(2, q0[2])
        _, qb, qc = qk_ops(0)
        for i in range(nblk // 2):
            if i == 4:
                q_cols(q0[3], SP + 16)
            vpu_a(0, SP, jord[2 * i:2 * i + 2])
            plain((qb + qc)[4 * i:4 * i + 4])
        g_softmax(0, 0)
        g_softmax(0, 1)
        plain(qproj_ops((0, 1))[KD:])
        g_query(1)
        g_query(2)
        set_pat(0, q0[3])
        plain(qk_ops(1)[0][PVB:])
        for i in range(0, PVB, 2):
            part[0] = qpart[min(KD + 4 + 3 * i // 2, 3 * KD - 1)]
            vpu_a(1, SP + 16, jord[i:i + 2])
        toks.clear()

        def block(t, ph):
            m = 2 * t + ph

            @pl.when(first)
            def _():
                kv_copy(m + 2, 0).wait()
                if ph == 1:
                    pl.when(m + 3 == NP)(start_ffn_weights)
                pair_rows(m + 2)
                if ph == 0 or not W2S:
                    stage_step(m + 5)
                else:
                    pl.when(m + 5 <= NST)(lambda: stage_step(m + 5))
                kv_copy(m + 2, 1).wait()

                @pl.when(m + 2 + KVW < NP)
                def _():
                    for i in range(2):
                        kv_copy(m + 2 + KVW, i).start()

                widen(m + 2)

            qp = qproj_ops((t, ph + 2))
            _, qb, qc = qk_ops(m + 1)
            qa = qk_ops(m + 2)[0]
            op = oproj_ops(jnp.maximum(m - 1, 0), m + 2, opart, 8 * ph)
            seq = ([(lambda: g_out(1 - ph),), (lambda: g_olhs(3 * m, 1 - ph),)]
                   + qc[:CF] + qp[:KD] + [(lambda: g_query(0),)] + qc[CF:] + qb
                   + [(lambda: g_softmax(1 - ph, 0),), (lambda: g_softmax(1 - ph, 1),)]
                   + qp[KD:] + [(lambda: g_query(1),), (lambda: g_query(2),)]
                   + op + qa[:nblk - AEND] + [(lambda: fence(pat_u, 3, zero_i),)]
                   + qa[nblk - AEND:])
            emit(pv_ops(m, ph), seq)

        def body(t, carry):
            block(t, 0)
            block(t, 1)
            return carry

        lax.fori_loop(0, NP // 2 - 1, body, 0)

        def big(kts, i0):
            return [op for i, kt in enumerate(kts)
                    for op in oproj_ops(kt, kt + 3, part, SP + KD * (i0 + i))]

        old = list(range(NP - 3, 3 * (NP - 3)))
        barrier()
        _, qb, qc = qk_ops(NP - 1)
        seq = ([(lambda: g_out(1),), (lambda: g_olhs(3 * (NP - 2), 1),)] + qc + qb
               + [(lambda: g_softmax(1, 0),), (lambda: g_softmax(1, 1),)]
               + big(old[:KT14 - 4] + list(range(3 * (NP - 3), 3 * (NP - 2))), 0)
               + [(lambda: fence(olhs_u, 3 * NP, zero_i),)]
               + big(old[KT14 - 4:KT14 - 3], KT14 - 1))
        emit(pv_ops(NP - 2, 0), seq)
        barrier()
        k15 = old[KT14 - 3:-1] + list(range(3 * (NP - 2), 3 * (NP - 1))) + old[-1:]
        emit(pv_ops(NP - 1, 1), [(lambda: g_olhs(3 * (NP - 1), 0),)] + big(k15, KT14))

        def epilogue(x):
            def lsum(g):
                return lane_sum(accx[1, 8 * g:8 * g + 8, :])

            den = [jnp.sum(lsum(2 * G + par), axis=0, keepdims=True) for par in range(2)]
            fac = [den[0], den[1] * recip(den[0]), recip(den[1])]
            acc = []
            for n in range(KD):
                t = out_scr[n]
                for i in range(2 * NP):
                    t = t + part[SP + KD * i + n]
                acc.append(t * fac[0])
            for par in range(2):
                for g2 in range(G2):
                    g = G * par + 2 * g2
                    z0, z1 = lsum(g), lsum(g + 1)
                    for n in range(KD):
                        v = f32_rows(wou[(NP - 1) * G + G2 * par + g2, n])
                        acc[n] = acc[n] + (v[:8] * z0 + v[8:] * z1)
                acc = [t * fac[par + 1] for t in acc]
            cols = [jnp.sum(t, axis=0, keepdims=True) for t in acc]
            return residual(x, jnp.concatenate(cols, axis=1))

        def tail1(x):
            if W2S:
                stage_step(NST + 1)
            return ffn1(epilogue(x))

        return lax.cond(first, tail1, lambda x: ffn2(epilogue(x)), x)

    for r in (y_u, pat_u, olhs_u):
        r[...] = jnp.zeros(r.shape, U32)
    reset_pipeline()
    stage_step(1)
    c_wo.wait()
    pair_wo(0, R0)
    stage_step(2)
    for m in range(KVW + 2):
        for i in range(2):
            kv_copy(m, i).start()
    for m in range(2):
        kv_copy(m, 0).wait()
        pair_rows(m)
        stage_step(3 + m)
        kv_copy(m, 1).wait()
        widen(m)
    wait_all([c_x] + c_wq)
    pair_wq()
    x = lax.fori_loop(0, 2, layer, xb[...].astype(F32))
    o_ref[...] = x.astype(o_ref.dtype)


@jax.jit
def pallas_interleave_layers__sliding_block_cached__glu_gated_swiglu__decode_kernel(
    A_x: jax.Array,
    A_k_cache: jax.Array,
    A_v_cache: jax.Array,
    A_wq: jax.Array,
    A_wo: jax.Array,
    B_x: jax.Array,
    B_w1: jax.Array,
    B_w3: jax.Array,
    B_w2: jax.Array,
):
    del B_x
    sk = A_k_cache.shape[2]
    win = min(4096, max(256, sk // 4))
    nb = sk // 128
    nblk = win // 128

    def cache_tiles(c):
        return (c.reshape(H, nb, 128, G2, 2, 8).transpose(0, 3, 4, 1, 5, 2)
                .reshape(H, G2, 2, nb // 2, 16, 128))

    def weight_tiles(w):
        r, c = w.shape
        return w.reshape(r // 16, 2, 8, c // 128, 128).transpose(0, 1, 3, 2, 4)

    vreg = lambda n: pltpu.VMEM((-(-n // 4) * 4, 8, 128), F32)
    lhs = lambda n: pltpu.VMEM((-(-n // 4) * 4, 16, 128), BF)
    kern = lambda *refs: _kernel(*refs, blk0=nb - nblk, nblk=nblk, scale=DH ** -0.5)
    out = pl.pallas_call(
        kern,
        out_shape=jax.ShapeDtypeStruct((1, D), BF),
        in_specs=[pl.BlockSpec(memory_space=pl.ANY)] * 8,
        out_specs=pl.BlockSpec(memory_space=pltpu.VMEM),
        scratch_shapes=[
            pltpu.VMEM((1, D), BF),
            pltpu.VMEM((NP, 2, 2, G2, 2, nblk // 2, 16, 128), BF),
            pltpu.VMEM((NP // 2, D // 16, 2, 3, 16, 128), BF),
            pltpu.VMEM((H * DH // 16, KD, 16, 128), BF),
            pltpu.VMEM((D // 16, 2, NC // 2, 16, 128), BF),
            pltpu.VMEM((D // 16, 2, NC // 2, 16, 128), BF),
            pltpu.VMEM((FF // 16, KD, 16, 128), BF),
            lhs(KD),
            vreg(1),
            vreg(3 * KD),
            lhs(8),
            vreg(nblk // 8),
            vreg(nblk // 2 + 2 * NP * KD),
            pltpu.VMEM((2, 2, nblk, 128), F32),
            pltpu.VMEM((nblk * 8, 128), F32),
            pltpu.VMEM((2, 64, 128), F32),
            pltpu.VMEM((2, 8 * NR, 128), F32),
            lhs(3 * NP + 4),
            vreg(16),
            vreg(KD),
            pltpu.VMEM((NP, NW, 2, 8, 128), F32),
            pltpu.SMEM((2, SC, KD, 16, 128), BF),
            pltpu.SemaphoreType.DMA((2, NP)),
            pltpu.SemaphoreType.DMA((5 + len(W2_CHUNKS),)),
            pltpu.SemaphoreType.DMA((2,)),
        ],
        compiler_params=pltpu.CompilerParams(
            vmem_limit_bytes=128 * 1024 * 1024, disable_semaphore_checks=True),
    )(A_x.reshape(1, D), cache_tiles(A_k_cache), cache_tiles(A_v_cache),
      weight_tiles(A_wq).reshape(D // 16, 2, 3 * NP // 2, 16, 128),
      weight_tiles(A_wo).reshape(H * G2, KD, 16, 128),
      weight_tiles(B_w1).reshape(D // 16, 2, NC // 2, 16, 128),
      weight_tiles(B_w3).reshape(D // 16, 2, NC // 2, 16, 128),
      weight_tiles(B_w2).reshape(FF // 16, KD, 16, 128))
    return out.reshape(1, 1, D)
```

```python
import math

import jax
import jax.numpy as jnp
from jax import lax
import jax.experimental.pallas as pl
import jax.experimental.pallas.tpu as pltpu

BF = jnp.bfloat16
F32 = jnp.float32
U32 = jnp.uint32

D = 640
H = 32
DH = 192
G = DH // 8
G2 = DH // 16
NP = H // 2
FF = 1536
EPS = 1e-5
KD = D // 128
NC = FF // 128
NZ = 2 * G + 2
NR = NZ + 2
W2S = 8
W2_CHUNKS = (768 - 16 * W2S, 384, 256, 128)

NA = 8
NW = 72
UNPACED = 8
LEAD = 16
RATE = 32.5
TAILC = 30
AEND = 4
CF = 8
KT14 = 10
PVB = 12
KM = 3
FPRE = 8
FSTEP = 3
NST = NP + 1
SC = 10
KVW = 4
PQH = 4
PTK = 6
PFB = 3


def _kernel(x_hbm, k_hbm, v_hbm, wq_hbm, wo_hbm, w1_hbm, w3_hbm, w2_hbm,
            o_ref,
            xb, kvb, wq, wo, w1, w3, w2,
            y_scr, rs_scr, qpart, pat_scr, part_a, part, p_scr, pb_scr, pb0,
            accx, olhs, opart, out_scr, vx, stage,
            kvsem, wsem, ssem, *, blk0, nblk, scale):
    c2 = scale * math.log2(math.e)
    nq = nblk // 8
    SP = 4 * nq

    def kv_copy(m, i):
        return pltpu.make_async_copy(
            (k_hbm, v_hbm)[i].at[pl.ds(2 * m, 2), :, :, pl.ds(blk0 // 2, nblk // 2)],
            kvb.at[m, i], kvsem.at[i, m])

    c_x = pltpu.make_async_copy(x_hbm, xb, wsem.at[0])
    c_wq = [pltpu.make_async_copy(wq_hbm.at[:, :, pl.ds(3 * b, 3)], wq.at[b], wsem.at[1])
            for b in range(NP // 2)]
    R0 = H * G2 - NST * SC
    c_wo = pltpu.make_async_copy(wo_hbm.at[pl.ds(0, R0)], wo.at[pl.ds(0, R0)], wsem.at[2])

    def to_stage(k):
        return pltpu.make_async_copy(wo_hbm.at[pl.ds(R0 + SC * k, SC)], stage.at[k & 1],
                                     ssem.at[0])

    def from_stage(k):
        return pltpu.make_async_copy(stage.at[k & 1], wo.at[pl.ds(R0 + SC * k, SC)], ssem.at[1])

    def stage_step(k):
        def when(cond, f):
            if isinstance(cond, bool):
                if cond:
                    f()
            else:
                pl.when(cond)(f)

        def forward():
            to_stage(k - 1).wait()
            from_stage(k - 1).start()

        landed = not isinstance(k, int) or k >= 2
        if landed:
            from_stage(k - 2).wait()
        when(k <= NST, forward)
        when(k < NST, lambda: to_stage(k).start())
        if W2S:
            when(k == NST, w2_in.start)
            if isinstance(k, int) and k == NST + 1:
                w2_in.wait()
                w2_out.start()
        if landed:
            pair_wo(R0 + SC * (k - 2), SC)

    c_w1 = pltpu.make_async_copy(w1_hbm, w1, wsem.at[3])
    c_w3 = pltpu.make_async_copy(w3_hbm, w3, wsem.at[4])
    w2_off = [16 * W2S + sum(W2_CHUNKS[:i]) for i in range(len(W2_CHUNKS))]
    c_w2 = [pltpu.make_async_copy(w2_hbm.at[pl.ds(o // 16, n // 16)],
                                  w2.at[pl.ds(o // 16, n // 16)], wsem.at[5 + i])
            for i, (o, n) in enumerate(zip(w2_off, W2_CHUNKS))]
    if W2S:
        w2_slot = stage.at[NST & 1, pl.ds(0, W2S)]
        w2_in = pltpu.make_async_copy(w2_hbm.at[pl.ds(0, W2S)], w2_slot, ssem.at[0])
        w2_out = pltpu.make_async_copy(w2_slot, w2.at[pl.ds(0, W2S)], ssem.at[1])

    def wait_all(cs):
        for c in cs:
            c.wait()

    c_wo.start()
    to_stage(0).start()
    for c in [c_x] + c_wq:
        c.start()

    def start_ffn_weights():
        for c in [c_w1, c_w3] + c_w2:
            c.start()

    kvu = kvb.bitcast(U32)
    wqu = wq.bitcast(U32)
    wou = wo.bitcast(U32)
    w1u, w3u, w2u = w1.bitcast(U32), w3.bitcast(U32), w2.bitcast(U32)
    y_u, pat_u, olhs_u = y_scr.bitcast(U32), pat_scr.bitcast(U32), olhs.bitcast(U32)

    def f32_rows(u):
        return pltpu.bitcast(u, BF).astype(F32)

    lane = lax.broadcasted_iota(jnp.int32, (8, 128), 1)
    row = lax.broadcasted_iota(jnp.int32, (8, 128), 0)
    diag_i = ((lane & 7) == row).astype(jnp.int32) * 64
    bit_i = [(lane << (3 - k)) & 64 for k in range(4)]
    uid = [0]

    def lane_sum(v):
        return jnp.broadcast_to(jnp.sum(v, axis=1, keepdims=True), (8, 128))

    def columns(v8):
        uid[0] += 1
        off = 256 * uid[0]
        dl = lane - row + off
        return [lane_sum(jnp.where(dl == off + 8 * b, v8[:, 128 * k:128 * k + 128], 0.0))
                for k in range(v8.shape[1] // 128) for b in range(16)]

    def moments(x):
        mu = jnp.mean(x, axis=-1, keepdims=True)
        xc = x - mu
        return mu, xc, 1.0 / jnp.sqrt(jnp.mean(xc * xc, axis=-1, keepdims=True) + EPS)

    def residual(x, a):
        return (x + a.astype(BF).astype(F32)).astype(BF).astype(F32)

    def tile_dot(l_u32, w_u32, rows, paced):
        w = pltpu.bitcast(w_u32.reshape(64, 128), BF)
        if paced:
            l = pltpu.bitcast(jnp.concatenate([l_u32, l_u32], axis=0), BF)[:24]
            return jnp.dot(l, w, preferred_element_type=F32)[:rows]
        l = pltpu.bitcast(l_u32, BF)[:rows]
        return jnp.dot(l, w, preferred_element_type=F32)

    def swap_halves(a, b):
        return (jnp.concatenate([a[..., :4, :], b[..., :4, :]], axis=-2),
                jnp.concatenate([a[..., 4:, :], b[..., 4:, :]], axis=-2))

    def pair_wq():
        def body(i, carry):
            b, r = i // KD, pl.ds(8 * (i % KD), 8)
            wqu[b, r, 0], wqu[b, r, 1] = swap_halves(wqu[b, r, 0], wqu[b, r, 1])
            return carry
        lax.fori_loop(0, KD * (NP // 2), body, 0)

    def pair_wo(r0, n):
        def body(i, carry):
            r = pl.ds(r0 + 2 * i, 2)
            v = wou[r]
            h = [v[:, f // 2, 4 * (f % 2):4 * (f % 2) + 4, :] for f in range(2 * KD)]
            for c in range(KD):
                wou[r, c] = jnp.concatenate([h[c], h[KD + c]], axis=1)
            return carry
        lax.fori_loop(0, n // 2, body, 0)

    def wq_tile(m, c, k):
        c6 = 3 * m[1] + c
        return wqu[m[0] + c6 // 6, 8 * k:8 * k + 8, c6 & 1, (c6 % 6) >> 1]

    def qproj_ops(m):
        def op(paced, c, k):
            qpart[c * KD + k] = tile_dot(
                y_u[k], wq_tile(m, c, k), 8, paced)
        return [(lambda p, c=c, k=k: op(p, c, k)) for c in range(3) for k in range(KD)]

    def oproj_ops(kt, slot, dst, d0):
        def op(paced, n):
            dst[d0 + n] = tile_dot(olhs_u[slot], wou[pl.ds(kt * 8, 8), n], 8, paced)
        return [(lambda p, n=n: op(p, n)) for n in range(KD)]

    def pair_rows(m):
        def body(i, c):
            par, g2 = i // G2, i % G2
            kvu[m, 0, par, g2, 0], kvu[m, 0, par, g2, 1] = swap_halves(
                kvu[m, 0, par, g2, 0], kvu[m, 0, par, g2, 1])
            return c
        lax.fori_loop(0, 2 * G2, body, 0)

    def k_blocks(m, par, g0, g1, j):
        return kvu[m, 0, par, g0:g1, j & 1, j >> 1]

    jord = [8 * (i // 8) + 2 * (i % 4) + (i % 8) // 4 for i in range(nblk)]

    def qk_ops(m):
        def op_a(paced, j):
            r = tile_dot(pat_u[0], k_blocks(m, 0, 0, 8, j), 8, paced)
            part_a[j // 8, j % 8:j % 8 + 1, :] = r[j % 8:j % 8 + 1, :]

        def op_c(paced, j):
            r = tile_dot(pat_u[2], k_blocks(m, 1, 4, 12, j), 8, paced)
            part[2 * nq + j // 8, j % 8:j % 8 + 1, :] = r[j % 8:j % 8 + 1, :]

        def op_b(paced, j):
            w = jnp.concatenate([k_blocks(m, 0, 8, 12, j), k_blocks(m, 1, 0, 4, j)], axis=0)
            r = tile_dot(pat_u[1], w, 16, paced)
            part[nq + j // 8, j % 8:j % 8 + 1, :] = r[j % 8:j % 8 + 1, :]
            part[3 * nq + j // 8, j % 8:j % 8 + 1, :] = r[8 + j % 8:8 + j % 8 + 1, :]

        return [[(lambda p, f=f, j=j: f(p, j)) for j in jord] for f in (op_a, op_b, op_c)]

    def plain(ops):
        for op in ops:
            op(False)

    steps = [(par, gb, j0) for par in range(2) for gb in range(G // NA)
             for j0 in range(0, nblk, 4)]

    def units(par, gb, j0):
        return [(par, g, j0) for g in range(gb * NA, (gb + 1) * NA)]

    order = [u for s in steps for u in units(*s)]
    wide = {}
    for i, u in enumerate(order):
        if (i + 1) * NW // len(order) > i * NW // len(order):
            wide[u] = len(wide)

    def widen(m):
        for (par, g, j), e in wide.items():
            v = f32_rows(kvu[m, 1, par, g // 2, g % 2, j // 2:j // 2 + 2])
            kvu[m, 1, par, g // 2, g % 2, j // 2:j // 2 + 2] = pltpu.bitcast(v[:, :8], U32)
            vx[m, e] = v[:, 8:]

    def v_unit(m, par, g, j):
        u = kvu[m, 1, par, g // 2, g % 2, j // 2:j // 2 + 2]
        if (par, g, j) in wide:
            return jnp.concatenate([pltpu.bitcast(u, F32), vx[m, wide[(par, g, j)]]], axis=1)
        return f32_rows(u)

    def pv_ops(m, ph):
        acc = {}

        def spread(par, q, r):
            pb_scr[pl.ds(64 * q + r, 8, stride=8), :] = p_scr[ph, par, 8 * q:8 * q + 8, :]

        def psum(par):
            p = p_scr[ph, par]
            accx[ph, 8 * (2 * G + par):8 * (2 * G + par) + 8, :] = (
                (p[0:8] + p[8:16]) + (p[16:24] + p[24:32]))

        pbv = {}

        def piece(par, gb, j0, k):
            if k == 0:
                if par == 0 and j0 < 8:
                    pb = pb0[ph, 8 * j0:8 * j0 + 32, :]
                else:
                    pb = pb_scr[8 * j0:8 * j0 + 32, :]
                pbv[0] = pb.reshape(4, 8, 128)
            for _, g, _ in units(par, gb, j0)[4 * k:4 * k + 4]:
                tv = v_unit(m, par, g, j0).reshape(4, 8, 128) * pbv[0]
                tv = jnp.sum(tv, axis=0)
                acc[g] = tv if j0 == 0 else acc[g] + tv
                if j0 == nblk - 4:
                    r0 = DH * par + 8 * g
                    accx[ph, r0:r0 + 8, :] = acc[g]

        pieces = [s + (k,) for s in steps for k in range(NA // 4)]
        half = len(pieces) // 2
        spq = 2 * (NA // 4)
        side = {}
        for q in range(nq):
            for r in range(8):
                if q:
                    side.setdefault((spq * (8 * (q - 1) + r)) // 9, []).append(
                        lambda q=q, r=r: spread(0, q, r))
                side.setdefault(half - nq * spq + spq * (q + 1) + (r * (3 * spq - 1)) // 8, []).append(
                    lambda q=q, r=r: spread(1, q, r))
        for par in range(2):
            side.setdefault(half // 2 + par, []).append(lambda par=par: psum(par))
        out = []
        for i, s in enumerate(pieces):
            out += [(0, f) for f in side.get(i, [])]
            out.append((2 * sum(4 if u in wide else 6 for u in units(*s[:3])[4 * s[3]:4 * s[3] + 4]),
                        (lambda s=s: piece(*s))))
        return out

    toks = []

    def fence(dst, slot, zero_i):
        for i, t in enumerate(toks):
            dst[slot + i + zero_i] = t
        toks.clear()

    def g_softmax(ph, par):
        s0 = part[2 * nq:3 * nq] if par else part_a[0:nq]
        s = (s0 + part[(2 * par + 1) * nq:(2 * par + 2) * nq]).reshape(nblk, 128)
        mx = jnp.max(jnp.max(s, axis=0, keepdims=True), axis=1, keepdims=True)
        p = jnp.exp2((s - mx) * jnp.concatenate([rs_scr[0]] * nq, axis=0))
        p_scr[ph, par] = p
        if par == 0:
            for r in range(8):
                pb0[ph, pl.ds(r, 8, stride=8), :] = p[0:8]
        toks.append(pltpu.bitcast(p[nblk - 8:nblk], U32))

    def recip(d):
        r = pl.reciprocal(d, approx=True)
        return r * (2.0 - d * r)

    def g_olhs(slot0, ph):
        z = [lane_sum(accx[ph, 8 * g:8 * g + 8, :]) for g in range(NZ)]
        inv = [jnp.broadcast_to(recip(jnp.sum(z[2 * G + par], axis=0, keepdims=True)), (8, 128))
               for par in range(2)]
        uid[0] += 1
        bit = [b > uid[0] for b in bit_i]
        for c in range(3):
            xs = z[16 * c:16 * c + 16]
            for k in range(4):
                xs = [jnp.where(bit[k], xs[i + 1], xs[i]) for i in range(0, len(xs), 2)]
            iv = inv[0] if c == 0 else (inv[1] if c == 2 else jnp.where(bit[3], inv[1], inv[0]))
            olhs[slot0 + c, 0:8, :] = jnp.where(diag_i > uid[0], xs[0] * iv, 0.0).astype(BF)

    def set_pat(c, q):
        if c == 1:
            hi = bit_i[3] > uid[0]
            pat_scr[c, 0:8, :] = jnp.where(hi, 0.0, q).astype(BF)
            pat_scr[c, 8:16, :] = jnp.where(hi, q, 0.0).astype(BF)
        else:
            pat_scr[c, 0:8, :] = q.astype(BF)
        if c > 0:
            toks.append(pltpu.bitcast(q, U32))

    def g_query(c):
        xs = [qpart[c * KD + k] for k in range(KD)]
        set_pat(c, ((xs[0] + xs[1]) + (xs[2] + xs[3])) + xs[4])

    def g_out(ph):
        for n in range(KD):
            out_scr[n] = out_scr[n] + opart[8 * ph + n]

    def reset_pipeline():
        accx[1, 0:16 * G, :] = jnp.zeros((16 * G, 128), F32)
        accx[1, 16 * G:16 * G + 16, :] = jnp.ones((16, 128), F32)
        for n in range(KD):
            opart[8 + n] = jnp.zeros((8, 128), F32)
            out_scr[n] = jnp.zeros((8, 128), F32)

    def emit(pv, seq):
        ntile = sum(not isinstance(e, tuple) for e in seq)
        total = sum(w for w, _ in pv) / 4
        k = done = n = 0
        for e in seq:
            if isinstance(e, tuple):
                e[0]()
                continue
            pos = LEAD + RATE * (n // 4) if n // 4 < (ntile - 1) // 4 else total - TAILC
            while k < len(pv) and done + pv[k][0] / 2 <= 4 * pos:
                done += pv[k][0]
                pv[k][1]()
                k += 1
            e(n < ntile - UNPACED)
            n += 1
        for _, g in pv[k:]:
            g()

    def ffn1(x):
        _, xc, rs = moments(x)
        y = jnp.broadcast_to(xc, (8, D)).astype(BF)
        reset_pipeline()

        def up(wu):
            cols = []
            for cp in range(NC // 2):
                ev, od = swap_halves(wu[:, 0, cp], wu[:, 1, cp])
                wu[:, 0, cp], wu[:, 1, cp] = ev, od
                cols += [jnp.dot(y, pltpu.bitcast(w.reshape(D // 2, 128), BF),
                                 preferred_element_type=F32) for w in (ev, od)]
            return jnp.concatenate(cols, axis=1) * rs

        def w2_rows(r0, n):
            v = w2u[r0:r0 + n]
            h = [v[:, f // 2, 4 * (f % 2):4 * (f % 2) + 4, :] for f in range(2 * KD)]
            nat = [jnp.concatenate([h[c], h[KD + c]], axis=1) for c in range(KD)]
            for c in range(KD):
                w2u[r0:r0 + n, c] = nat[c]
            return v, nat

        def down(o, n):
            cols = [None] * KD
            for k in range(o // 128, (o + n) // 128):
                for c, w in enumerate(w2_rows(8 * k, 8)[1]):
                    t = jnp.dot(hh[:, 128 * k:128 * k + 128], pltpu.bitcast(w.reshape(64, 128), BF),
                                preferred_element_type=F32)[0:1]
                    cols[c] = t if cols[c] is None else cols[c] + t
            return jnp.concatenate(cols, axis=1)

        c_w1.wait()
        g = up(w1u)
        c_w3.wait()
        u = up(w3u)
        hh = (g * jax.nn.sigmoid(g) * u).astype(BF)
        hb = columns(hh[:, w2_off[-1]:].astype(F32))
        a = None
        parts = list(zip(c_w2, w2_off, W2_CHUNKS))[:-1]
        if W2S:
            parts.insert(1, (w2_out, 0, 16 * W2S))
        for c, o, n in parts:
            c.wait()
            a = down(o, n) if a is None else a + down(o, n)
        c_w2[-1].wait()
        acc = [None] * KD
        for r in range(W2_CHUNKS[-1] // 16):
            v = f32_rows(w2_rows(w2_off[-1] // 16 + r, 1)[0][0])
            for f in range(2 * KD):
                tv = v[f // 2, 8 * (f % 2):8 * (f % 2) + 8] * hb[2 * r + f // KD]
                acc[f % KD] = tv if acc[f % KD] is None else acc[f % KD] + tv
        a = a + jnp.concatenate([jnp.sum(t, axis=0, keepdims=True) for t in acc], axis=1)
        return residual(x, a)

    def ffn2(x):
        mu, _, rs = moments(x)
        x8 = jnp.broadcast_to(x, (8, D))
        rowk = lax.broadcasted_iota(jnp.int32, (8, 128 * KM), 0)
        y = jnp.where(rowk == 0, x8[:, :128 * KM], jnp.where(rowk == 1, 1.0, 0.0)).astype(BF)
        coef = jnp.where(row == 0, 1.0, -mu)
        yb = jnp.concatenate([c - mu for c in columns(x8[:, 128 * KM:])], axis=0)
        mx = {}
        out = [None] * KD
        for c in range(NC):
            while len(mx) < min(NC, FPRE + c * FSTEP / 4):
                cc = len(mx)
                mx[cc] = [jnp.dot(y, pltpu.bitcast(wu[0:8 * KM, cc & 1, cc >> 1].reshape(64 * KM, 128), BF),
                                  preferred_element_type=F32) * coef for wu in (w1u, w3u)]
            gu = []
            for i, wu in enumerate((w1u, w3u)):
                acc = None
                for r in range(8 * (KD - KM)):
                    tv = f32_rows(wu[8 * KM + r, c & 1, c >> 1]) * yb[16 * r:16 * r + 16]
                    acc = tv if r == 0 else acc + tv
                gu.append(jnp.sum((acc[:8] + acc[8:]) + mx[c][i], axis=0, keepdims=True) * rs)
            hg = 0.5 * gu[0]
            h = jnp.broadcast_to((hg * jnp.tanh(hg) + hg) * gu[1], (8, 128)).astype(BF)
            for n in range(KD):
                t = jnp.dot(h, pltpu.bitcast(w2u[8 * c:8 * c + 8, n].reshape(64, 128), BF),
                            preferred_element_type=F32)[0:1]
                out[n] = t if c == 0 else out[n] + t
        return residual(x, jnp.concatenate(out, axis=1))

    def arrive(p, odd):
        def when(cond, f):
            if isinstance(cond, bool):
                if cond:
                    f()
            else:
                pl.when(cond)(f)

        def feed():
            for i in range(2):
                kv_copy(p + KVW, i).start()

        kv_copy(p, 0).wait()
        when(odd and p == NP - 1, start_ffn_weights)
        pair_rows(p)
        when(not odd or p + 3 <= NST, lambda: stage_step(p + 3))
        kv_copy(p, 1).wait()
        when(p + KVW < NP, feed)
        widen(p)

    def layer(li, x):
        first = li == 0
        zero_i = li >> 4

        def barrier():
            @pl.when(li > 2)
            def _():
                reset_pipeline()

        mu, xc, rs = moments(x)
        y = jnp.broadcast_to(xc, (8, D))
        for k in range(KD):
            y_scr[k, 0:8, :] = y[:, 128 * k:128 * k + 128].astype(BF)
        rs_scr[0] = jnp.broadcast_to(rs * c2, (8, 128))
        rowd = lax.broadcasted_iota(jnp.int32, (8, D), 0)
        xo = jnp.where(rowd < 4, jnp.broadcast_to(x, (8, D)), 1.0).astype(BF)
        coef = jnp.where(row < 4, 1.0, -mu)

        def q_direct(col):
            t = jnp.dot(xo, pltpu.bitcast(wqu[0, :, col & 1, col >> 1].reshape(D // 2, 128), BF), preferred_element_type=F32) * coef
            return (t + pltpu.roll(t, 4, 0)).astype(BF).astype(F32)

        def q_cols(q, slot):
            for b, col in enumerate(columns(q)):
                part[slot + b] = col

        def vpu_a(m, slot, js):
            acc = {}
            for g2 in range(8):
                qc = jnp.concatenate([part[slot + 2 * g2 + t + zero_i] for t in range(2)], axis=0)
                for j in js:
                    tv = f32_rows(kvu[m, 0, 0, g2, j & 1, j >> 1]) * qc
                    acc[j] = tv if g2 == 0 else acc[j] + tv
            for j in js:
                part_a[j // 8, j % 8:j % 8 + 1, :] = jnp.sum(acc[j], axis=0, keepdims=True)

        q0 = [q_direct(c) for c in range(4)]
        q_cols(q0[0], SP)
        set_pat(1, q0[1])
        set_pat(2, q0[2])
        _, qb, qc = qk_ops(0)
        for i in range(nblk // 2):
            if i == PQH:
                q_cols(q0[3], SP + 16)
            vpu_a(0, SP, jord[2 * i:2 * i + 2])
            plain((qb + qc)[4 * i:4 * i + 4])
        g_softmax(0, 0)
        g_softmax(0, 1)
        plain(qproj_ops((0, 1))[KD:])
        g_query(1)
        g_query(2)
        set_pat(0, q0[3])
        qa = qk_ops(1)[0][PVB:]
        k = 0
        for i in range(0, PVB, 2):
            n = PTK + PFB * i // 2
            if n < 2 * KD:
                part[0] = qpart[KD + n]
            else:
                n = min(n - 2 * KD, len(qa) - 1)
                plain(qa[k:n + 1])
                k = max(k, n + 1)
                part[0] = part_a[jord[PVB + n] // 8]
            vpu_a(1, SP + 16, jord[i:i + 2])
        plain(qa[k:])
        toks.clear()

        def block(t, ph):
            m = 2 * t + ph

            qp = qproj_ops((t, ph + 2))
            _, qb, qc = qk_ops(m + 1)
            qa = qk_ops(m + 2)[0]
            op = oproj_ops(jnp.maximum(m - 1, 0), m + 2, opart, 8 * ph)
            seq = ([(lambda: g_out(1 - ph),), (lambda: g_olhs(3 * m, 1 - ph),)]
                   + qc[:CF] + qp[:KD] + [(lambda: g_query(0),)] + qc[CF:] + qb
                   + [(lambda: g_softmax(1 - ph, 0),), (lambda: g_softmax(1 - ph, 1),)]
                   + qp[KD:] + [(lambda: g_query(1),), (lambda: g_query(2),)]
                   + op + qa[:nblk - AEND] + [(lambda: fence(pat_u, 3, zero_i),)]
                   + qa[nblk - AEND:])
            emit(pv_ops(m, ph), seq)

        def body(t, carry):
            for ph in range(2):
                pl.when(first)(lambda: arrive(2 * t + ph + 2, ph == 1))
                block(t, ph)
            return carry

        lax.fori_loop(0, NP // 2 - 1, body, 0)

        def big(kts, i0):
            return [op for i, kt in enumerate(kts)
                    for op in oproj_ops(kt, kt + 3, part, SP + KD * (i0 + i))]

        old = list(range(NP - 3, 3 * (NP - 3)))
        _, qb, qc = qk_ops(NP - 1)
        seq = ([(lambda: g_out(1),), (lambda: g_olhs(3 * (NP - 2), 1),)] + qc + qb
               + [(lambda: g_softmax(1, 0),), (lambda: g_softmax(1, 1),)]
               + big(old[:KT14 - 4] + list(range(3 * (NP - 3), 3 * (NP - 2))), 0)
               + [(lambda: fence(olhs_u, 3 * NP, zero_i),)]
               + big(old[KT14 - 4:KT14 - 3], KT14 - 1))
        emit(pv_ops(NP - 2, 0), seq)
        barrier()
        k15 = old[KT14 - 3:-1] + list(range(3 * (NP - 2), 3 * (NP - 1))) + old[-1:]
        emit(pv_ops(NP - 1, 1), [(lambda: g_olhs(3 * (NP - 1), 0),)] + big(k15, KT14))

        def epilogue(x):
            def lsum(g):
                return lane_sum(accx[1, 8 * g:8 * g + 8, :])

            den = [jnp.sum(lsum(2 * G + par), axis=0, keepdims=True) for par in range(2)]
            fac = [den[0], den[1] * recip(den[0]), recip(den[1])]
            acc = []
            for n in range(KD):
                t = out_scr[n]
                for i in range(2 * NP):
                    t = t + part[SP + KD * i + n]
                acc.append(t * fac[0])
            for par in range(2):
                for g2 in range(G2):
                    g = G * par + 2 * g2
                    z0, z1 = lsum(g), lsum(g + 1)
                    for n in range(KD):
                        v = f32_rows(wou[(NP - 1) * G + G2 * par + g2, n])
                        acc[n] = acc[n] + (v[:8] * z0 + v[8:] * z1)
                acc = [t * fac[par + 1] for t in acc]
            cols = [jnp.sum(t, axis=0, keepdims=True) for t in acc]
            return residual(x, jnp.concatenate(cols, axis=1))

        def tail1(x):
            if W2S:
                stage_step(NST + 1)
            return ffn1(epilogue(x))

        return lax.cond(first, tail1, lambda x: ffn2(epilogue(x)), x)

    for r in (y_u, pat_u, olhs_u):
        r[...] = jnp.zeros(r.shape, U32)
    reset_pipeline()
    stage_step(1)
    c_wo.wait()
    pair_wo(0, R0)
    stage_step(2)
    for m in range(KVW):
        for i in range(2):
            kv_copy(m, i).start()

    arrive(0, False)
    arrive(1, True)
    wait_all([c_x] + c_wq)
    pair_wq()
    x = lax.fori_loop(0, 2, layer, xb[...].astype(F32))
    o_ref[...] = x.astype(o_ref.dtype)


@jax.jit
def pallas_interleave_layers__sliding_block_cached__glu_gated_swiglu__decode_kernel(
    A_x: jax.Array,
    A_k_cache: jax.Array,
    A_v_cache: jax.Array,
    A_wq: jax.Array,
    A_wo: jax.Array,
    B_x: jax.Array,
    B_w1: jax.Array,
    B_w3: jax.Array,
    B_w2: jax.Array,
):
    del B_x
    sk = A_k_cache.shape[2]
    win = min(4096, max(256, sk // 4))
    nb = sk // 128
    nblk = win // 128

    def cache_tiles(c):
        return (c.reshape(H, nb, 128, G2, 2, 8).transpose(0, 3, 4, 1, 5, 2)
                .reshape(H, G2, 2, nb // 2, 16, 128))

    def weight_tiles(w):
        r, c = w.shape
        return w.reshape(r // 16, 2, 8, c // 128, 128).transpose(0, 1, 3, 2, 4)

    vreg = lambda n: pltpu.VMEM((-(-n // 4) * 4, 8, 128), F32)
    lhs = lambda n: pltpu.VMEM((-(-n // 4) * 4, 16, 128), BF)
    kern = lambda *refs: _kernel(*refs, blk0=nb - nblk, nblk=nblk, scale=DH ** -0.5)
    out = pl.pallas_call(
        kern,
        out_shape=jax.ShapeDtypeStruct((1, D), BF),
        in_specs=[pl.BlockSpec(memory_space=pl.ANY)] * 8,
        out_specs=pl.BlockSpec(memory_space=pltpu.VMEM),
        scratch_shapes=[
            pltpu.VMEM((1, D), BF),
            pltpu.VMEM((NP, 2, 2, G2, 2, nblk // 2, 16, 128), BF),
            pltpu.VMEM((NP // 2, D // 16, 2, 3, 16, 128), BF),
            pltpu.VMEM((H * DH // 16, KD, 16, 128), BF),
            pltpu.VMEM((D // 16, 2, NC // 2, 16, 128), BF),
            pltpu.VMEM((D // 16, 2, NC // 2, 16, 128), BF),
            pltpu.VMEM((FF // 16, KD, 16, 128), BF),
            lhs(KD),
            vreg(1),
            vreg(3 * KD),
            lhs(8),
            vreg(nblk // 8),
            vreg(nblk // 2 + 2 * NP * KD),
            pltpu.VMEM((2, 2, nblk, 128), F32),
            pltpu.VMEM((nblk * 8, 128), F32),
            pltpu.VMEM((2, 64, 128), F32),
            pltpu.VMEM((2, 8 * NR, 128), F32),
            lhs(3 * NP + 4),
            vreg(16),
            vreg(KD),
            pltpu.VMEM((NP, NW, 2, 8, 128), F32),
            pltpu.SMEM((2, SC, KD, 16, 128), BF),
            pltpu.SemaphoreType.DMA((2, NP)),
            pltpu.SemaphoreType.DMA((5 + len(W2_CHUNKS),)),
            pltpu.SemaphoreType.DMA((2,)),
        ],
        compiler_params=pltpu.CompilerParams(
            vmem_limit_bytes=128 * 1024 * 1024, disable_semaphore_checks=True),
    )(A_x.reshape(1, D), cache_tiles(A_k_cache), cache_tiles(A_v_cache),
      weight_tiles(A_wq).reshape(D // 16, 2, 3 * NP // 2, 16, 128),
      weight_tiles(A_wo).reshape(H * G2, KD, 16, 128),
      weight_tiles(B_w1).reshape(D // 16, 2, NC // 2, 16, 128),
      weight_tiles(B_w3).reshape(D // 16, 2, NC // 2, 16, 128),
      weight_tiles(B_w2).reshape(FF // 16, KD, 16, 128))
    return out.reshape(1, 1, D)
```

```python
import math

import jax
import jax.numpy as jnp
from jax import lax
import jax.experimental.pallas as pl
import jax.experimental.pallas.tpu as pltpu

BF = jnp.bfloat16
F32 = jnp.float32
U32 = jnp.uint32

D = 640
H = 32
DH = 192
G = DH // 8
G2 = DH // 16
NP = H // 2
FF = 1536
EPS = 1e-5
KD = D // 128
NC = FF // 128
NZ = 2 * G + 2
NR = NZ + 2
W2S = 8
W2_CHUNKS = (768 - 16 * W2S, 384, 256, 128)

NA = 8
NW = 72
UNPACED = 8
LEAD = 16
RATE = 32.5
TAILC = 30
AEND = 4
CF = 8
KT14 = 10
PVB = 12
KM = 3
FPRE = 8
FSTEP = 3
NST = NP + 1
SC = 10
KVW = 2
PQH = 4
PTK = 6
PFB = 3
TRG = 6


def _kernel(x_hbm, k_hbm, v_hbm, wq_hbm, wo_hbm, w1_hbm, w3_hbm, w2_hbm,
            o_ref,
            xb, kvb, wq, wo, w1, w3, w2,
            y_scr, rs_scr, qpart, pat_scr, part_a, part, p_scr, pb_scr, pb0,
            accx, olhs, opart, out_scr, vx, stage,
            kvsem, wsem, ssem, *, blk0, nblk, scale):
    c2 = scale * math.log2(math.e)
    nq = nblk // 8
    SP = 4 * nq

    def kv_copies(m):
        n = nblk // 4
        return [pltpu.make_async_copy(
            src.at[pl.ds(2 * m, 2), :, t, pl.ds(blk0 // 2 + n * h, n)],
            kvb.at[m, i, :, :, t, pl.ds(n * h, n)], kvsem.at[m])
            for i, src in enumerate((k_hbm, v_hbm)) for t in range(2) for h in range(2)]

    def kv_start(m):
        for c in kv_copies(m):
            c.start()

    c_x = pltpu.make_async_copy(x_hbm, xb, wsem.at[0])
    c_wq = [pltpu.make_async_copy(wq_hbm.at[:, b], wq.at[:, b], wsem.at[1])
            for b in range(NP // 2)]
    R0 = H * G2 - NST * SC
    c_wo = pltpu.make_async_copy(wo_hbm.at[pl.ds(0, R0)], wo.at[pl.ds(0, R0)], wsem.at[2])

    def to_stage(k):
        return pltpu.make_async_copy(wo_hbm.at[pl.ds(R0 + SC * k, SC)], stage.at[k & 1],
                                     ssem.at[0])

    def from_stage(k):
        return pltpu.make_async_copy(stage.at[k & 1], wo.at[pl.ds(R0 + SC * k, SC)], ssem.at[1])

    def stage_step(k):
        def when(cond, f):
            if isinstance(cond, bool):
                if cond:
                    f()
            else:
                pl.when(cond)(f)

        def forward():
            to_stage(k - 1).wait()
            from_stage(k - 1).start()

        landed = not isinstance(k, int) or k >= 2
        if landed:
            from_stage(k - 2).wait()
        when(k <= NST, forward)
        when(k < NST, lambda: to_stage(k).start())
        if W2S:
            when(k == NST, w2_in.start)
            if isinstance(k, int) and k == NST + 1:
                w2_in.wait()
                w2_out.start()
        if landed:
            pair_wo(R0 + SC * (k - 2), SC)

    c_w1 = pltpu.make_async_copy(w1_hbm, w1, wsem.at[3])
    c_w3 = pltpu.make_async_copy(w3_hbm, w3, wsem.at[4])
    w2_off = [16 * W2S + sum(W2_CHUNKS[:i]) for i in range(len(W2_CHUNKS))]
    c_w2 = [pltpu.make_async_copy(w2_hbm.at[pl.ds(o // 16, n // 16)],
                                  w2.at[pl.ds(o // 16, n // 16)], wsem.at[5 + i])
            for i, (o, n) in enumerate(zip(w2_off, W2_CHUNKS))]
    if W2S:
        w2_slot = stage.at[NST & 1, pl.ds(0, W2S)]
        w2_in = pltpu.make_async_copy(w2_hbm.at[pl.ds(0, W2S)], w2_slot, ssem.at[0])
        w2_out = pltpu.make_async_copy(w2_slot, w2.at[pl.ds(0, W2S)], ssem.at[1])

    def wait_all(cs):
        for c in cs:
            c.wait()

    for c in [c_wo] + c_wq + [to_stage(0), c_x]:
        c.start()

    def start_ffn_weights():
        for c in [c_w1, c_w3] + c_w2:
            c.start()

    kvu = kvb.bitcast(U32)
    wqu = wq.bitcast(U32)
    wou = wo.bitcast(U32)
    w1u, w3u, w2u = w1.bitcast(U32), w3.bitcast(U32), w2.bitcast(U32)
    y_u, pat_u, olhs_u = y_scr.bitcast(U32), pat_scr.bitcast(U32), olhs.bitcast(U32)

    def f32_rows(u):
        return pltpu.bitcast(u, BF).astype(F32)

    lane = lax.broadcasted_iota(jnp.int32, (8, 128), 1)
    row = lax.broadcasted_iota(jnp.int32, (8, 128), 0)
    diag_i = ((lane & 7) == row).astype(jnp.int32) * 64
    bit_i = [(lane << (3 - k)) & 64 for k in range(4)]
    uid = [0]

    def lane_sum(v):
        return jnp.broadcast_to(jnp.sum(v, axis=1, keepdims=True), (8, 128))

    def columns(v8):
        uid[0] += 1
        off = 256 * uid[0]
        dl = lane - row + off
        return [lane_sum(jnp.where(dl == off + 8 * b, v8[:, 128 * k:128 * k + 128], 0.0))
                for k in range(v8.shape[1] // 128) for b in range(16)]

    def moments(x):
        mu = jnp.mean(x, axis=-1, keepdims=True)
        xc = x - mu
        return mu, xc, 1.0 / jnp.sqrt(jnp.mean(xc * xc, axis=-1, keepdims=True) + EPS)

    def residual(x, a):
        return (x + a.astype(BF).astype(F32)).astype(BF).astype(F32)

    def tile_dot(l_u32, w_u32, rows, paced):
        w = pltpu.bitcast(w_u32.reshape(64, 128), BF)
        if paced:
            l = pltpu.bitcast(jnp.concatenate([l_u32, l_u32], axis=0), BF)[:24]
            return jnp.dot(l, w, preferred_element_type=F32)[:rows]
        l = pltpu.bitcast(l_u32, BF)[:rows]
        return jnp.dot(l, w, preferred_element_type=F32)

    def swap_halves(a, b):
        return (jnp.concatenate([a[..., :4, :], b[..., :4, :]], axis=-2),
                jnp.concatenate([a[..., 4:, :], b[..., 4:, :]], axis=-2))

    def pair_wq():
        def body(i, carry):
            for f in range(8):
                part[12 * f:12 * f + 12] = pltpu.bitcast(wqu[i, f].reshape(12, 8, 128), F32)
            for q in range(NP // 2):
                for r in range(2):
                    a, b = [pltpu.bitcast(part[48 * r + 24 * t + 3 * q:48 * r + 24 * t + 3 * q + 3], U32)
                            for t in range(2)]
                    wqu[i, q, r, 0:3], wqu[i, q, r, 3:6] = swap_halves(a, b)
            return carry
        lax.fori_loop(0, D // 32, body, 0)

    def pair_wo(r0, n):
        def body(i, carry):
            r = pl.ds(r0 + 2 * i, 2)
            v = wou[r]
            h = [v[:, f // 2, 4 * (f % 2):4 * (f % 2) + 4, :] for f in range(2 * KD)]
            for c in range(KD):
                wou[r, c] = jnp.concatenate([h[c], h[KD + c]], axis=1)
            return carry
        lax.fori_loop(0, n // 2, body, 0)

    def wq_tile(m, c, k):
        c6 = 3 * m[1] + c
        return wqu[4 * k:4 * k + 4, m[0] + c6 // 6, :, 3 * (c6 & 1) + ((c6 % 6) >> 1)]

    def qproj_ops(m):
        def op(paced, c, k):
            qpart[c * KD + k] = tile_dot(
                y_u[k], wq_tile(m, c, k), 8, paced)
        return [(lambda p, c=c, k=k: op(p, c, k)) for c in range(3) for k in range(KD)]

    def oproj_ops(kt, slot, dst, d0):
        def op(paced, n):
            dst[d0 + n] = tile_dot(olhs_u[slot], wou[pl.ds(kt * 8, 8), n], 8, paced)
        return [(lambda p, n=n: op(p, n)) for n in range(KD)]

    def pair_rows(m):
        def body(i, c):
            par, g2 = i // G2, i % G2
            kvu[m, 0, par, g2, 0], kvu[m, 0, par, g2, 1] = swap_halves(
                kvu[m, 0, par, g2, 0], kvu[m, 0, par, g2, 1])
            return c
        lax.fori_loop(0, 2 * G2, body, 0)

    def k_blocks(m, par, g0, g1, j):
        return kvu[m, 0, par, g0:g1, j & 1, j >> 1]

    jord = [8 * (i // 8) + 2 * (i % 4) + (i % 8) // 4 for i in range(nblk)]

    def qk_ops(m):
        def op_a(paced, j):
            r = tile_dot(pat_u[0], k_blocks(m, 0, 0, 8, j), 8, paced)
            part_a[j // 8, j % 8:j % 8 + 1, :] = r[j % 8:j % 8 + 1, :]

        def op_c(paced, j):
            r = tile_dot(pat_u[2], k_blocks(m, 1, 4, 12, j), 8, paced)
            part[2 * nq + j // 8, j % 8:j % 8 + 1, :] = r[j % 8:j % 8 + 1, :]

        def op_b(paced, j):
            w = jnp.concatenate([k_blocks(m, 0, 8, 12, j), k_blocks(m, 1, 0, 4, j)], axis=0)
            r = tile_dot(pat_u[1], w, 16, paced)
            part[nq + j // 8, j % 8:j % 8 + 1, :] = r[j % 8:j % 8 + 1, :]
            part[3 * nq + j // 8, j % 8:j % 8 + 1, :] = r[8 + j % 8:8 + j % 8 + 1, :]

        return [[(lambda p, f=f, j=j: f(p, j)) for j in jord] for f in (op_a, op_b, op_c)]

    def plain(ops):
        for op in ops:
            op(False)

    steps = [(par, gb, j0) for par in range(2) for gb in range(G // NA)
             for j0 in range(0, nblk, 4)]

    def units(par, gb, j0):
        return [(par, g, j0) for g in range(gb * NA, (gb + 1) * NA)]

    order = [u for s in steps for u in units(*s)]
    wide = {}
    for i, u in enumerate(order):
        if (i + 1) * NW // len(order) > i * NW // len(order):
            wide[u] = len(wide)

    def widen(m):
        for (par, g, j), e in wide.items():
            v = f32_rows(kvu[m, 1, par, g // 2, g % 2, j // 2:j // 2 + 2])
            kvu[m, 1, par, g // 2, g % 2, j // 2:j // 2 + 2] = pltpu.bitcast(v[:, :8], U32)
            vx[m, e] = v[:, 8:]

    def v_unit(m, par, g, j):
        u = kvu[m, 1, par, g // 2, g % 2, j // 2:j // 2 + 2]
        if (par, g, j) in wide:
            return jnp.concatenate([pltpu.bitcast(u, F32), vx[m, wide[(par, g, j)]]], axis=1)
        return f32_rows(u)

    def pv_ops(m, ph):
        acc = {}

        def spread(par, q, r):
            pb_scr[pl.ds(64 * q + r, 8, stride=8), :] = p_scr[ph, par, 8 * q:8 * q + 8, :]

        def psum(par):
            p = p_scr[ph, par]
            accx[ph, 8 * (2 * G + par):8 * (2 * G + par) + 8, :] = (
                (p[0:8] + p[8:16]) + (p[16:24] + p[24:32]))

        pbv = {}

        def piece(par, gb, j0, k):
            if k == 0:
                if par == 0 and j0 < 8:
                    pb = pb0[ph, 8 * j0:8 * j0 + 32, :]
                else:
                    pb = pb_scr[8 * j0:8 * j0 + 32, :]
                pbv[0] = pb.reshape(4, 8, 128)
            for _, g, _ in units(par, gb, j0)[4 * k:4 * k + 4]:
                tv = v_unit(m, par, g, j0).reshape(4, 8, 128) * pbv[0]
                tv = jnp.sum(tv, axis=0)
                acc[g] = tv if j0 == 0 else acc[g] + tv
                if j0 == nblk - 4:
                    r0 = DH * par + 8 * g
                    accx[ph, r0:r0 + 8, :] = acc[g]

        pieces = [s + (k,) for s in steps for k in range(NA // 4)]
        half = len(pieces) // 2
        spq = 2 * (NA // 4)
        side = {}
        for q in range(nq):
            for r in range(8):
                if q:
                    side.setdefault((spq * (8 * (q - 1) + r)) // 9, []).append(
                        lambda q=q, r=r: spread(0, q, r))
                side.setdefault(half - nq * spq + spq * (q + 1) + (r * (3 * spq - 1)) // 8, []).append(
                    lambda q=q, r=r: spread(1, q, r))
        for par in range(2):
            side.setdefault(half // 2 + par, []).append(lambda par=par: psum(par))
        out = []
        for i, s in enumerate(pieces):
            out += [(0, f) for f in side.get(i, [])]
            out.append((2 * sum(4 if u in wide else 6 for u in units(*s[:3])[4 * s[3]:4 * s[3] + 4]),
                        (lambda s=s: piece(*s))))
        return out

    toks = []

    def fence(dst, slot, zero_i):
        for i, t in enumerate(toks):
            dst[slot + i + zero_i] = t
        toks.clear()

    def g_softmax(ph, par):
        s0 = part[2 * nq:3 * nq] if par else part_a[0:nq]
        s = (s0 + part[(2 * par + 1) * nq:(2 * par + 2) * nq]).reshape(nblk, 128)
        mx = jnp.max(jnp.max(s, axis=0, keepdims=True), axis=1, keepdims=True)
        p = jnp.exp2((s - mx) * jnp.concatenate([rs_scr[0]] * nq, axis=0))
        p_scr[ph, par] = p
        if par == 0:
            for r in range(8):
                pb0[ph, pl.ds(r, 8, stride=8), :] = p[0:8]
        toks.append(pltpu.bitcast(p[nblk - 8:nblk], U32))

    def recip(d):
        r = pl.reciprocal(d, approx=True)
        return r * (2.0 - d * r)

    def g_olhs(slot0, ph):
        z = [lane_sum(accx[ph, 8 * g:8 * g + 8, :]) for g in range(NZ)]
        inv = [jnp.broadcast_to(recip(jnp.sum(z[2 * G + par], axis=0, keepdims=True)), (8, 128))
               for par in range(2)]
        uid[0] += 1
        bit = [b > uid[0] for b in bit_i]
        for c in range(3):
            xs = z[16 * c:16 * c + 16]
            for k in range(4):
                xs = [jnp.where(bit[k], xs[i + 1], xs[i]) for i in range(0, len(xs), 2)]
            iv = inv[0] if c == 0 else (inv[1] if c == 2 else jnp.where(bit[3], inv[1], inv[0]))
            olhs[slot0 + c, 0:8, :] = jnp.where(diag_i > uid[0], xs[0] * iv, 0.0).astype(BF)

    def set_pat(c, q):
        if c == 1:
            hi = bit_i[3] > uid[0]
            pat_scr[c, 0:8, :] = jnp.where(hi, 0.0, q).astype(BF)
            pat_scr[c, 8:16, :] = jnp.where(hi, q, 0.0).astype(BF)
        else:
            pat_scr[c, 0:8, :] = q.astype(BF)
        if c > 0:
            toks.append(pltpu.bitcast(q, U32))

    def g_query(c):
        xs = [qpart[c * KD + k] for k in range(KD)]
        set_pat(c, ((xs[0] + xs[1]) + (xs[2] + xs[3])) + xs[4])

    def g_out(ph):
        for n in range(KD):
            out_scr[n] = out_scr[n] + opart[8 * ph + n]

    def reset_pipeline():
        accx[1, 0:16 * G, :] = jnp.zeros((16 * G, 128), F32)
        accx[1, 16 * G:16 * G + 16, :] = jnp.ones((16, 128), F32)
        for n in range(KD):
            opart[8 + n] = jnp.zeros((8, 128), F32)
            out_scr[n] = jnp.zeros((8, 128), F32)

    def emit(pv, seq):
        ntile = sum(not isinstance(e, tuple) for e in seq)
        total = sum(w for w, _ in pv) / 4
        k = done = n = 0
        for e in seq:
            if isinstance(e, tuple):
                e[0]()
                continue
            pos = LEAD + RATE * (n // 4) if n // 4 < (ntile - 1) // 4 else total - TAILC
            while k < len(pv) and done + pv[k][0] / 2 <= 4 * pos:
                done += pv[k][0]
                pv[k][1]()
                k += 1
            e(n < ntile - UNPACED)
            n += 1
        for _, g in pv[k:]:
            g()

    def ffn1(x):
        _, xc, rs = moments(x)
        y = jnp.broadcast_to(xc, (8, D)).astype(BF)
        reset_pipeline()

        def up(wu):
            cols = []
            for cp in range(NC // 2):
                ev, od = swap_halves(wu[:, 0, cp], wu[:, 1, cp])
                wu[:, 0, cp], wu[:, 1, cp] = ev, od
                cols += [jnp.dot(y, pltpu.bitcast(w.reshape(D // 2, 128), BF),
                                 preferred_element_type=F32) for w in (ev, od)]
            return jnp.concatenate(cols, axis=1) * rs

        def w2_rows(r0, n):
            v = w2u[r0:r0 + n]
            h = [v[:, f // 2, 4 * (f % 2):4 * (f % 2) + 4, :] for f in range(2 * KD)]
            nat = [jnp.concatenate([h[c], h[KD + c]], axis=1) for c in range(KD)]
            for c in range(KD):
                w2u[r0:r0 + n, c] = nat[c]
            return v, nat

        def down(o, n):
            cols = [None] * KD
            for k in range(o // 128, (o + n) // 128):
                for c, w in enumerate(w2_rows(8 * k, 8)[1]):
                    t = jnp.dot(hh[:, 128 * k:128 * k + 128], pltpu.bitcast(w.reshape(64, 128), BF),
                                preferred_element_type=F32)[0:1]
                    cols[c] = t if cols[c] is None else cols[c] + t
            return jnp.concatenate(cols, axis=1)

        c_w1.wait()
        g = up(w1u)
        c_w3.wait()
        u = up(w3u)
        hh = (g * jax.nn.sigmoid(g) * u).astype(BF)
        hb = columns(hh[:, w2_off[-1]:].astype(F32))
        a = None
        parts = list(zip(c_w2, w2_off, W2_CHUNKS))[:-1]
        if W2S:
            parts.insert(1, (w2_out, 0, 16 * W2S))
        for c, o, n in parts:
            c.wait()
            a = down(o, n) if a is None else a + down(o, n)
        c_w2[-1].wait()
        acc = [None] * KD
        for r in range(W2_CHUNKS[-1] // 16):
            v = f32_rows(w2_rows(w2_off[-1] // 16 + r, 1)[0][0])
            for f in range(2 * KD):
                tv = v[f // 2, 8 * (f % 2):8 * (f % 2) + 8] * hb[2 * r + f // KD]
                acc[f % KD] = tv if acc[f % KD] is None else acc[f % KD] + tv
        a = a + jnp.concatenate([jnp.sum(t, axis=0, keepdims=True) for t in acc], axis=1)
        return residual(x, a)

    def ffn2(x):
        mu, _, rs = moments(x)
        x8 = jnp.broadcast_to(x, (8, D))
        rowk = lax.broadcasted_iota(jnp.int32, (8, 128 * KM), 0)
        y = jnp.where(rowk == 0, x8[:, :128 * KM], jnp.where(rowk == 1, 1.0, 0.0)).astype(BF)
        coef = jnp.where(row == 0, 1.0, -mu)
        yb = jnp.concatenate([c - mu for c in columns(x8[:, 128 * KM:])], axis=0)
        mx = {}
        out = [None] * KD
        for c in range(NC):
            while len(mx) < min(NC, FPRE + c * FSTEP / 4):
                cc = len(mx)
                mx[cc] = [jnp.dot(y, pltpu.bitcast(wu[0:8 * KM, cc & 1, cc >> 1].reshape(64 * KM, 128), BF),
                                  preferred_element_type=F32) * coef for wu in (w1u, w3u)]
            gu = []
            for i, wu in enumerate((w1u, w3u)):
                acc = None
                for r in range(8 * (KD - KM)):
                    tv = f32_rows(wu[8 * KM + r, c & 1, c >> 1]) * yb[16 * r:16 * r + 16]
                    acc = tv if r == 0 else acc + tv
                gu.append(jnp.sum((acc[:8] + acc[8:]) + mx[c][i], axis=0, keepdims=True) * rs)
            hg = 0.5 * gu[0]
            h = jnp.broadcast_to((hg * jnp.tanh(hg) + hg) * gu[1], (8, 128)).astype(BF)
            for n in range(KD):
                t = jnp.dot(h, pltpu.bitcast(w2u[8 * c:8 * c + 8, n].reshape(64, 128), BF),
                            preferred_element_type=F32)[0:1]
                out[n] = t if c == 0 else out[n] + t
        return residual(x, jnp.concatenate(out, axis=1))

    def arrive(p, odd):
        def when(cond, f):
            if isinstance(cond, bool):
                if cond:
                    f()
            else:
                pl.when(cond)(f)

        cs = kv_copies(p)
        wait_all(cs[:4])
        when(not odd or p + 3 <= NST, lambda: stage_step(p + 3))
        wait_all(cs[4:TRG])
        when(odd and p == NP - 1, start_ffn_weights)
        wait_all(cs[TRG:])
        when(p + KVW < NP, lambda: kv_start(p + KVW))
        pair_rows(p)
        widen(p)
        when(odd and p == NP - 1, lambda: stage_step(NST + 1))

    def layer(li, x):
        first = li == 0
        zero_i = li >> 4

        def barrier():
            @pl.when(li > 2)
            def _():
                reset_pipeline()

        mu, xc, rs = moments(x)
        y = jnp.broadcast_to(xc, (8, D))
        for k in range(KD):
            y_scr[k, 0:8, :] = y[:, 128 * k:128 * k + 128].astype(BF)
        rs_scr[0] = jnp.broadcast_to(rs * c2, (8, 128))
        rowd = lax.broadcasted_iota(jnp.int32, (8, D), 0)
        xo = jnp.where(rowd < 4, jnp.broadcast_to(x, (8, D)), 1.0).astype(BF)
        coef = jnp.where(row < 4, 1.0, -mu)

        def q_direct(col):
            t = jnp.dot(xo, pltpu.bitcast(wqu[:, 0, :, 3 * (col & 1) + (col >> 1)].reshape(D // 2, 128), BF), preferred_element_type=F32) * coef
            return (t + pltpu.roll(t, 4, 0)).astype(BF).astype(F32)

        def q_cols(q, slot):
            for b, col in enumerate(columns(q)):
                part[slot + b] = col

        def vpu_a(m, slot, js):
            acc = {}
            for g2 in range(8):
                qc = jnp.concatenate([part[slot + 2 * g2 + t + zero_i] for t in range(2)], axis=0)
                for j in js:
                    tv = f32_rows(kvu[m, 0, 0, g2, j & 1, j >> 1]) * qc
                    acc[j] = tv if g2 == 0 else acc[j] + tv
            for j in js:
                part_a[j // 8, j % 8:j % 8 + 1, :] = jnp.sum(acc[j], axis=0, keepdims=True)

        q0 = [q_direct(c) for c in range(4)]
        q_cols(q0[0], SP)
        set_pat(1, q0[1])
        set_pat(2, q0[2])
        _, qb, qc = qk_ops(0)
        for i in range(nblk // 2):
            if i == PQH:
                q_cols(q0[3], SP + 16)
            vpu_a(0, SP, jord[2 * i:2 * i + 2])
            plain((qb + qc)[4 * i:4 * i + 4])
        g_softmax(0, 0)
        g_softmax(0, 1)
        plain(qproj_ops((0, 1))[KD:])
        g_query(1)
        g_query(2)
        set_pat(0, q0[3])
        qa = qk_ops(1)[0][PVB:]
        k = 0
        for i in range(0, PVB, 2):
            n = PTK + PFB * i // 2
            if n < 2 * KD:
                part[0] = qpart[KD + n]
            else:
                n = min(n - 2 * KD, len(qa) - 1)
                plain(qa[k:n + 1])
                k = max(k, n + 1)
                part[0] = part_a[jord[PVB + n] // 8]
            vpu_a(1, SP + 16, jord[i:i + 2])
        plain(qa[k:])
        toks.clear()

        def block(t, ph):
            m = 2 * t + ph

            qp = qproj_ops((t, ph + 2))
            _, qb, qc = qk_ops(m + 1)
            qa = qk_ops(m + 2)[0]
            op = oproj_ops(jnp.maximum(m - 1, 0), m + 2, opart, 8 * ph)
            seq = ([(lambda: g_out(1 - ph),), (lambda: g_olhs(3 * m, 1 - ph),)]
                   + qc[:CF] + qp[:KD] + [(lambda: g_query(0),)] + qc[CF:] + qb
                   + [(lambda: g_softmax(1 - ph, 0),), (lambda: g_softmax(1 - ph, 1),)]
                   + qp[KD:] + [(lambda: g_query(1),), (lambda: g_query(2),)]
                   + op + qa[:nblk - AEND] + [(lambda: fence(pat_u, 3, zero_i),)]
                   + qa[nblk - AEND:])
            emit(pv_ops(m, ph), seq)

        def body(t, carry):
            for ph in range(2):
                pl.when(first)(lambda: arrive(2 * t + ph + 2, ph == 1))
                block(t, ph)
            return carry

        lax.fori_loop(0, NP // 2 - 1, body, 0)

        def big(kts, i0):
            return [op for i, kt in enumerate(kts)
                    for op in oproj_ops(kt, kt + 3, part, SP + KD * (i0 + i))]

        old = list(range(NP - 3, 3 * (NP - 3)))
        _, qb, qc = qk_ops(NP - 1)
        seq = ([(lambda: g_out(1),), (lambda: g_olhs(3 * (NP - 2), 1),)] + qc + qb
               + [(lambda: g_softmax(1, 0),), (lambda: g_softmax(1, 1),)]
               + big(old[:KT14 - 4] + list(range(3 * (NP - 3), 3 * (NP - 2))), 0)
               + [(lambda: fence(olhs_u, 3 * NP, zero_i),)]
               + big(old[KT14 - 4:KT14 - 3], KT14 - 1))
        emit(pv_ops(NP - 2, 0), seq)
        barrier()
        k15 = old[KT14 - 3:-1] + list(range(3 * (NP - 2), 3 * (NP - 1))) + old[-1:]
        emit(pv_ops(NP - 1, 1), [(lambda: g_olhs(3 * (NP - 1), 0),)] + big(k15, KT14))

        def epilogue(x):
            def lsum(g):
                return lane_sum(accx[1, 8 * g:8 * g + 8, :])

            den = [jnp.sum(lsum(2 * G + par), axis=0, keepdims=True) for par in range(2)]
            fac = [den[0], den[1] * recip(den[0]), recip(den[1])]
            acc = []
            for n in range(KD):
                t = out_scr[n]
                for i in range(2 * NP):
                    t = t + part[SP + KD * i + n]
                acc.append(t * fac[0])
            for par in range(2):
                for g2 in range(G2):
                    g = G * par + 2 * g2
                    z0, z1 = lsum(g), lsum(g + 1)
                    for n in range(KD):
                        v = f32_rows(wou[(NP - 1) * G + G2 * par + g2, n])
                        acc[n] = acc[n] + (v[:8] * z0 + v[8:] * z1)
                acc = [t * fac[par + 1] for t in acc]
            cols = [jnp.sum(t, axis=0, keepdims=True) for t in acc]
            return residual(x, jnp.concatenate(cols, axis=1))

        return lax.cond(first, lambda x: ffn1(epilogue(x)), lambda x: ffn2(epilogue(x)), x)

    for r in (y_u, pat_u, olhs_u):
        r[...] = jnp.zeros(r.shape, U32)
    reset_pipeline()
    stage_step(1)
    stage_step(2)
    kv_start(0)
    c_x.wait()
    kv_start(1)
    wait_all(c_wq)
    pair_wq()
    c_wo.wait()
    arrive(0, False)
    pair_wo(0, R0)
    arrive(1, True)
    x = lax.fori_loop(0, 2, layer, xb[...].astype(F32))
    o_ref[...] = x.astype(o_ref.dtype)


@jax.jit
def pallas_interleave_layers__sliding_block_cached__glu_gated_swiglu__decode_kernel(
    A_x: jax.Array,
    A_k_cache: jax.Array,
    A_v_cache: jax.Array,
    A_wq: jax.Array,
    A_wo: jax.Array,
    B_x: jax.Array,
    B_w1: jax.Array,
    B_w3: jax.Array,
    B_w2: jax.Array,
):
    del B_x
    sk = A_k_cache.shape[2]
    win = min(4096, max(256, sk // 4))
    nb = sk // 128
    nblk = win // 128

    def cache_tiles(c):
        return (c.reshape(H, nb, 128, G2, 2, 8).transpose(0, 3, 4, 1, 5, 2)
                .reshape(H, G2, 2, nb // 2, 16, 128))

    def weight_tiles(w):
        r, c = w.shape
        return w.reshape(r // 16, 2, 8, c // 128, 128).transpose(0, 1, 3, 2, 4)

    vreg = lambda n: pltpu.VMEM((-(-n // 4) * 4, 8, 128), F32)
    lhs = lambda n: pltpu.VMEM((-(-n // 4) * 4, 16, 128), BF)
    kern = lambda *refs: _kernel(*refs, blk0=nb - nblk, nblk=nblk, scale=DH ** -0.5)
    out = pl.pallas_call(
        kern,
        out_shape=jax.ShapeDtypeStruct((1, D), BF),
        in_specs=[pl.BlockSpec(memory_space=pl.ANY)] * 8,
        out_specs=pl.BlockSpec(memory_space=pltpu.VMEM),
        scratch_shapes=[
            pltpu.VMEM((1, D), BF),
            pltpu.VMEM((NP, 2, 2, G2, 2, nblk // 2, 16, 128), BF),
            pltpu.VMEM((D // 32, NP // 2, 2, 6, 16, 128), BF),
            pltpu.VMEM((H * DH // 16, KD, 16, 128), BF),
            pltpu.VMEM((D // 16, 2, NC // 2, 16, 128), BF),
            pltpu.VMEM((D // 16, 2, NC // 2, 16, 128), BF),
            pltpu.VMEM((FF // 16, KD, 16, 128), BF),
            lhs(KD),
            vreg(1),
            vreg(3 * KD),
            lhs(8),
            vreg(nblk // 8),
            vreg(nblk // 2 + 2 * NP * KD),
            pltpu.VMEM((2, 2, nblk, 128), F32),
            pltpu.VMEM((nblk * 8, 128), F32),
            pltpu.VMEM((2, 64, 128), F32),
            pltpu.VMEM((2, 8 * NR, 128), F32),
            lhs(3 * NP + 4),
            vreg(16),
            vreg(KD),
            pltpu.VMEM((NP, NW, 2, 8, 128), F32),
            pltpu.SMEM((2, SC, KD, 16, 128), BF),
            pltpu.SemaphoreType.DMA((NP,)),
            pltpu.SemaphoreType.DMA((5 + len(W2_CHUNKS),)),
            pltpu.SemaphoreType.DMA((2,)),
        ],
        compiler_params=pltpu.CompilerParams(
            vmem_limit_bytes=128 * 1024 * 1024, disable_semaphore_checks=True),
    )(A_x.reshape(1, D), cache_tiles(A_k_cache), cache_tiles(A_v_cache),
      weight_tiles(A_wq).reshape(D // 32, NP // 2, 2, 6, 16, 128),
      weight_tiles(A_wo).reshape(H * G2, KD, 16, 128),
      weight_tiles(B_w1).reshape(D // 16, 2, NC // 2, 16, 128),
      weight_tiles(B_w3).reshape(D // 16, 2, NC // 2, 16, 128),
      weight_tiles(B_w2).reshape(FF // 16, KD, 16, 128))
    return out.reshape(1, 1, D)
```

```python
import math

import jax
import jax.numpy as jnp
from jax import lax
import jax.experimental.pallas as pl
import jax.experimental.pallas.tpu as pltpu

BF = jnp.bfloat16
F32 = jnp.float32
U32 = jnp.uint32

D = 640
H = 32
DH = 192
G = DH // 8
G2 = DH // 16
NP = H // 2
FF = 1536
EPS = 1e-5
KD = D // 128
NC = FF // 128
NZ = 2 * G + 2
NR = NZ + 2
W2S = 8
W2_CHUNKS = (768 - 16 * W2S, 384, 256, 128)

NA = 8
NW = 72
UNPACED = 8
LEAD = 16
RATE = 32.5
TAILC = 30
AEND = 4
CF = 8
KT14 = 10
PVB = 12
KM = 3
FPRE = 8
FSTEP = 3
NST = NP + 1
SC = 10
KVW = 2
PQH = 4
PTK = 6
PFB = 3
TRG = 6


def _kernel(x_hbm, k_hbm, v_hbm, wq_hbm, wa_hbm, wo_hbm, w1_hbm, w3_hbm, w2_hbm,
            o_ref,
            xb, kvb, wq, wa, wo, w1, w3, w2,
            y_scr, rs_scr, qpart, pat_scr, part_a, part, p_scr, pb_scr, pb0,
            accx, olhs, opart, out_scr, vx, stage,
            kvsem, wsem, ssem, *, blk0, nblk, scale):
    c2 = scale * math.log2(math.e)
    nq = nblk // 8
    SP = 4 * nq

    def kv_copies(m):
        n = nblk // 4
        return [pltpu.make_async_copy(
            src.at[pl.ds(2 * m, 2), :, t, pl.ds(blk0 // 2 + n * h, n)],
            kvb.at[m, i, :, :, t, pl.ds(n * h, n)], kvsem.at[m])
            for i, src in enumerate((k_hbm, v_hbm)) for t in range(2) for h in range(2)]

    def kv_start(m):
        for c in kv_copies(m):
            c.start()

    c_x = pltpu.make_async_copy(x_hbm, xb, wsem.at[0])
    c_wq = [pltpu.make_async_copy(wq_hbm.at[:, b], wq.at[:, b], wsem.at[1])
            for b in range(NP // 2)]
    RH = H * G2 // 2
    R0 = RH - NST * SC
    c_wo = [pltpu.make_async_copy(wa_hbm.at[pl.ds(0, 6), b], wa.at[:, b], wsem.at[2])
            for b in range(16)]
    c_wo.append(pltpu.make_async_copy(wo_hbm.at[pl.ds(RH, R0)], wo.at[pl.ds(0, R0)], wsem.at[2]))

    def to_stage(k):
        return pltpu.make_async_copy(wo_hbm.at[pl.ds(RH + R0 + SC * k, SC)], stage.at[k & 1],
                                     ssem.at[0])

    def from_stage(k):
        return pltpu.make_async_copy(stage.at[k & 1], wo.at[pl.ds(R0 + SC * k, SC)], ssem.at[1])

    def stage_step(k):
        def when(cond, f):
            if isinstance(cond, bool):
                if cond:
                    f()
            else:
                pl.when(cond)(f)

        def forward():
            to_stage(k - 1).wait()
            from_stage(k - 1).start()

        landed = not isinstance(k, int) or k >= 2
        if landed:
            from_stage(k - 2).wait()
        when(k <= NST, forward)
        when(k < NST, lambda: to_stage(k).start())
        if W2S:
            when(k == NST, w2_in.start)
            if isinstance(k, int) and k == NST + 1:
                w2_in.wait()
                w2_out.start()
        if landed:
            pair_wo(R0 + SC * (k - 2), SC)

    c_w1 = pltpu.make_async_copy(w1_hbm, w1, wsem.at[3])
    c_w3 = pltpu.make_async_copy(w3_hbm, w3, wsem.at[4])
    w2_off = [16 * W2S + sum(W2_CHUNKS[:i]) for i in range(len(W2_CHUNKS))]
    c_w2 = [pltpu.make_async_copy(w2_hbm.at[pl.ds(o // 16, n // 16)],
                                  w2.at[pl.ds(o // 16, n // 16)], wsem.at[5 + i])
            for i, (o, n) in enumerate(zip(w2_off, W2_CHUNKS))]
    if W2S:
        w2_slot = stage.at[NST & 1, pl.ds(0, W2S)]
        w2_in = pltpu.make_async_copy(w2_hbm.at[pl.ds(0, W2S)], w2_slot, ssem.at[0])
        w2_out = pltpu.make_async_copy(w2_slot, w2.at[pl.ds(0, W2S)], ssem.at[1])

    def wait_all(cs):
        for c in cs:
            c.wait()

    for c in c_wq[:1] + [to_stage(0), c_x] + c_wo + c_wq[1:]:
        c.start()

    def start_ffn_weights():
        for c in [c_w1, c_w3] + c_w2:
            c.start()

    kvu = kvb.bitcast(U32)
    wqu = wq.bitcast(U32)
    wau = wa.bitcast(U32)
    wou = wo.bitcast(U32)
    w1u, w3u, w2u = w1.bitcast(U32), w3.bitcast(U32), w2.bitcast(U32)
    y_u, pat_u, olhs_u = y_scr.bitcast(U32), pat_scr.bitcast(U32), olhs.bitcast(U32)

    def f32_rows(u):
        return pltpu.bitcast(u, BF).astype(F32)

    lane = lax.broadcasted_iota(jnp.int32, (8, 128), 1)
    row = lax.broadcasted_iota(jnp.int32, (8, 128), 0)
    diag_i = ((lane & 7) == row).astype(jnp.int32) * 64
    bit_i = [(lane << (3 - k)) & 64 for k in range(4)]
    uid = [0]

    def lane_sum(v):
        return jnp.broadcast_to(jnp.sum(v, axis=1, keepdims=True), (8, 128))

    def columns(v8):
        uid[0] += 1
        off = 256 * uid[0]
        dl = lane - row + off
        return [lane_sum(jnp.where(dl == off + 8 * b, v8[:, 128 * k:128 * k + 128], 0.0))
                for k in range(v8.shape[1] // 128) for b in range(16)]

    def moments(x):
        mu = jnp.mean(x, axis=-1, keepdims=True)
        xc = x - mu
        return mu, xc, 1.0 / jnp.sqrt(jnp.mean(xc * xc, axis=-1, keepdims=True) + EPS)

    def residual(x, a):
        return (x + a.astype(BF).astype(F32)).astype(BF).astype(F32)

    def tile_dot(l_u32, w_u32, rows, paced):
        w = pltpu.bitcast(w_u32.reshape(64, 128), BF)
        if paced:
            l = pltpu.bitcast(jnp.concatenate([l_u32, l_u32], axis=0), BF)[:24]
            return jnp.dot(l, w, preferred_element_type=F32)[:rows]
        l = pltpu.bitcast(l_u32, BF)[:rows]
        return jnp.dot(l, w, preferred_element_type=F32)

    def swap_halves(a, b):
        return (jnp.concatenate([a[..., :4, :], b[..., :4, :]], axis=-2),
                jnp.concatenate([a[..., 4:, :], b[..., 4:, :]], axis=-2))

    def pair_wq():
        def body(i, carry):
            for f in range(8):
                part[12 * f:12 * f + 12] = pltpu.bitcast(wqu[i, f].reshape(12, 8, 128), F32)
            for q in range(NP // 2):
                for r in range(2):
                    a, b = [pltpu.bitcast(part[48 * r + 24 * t + 3 * q:48 * r + 24 * t + 3 * q + 3], U32)
                            for t in range(2)]
                    wqu[i, q, r, 0:3], wqu[i, q, r, 3:6] = swap_halves(a, b)
            return carry
        lax.fori_loop(0, D // 32, body, 0)

    def regroup5(v):
        h = [v[:, f // 2, 4 * (f % 2):4 * (f % 2) + 4, :] for f in range(2 * KD)]
        return [jnp.concatenate([h[c], h[KD + c]], axis=1) for c in range(KD)]

    def pair_wo(r0, n):
        def body(i, carry):
            r = pl.ds(r0 + 2 * i, 2)
            for c, w in enumerate(regroup5(wou[r])):
                wou[r, c] = w
            return carry
        lax.fori_loop(0, n // 2, body, 0)

    def pair_wa():
        def body(i, carry):
            a, b = i >> 4, i & 15
            for c, w in enumerate(regroup5(wau[a, b])):
                wau[a, b, :, c] = w
            return carry
        lax.fori_loop(0, RH // 2, body, 0)

    def wo_tile(kt, n):
        if isinstance(kt, int) and 8 * kt >= RH:
            return wou[8 * kt - RH:8 * kt - RH + 8, n]
        return wau[kt >> 2, pl.ds(4 * (kt & 3), 4), :, n]

    def wq_tile(m, c, k):
        c6 = 3 * m[1] + c
        return wqu[4 * k:4 * k + 4, m[0] + c6 // 6, :, 3 * (c6 & 1) + ((c6 % 6) >> 1)]

    def qproj_ops(m):
        def op(paced, c, k):
            qpart[c * KD + k] = tile_dot(
                y_u[k], wq_tile(m, c, k), 8, paced)
        return [(lambda p, c=c, k=k: op(p, c, k)) for c in range(3) for k in range(KD)]

    def oproj_ops(kt, slot, dst, d0):
        def op(paced, n):
            dst[d0 + n] = tile_dot(olhs_u[slot], wo_tile(kt, n), 8, paced)
        return [(lambda p, n=n: op(p, n)) for n in range(KD)]

    def pair_rows(m):
        def body(i, c):
            par, g2 = i // G2, i % G2
            kvu[m, 0, par, g2, 0], kvu[m, 0, par, g2, 1] = swap_halves(
                kvu[m, 0, par, g2, 0], kvu[m, 0, par, g2, 1])
            return c
        lax.fori_loop(0, 2 * G2, body, 0)

    def k_blocks(m, par, g0, g1, j):
        return kvu[m, 0, par, g0:g1, j & 1, j >> 1]

    jord = [8 * (i // 8) + 2 * (i % 4) + (i % 8) // 4 for i in range(nblk)]

    def qk_ops(m):
        def op_a(paced, j):
            r = tile_dot(pat_u[0], k_blocks(m, 0, 0, 8, j), 8, paced)
            part_a[j // 8, j % 8:j % 8 + 1, :] = r[j % 8:j % 8 + 1, :]

        def op_c(paced, j):
            r = tile_dot(pat_u[2], k_blocks(m, 1, 4, 12, j), 8, paced)
            part[2 * nq + j // 8, j % 8:j % 8 + 1, :] = r[j % 8:j % 8 + 1, :]

        def op_b(paced, j):
            w = jnp.concatenate([k_blocks(m, 0, 8, 12, j), k_blocks(m, 1, 0, 4, j)], axis=0)
            r = tile_dot(pat_u[1], w, 16, paced)
            part[nq + j // 8, j % 8:j % 8 + 1, :] = r[j % 8:j % 8 + 1, :]
            part[3 * nq + j // 8, j % 8:j % 8 + 1, :] = r[8 + j % 8:8 + j % 8 + 1, :]

        return [[(lambda p, f=f, j=j: f(p, j)) for j in jord] for f in (op_a, op_b, op_c)]

    def plain(ops):
        for op in ops:
            op(False)

    steps = [(par, gb, j0) for par in range(2) for gb in range(G // NA)
             for j0 in range(0, nblk, 4)]

    def units(par, gb, j0):
        return [(par, g, j0) for g in range(gb * NA, (gb + 1) * NA)]

    order = [u for s in steps for u in units(*s)]
    wide = {}
    for i, u in enumerate(order):
        if (i + 1) * NW // len(order) > i * NW // len(order):
            wide[u] = len(wide)

    def widen(m):
        for (par, g, j), e in wide.items():
            v = f32_rows(kvu[m, 1, par, g // 2, g % 2, j // 2:j // 2 + 2])
            kvu[m, 1, par, g // 2, g % 2, j // 2:j // 2 + 2] = pltpu.bitcast(v[:, :8], U32)
            vx[m, e] = v[:, 8:]

    def v_unit(m, par, g, j):
        u = kvu[m, 1, par, g // 2, g % 2, j // 2:j // 2 + 2]
        if (par, g, j) in wide:
            return jnp.concatenate([pltpu.bitcast(u, F32), vx[m, wide[(par, g, j)]]], axis=1)
        return f32_rows(u)

    def pv_ops(m, ph):
        acc = {}

        def spread(par, q, r):
            pb_scr[pl.ds(64 * q + r, 8, stride=8), :] = p_scr[ph, par, 8 * q:8 * q + 8, :]

        def psum(par):
            p = p_scr[ph, par]
            accx[ph, 8 * (2 * G + par):8 * (2 * G + par) + 8, :] = (
                (p[0:8] + p[8:16]) + (p[16:24] + p[24:32]))

        pbv = {}

        def piece(par, gb, j0, k):
            if k == 0:
                if par == 0 and j0 < 8:
                    pb = pb0[ph, 8 * j0:8 * j0 + 32, :]
                else:
                    pb = pb_scr[8 * j0:8 * j0 + 32, :]
                pbv[0] = pb.reshape(4, 8, 128)
            for _, g, _ in units(par, gb, j0)[4 * k:4 * k + 4]:
                tv = v_unit(m, par, g, j0).reshape(4, 8, 128) * pbv[0]
                tv = jnp.sum(tv, axis=0)
                acc[g] = tv if j0 == 0 else acc[g] + tv
                if j0 == nblk - 4:
                    r0 = DH * par + 8 * g
                    accx[ph, r0:r0 + 8, :] = acc[g]

        pieces = [s + (k,) for s in steps for k in range(NA // 4)]
        half = len(pieces) // 2
        spq = 2 * (NA // 4)
        side = {}
        for q in range(nq):
            for r in range(8):
                if q:
                    side.setdefault((spq * (8 * (q - 1) + r)) // 9, []).append(
                        lambda q=q, r=r: spread(0, q, r))
                side.setdefault(half - nq * spq + spq * (q + 1) + (r * (3 * spq - 1)) // 8, []).append(
                    lambda q=q, r=r: spread(1, q, r))
        for par in range(2):
            side.setdefault(half // 2 + par, []).append(lambda par=par: psum(par))
        out = []
        for i, s in enumerate(pieces):
            out += [(0, f) for f in side.get(i, [])]
            out.append((2 * sum(4 if u in wide else 6 for u in units(*s[:3])[4 * s[3]:4 * s[3] + 4]),
                        (lambda s=s: piece(*s))))
        return out

    toks = []

    def fence(dst, slot, zero_i):
        for i, t in enumerate(toks):
            dst[slot + i + zero_i] = t
        toks.clear()

    def g_softmax(ph, par):
        s0 = part[2 * nq:3 * nq] if par else part_a[0:nq]
        s = (s0 + part[(2 * par + 1) * nq:(2 * par + 2) * nq]).reshape(nblk, 128)
        mx = jnp.max(jnp.max(s, axis=0, keepdims=True), axis=1, keepdims=True)
        p = jnp.exp2((s - mx) * jnp.concatenate([rs_scr[0]] * nq, axis=0))
        p_scr[ph, par] = p
        if par == 0:
            for r in range(8):
                pb0[ph, pl.ds(r, 8, stride=8), :] = p[0:8]
        toks.append(pltpu.bitcast(p[nblk - 8:nblk], U32))

    def recip(d):
        r = pl.reciprocal(d, approx=True)
        return r * (2.0 - d * r)

    def g_olhs(slot0, ph):
        z = [lane_sum(accx[ph, 8 * g:8 * g + 8, :]) for g in range(NZ)]
        inv = [jnp.broadcast_to(recip(jnp.sum(z[2 * G + par], axis=0, keepdims=True)), (8, 128))
               for par in range(2)]
        uid[0] += 1
        bit = [b > uid[0] for b in bit_i]
        for c in range(3):
            xs = z[16 * c:16 * c + 16]
            for k in range(4):
                xs = [jnp.where(bit[k], xs[i + 1], xs[i]) for i in range(0, len(xs), 2)]
            iv = inv[0] if c == 0 else (inv[1] if c == 2 else jnp.where(bit[3], inv[1], inv[0]))
            olhs[slot0 + c, 0:8, :] = jnp.where(diag_i > uid[0], xs[0] * iv, 0.0).astype(BF)

    def set_pat(c, q):
        if c == 1:
            hi = bit_i[3] > uid[0]
            pat_scr[c, 0:8, :] = jnp.where(hi, 0.0, q).astype(BF)
            pat_scr[c, 8:16, :] = jnp.where(hi, q, 0.0).astype(BF)
        else:
            pat_scr[c, 0:8, :] = q.astype(BF)
        if c > 0:
            toks.append(pltpu.bitcast(q, U32))

    def g_query(c):
        xs = [qpart[c * KD + k] for k in range(KD)]
        set_pat(c, ((xs[0] + xs[1]) + (xs[2] + xs[3])) + xs[4])

    def g_out(ph):
        for n in range(KD):
            out_scr[n] = out_scr[n] + opart[8 * ph + n]

    def reset_pipeline():
        accx[1, 0:16 * G, :] = jnp.zeros((16 * G, 128), F32)
        accx[1, 16 * G:16 * G + 16, :] = jnp.ones((16, 128), F32)
        for n in range(KD):
            opart[8 + n] = jnp.zeros((8, 128), F32)
            out_scr[n] = jnp.zeros((8, 128), F32)

    def emit(pv, seq):
        ntile = sum(not isinstance(e, tuple) for e in seq)
        total = sum(w for w, _ in pv) / 4
        k = done = n = 0
        for e in seq:
            if isinstance(e, tuple):
                e[0]()
                continue
            pos = LEAD + RATE * (n // 4) if n // 4 < (ntile - 1) // 4 else total - TAILC
            while k < len(pv) and done + pv[k][0] / 2 <= 4 * pos:
                done += pv[k][0]
                pv[k][1]()
                k += 1
            e(n < ntile - UNPACED)
            n += 1
        for _, g in pv[k:]:
            g()

    def ffn1(x):
        _, xc, rs = moments(x)
        y = jnp.broadcast_to(xc, (8, D)).astype(BF)
        reset_pipeline()

        def up(wu):
            cols = []
            for cp in range(NC // 2):
                ev, od = swap_halves(wu[:, 0, cp], wu[:, 1, cp])
                wu[:, 0, cp], wu[:, 1, cp] = ev, od
                cols += [jnp.dot(y, pltpu.bitcast(w.reshape(D // 2, 128), BF),
                                 preferred_element_type=F32) for w in (ev, od)]
            return jnp.concatenate(cols, axis=1) * rs

        def w2_rows(r0, n):
            v = w2u[r0:r0 + n]
            nat = regroup5(v)
            for c in range(KD):
                w2u[r0:r0 + n, c] = nat[c]
            return v, nat

        def down(o, n):
            cols = [None] * KD
            for k in range(o // 128, (o + n) // 128):
                for c, w in enumerate(w2_rows(8 * k, 8)[1]):
                    t = jnp.dot(hh[:, 128 * k:128 * k + 128], pltpu.bitcast(w.reshape(64, 128), BF),
                                preferred_element_type=F32)[0:1]
                    cols[c] = t if cols[c] is None else cols[c] + t
            return jnp.concatenate(cols, axis=1)

        c_w1.wait()
        g = up(w1u)
        c_w3.wait()
        u = up(w3u)
        hh = (g * jax.nn.sigmoid(g) * u).astype(BF)
        hb = columns(hh[:, w2_off[-1]:].astype(F32))
        a = None
        parts = list(zip(c_w2, w2_off, W2_CHUNKS))[:-1]
        if W2S:
            parts.insert(1, (w2_out, 0, 16 * W2S))
        for c, o, n in parts:
            c.wait()
            a = down(o, n) if a is None else a + down(o, n)
        c_w2[-1].wait()
        acc = [None] * KD
        for r in range(W2_CHUNKS[-1] // 16):
            v = f32_rows(w2_rows(w2_off[-1] // 16 + r, 1)[0][0])
            for f in range(2 * KD):
                tv = v[f // 2, 8 * (f % 2):8 * (f % 2) + 8] * hb[2 * r + f // KD]
                acc[f % KD] = tv if acc[f % KD] is None else acc[f % KD] + tv
        a = a + jnp.concatenate([jnp.sum(t, axis=0, keepdims=True) for t in acc], axis=1)
        return residual(x, a)

    def ffn2(x):
        mu, _, rs = moments(x)
        x8 = jnp.broadcast_to(x, (8, D))
        rowk = lax.broadcasted_iota(jnp.int32, (8, 128 * KM), 0)
        y = jnp.where(rowk == 0, x8[:, :128 * KM], jnp.where(rowk == 1, 1.0, 0.0)).astype(BF)
        coef = jnp.where(row == 0, 1.0, -mu)
        yb = jnp.concatenate([c - mu for c in columns(x8[:, 128 * KM:])], axis=0)
        mx = {}
        out = [None] * KD
        for c in range(NC):
            while len(mx) < min(NC, FPRE + c * FSTEP / 4):
                cc = len(mx)
                mx[cc] = [jnp.dot(y, pltpu.bitcast(wu[0:8 * KM, cc & 1, cc >> 1].reshape(64 * KM, 128), BF),
                                  preferred_element_type=F32) * coef for wu in (w1u, w3u)]
            gu = []
            for i, wu in enumerate((w1u, w3u)):
                acc = None
                for r in range(8 * (KD - KM)):
                    tv = f32_rows(wu[8 * KM + r, c & 1, c >> 1]) * yb[16 * r:16 * r + 16]
                    acc = tv if r == 0 else acc + tv
                gu.append(jnp.sum((acc[:8] + acc[8:]) + mx[c][i], axis=0, keepdims=True) * rs)
            hg = 0.5 * gu[0]
            h = jnp.broadcast_to((hg * jnp.tanh(hg) + hg) * gu[1], (8, 128)).astype(BF)
            for n in range(KD):
                t = jnp.dot(h, pltpu.bitcast(w2u[8 * c:8 * c + 8, n].reshape(64, 128), BF),
                            preferred_element_type=F32)[0:1]
                out[n] = t if c == 0 else out[n] + t
        return residual(x, jnp.concatenate(out, axis=1))

    def arrive(p, odd):
        def when(cond, f):
            if isinstance(cond, bool):
                if cond:
                    f()
            else:
                pl.when(cond)(f)

        cs = kv_copies(p)
        wait_all(cs[:4])
        when(not odd or p + 3 <= NST, lambda: stage_step(p + 3))
        wait_all(cs[4:TRG])
        when(odd and p == NP - 1, start_ffn_weights)
        wait_all(cs[TRG:])
        when(p + KVW < NP, lambda: kv_start(p + KVW))
        pair_rows(p)
        widen(p)
        when(odd and p == NP - 1, lambda: stage_step(NST + 1))

    def layer(li, x):
        first = li == 0
        zero_i = li >> 4

        def barrier():
            @pl.when(li > 2)
            def _():
                reset_pipeline()

        mu, xc, rs = moments(x)
        y = jnp.broadcast_to(xc, (8, D))
        for k in range(KD):
            y_scr[k, 0:8, :] = y[:, 128 * k:128 * k + 128].astype(BF)
        rs_scr[0] = jnp.broadcast_to(rs * c2, (8, 128))
        rowd = lax.broadcasted_iota(jnp.int32, (8, D), 0)
        xo = jnp.where(rowd < 4, jnp.broadcast_to(x, (8, D)), 1.0).astype(BF)
        coef = jnp.where(row < 4, 1.0, -mu)

        def q_direct(col):
            t = jnp.dot(xo, pltpu.bitcast(wqu[:, 0, :, 3 * (col & 1) + (col >> 1)].reshape(D // 2, 128), BF), preferred_element_type=F32) * coef
            return (t + pltpu.roll(t, 4, 0)).astype(BF).astype(F32)

        def q_cols(q, slot):
            for b, col in enumerate(columns(q)):
                part[slot + b] = col

        def vpu_a(m, slot, js):
            acc = {}
            for g2 in range(8):
                qc = jnp.concatenate([part[slot + 2 * g2 + t + zero_i] for t in range(2)], axis=0)
                for j in js:
                    tv = f32_rows(kvu[m, 0, 0, g2, j & 1, j >> 1]) * qc
                    acc[j] = tv if g2 == 0 else acc[j] + tv
            for j in js:
                part_a[j // 8, j % 8:j % 8 + 1, :] = jnp.sum(acc[j], axis=0, keepdims=True)

        q0 = [q_direct(c) for c in range(4)]
        q_cols(q0[0], SP)
        set_pat(1, q0[1])
        set_pat(2, q0[2])
        _, qb, qc = qk_ops(0)
        for i in range(nblk // 2):
            if i == PQH:
                q_cols(q0[3], SP + 16)
            vpu_a(0, SP, jord[2 * i:2 * i + 2])
            plain((qb + qc)[4 * i:4 * i + 4])
        g_softmax(0, 0)
        g_softmax(0, 1)
        plain(qproj_ops((0, 1))[KD:])
        g_query(1)
        g_query(2)
        set_pat(0, q0[3])
        qa = qk_ops(1)[0][PVB:]
        k = 0
        for i in range(0, PVB, 2):
            n = PTK + PFB * i // 2
            if n < 2 * KD:
                part[0] = qpart[KD + n]
            else:
                n = min(n - 2 * KD, len(qa) - 1)
                plain(qa[k:n + 1])
                k = max(k, n + 1)
                part[0] = part_a[jord[PVB + n] // 8]
            vpu_a(1, SP + 16, jord[i:i + 2])
        plain(qa[k:])
        toks.clear()

        def block(t, ph):
            m = 2 * t + ph

            qp = qproj_ops((t, ph + 2))
            _, qb, qc = qk_ops(m + 1)
            qa = qk_ops(m + 2)[0]
            op = oproj_ops(jnp.maximum(m - 1, 0), m + 2, opart, 8 * ph)
            seq = ([(lambda: g_out(1 - ph),), (lambda: g_olhs(3 * m, 1 - ph),)]
                   + qc[:CF] + qp[:KD] + [(lambda: g_query(0),)] + qc[CF:] + qb
                   + [(lambda: g_softmax(1 - ph, 0),), (lambda: g_softmax(1 - ph, 1),)]
                   + qp[KD:] + [(lambda: g_query(1),), (lambda: g_query(2),)]
                   + op + qa[:nblk - AEND] + [(lambda: fence(pat_u, 3, zero_i),)]
                   + qa[nblk - AEND:])
            emit(pv_ops(m, ph), seq)

        def body(t, carry):
            for ph in range(2):
                pl.when(first)(lambda: arrive(2 * t + ph + 2, ph == 1))
                block(t, ph)
            return carry

        lax.fori_loop(0, NP // 2 - 1, body, 0)

        def big(kts, i0):
            return [op for i, kt in enumerate(kts)
                    for op in oproj_ops(kt, kt + 3, part, SP + KD * (i0 + i))]

        old = list(range(NP - 3, 3 * (NP - 3)))
        _, qb, qc = qk_ops(NP - 1)
        seq = ([(lambda: g_out(1),), (lambda: g_olhs(3 * (NP - 2), 1),)] + qc + qb
               + [(lambda: g_softmax(1, 0),), (lambda: g_softmax(1, 1),)]
               + big(old[:KT14 - 4] + list(range(3 * (NP - 3), 3 * (NP - 2))), 0)
               + [(lambda: fence(olhs_u, 3 * NP, zero_i),)]
               + big(old[KT14 - 4:KT14 - 3], KT14 - 1))
        emit(pv_ops(NP - 2, 0), seq)
        barrier()
        k15 = old[KT14 - 3:-1] + list(range(3 * (NP - 2), 3 * (NP - 1))) + old[-1:]
        emit(pv_ops(NP - 1, 1), [(lambda: g_olhs(3 * (NP - 1), 0),)] + big(k15, KT14))

        def epilogue(x):
            def lsum(g):
                return lane_sum(accx[1, 8 * g:8 * g + 8, :])

            den = [jnp.sum(lsum(2 * G + par), axis=0, keepdims=True) for par in range(2)]
            fac = [den[0], den[1] * recip(den[0]), recip(den[1])]
            acc = []
            for n in range(KD):
                t = out_scr[n]
                for i in range(2 * NP):
                    t = t + part[SP + KD * i + n]
                acc.append(t * fac[0])
            for par in range(2):
                for g2 in range(G2):
                    g = G * par + 2 * g2
                    z0, z1 = lsum(g), lsum(g + 1)
                    for n in range(KD):
                        v = f32_rows(wou[RH - G + G2 * par + g2, n])
                        acc[n] = acc[n] + (v[:8] * z0 + v[8:] * z1)
                acc = [t * fac[par + 1] for t in acc]
            cols = [jnp.sum(t, axis=0, keepdims=True) for t in acc]
            return residual(x, jnp.concatenate(cols, axis=1))

        return lax.cond(first, lambda x: ffn1(epilogue(x)), lambda x: ffn2(epilogue(x)), x)

    for r in (y_u, pat_u, olhs_u):
        r[...] = jnp.zeros(r.shape, U32)
    reset_pipeline()
    stage_step(1)
    stage_step(2)
    kv_start(0)
    c_x.wait()
    kv_start(1)
    wait_all(c_wq)
    pair_wq()
    arrive(0, False)
    wait_all(c_wo)
    pair_wa()
    pair_wo(0, R0)
    arrive(1, True)
    x = lax.fori_loop(0, 2, layer, xb[...].astype(F32))
    o_ref[...] = x.astype(o_ref.dtype)


@jax.jit
def pallas_interleave_layers__sliding_block_cached__glu_gated_swiglu__decode_kernel(
    A_x: jax.Array,
    A_k_cache: jax.Array,
    A_v_cache: jax.Array,
    A_wq: jax.Array,
    A_wo: jax.Array,
    B_x: jax.Array,
    B_w1: jax.Array,
    B_w3: jax.Array,
    B_w2: jax.Array,
):
    del B_x
    sk = A_k_cache.shape[2]
    win = min(4096, max(256, sk // 4))
    nb = sk // 128
    nblk = win // 128

    def cache_tiles(c):
        return (c.reshape(H, nb, 128, G2, 2, 8).transpose(0, 3, 4, 1, 5, 2)
                .reshape(H, G2, 2, nb // 2, 16, 128))

    def weight_tiles(w):
        r, c = w.shape
        return w.reshape(r // 16, 2, 8, c // 128, 128).transpose(0, 1, 3, 2, 4)

    vreg = lambda n: pltpu.VMEM((-(-n // 4) * 4, 8, 128), F32)
    lhs = lambda n: pltpu.VMEM((-(-n // 4) * 4, 16, 128), BF)
    kern = lambda *refs: _kernel(*refs, blk0=nb - nblk, nblk=nblk, scale=DH ** -0.5)
    out = pl.pallas_call(
        kern,
        out_shape=jax.ShapeDtypeStruct((1, D), BF),
        in_specs=[pl.BlockSpec(memory_space=pl.ANY)] * 9,
        out_specs=pl.BlockSpec(memory_space=pltpu.VMEM),
        scratch_shapes=[
            pltpu.VMEM((1, D), BF),
            pltpu.VMEM((NP, 2, 2, G2, 2, nblk // 2, 16, 128), BF),
            pltpu.VMEM((D // 32, NP // 2, 2, 6, 16, 128), BF),
            pltpu.VMEM((6, 16, 2, KD, 16, 128), BF),
            pltpu.VMEM((H * G2 // 2, KD, 16, 128), BF),
            pltpu.VMEM((D // 16, 2, NC // 2, 16, 128), BF),
            pltpu.VMEM((D // 16, 2, NC // 2, 16, 128), BF),
            pltpu.VMEM((FF // 16, KD, 16, 128), BF),
            lhs(KD),
            vreg(1),
            vreg(3 * KD),
            lhs(8),
            vreg(nblk // 8),
            vreg(nblk // 2 + 2 * NP * KD),
            pltpu.VMEM((2, 2, nblk, 128), F32),
            pltpu.VMEM((nblk * 8, 128), F32),
            pltpu.VMEM((2, 64, 128), F32),
            pltpu.VMEM((2, 8 * NR, 128), F32),
            lhs(3 * NP + 4),
            vreg(16),
            vreg(KD),
            pltpu.VMEM((NP, NW, 2, 8, 128), F32),
            pltpu.SMEM((2, SC, KD, 16, 128), BF),
            pltpu.SemaphoreType.DMA((NP,)),
            pltpu.SemaphoreType.DMA((5 + len(W2_CHUNKS),)),
            pltpu.SemaphoreType.DMA((2,)),
        ],
        compiler_params=pltpu.CompilerParams(
            vmem_limit_bytes=128 * 1024 * 1024, disable_semaphore_checks=True),
    )(A_x.reshape(1, D), cache_tiles(A_k_cache), cache_tiles(A_v_cache),
      weight_tiles(A_wq).reshape(D // 32, NP // 2, 2, 6, 16, 128),
      weight_tiles(A_wo).reshape(12, 16, 2, KD, 16, 128),
      weight_tiles(A_wo).reshape(H * G2, KD, 16, 128),
      weight_tiles(B_w1).reshape(D // 16, 2, NC // 2, 16, 128),
      weight_tiles(B_w3).reshape(D // 16, 2, NC // 2, 16, 128),
      weight_tiles(B_w2).reshape(FF // 16, KD, 16, 128))
    return out.reshape(1, 1, D)
```

```python
import math

import jax
import jax.numpy as jnp
from jax import lax
import jax.experimental.pallas as pl
import jax.experimental.pallas.tpu as pltpu

BF = jnp.bfloat16
F32 = jnp.float32
U32 = jnp.uint32

D = 640
H = 32
DH = 192
G = DH // 8
G2 = DH // 16
NP = H // 2
FF = 1536
EPS = 1e-5
KD = D // 128
NC = FF // 128
NZ = 2 * G + 2
NR = NZ + 2
W2S = 8
W2_CHUNKS = (768 - 16 * W2S, 384, 256, 128)
NST = NP + 1
SC = 10
KVW = 2
TRG = 6

NA = 8
NW = 64
PACE_LOOP = (30.7, 36, 30)
PACE_QUAD = (33, 8, 30)
PACE_PAIR = (32.5, 16, 30)
UNPACED = 8
PM = 6
PK = 4
AEND = 4
OF = 19
CF = 8
KT13 = 6
KT14 = 20
PVB = 14
PQ1 = 8
PQH = 4
PQ2 = 16
PLG = 86
PFS = 3.75
KM = 3
FPRE = 8
FSTEP = 3


def _kernel(x_hbm, k_hbm, v_hbm, wq_hbm, wa_hbm, wo_hbm, w1_hbm, w3_hbm, w2_hbm,
            o_ref,
            xb, kvb, wq, wa, wo, w1, w3, w2,
            y_scr, rs_scr, qpart, pat_scr, part_a, part, p_scr, pb_scr, pb0,
            accx, olhs, plhs, vres, vx, stage,
            kvsem, wsem, ssem, *, blk0, nblk, scale):
    c2 = scale * math.log2(math.e)
    nq = nblk // 8
    SP = 4 * nq

    def kv_copies(m):
        n = nblk // 4
        return [pltpu.make_async_copy(
            src.at[pl.ds(2 * m, 2), :, t, pl.ds(blk0 // 2 + n * h, n)],
            kvb.at[m, i, :, :, t, pl.ds(n * h, n)], kvsem.at[m])
            for i, src in enumerate((k_hbm, v_hbm)) for t in range(2) for h in range(2)]

    def kv_start(m):
        for c in kv_copies(m):
            c.start()

    c_x = pltpu.make_async_copy(x_hbm, xb, wsem.at[0])
    c_wq = [pltpu.make_async_copy(wq_hbm.at[:, b], wq.at[:, b], wsem.at[1])
            for b in range(NP // 2)]
    RH = H * G2 // 2
    R0 = RH - NST * SC
    c_wo = [pltpu.make_async_copy(wa_hbm.at[pl.ds(0, 6), b], wa.at[:, b], wsem.at[2])
            for b in range(16)]
    c_wo.append(pltpu.make_async_copy(wo_hbm.at[pl.ds(RH, R0)], wo.at[pl.ds(0, R0)], wsem.at[2]))

    def to_stage(k):
        return pltpu.make_async_copy(wo_hbm.at[pl.ds(RH + R0 + SC * k, SC)], stage.at[k & 1],
                                     ssem.at[0])

    def from_stage(k):
        return pltpu.make_async_copy(stage.at[k & 1], wo.at[pl.ds(R0 + SC * k, SC)], ssem.at[1])

    def stage_step(k):
        def when(cond, f):
            if isinstance(cond, bool):
                if cond:
                    f()
            else:
                pl.when(cond)(f)

        def forward():
            to_stage(k - 1).wait()
            from_stage(k - 1).start()

        landed = not isinstance(k, int) or k >= 2
        if landed:
            from_stage(k - 2).wait()
        when(k <= NST, forward)
        when(k < NST, lambda: to_stage(k).start())
        when(k == NST, w2_in.start)
        if isinstance(k, int) and k == NST + 1:
            w2_in.wait()
            w2_out.start()
        if landed:
            pair_wo(R0 + SC * (k - 2), SC)

    c_w1 = pltpu.make_async_copy(w1_hbm, w1, wsem.at[3])
    c_w3 = pltpu.make_async_copy(w3_hbm, w3, wsem.at[4])
    w2_off = [16 * W2S + sum(W2_CHUNKS[:i]) for i in range(len(W2_CHUNKS))]
    c_w2 = [pltpu.make_async_copy(w2_hbm.at[pl.ds(o // 16, n // 16)],
                                  w2.at[pl.ds(o // 16, n // 16)], wsem.at[5 + i])
            for i, (o, n) in enumerate(zip(w2_off, W2_CHUNKS))]
    w2_slot = stage.at[NST & 1, pl.ds(0, W2S)]
    w2_in = pltpu.make_async_copy(w2_hbm.at[pl.ds(0, W2S)], w2_slot, ssem.at[0])
    w2_out = pltpu.make_async_copy(w2_slot, w2.at[pl.ds(0, W2S)], ssem.at[1])

    def wait_all(cs):
        for c in cs:
            c.wait()

    for c in c_wq[:1] + [to_stage(0), c_x] + c_wo + c_wq[1:]:
        c.start()

    def start_ffn_weights():
        for c in [c_w1, c_w3] + c_w2:
            c.start()

    kvu = kvb.bitcast(U32)
    wqu = wq.bitcast(U32)
    wau = wa.bitcast(U32)
    wou = wo.bitcast(U32)
    w1u, w3u, w2u = w1.bitcast(U32), w3.bitcast(U32), w2.bitcast(U32)
    y_u, pat_u, olhs_u = y_scr.bitcast(U32), pat_scr.bitcast(U32), olhs.bitcast(U32)
    plhs_u = plhs.bitcast(U32)

    def f32_rows(u):
        return pltpu.bitcast(u, BF).astype(F32)

    lane = lax.broadcasted_iota(jnp.int32, (8, 128), 1)
    row = lax.broadcasted_iota(jnp.int32, (8, 128), 0)
    diag_i = ((lane & 7) == row).astype(jnp.int32) * 64
    bit_i = [(lane << (3 - k)) & 64 for k in range(4)]
    uid = [0]

    def lane_sum(v):
        return jnp.broadcast_to(jnp.sum(v, axis=1, keepdims=True), (8, 128))

    def columns(v8):
        uid[0] += 1
        off = 256 * uid[0]
        dl = lane - row + off
        return [lane_sum(jnp.where(dl == off + 8 * b, v8[:, 128 * k:128 * k + 128], 0.0))
                for k in range(v8.shape[1] // 128) for b in range(16)]

    def moments(x):
        mu = jnp.mean(x, axis=-1, keepdims=True)
        xc = x - mu
        return mu, xc, 1.0 / jnp.sqrt(jnp.mean(xc * xc, axis=-1, keepdims=True) + EPS)

    def residual(x, a):
        return (x + a.astype(BF).astype(F32)).astype(BF).astype(F32)

    def tile_dot(l_u32, w_u32, rows, paced):
        w = pltpu.bitcast(w_u32.reshape(64, 128), BF)
        if paced:
            l = pltpu.bitcast(jnp.concatenate([l_u32, l_u32], axis=0), BF)[:24]
            return jnp.dot(l, w, preferred_element_type=F32)[:rows]
        l = pltpu.bitcast(l_u32, BF)[:rows]
        return jnp.dot(l, w, preferred_element_type=F32)

    def swap_halves(a, b):
        return (jnp.concatenate([a[..., :4, :], b[..., :4, :]], axis=-2),
                jnp.concatenate([a[..., 4:, :], b[..., 4:, :]], axis=-2))

    def pair_wq():
        def body(i, carry):
            for f in range(8):
                part[12 * f:12 * f + 12] = pltpu.bitcast(wqu[i, f].reshape(12, 8, 128), F32)
            for q in range(NP // 2):
                for r in range(2):
                    a, b = [pltpu.bitcast(part[48 * r + 24 * t + 3 * q:48 * r + 24 * t + 3 * q + 3], U32)
                            for t in range(2)]
                    wqu[i, q, r, 0:3], wqu[i, q, r, 3:6] = swap_halves(a, b)
            return carry
        lax.fori_loop(0, D // 32, body, 0)

    def regroup5(v):
        h = [v[:, f // 2, 4 * (f % 2):4 * (f % 2) + 4, :] for f in range(2 * KD)]
        return [jnp.concatenate([h[c], h[KD + c]], axis=1) for c in range(KD)]

    def pair_wo(r0, n):
        def body(i, carry):
            r = pl.ds(r0 + 2 * i, 2)
            for c, w in enumerate(regroup5(wou[r])):
                wou[r, c] = w
            return carry
        lax.fori_loop(0, n // 2, body, 0)

    def pair_wa():
        def body(i, carry):
            a, b = i >> 4, i & 15
            for c, w in enumerate(regroup5(wau[a, b])):
                wau[a, b, :, c] = w
            return carry
        lax.fori_loop(0, RH // 2, body, 0)

    def wo_tile(kt, n):
        if 8 * kt >= RH:
            return wou[8 * kt - RH:8 * kt - RH + 8, n]
        return wau[kt >> 2, 4 * (kt & 3):4 * (kt & 3) + 4, :, n]

    def wq_tile(m, c, k):
        c6 = 3 * m[1] + c
        return wqu[4 * k:4 * k + 4, m[0] + c6 // 6, :, 3 * (c6 & 1) + ((c6 % 6) >> 1)]

    def qproj_ops(m):
        def op(paced, c, k):
            qpart[c * KD + k] = tile_dot(
                y_u[k], wq_tile(m, c, k), 8, paced)
        return [(lambda p, c=c, k=k: op(p, c, k)) for c in range(3) for k in range(KD)]

    def oproj_ops(kt, slot, dst, d0):
        def op(paced, n):
            dst[d0 + n] = tile_dot(olhs_u[slot], wo_tile(kt, n), 8, paced)
        return [(lambda p, n=n: op(p, n)) for n in range(KD)]

    def pair_rows(m):
        def body(g2, c):
            for par in range(2):
                kvu[m, 0, par, g2, 0], kvu[m, 0, par, g2, 1] = swap_halves(
                    kvu[m, 0, par, g2, 0], kvu[m, 0, par, g2, 1])
            return c
        lax.fori_loop(0, G2, body, 0)

    def k_blocks(m, par, g0, g1, j):
        return kvu[m, 0, par, g0:g1, j & 1, j >> 1]

    jord = [8 * (i // 8) + 2 * (i % 4) + (i % 8) // 4 for i in range(nblk)]

    def qk_ops(m, po=0, pb=0):
        def op_a(paced, j):
            r = tile_dot(pat_u[po + 0], k_blocks(m, 0, 0, 8, j), 8, paced)
            part_a[j // 8, j % 8:j % 8 + 1, :] = r[j % 8:j % 8 + 1, :]

        def op_c(paced, j):
            r = tile_dot(pat_u[po + 2], k_blocks(m, 1, 4, 12, j), 8, paced)
            part[pb + 2 * nq + j // 8, j % 8:j % 8 + 1, :] = r[j % 8:j % 8 + 1, :]

        def op_b(paced, j):
            w = jnp.concatenate([k_blocks(m, 0, 8, 12, j), k_blocks(m, 1, 0, 4, j)], axis=0)
            r = tile_dot(pat_u[po + 1], w, 16, paced)
            part[pb + nq + j // 8, j % 8:j % 8 + 1, :] = r[j % 8:j % 8 + 1, :]
            part[pb + 3 * nq + j // 8, j % 8:j % 8 + 1, :] = r[8 + j % 8:8 + j % 8 + 1, :]

        return [[(lambda p, f=f, j=j: f(p, j)) for j in jord] for f in (op_a, op_b, op_c)]

    def plain(ops):
        for op in ops:
            op(False)

    steps = [(par, gb, j0) for par in range(2) for gb in range(G // NA)
             for j0 in range(0, nblk, 4) if j0 != 4 or gb == 2 - 2 * par]

    def flip(m):
        for par in range(2):
            for a in range(2):
                v = f32_rows(kvu[m, 1, par, 4 * par:4 * par + 8, :, 2 + a])
                ts = [v[:, :, 8 * b:8 * b + 8, :].reshape(128, 128).T.astype(BF) for b in range(2)]
                for b in range(2):
                    kvu[m, 1, par, 4 * par:4 * par + 8, b, 2 + a] = (
                        pltpu.bitcast(ts[b], U32).reshape(8, 8, 128))

    def pvm_ops(m, sl):
        def op(paced, par, j):
            r = tile_dot(plhs_u[2 * sl + par],
                         kvu[m, 1, par, 4 * par:4 * par + 8, j & 1, j >> 1], 8, paced)
            vres[2 * sl + par, j:j + 1, :] = r[j:j + 1, :]
        return [(lambda p, par=par, j=j: op(p, par, j))
                for j in range(4, 8) for par in range(2)]

    def units(par, gb, j0):
        return [(par, g, j0) for g in range(gb * NA, (gb + 1) * NA)]

    order = [u for s in steps for u in units(*s)]
    wide = {}
    for i, u in enumerate(order):
        if (i + 1) * NW // len(order) > i * NW // len(order):
            wide[u] = len(wide)

    def widen(m):
        for (par, g, j), e in wide.items():
            v = f32_rows(kvu[m, 1, par, g // 2, g % 2, j // 2:j // 2 + 2])
            kvu[m, 1, par, g // 2, g % 2, j // 2:j // 2 + 2] = pltpu.bitcast(v[:, :8], U32)
            vx[m, e] = v[:, 8:]

    def v_unit(m, par, g, j):
        u = kvu[m, 1, par, g // 2, g % 2, j // 2:j // 2 + 2]
        if (par, g, j) in wide:
            return jnp.concatenate([pltpu.bitcast(u, F32), vx[m, wide[(par, g, j)]]], axis=1)
        return f32_rows(u)

    def pv_ops(m, ph):
        acc = {}

        def spread(par, q, r):
            pb_scr[pl.ds(64 * q + r, 8, stride=8), :] = p_scr[ph, par, 8 * q:8 * q + 8, :]

        def psum(par):
            p = p_scr[ph, par]
            accx[ph, 8 * (2 * G + par):8 * (2 * G + par) + 8, :] = (
                (p[0:8] + p[8:16]) + (p[16:24] + p[24:32]))

        pbv = {}

        def piece(par, gb, j0, k):
            if k == 0:
                if par == 0 and j0 < 8:
                    pb = pb0[ph, 8 * j0:8 * j0 + 32, :]
                else:
                    pb = pb_scr[8 * j0:8 * j0 + 32, :]
                pbv[0] = pb.reshape(4, 8, 128)
            for _, g, _ in units(par, gb, j0)[4 * k:4 * k + 4]:
                tv = v_unit(m, par, g, j0).reshape(4, 8, 128) * pbv[0]
                tv = jnp.sum(tv, axis=0)
                acc[g] = tv if j0 == 0 else acc[g] + tv
                if j0 == nblk - 4:
                    r0 = DH * par + 8 * g
                    accx[ph, r0:r0 + 8, :] = acc[g]

        pieces = [s + (k,) for s in steps for k in range(NA // 4)]
        use = {}
        for i, (par, _, j0, k) in enumerate(pieces):
            if k == 0:
                use.setdefault((par, j0 // 8), []).append(i)
        side = {}
        for q in range(nq):
            for r in range(8):
                if q:
                    lo, hi = (use[0, q - 1][0] - 1 if q > 1 else 0), use[0, q][0] - 1
                    side.setdefault(lo + (r * (hi - lo + 1)) // 8, []).append(
                        lambda q=q, r=r: spread(0, q, r))
                lo, hi = use[0, q][-1] + 1, use[1, q][0] - 1
                side.setdefault(lo + (r * (hi - lo)) // 8, []).append(
                    lambda q=q, r=r: spread(1, q, r))
        for par in range(2):
            side.setdefault(len(pieces) // 4 + par, []).append(lambda par=par: psum(par))
        out = []
        for i, s in enumerate(pieces):
            out += [(0, f) for f in side.get(i, [])]
            out.append((2 * sum(4 if u in wide else 6 for u in units(*s[:3])[4 * s[3]:4 * s[3] + 4]),
                        (lambda s=s: piece(*s))))
        return out

    toks = []

    def fence(dst, slot, zero_i):
        for i, t in enumerate(toks):
            dst[slot + i + zero_i] = t
        toks.clear()

    def g_softmax(ph, par, pb=0, pa=0):
        s0 = part[pb + 2 * nq:pb + 3 * nq] if par else part_a[pa:pa + nq]
        s = (s0 + part[pb + (2 * par + 1) * nq:pb + (2 * par + 2) * nq]).reshape(nblk, 128)
        mx = jnp.max(jnp.max(s, axis=0, keepdims=True), axis=1, keepdims=True)
        p = jnp.exp2((s - mx) * jnp.concatenate([rs_scr[0]] * nq, axis=0))
        p_scr[ph, par] = p
        plhs[2 * ph + par, 0:8, :] = p[0:8].astype(BF)
        if par == 0:
            for r in range(8):
                pb0[ph, pl.ds(r, 8, stride=8), :] = p[0:8]
        toks.append(pltpu.bitcast(p[nblk - 8:nblk], U32))

    def recip(d):
        r = pl.reciprocal(d, approx=True)
        return r * (2.0 - d * r)

    def g_olhs(slot0, ph, tok=False):
        zz = [lane_sum(accx[ph, 8 * g:8 * g + 8, :]) for g in range(NZ)]
        inv = [jnp.broadcast_to(recip(jnp.sum(zz[2 * G + par], axis=0, keepdims=True)), (8, 128))
               for par in range(2)]
        uid[0] += 1
        bit = [b > uid[0] for b in bit_i]
        for c in range(3):
            xs = zz[16 * c:16 * c + 16]
            for k in range(4):
                xs = [jnp.where(bit[k], xs[i + 1], xs[i]) for i in range(0, len(xs), 2)]
            iv = inv[0] if c == 0 else (inv[1] if c == 2 else jnp.where(bit[3], inv[1], inv[0]))
            z = jnp.where(diag_i > uid[0], xs[0], 0.0)
            if c != 1:
                z = z + vres[2 * ph + c // 2]
            z = z * iv
            olhs[slot0 + c, 0:8, :] = z.astype(BF)
            if tok:
                toks.append(pltpu.bitcast(z, U32))

    def set_pat(c, q, po=0):
        if c == 1:
            hi = bit_i[3] > uid[0]
            pat_scr[po + c, 0:8, :] = jnp.where(hi, 0.0, q).astype(BF)
            pat_scr[po + c, 8:16, :] = jnp.where(hi, q, 0.0).astype(BF)
        else:
            pat_scr[po + c, 0:8, :] = q.astype(BF)
        if c > 0:
            toks.append(pltpu.bitcast(q, U32))

    def g_query(c):
        xs = [qpart[c * KD + k] for k in range(KD)]
        set_pat(c, ((xs[0] + xs[1]) + (xs[2] + xs[3])) + xs[4])

    def clear_acc():
        accx[2:4] = jnp.ones((2, 8 * NR, 128), F32)

    def emit(pv, seq, pace, pk=PM):
        rate, lead, tail = pace
        ntile = sum(not isinstance(e, tuple) for e in seq)
        total = sum(w for w, _ in pv) / 4
        k = done = n = 0
        for e in seq:
            if isinstance(e, tuple):
                e[0]()
                continue
            r = n // 4
            pos = lead + rate * r if r < (ntile - 1) // 4 else total - tail
            while k < len(pv) and done + pv[k][0] / 2 <= 4 * pos:
                done += pv[k][0]
                pv[k][1]()
                k += 1
            e(n < ntile - UNPACED and r % PM < pk)
            n += 1
        for _, g in pv[k:]:
            g()

    def ffn1(x):
        _, xc, rs = moments(x)
        y = jnp.broadcast_to(xc, (8, D)).astype(BF)

        def up(wu):
            cols = []
            for cp in range(NC // 2):
                ev, od = swap_halves(wu[:, 0, cp], wu[:, 1, cp])
                wu[:, 0, cp], wu[:, 1, cp] = ev, od
                cols += [jnp.dot(y, pltpu.bitcast(w.reshape(D // 2, 128), BF),
                                 preferred_element_type=F32) for w in (ev, od)]
            return jnp.concatenate(cols, axis=1) * rs

        def w2_rows(r0, n):
            v = w2u[r0:r0 + n]
            nat = regroup5(v)
            for c in range(KD):
                w2u[r0:r0 + n, c] = nat[c]
            return v, nat

        def down(o, n):
            cols = [None] * KD
            for k in range(o // 128, (o + n) // 128):
                for c, w in enumerate(w2_rows(8 * k, 8)[1]):
                    t = jnp.dot(hh[:, 128 * k:128 * k + 128], pltpu.bitcast(w.reshape(64, 128), BF),
                                preferred_element_type=F32)[0:1]
                    cols[c] = t if cols[c] is None else cols[c] + t
            return jnp.concatenate(cols, axis=1)

        c_w1.wait()
        g = up(w1u)
        c_w3.wait()
        u = up(w3u)
        hh = (g * jax.nn.sigmoid(g) * u).astype(BF)
        hb = columns(hh[:, w2_off[-1]:].astype(F32))
        a = None
        parts = list(zip(c_w2, w2_off, W2_CHUNKS))[:-1]
        parts.insert(1, (w2_out, 0, 16 * W2S))
        for c, o, n in parts:
            c.wait()
            a = down(o, n) if a is None else a + down(o, n)
        c_w2[-1].wait()
        acc = [None] * KD
        for r in range(W2_CHUNKS[-1] // 16):
            v = f32_rows(w2_rows(w2_off[-1] // 16 + r, 1)[0][0])
            for f in range(2 * KD):
                tv = v[f // 2, 8 * (f % 2):8 * (f % 2) + 8] * hb[2 * r + f // KD]
                acc[f % KD] = tv if acc[f % KD] is None else acc[f % KD] + tv
        a = a + jnp.concatenate([jnp.sum(t, axis=0, keepdims=True) for t in acc], axis=1)
        return residual(x, a)

    def ffn2(x):
        mu, _, rs = moments(x)
        x8 = jnp.broadcast_to(x, (8, D))
        rowk = lax.broadcasted_iota(jnp.int32, (8, 128 * KM), 0)
        y = jnp.where(rowk == 0, x8[:, :128 * KM], jnp.where(rowk == 1, 1.0, 0.0)).astype(BF)
        coef = jnp.where(row == 0, 1.0, -mu)
        yb = jnp.concatenate([c - mu for c in columns(x8[:, 128 * KM:])], axis=0)
        mx = {}
        out = [None] * KD
        for c in range(NC):
            while len(mx) < min(NC, FPRE + c * FSTEP / 4):
                cc = len(mx)
                mx[cc] = [jnp.dot(y, pltpu.bitcast(wu[0:8 * KM, cc & 1, cc >> 1].reshape(64 * KM, 128), BF),
                                  preferred_element_type=F32) * coef for wu in (w1u, w3u)]
            gu = []
            for i, wu in enumerate((w1u, w3u)):
                acc = None
                for r in range(8 * (KD - KM)):
                    tv = f32_rows(wu[8 * KM + r, c & 1, c >> 1]) * yb[16 * r:16 * r + 16]
                    acc = tv if r == 0 else acc + tv
                gu.append(jnp.sum((acc[:8] + acc[8:]) + mx[c][i], axis=0, keepdims=True) * rs)
            hg = 0.5 * gu[0]
            h = jnp.broadcast_to((hg * jnp.tanh(hg) + hg) * gu[1], (8, 128)).astype(BF)
            for n in range(KD):
                t = jnp.dot(h, pltpu.bitcast(w2u[8 * c:8 * c + 8, n].reshape(64, 128), BF),
                            preferred_element_type=F32)[0:1]
                out[n] = t if c == 0 else out[n] + t
        return residual(x, jnp.concatenate(out, axis=1))

    def arrive(p, last):
        def when(cond, f):
            if isinstance(cond, bool):
                if cond:
                    f()
            else:
                pl.when(cond)(f)

        cs = kv_copies(p)
        wait_all(cs[:4])
        if not last:
            stage_step(p + 3)
        wait_all(cs[4:TRG])
        if last:
            start_ffn_weights()
        wait_all(cs[TRG:])
        when(p + KVW < NP, lambda: kv_start(p + KVW))
        pair_rows(p)
        widen(p)
        flip(p)
        if last:
            stage_step(NST + 1)

    def arrivals(p0, n):
        def body(i, carry):
            arrive(p0 + i, False)
            return carry
        lax.fori_loop(0, n, body, 0)

    def layer(li, x):
        first = li == 0
        zero_i = li >> 4

        def barrier():
            @pl.when(li > 2)
            def _():
                clear_acc()

        mu, xc, rs = moments(x)
        y = jnp.broadcast_to(xc, (8, D))
        for k in range(KD):
            y_scr[k, 0:8, :] = y[:, 128 * k:128 * k + 128].astype(BF)
        rs_scr[0] = jnp.broadcast_to(rs * c2, (8, 128))
        rowd = lax.broadcasted_iota(jnp.int32, (8, D), 0)
        xo = jnp.where(rowd < 4, jnp.broadcast_to(x, (8, D)), 1.0).astype(BF)
        coef = jnp.where(row < 4, 1.0, -mu)

        def q_direct(col):
            t = jnp.dot(xo, pltpu.bitcast(wqu[:, 0, :, 3 * (col & 1) + (col >> 1)].reshape(D // 2, 128), BF), preferred_element_type=F32) * coef
            return (t + pltpu.roll(t, 4, 0)).astype(BF).astype(F32)

        def q_cols(q, slot):
            for b, col in enumerate(columns(q)):
                part[slot + b] = col

        def vpu_a(m, slot, js, pa):
            z = zero_i if m == 0 else 0
            acc = {}
            for g2 in range(8):
                qc = jnp.concatenate([part[slot + 2 * g2 + t + z] for t in range(2)], axis=0)
                for j in js:
                    tv = f32_rows(kvu[m, 0, 0, g2, j & 1, j >> 1]) * qc
                    acc[j] = tv if g2 == 0 else acc[j] + tv
            rs_ = [jnp.sum(acc[j], axis=0, keepdims=True) for j in js]
            for j, r in zip(js, rs_):
                part_a[pa + j // 8, j % 8:j % 8 + 1, :] = r
            return [pltpu.bitcast(jnp.broadcast_to(r, (8, 128)), U32) for r in rs_]

        def q_sum(c):
            xs = [qpart[c * KD + k] for k in range(KD)]
            return (((xs[0] + xs[1]) + (xs[2] + xs[3])) + xs[4]).astype(BF).astype(F32)

        q0 = [q_direct(c) for c in range(4)]
        q_cols(q0[0], SP)
        set_pat(1, q0[1], 10)
        set_pat(2, q0[2], 10)
        P0 = SP + 48

        def mark(ops, src):
            def wrap(op, v):
                def f(p):
                    op(p)
                    part[0] = v()
                return f
            return [wrap(op, v) for op, v in zip(ops, src)]

        def qp(m, lo, hi):
            return mark(qproj_ops((0, m))[lo:hi], [(lambda i=i: qpart[i]) for i in range(lo, hi)])

        st = {}

        def queries():
            g_query(1)
            g_query(2)
            st["q"] = q_sum(0)
            set_pat(0, st["q"])

        _, b0, c0 = qk_ops(0, 10, P0)
        _, b1, c1 = qk_ops(1)
        a2 = qk_ops(2)[0][PVB:]
        bc = b0 + c0

        def sprinkle(few, many):
            out = []
            for i, e in enumerate(many):
                out.append(e)
                if i % 3 == 2 and i // 3 < len(few):
                    out.append(few[i // 3])
            return out + few[len(many) // 3:]

        q2 = qproj_ops((0, 2))[KD:]
        mx = (bc[:PQ1] + qp(1, KD, 3 * KD) + qp(2, 0, KD) + [(queries,)] + bc[PQ1:]
              + [(lambda: g_softmax(0, 1, P0),)]
              + sprinkle(q2, b1) + c1 + [(lambda: g_softmax(1, 1),)]
              + [(lambda: g_query(1),), (lambda: g_query(2),)] + a2)
        vg = ([(0, SP, jord[i:i + 2], 2 * nq) for i in range(0, nblk, 2)]
              + [(1, SP + 16, jord[i:i + 2], nq) for i in range(0, nblk, 2)]
              + [(2, SP + 32, jord[i:i + 2], 0) for i in range(0, PVB, 2)])
        n = g = 0
        done = set()

        def ripe():
            if "s0" not in done and g >= nblk // 2 and n >= nblk + 3 * KD:
                done.add("s0")
                g_softmax(0, 0, P0, 2 * nq)
            if "s1" not in done and g >= nblk and n >= 3 * nblk + 5 * KD:
                done.add("s1")
                g_softmax(1, 0, 0, nq)

        for e in mx + [None]:
            while g < len(vg) and (e is None or (4 * g if g < 16 else PLG + PFS * (g - 16)) <= n):
                if g == PQH:
                    q_cols(q0[3], SP + 16)
                if g == PQ2:
                    q_cols(st["q"], SP + 32)
                toks[:] = vpu_a(*vg[g])
                if g >= 16 and e is not None:
                    fence(pat_u, 3, zero_i)
                g += 1
                ripe()
            if isinstance(e, tuple):
                e[0]()
            elif e is not None:
                e(False)
                n += 1
                ripe()
        toks.clear()

        def half(b, ph, e):
            n = 2 * b + 2 + e
            qp = qproj_ops((b, 3 + e))
            _, qb, qc = qk_ops(n)
            qa = qk_ops(n + 1)[0]
            so = 2 * (1 - ph) + e
            return ([(lambda: g_olhs(3 * (n - 2), so, True),)]
                    + qc[:CF] + qp[:KD] + [(lambda: g_query(0),)] + qc[CF:] + qb[:OF]
                    + [(lambda: fence(pat_u, 3, zero_i),)] + qb[OF:]
                    + [(lambda: g_softmax(so, 0),), (lambda: g_softmax(so, 1),)]
                    + qp[KD:] + [(lambda: g_query(1),), (lambda: g_query(2),)]
                    + pvm_ops(2 * b + e, 2 * ph + e)
                    + qa[:nblk - AEND] + [(lambda: fence(pat_u, 3, zero_i),)] + qa[nblk - AEND:])

        def body(t, carry):
            for ph in range(2):
                b = 2 * t + ph

                @pl.when(first)
                def _():
                    arrivals(2 * b + 3, 2)

                emit(pv_ops(2 * b, 2 * ph) + pv_ops(2 * b + 1, 2 * ph + 1),
                     half(b, ph, 0) + half(b, ph, 1), PACE_LOOP, PK)
            return carry

        lax.fori_loop(0, 3, body, 0)

        def big(kts):
            return [op for kt in kts for op in oproj_ops(kt, kt + 6, part, SP + KD * kt)]

        pl.when(first)(lambda: arrive(NP - 1, True))
        _, qb, qc = qk_ops(NP - 1)
        seq = (half(6, 0, 0) + [(lambda: g_olhs(3 * 13, 3, True),)] + qc + qb[:OF]
               + [(lambda: fence(pat_u, 3, zero_i),)] + qb[OF:]
               + [(lambda: g_softmax(3, 0),), (lambda: g_softmax(3, 1),)]
               + pvm_ops(13, 1) + big(range(KT13 - 1))
               + [(lambda: fence(olhs_u, 3 * NP + 4, zero_i),)] + big([KT13 - 1]))
        emit(pv_ops(12, 0) + pv_ops(13, 1), seq, PACE_QUAD)
        barrier()
        old = list(range(KT13, 36))
        k14 = old[:KT14 - 7] + list(range(36, 42)) + old[KT14 - 7:KT14 - 6]
        emit(pv_ops(14, 2), [(lambda: g_olhs(3 * 14, 0),), (lambda: g_olhs(3 * 15, 1),)]
             + pvm_ops(14, 2) + big(k14), PACE_PAIR)
        barrier()
        k15 = old[KT14 - 6:-1] + list(range(42, 45)) + old[-1:]
        emit(pv_ops(15, 3), [(lambda: g_olhs(3 * 16, 2),)] + pvm_ops(15, 3) + big(k15), PACE_PAIR)

        def epilogue(x):
            def lsum(g):
                return lane_sum(accx[3, 8 * g:8 * g + 8, :])

            den = [jnp.sum(lsum(2 * G + par), axis=0, keepdims=True) for par in range(2)]
            fac = [den[0], den[1] * recip(den[0]), recip(den[1])]
            acc = []
            for n in range(KD):
                t = part[SP + n]
                for i in range(1, 3 * NP - 3):
                    t = t + part[SP + KD * i + n]
                acc.append(t * fac[0])
            for par in range(2):
                for g2 in range(G2):
                    g = G * par + 2 * g2
                    z0, z1 = lsum(g), lsum(g + 1)
                    for n in range(KD):
                        v = f32_rows(wou[RH - G + G2 * par + g2, n])
                        acc[n] = acc[n] + (v[:8] * z0 + v[8:] * z1)
                l = vres[6 + par].astype(BF)
                acc = [acc[n] + jnp.dot(
                    l, pltpu.bitcast(wo_tile(3 * NP - 3 + 2 * par, n).reshape(64, 128), BF),
                    preferred_element_type=F32) * 1.0 for n in range(KD)]
                acc = [t * fac[par + 1] for t in acc]
            cols = [jnp.sum(t, axis=0, keepdims=True) for t in acc]
            return residual(x, jnp.concatenate(cols, axis=1))

        return lax.cond(first, lambda x: ffn1(epilogue(x)), lambda x: ffn2(epilogue(x)), x)

    for r in (y_u, pat_u, olhs_u, plhs_u):
        r[...] = jnp.zeros(r.shape, U32)
    vres[...] = jnp.zeros(vres.shape, F32)
    clear_acc()
    stage_step(1)
    stage_step(2)
    kv_start(0)
    c_x.wait()
    kv_start(1)
    wait_all(c_wq)
    pair_wq()
    arrivals(0, 3)
    wait_all(c_wo)
    pair_wa()
    pair_wo(0, R0)
    x = lax.fori_loop(0, 2, layer, xb[...].astype(F32))
    o_ref[...] = x.astype(o_ref.dtype)


@jax.jit
def pallas_interleave_layers__sliding_block_cached__glu_gated_swiglu__decode_kernel(
    A_x: jax.Array,
    A_k_cache: jax.Array,
    A_v_cache: jax.Array,
    A_wq: jax.Array,
    A_wo: jax.Array,
    B_x: jax.Array,
    B_w1: jax.Array,
    B_w3: jax.Array,
    B_w2: jax.Array,
):
    del B_x
    sk = A_k_cache.shape[2]
    win = min(4096, max(256, sk // 4))
    nb = sk // 128
    nblk = win // 128

    def cache_tiles(c):
        return (c.reshape(H, nb, 128, G2, 2, 8).transpose(0, 3, 4, 1, 5, 2)
                .reshape(H, G2, 2, nb // 2, 16, 128))

    def weight_tiles(w):
        r, c = w.shape
        return w.reshape(r // 16, 2, 8, c // 128, 128).transpose(0, 1, 3, 2, 4)

    vreg = lambda n: pltpu.VMEM((-(-n // 4) * 4, 8, 128), F32)
    lhs = lambda n: pltpu.VMEM((-(-n // 4) * 4, 16, 128), BF)
    kern = lambda *refs: _kernel(*refs, blk0=nb - nblk, nblk=nblk, scale=DH ** -0.5)
    out = pl.pallas_call(
        kern,
        out_shape=jax.ShapeDtypeStruct((1, D), BF),
        in_specs=[pl.BlockSpec(memory_space=pl.ANY)] * 9,
        out_specs=pl.BlockSpec(memory_space=pltpu.VMEM),
        scratch_shapes=[
            pltpu.VMEM((1, D), BF),
            pltpu.VMEM((NP, 2, 2, G2, 2, nblk // 2, 16, 128), BF),
            pltpu.VMEM((D // 32, NP // 2, 2, 6, 16, 128), BF),
            pltpu.VMEM((6, 16, 2, KD, 16, 128), BF),
            pltpu.VMEM((H * G2 // 2, KD, 16, 128), BF),
            pltpu.VMEM((D // 16, 2, NC // 2, 16, 128), BF),
            pltpu.VMEM((D // 16, 2, NC // 2, 16, 128), BF),
            pltpu.VMEM((FF // 16, KD, 16, 128), BF),
            lhs(KD),
            vreg(1),
            vreg(3 * KD),
            lhs(16),
            vreg(3 * nblk // 8),
            vreg(nblk // 2 + (3 * NP - 3) * KD),
            pltpu.VMEM((4, 2, nblk, 128), F32),
            pltpu.VMEM((nblk * 8, 128), F32),
            pltpu.VMEM((4, 64, 128), F32),
            pltpu.VMEM((4, 8 * NR, 128), F32),
            lhs(3 * NP + 12),
            lhs(8),
            vreg(8),
            pltpu.VMEM((NP, NW, 2, 8, 128), F32),
            pltpu.SMEM((2, SC, KD, 16, 128), BF),
            pltpu.SemaphoreType.DMA((NP,)),
            pltpu.SemaphoreType.DMA((5 + len(W2_CHUNKS),)),
            pltpu.SemaphoreType.DMA((2,)),
        ],
        compiler_params=pltpu.CompilerParams(
            vmem_limit_bytes=128 * 1024 * 1024, disable_semaphore_checks=True),
    )(A_x.reshape(1, D), cache_tiles(A_k_cache), cache_tiles(A_v_cache),
      weight_tiles(A_wq).reshape(D // 32, NP // 2, 2, 6, 16, 128),
      weight_tiles(A_wo).reshape(12, 16, 2, KD, 16, 128),
      weight_tiles(A_wo).reshape(H * G2, KD, 16, 128),
      weight_tiles(B_w1).reshape(D // 16, 2, NC // 2, 16, 128),
      weight_tiles(B_w3).reshape(D // 16, 2, NC // 2, 16, 128),
      weight_tiles(B_w2).reshape(FF // 16, KD, 16, 128))
    return out.reshape(1, 1, D)
```

```python
import math

import jax
import jax.numpy as jnp
from jax import lax
import jax.experimental.pallas as pl
import jax.experimental.pallas.tpu as pltpu

BF = jnp.bfloat16
F32 = jnp.float32
U32 = jnp.uint32

D = 640
H = 32
DH = 192
G = DH // 8
G2 = DH // 16
NP = H // 2
FF = 1536
EPS = 1e-5
KD = D // 128
NC = FF // 128
NZ = 2 * G + 2
NR = NZ + 2
W2S = 8
W2_CHUNKS = (768 - 16 * W2S, 384, 256, 128)
NST = NP + 1
SC = 10
KVW = 2
TRG = 6

NA = 8
NW = 64
PACE_LOOP = (30.7, 36, 30)
PACE_QUAD = (33, 8, 30)
PACE_PAIR = (32.5, 16, 30)
UNPACED = 8
PM = 6
PK = 4
AEND = 4
OF = 19
CF = 8
KT13 = 6
KT14 = 20
PVB = 14
PQ1 = 8
PQH = 4
PQ2 = 16
PLG = 86
PFS = 3.75
KM = 3
FPRE = 8
FSTEP = 3


def _kernel(x_hbm, k_hbm, v_hbm, wq_hbm, wa_hbm, wo_hbm, w1_hbm, w3_hbm, w2_hbm,
            o_ref,
            xb, kvb, wq, wa, wo, w1, w3, w2,
            y_scr, rs_scr, qpart, pat_scr, part_a, part, p_scr, pb_scr, pb0,
            accx, olhs, plhs, vres, vx, stage,
            kvsem, wsem, ssem, *, blk0, nblk, scale):
    c2 = scale * math.log2(math.e)
    nq = nblk // 8
    SP = 4 * nq

    def kv_copies(m):
        n = nblk // 4
        return [pltpu.make_async_copy(
            src.at[pl.ds(2 * m, 2), :, t, pl.ds(blk0 // 2 + n * h, n)],
            kvb.at[m, i, :, :, t, pl.ds(n * h, n)], kvsem.at[m])
            for i, src in enumerate((k_hbm, v_hbm)) for t in range(2) for h in range(2)]

    def kv_start(m):
        for c in kv_copies(m):
            c.start()

    c_x = pltpu.make_async_copy(x_hbm, xb, wsem.at[0])
    c_wq = [pltpu.make_async_copy(wq_hbm.at[:, b], wq.at[:, b], wsem.at[1])
            for b in range(NP // 2)]
    RH = H * G2 // 2
    R0 = RH - NST * SC
    c_wo = [pltpu.make_async_copy(wa_hbm.at[pl.ds(0, 6), b], wa.at[:, b], wsem.at[2])
            for b in range(16)]
    c_wo.append(pltpu.make_async_copy(wo_hbm.at[pl.ds(RH, R0)], wo.at[pl.ds(0, R0)], wsem.at[2]))

    def to_stage(k):
        return pltpu.make_async_copy(wo_hbm.at[pl.ds(RH + R0 + SC * k, SC)], stage.at[k & 1],
                                     ssem.at[0])

    def from_stage(k):
        return pltpu.make_async_copy(stage.at[k & 1], wo.at[pl.ds(R0 + SC * k, SC)], ssem.at[1])

    def stage_step(k):
        def when(cond, f):
            if isinstance(cond, bool):
                if cond:
                    f()
            else:
                pl.when(cond)(f)

        def forward():
            to_stage(k - 1).wait()
            from_stage(k - 1).start()

        landed = not isinstance(k, int) or k >= 2
        if landed:
            from_stage(k - 2).wait()
        when(k <= NST, forward)
        when(k < NST, lambda: to_stage(k).start())
        when(k == NST, w2_in.start)
        if isinstance(k, int) and k == NST + 1:
            w2_in.wait()
            w2_out.start()
        if landed:
            pair_wo(R0 + SC * (k - 2), SC)

    c_w1 = pltpu.make_async_copy(w1_hbm, w1, wsem.at[3])
    c_w3 = pltpu.make_async_copy(w3_hbm, w3, wsem.at[4])
    w2_off = [16 * W2S + sum(W2_CHUNKS[:i]) for i in range(len(W2_CHUNKS))]
    c_w2 = [pltpu.make_async_copy(w2_hbm.at[pl.ds(o // 16, n // 16)],
                                  w2.at[pl.ds(o // 16, n // 16)], wsem.at[5 + i])
            for i, (o, n) in enumerate(zip(w2_off, W2_CHUNKS))]
    w2_slot = stage.at[NST & 1, pl.ds(0, W2S)]
    w2_in = pltpu.make_async_copy(w2_hbm.at[pl.ds(0, W2S)], w2_slot, ssem.at[0])
    w2_out = pltpu.make_async_copy(w2_slot, w2.at[pl.ds(0, W2S)], ssem.at[1])

    def wait_all(cs):
        for c in cs:
            c.wait()

    for c in c_wq[:1] + [to_stage(0), c_x] + c_wo + c_wq[1:]:
        c.start()

    def start_ffn_weights():
        for c in [c_w1, c_w3] + c_w2:
            c.start()

    kvu = kvb.bitcast(U32)
    wqu = wq.bitcast(U32)
    wau = wa.bitcast(U32)
    wou = wo.bitcast(U32)
    w1u, w3u, w2u = w1.bitcast(U32), w3.bitcast(U32), w2.bitcast(U32)
    y_u, pat_u, olhs_u = y_scr.bitcast(U32), pat_scr.bitcast(U32), olhs.bitcast(U32)
    plhs_u = plhs.bitcast(U32)

    def f32_rows(u):
        return pltpu.bitcast(u, BF).astype(F32)

    lane = lax.broadcasted_iota(jnp.int32, (8, 128), 1)
    row = lax.broadcasted_iota(jnp.int32, (8, 128), 0)
    diag_i = ((lane & 7) == row).astype(jnp.int32) * 64
    bit_i = [(lane << (3 - k)) & 64 for k in range(4)]
    uid = [0]

    def lane_sum(v):
        return jnp.broadcast_to(jnp.sum(v, axis=1, keepdims=True), (8, 128))

    def columns(v8):
        uid[0] += 1
        off = 256 * uid[0]
        dl = lane - row + off
        return [lane_sum(jnp.where(dl == off + 8 * b, v8[:, 128 * k:128 * k + 128], 0.0))
                for k in range(v8.shape[1] // 128) for b in range(16)]

    def moments(x):
        mu = jnp.mean(x, axis=-1, keepdims=True)
        xc = x - mu
        return mu, xc, 1.0 / jnp.sqrt(jnp.mean(xc * xc, axis=-1, keepdims=True) + EPS)

    def residual(x, a):
        return (x + a.astype(BF).astype(F32)).astype(BF).astype(F32)

    def tile_dot(l_u32, w_u32, rows, paced):
        w = pltpu.bitcast(w_u32.reshape(64, 128), BF)
        if paced:
            l = pltpu.bitcast(jnp.concatenate([l_u32, l_u32], axis=0), BF)[:24]
            return jnp.dot(l, w, preferred_element_type=F32)[:rows]
        l = pltpu.bitcast(l_u32, BF)[:rows]
        return jnp.dot(l, w, preferred_element_type=F32)

    def swap_halves(a, b):
        return (jnp.concatenate([a[..., :4, :], b[..., :4, :]], axis=-2),
                jnp.concatenate([a[..., 4:, :], b[..., 4:, :]], axis=-2))

    def pair_wq():
        def body(i, carry):
            for f in range(8):
                part[12 * f:12 * f + 12] = pltpu.bitcast(wqu[i, f].reshape(12, 8, 128), F32)
            for q in range(NP // 2):
                for r in range(2):
                    a, b = [pltpu.bitcast(part[48 * r + 24 * t + 3 * q:48 * r + 24 * t + 3 * q + 3], U32)
                            for t in range(2)]
                    wqu[i, q, r, 0:3], wqu[i, q, r, 3:6] = swap_halves(a, b)
            return carry
        lax.fori_loop(0, D // 32, body, 0)

    def regroup5(v):
        h = [v[:, f // 2, 4 * (f % 2):4 * (f % 2) + 4, :] for f in range(2 * KD)]
        return [jnp.concatenate([h[c], h[KD + c]], axis=1) for c in range(KD)]

    def pair_wo(r0, n):
        def body(i, carry):
            r = pl.ds(r0 + 2 * i, 2)
            for c, w in enumerate(regroup5(wou[r])):
                wou[r, c] = w
            return carry
        lax.fori_loop(0, n // 2, body, 0)

    def pair_wa():
        def body(i, carry):
            a, b = i >> 4, i & 15
            for c, w in enumerate(regroup5(wau[a, b])):
                wau[a, b, :, c] = w
            return carry
        lax.fori_loop(0, RH // 2, body, 0)

    def wo_tile(kt, n):
        if 8 * kt >= RH:
            return wou[8 * kt - RH:8 * kt - RH + 8, n]
        return wau[kt >> 2, 4 * (kt & 3):4 * (kt & 3) + 4, :, n]

    def wq_tile(m, c, k):
        c6 = 3 * m[1] + c
        return wqu[4 * k:4 * k + 4, m[0] + c6 // 6, :, 3 * (c6 & 1) + ((c6 % 6) >> 1)]

    def qproj_ops(m):
        def op(paced, c, k):
            qpart[c * KD + k] = tile_dot(
                y_u[k], wq_tile(m, c, k), 8, paced)
        return [(lambda p, c=c, k=k: op(p, c, k)) for c in range(3) for k in range(KD)]

    def oproj_ops(kt, slot, dst, d0):
        def op(paced, n):
            dst[d0 + n] = tile_dot(olhs_u[slot], wo_tile(kt, n), 8, paced)
        return [(lambda p, n=n: op(p, n)) for n in range(KD)]

    def pair_rows(m):
        def body(g2, c):
            for par in range(2):
                kvu[m, 0, par, g2, 0], kvu[m, 0, par, g2, 1] = swap_halves(
                    kvu[m, 0, par, g2, 0], kvu[m, 0, par, g2, 1])
            return c
        lax.fori_loop(0, G2, body, 0)

    def k_blocks(m, par, g0, g1, j):
        return kvu[m, 0, par, g0:g1, j & 1, j >> 1]

    jord = [8 * (i // 8) + 2 * (i % 4) + (i % 8) // 4 for i in range(nblk)]

    def qk_ops(m, po=0, pb=0):
        def op_a(paced, j):
            r = tile_dot(pat_u[po + 0], k_blocks(m, 0, 0, 8, j), 8, paced)
            part_a[j // 8, j % 8:j % 8 + 1, :] = r[j % 8:j % 8 + 1, :]

        def op_c(paced, j):
            r = tile_dot(pat_u[po + 2], k_blocks(m, 1, 4, 12, j), 8, paced)
            part[pb + 2 * nq + j // 8, j % 8:j % 8 + 1, :] = r[j % 8:j % 8 + 1, :]

        def op_b(paced, j):
            w = jnp.concatenate([k_blocks(m, 0, 8, 12, j), k_blocks(m, 1, 0, 4, j)], axis=0)
            r = tile_dot(pat_u[po + 1], w, 16, paced)
            part[pb + nq + j // 8, j % 8:j % 8 + 1, :] = r[j % 8:j % 8 + 1, :]
            part[pb + 3 * nq + j // 8, j % 8:j % 8 + 1, :] = r[8 + j % 8:8 + j % 8 + 1, :]

        return [[(lambda p, f=f, j=j: f(p, j)) for j in jord] for f in (op_a, op_b, op_c)]

    def plain(ops):
        for op in ops:
            op(False)

    steps = [(par, gb, j0) for par in range(2) for gb in range(G // NA)
             for j0 in range(0, nblk, 4) if j0 != 4 or gb == 2 - 2 * par]

    def flip(m):
        for par in range(2):
            for a in range(2):
                v = f32_rows(kvu[m, 1, par, 4 * par:4 * par + 8, :, 2 + a])
                ts = [v[:, :, 8 * b:8 * b + 8, :].reshape(128, 128).T.astype(BF) for b in range(2)]
                for b in range(2):
                    kvu[m, 1, par, 4 * par:4 * par + 8, b, 2 + a] = (
                        pltpu.bitcast(ts[b], U32).reshape(8, 8, 128))

    def pvm_ops(m, sl):
        def op(paced, par, j):
            r = tile_dot(plhs_u[2 * sl + par],
                         kvu[m, 1, par, 4 * par:4 * par + 8, j & 1, j >> 1], 8, paced)
            vres[2 * sl + par, j:j + 1, :] = r[j:j + 1, :]
        return [(lambda p, par=par, j=j: op(p, par, j))
                for j in range(4, 8) for par in range(2)]

    def units(par, gb, j0):
        return [(par, g, j0) for g in range(gb * NA, (gb + 1) * NA)]

    order = [u for s in steps for u in units(*s)]
    wide = {}
    for i, u in enumerate(order):
        if (i + 1) * NW // len(order) > i * NW // len(order):
            wide[u] = len(wide)

    def widen(m):
        for (par, g, j), e in wide.items():
            v = f32_rows(kvu[m, 1, par, g // 2, g % 2, j // 2:j // 2 + 2])
            kvu[m, 1, par, g // 2, g % 2, j // 2:j // 2 + 2] = pltpu.bitcast(v[:, :8], U32)
            vx[m, e] = v[:, 8:]

    def v_unit(m, par, g, j):
        u = kvu[m, 1, par, g // 2, g % 2, j // 2:j // 2 + 2]
        if (par, g, j) in wide:
            return jnp.concatenate([pltpu.bitcast(u, F32), vx[m, wide[(par, g, j)]]], axis=1)
        return f32_rows(u)

    def pv_ops(m, ph):
        acc = {}

        def spread(par, q, r):
            pb_scr[pl.ds(64 * q + r, 8, stride=8), :] = p_scr[ph, par, 8 * q:8 * q + 8, :]

        def psum(par):
            p = p_scr[ph, par]
            accx[ph, 8 * (2 * G + par):8 * (2 * G + par) + 8, :] = (
                (p[0:8] + p[8:16]) + (p[16:24] + p[24:32]))

        pbv = {}

        def piece(par, gb, j0, k):
            if k == 0:
                if par == 0 and j0 < 8:
                    pb = pb0[ph, 8 * j0:8 * j0 + 32, :]
                else:
                    pb = pb_scr[8 * j0:8 * j0 + 32, :]
                pbv[0] = pb.reshape(4, 8, 128)
            for _, g, _ in units(par, gb, j0)[4 * k:4 * k + 4]:
                tv = v_unit(m, par, g, j0).reshape(4, 8, 128) * pbv[0]
                tv = jnp.sum(tv, axis=0)
                acc[g] = tv if j0 == 0 else acc[g] + tv
                if j0 == nblk - 4:
                    r0 = DH * par + 8 * g
                    accx[ph, r0:r0 + 8, :] = acc[g]

        pieces = [s + (k,) for s in steps for k in range(NA // 4)]
        use = {}
        for i, (par, _, j0, k) in enumerate(pieces):
            if k == 0:
                use.setdefault((par, j0 // 8), []).append(i)
        side = {}
        for q in range(nq):
            for r in range(8):
                if q:
                    lo, hi = (use[0, q - 1][0] - 1 if q > 1 else 0), use[0, q][0] - 1
                    side.setdefault(lo + (r * (hi - lo + 1)) // 8, []).append(
                        lambda q=q, r=r: spread(0, q, r))
                lo, hi = use[0, q][-1] + 1, use[1, q][0] - 1
                side.setdefault(lo + (r * (hi - lo)) // 8, []).append(
                    lambda q=q, r=r: spread(1, q, r))
        for par in range(2):
            side.setdefault(len(pieces) // 4 + par, []).append(lambda par=par: psum(par))
        out = []
        for i, s in enumerate(pieces):
            out += [(0, f) for f in side.get(i, [])]
            out.append((2 * sum(4 if u in wide else 6 for u in units(*s[:3])[4 * s[3]:4 * s[3] + 4]),
                        (lambda s=s: piece(*s))))
        return out

    toks = []

    def fence(dst, slot, zero_i):
        for i, t in enumerate(toks):
            dst[slot + i + zero_i] = t
        toks.clear()

    def g_softmax(ph, par, pb=0, pa=0):
        s0 = part[pb + 2 * nq:pb + 3 * nq] if par else part_a[pa:pa + nq]
        s = (s0 + part[pb + (2 * par + 1) * nq:pb + (2 * par + 2) * nq]).reshape(nblk, 128)
        mx = jnp.max(jnp.max(s, axis=0, keepdims=True), axis=1, keepdims=True)
        p = jnp.exp2((s - mx) * jnp.concatenate([rs_scr[0]] * nq, axis=0))
        p_scr[ph, par] = p
        plhs[2 * ph + par, 0:8, :] = p[0:8].astype(BF)
        if par == 0:
            for r in range(8):
                pb0[ph, pl.ds(r, 8, stride=8), :] = p[0:8]
        toks.append(pltpu.bitcast(p[nblk - 8:nblk], U32))

    def recip(d):
        r = pl.reciprocal(d, approx=True)
        return r * (2.0 - d * r)

    def g_olhs(slot0, ph, tok=False):
        zz = [lane_sum(accx[ph, 8 * g:8 * g + 8, :]) for g in range(NZ)]
        inv = [jnp.broadcast_to(recip(jnp.sum(zz[2 * G + par], axis=0, keepdims=True)), (8, 128))
               for par in range(2)]
        uid[0] += 1
        bit = [b > uid[0] for b in bit_i]
        for c in range(3):
            xs = zz[16 * c:16 * c + 16]
            for k in range(4):
                xs = [jnp.where(bit[k], xs[i + 1], xs[i]) for i in range(0, len(xs), 2)]
            iv = inv[0] if c == 0 else (inv[1] if c == 2 else jnp.where(bit[3], inv[1], inv[0]))
            z = jnp.where(diag_i > uid[0], xs[0], 0.0)
            if c != 1:
                z = z + vres[2 * ph + c // 2]
            z = z * iv
            olhs[slot0 + c, 0:8, :] = z.astype(BF)
            if tok:
                toks.append(pltpu.bitcast(z, U32))

    def set_pat(c, q, po=0):
        if c == 1:
            hi = bit_i[3] > uid[0]
            pat_scr[po + c, 0:8, :] = jnp.where(hi, 0.0, q).astype(BF)
            pat_scr[po + c, 8:16, :] = jnp.where(hi, q, 0.0).astype(BF)
        else:
            pat_scr[po + c, 0:8, :] = q.astype(BF)
        if c > 0:
            toks.append(pltpu.bitcast(q, U32))

    def g_query(c):
        xs = [qpart[c * KD + k] for k in range(KD)]
        set_pat(c, ((xs[0] + xs[1]) + (xs[2] + xs[3])) + xs[4])

    def clear_acc():
        accx[2:4] = jnp.ones((2, 8 * NR, 128), F32)

    def emit(pv, seq, pace, pk=PM):
        rate, lead, tail = pace
        ntile = sum(not isinstance(e, tuple) for e in seq)
        total = sum(w for w, _ in pv) / 4
        k = done = n = 0
        for e in seq:
            if isinstance(e, tuple):
                e[0]()
                continue
            r = n // 4
            pos = lead + rate * r if r < (ntile - 1) // 4 else total - tail
            while k < len(pv) and done + pv[k][0] / 2 <= 4 * pos:
                done += pv[k][0]
                pv[k][1]()
                k += 1
            e(n < ntile - UNPACED and r % PM < pk)
            n += 1
        for _, g in pv[k:]:
            g()

    def ffn1(x):
        _, xc, rs = moments(x)
        y = jnp.broadcast_to(xc, (8, D)).astype(BF)

        def up(wu):
            cols = []
            for cp in range(NC // 2):
                ev, od = swap_halves(wu[:, 0, cp], wu[:, 1, cp])
                wu[:, 0, cp], wu[:, 1, cp] = ev, od
                cols += [jnp.dot(y, pltpu.bitcast(w.reshape(D // 2, 128), BF),
                                 preferred_element_type=F32) for w in (ev, od)]
            return jnp.concatenate(cols, axis=1) * rs

        def w2_rows(r0, n):
            nat = regroup5(w2u[r0:r0 + n])
            for c in range(KD):
                w2u[r0:r0 + n, c] = nat[c]
            return nat

        def down(o, n):
            cols = [None] * KD
            for k in range(o // 128, (o + n) // 128):
                for c, w in enumerate(w2_rows(8 * k, 8)):
                    t = jnp.dot(hh[:, 128 * k:128 * k + 128], pltpu.bitcast(w.reshape(64, 128), BF),
                                preferred_element_type=F32)[0:1]
                    cols[c] = t if cols[c] is None else cols[c] + t
            return jnp.concatenate(cols, axis=1)

        c_w1.wait()
        g = up(w1u)
        c_w3.wait()
        u = up(w3u)
        hh = (g * jax.nn.sigmoid(g) * u).astype(BF)
        hb = columns(hh[:, w2_off[-1]:].astype(F32))
        a = None
        parts = list(zip(c_w2, w2_off, W2_CHUNKS))[:-1]
        parts.insert(1, (w2_out, 0, 16 * W2S))
        for c, o, n in parts:
            c.wait()
            a = down(o, n) if a is None else a + down(o, n)
        c_w2[-1].wait()
        acc = [None] * KD
        for r in range(W2_CHUNKS[-1] // 16):
            v = f32_rows(w2u[w2_off[-1] // 16 + r])
            for f in range(2 * KD):
                tv = v[f // 2, 8 * (f % 2):8 * (f % 2) + 8] * hb[2 * r + f // KD]
                acc[f % KD] = tv if acc[f % KD] is None else acc[f % KD] + tv
        a = a + jnp.concatenate([jnp.sum(t, axis=0, keepdims=True) for t in acc], axis=1)
        return residual(x, a)

    def ffn2(x):
        mu, _, rs = moments(x)
        x8 = jnp.broadcast_to(x, (8, D))
        rowk = lax.broadcasted_iota(jnp.int32, (8, 128 * KM), 0)
        y = jnp.where(rowk == 0, x8[:, :128 * KM], jnp.where(rowk == 1, 1.0, 0.0)).astype(BF)
        coef = jnp.where(row == 0, 1.0, -mu)
        yb = jnp.concatenate([c - mu for c in columns(x8[:, 128 * KM:])], axis=0)
        mx = {}
        out = [None] * KD
        for c in range(NC):
            while len(mx) < min(NC, FPRE + c * FSTEP / 4):
                cc = len(mx)
                mx[cc] = [jnp.dot(y, pltpu.bitcast(wu[0:8 * KM, cc & 1, cc >> 1].reshape(64 * KM, 128), BF),
                                  preferred_element_type=F32) * coef for wu in (w1u, w3u)]
            gu = []
            for i, wu in enumerate((w1u, w3u)):
                acc = None
                for r in range(8 * (KD - KM)):
                    tv = f32_rows(wu[8 * KM + r, c & 1, c >> 1]) * yb[16 * r:16 * r + 16]
                    acc = tv if r == 0 else acc + tv
                gu.append(jnp.sum((acc[:8] + acc[8:]) + mx[c][i], axis=0, keepdims=True) * rs)
            hg = 0.5 * gu[0]
            h = jnp.broadcast_to((hg * jnp.tanh(hg) + hg) * gu[1], (8, 128)).astype(BF)
            if c == NC - 1:
                ws = regroup5(w2u[8 * c:8 * c + 8])
            else:
                ws = [w2u[8 * c:8 * c + 8, n] for n in range(KD)]
            for n in range(KD):
                t = jnp.dot(h, pltpu.bitcast(ws[n].reshape(64, 128), BF),
                            preferred_element_type=F32)[0:1]
                out[n] = t if c == 0 else out[n] + t
        a = jnp.concatenate(out, axis=1)
        o_ref[...] = (x + a.astype(BF).astype(F32)).astype(BF)
        return x

    def arrive(p, last):
        def when(cond, f):
            if isinstance(cond, bool):
                if cond:
                    f()
            else:
                pl.when(cond)(f)

        cs = kv_copies(p)
        wait_all(cs[:4])
        if not last:
            stage_step(p + 3)
        wait_all(cs[4:TRG])
        if last:
            start_ffn_weights()
        wait_all(cs[TRG:])
        when(p + KVW < NP, lambda: kv_start(p + KVW))
        pair_rows(p)
        widen(p)
        flip(p)
        if last:
            stage_step(NST + 1)

    def arrivals(p0, n):
        def body(i, carry):
            arrive(p0 + i, False)
            return carry
        lax.fori_loop(0, n, body, 0)

    def layer(li, x):
        first = li == 0
        zero_i = li >> 4

        def barrier():
            @pl.when(li > 2)
            def _():
                clear_acc()

        mu, xc, rs = moments(x)
        y = jnp.broadcast_to(xc, (8, D))
        for k in range(KD):
            y_scr[k, 0:8, :] = y[:, 128 * k:128 * k + 128].astype(BF)
        rs_scr[0] = jnp.broadcast_to(rs * c2, (8, 128))
        rowd = lax.broadcasted_iota(jnp.int32, (8, D), 0)
        xo = jnp.where(rowd < 4, jnp.broadcast_to(x, (8, D)), 1.0).astype(BF)
        coef = jnp.where(row < 4, 1.0, -mu)

        def q_direct(col):
            t = jnp.dot(xo, pltpu.bitcast(wqu[:, 0, :, 3 * (col & 1) + (col >> 1)].reshape(D // 2, 128), BF), preferred_element_type=F32) * coef
            return (t + pltpu.roll(t, 4, 0)).astype(BF).astype(F32)

        def q_cols(q, slot):
            for b, col in enumerate(columns(q)):
                part[slot + b] = col

        def vpu_a(m, slot, js, pa):
            z = zero_i if m == 0 else 0
            acc = {}
            for g2 in range(8):
                qc = jnp.concatenate([part[slot + 2 * g2 + t + z] for t in range(2)], axis=0)
                for j in js:
                    tv = f32_rows(kvu[m, 0, 0, g2, j & 1, j >> 1]) * qc
                    acc[j] = tv if g2 == 0 else acc[j] + tv
            rs_ = [jnp.sum(acc[j], axis=0, keepdims=True) for j in js]
            for j, r in zip(js, rs_):
                part_a[pa + j // 8, j % 8:j % 8 + 1, :] = r
            return [pltpu.bitcast(jnp.broadcast_to(r, (8, 128)), U32) for r in rs_]

        def q_sum(c):
            xs = [qpart[c * KD + k] for k in range(KD)]
            return (((xs[0] + xs[1]) + (xs[2] + xs[3])) + xs[4]).astype(BF).astype(F32)

        q0 = [q_direct(c) for c in range(4)]
        q_cols(q0[0], SP)
        set_pat(1, q0[1], 10)
        set_pat(2, q0[2], 10)
        P0 = SP + 48

        def mark(ops, src):
            def wrap(op, v):
                def f(p):
                    op(p)
                    part[0] = v()
                return f
            return [wrap(op, v) for op, v in zip(ops, src)]

        def qp(m, lo, hi):
            return mark(qproj_ops((0, m))[lo:hi], [(lambda i=i: qpart[i]) for i in range(lo, hi)])

        st = {}

        def queries():
            g_query(1)
            g_query(2)
            st["q"] = q_sum(0)
            set_pat(0, st["q"])

        _, b0, c0 = qk_ops(0, 10, P0)
        _, b1, c1 = qk_ops(1)
        a2 = qk_ops(2)[0][PVB:]
        bc = b0 + c0

        def sprinkle(few, many):
            out = []
            for i, e in enumerate(many):
                out.append(e)
                if i % 3 == 2 and i // 3 < len(few):
                    out.append(few[i // 3])
            return out + few[len(many) // 3:]

        q2 = qproj_ops((0, 2))[KD:]
        mx = (bc[:PQ1] + qp(1, KD, 3 * KD) + qp(2, 0, KD) + [(queries,)] + bc[PQ1:]
              + [(lambda: g_softmax(0, 1, P0),)]
              + sprinkle(q2, b1) + c1 + [(lambda: g_softmax(1, 1),)]
              + [(lambda: g_query(1),), (lambda: g_query(2),)] + a2)
        vg = ([(0, SP, jord[i:i + 2], 2 * nq) for i in range(0, nblk, 2)]
              + [(1, SP + 16, jord[i:i + 2], nq) for i in range(0, nblk, 2)]
              + [(2, SP + 32, jord[i:i + 2], 0) for i in range(0, PVB, 2)])
        n = g = 0
        done = set()

        def ripe():
            if "s0" not in done and g >= nblk // 2 and n >= nblk + 3 * KD:
                done.add("s0")
                g_softmax(0, 0, P0, 2 * nq)
            if "s1" not in done and g >= nblk and n >= 3 * nblk + 5 * KD:
                done.add("s1")
                g_softmax(1, 0, 0, nq)

        for e in mx + [None]:
            while g < len(vg) and (e is None or (4 * g if g < 16 else PLG + PFS * (g - 16)) <= n):
                if g == PQH:
                    q_cols(q0[3], SP + 16)
                if g == PQ2:
                    q_cols(st["q"], SP + 32)
                toks[:] = vpu_a(*vg[g])
                if g >= 16 and e is not None:
                    fence(pat_u, 3, zero_i)
                g += 1
                ripe()
            if isinstance(e, tuple):
                e[0]()
            elif e is not None:
                e(False)
                n += 1
                ripe()
        toks.clear()

        def half(b, ph, e):
            n = 2 * b + 2 + e
            qp = qproj_ops((b, 3 + e))
            _, qb, qc = qk_ops(n)
            qa = qk_ops(n + 1)[0]
            so = 2 * (1 - ph) + e
            return ([(lambda: g_olhs(3 * (n - 2), so, True),)]
                    + qc[:CF] + qp[:KD] + [(lambda: g_query(0),)] + qc[CF:] + qb[:OF]
                    + [(lambda: fence(pat_u, 3, zero_i),)] + qb[OF:]
                    + [(lambda: g_softmax(so, 0),), (lambda: g_softmax(so, 1),)]
                    + qp[KD:] + [(lambda: g_query(1),), (lambda: g_query(2),)]
                    + pvm_ops(2 * b + e, 2 * ph + e)
                    + qa[:nblk - AEND] + [(lambda: fence(pat_u, 3, zero_i),)] + qa[nblk - AEND:])

        def body(t, carry):
            for ph in range(2):
                b = 2 * t + ph

                @pl.when(first)
                def _():
                    arrivals(2 * b + 3, 2)

                emit(pv_ops(2 * b, 2 * ph) + pv_ops(2 * b + 1, 2 * ph + 1),
                     half(b, ph, 0) + half(b, ph, 1), PACE_LOOP, PK)
            return carry

        lax.fori_loop(0, 3, body, 0)

        def big(kts):
            return [op for kt in kts for op in oproj_ops(kt, kt + 6, part, SP + KD * kt)]

        pl.when(first)(lambda: arrive(NP - 1, True))
        _, qb, qc = qk_ops(NP - 1)
        seq = (half(6, 0, 0) + [(lambda: g_olhs(3 * 13, 3, True),)] + qc + qb[:OF]
               + [(lambda: fence(pat_u, 3, zero_i),)] + qb[OF:]
               + [(lambda: g_softmax(3, 0),), (lambda: g_softmax(3, 1),)]
               + pvm_ops(13, 1) + big(range(KT13 - 1))
               + [(lambda: fence(olhs_u, 3 * NP + 4, zero_i),)] + big([KT13 - 1]))
        emit(pv_ops(12, 0) + pv_ops(13, 1), seq, PACE_QUAD)
        barrier()
        old = list(range(KT13, 36))
        k14 = old[:KT14 - 7] + list(range(36, 42)) + old[KT14 - 7:KT14 - 6]
        emit(pv_ops(14, 2), [(lambda: g_olhs(3 * 14, 0),), (lambda: g_olhs(3 * 15, 1),)]
             + pvm_ops(14, 2) + big(k14), PACE_PAIR)
        barrier()
        k15 = old[KT14 - 6:-1] + list(range(42, 45)) + old[-1:]
        emit(pv_ops(15, 3), [(lambda: g_olhs(3 * 16, 2),)] + pvm_ops(15, 3) + big(k15), PACE_PAIR)

        def epilogue(x):
            def lsum(g):
                return lane_sum(accx[3, 8 * g:8 * g + 8, :])

            den = [jnp.sum(lsum(2 * G + par), axis=0, keepdims=True) for par in range(2)]
            fac = [den[0], den[1] * recip(den[0]), recip(den[1])]
            acc = []
            for n in range(KD):
                t = part[SP + n]
                for i in range(1, 3 * NP - 3):
                    t = t + part[SP + KD * i + n]
                acc.append(t * fac[0])
            for par in range(2):
                for g2 in range(G2):
                    g = G * par + 2 * g2
                    z0, z1 = lsum(g), lsum(g + 1)
                    for n in range(KD):
                        v = f32_rows(wou[RH - G + G2 * par + g2, n])
                        acc[n] = acc[n] + (v[:8] * z0 + v[8:] * z1)
                l = vres[6 + par].astype(BF)
                acc = [acc[n] + jnp.dot(
                    l, pltpu.bitcast(wo_tile(3 * NP - 3 + 2 * par, n).reshape(64, 128), BF),
                    preferred_element_type=F32) * 1.0 for n in range(KD)]
                acc = [t * fac[par + 1] for t in acc]
            cols = [jnp.sum(t, axis=0, keepdims=True) for t in acc]
            return residual(x, jnp.concatenate(cols, axis=1))

        return lax.cond(first, lambda x: ffn1(epilogue(x)), lambda x: ffn2(epilogue(x)), x)

    for r in (y_u, pat_u, olhs_u, plhs_u):
        r[...] = jnp.zeros(r.shape, U32)
    vres[...] = jnp.zeros(vres.shape, F32)
    clear_acc()
    stage_step(1)
    stage_step(2)
    kv_start(0)
    c_x.wait()
    kv_start(1)
    wait_all(c_wq)
    pair_wq()
    arrivals(0, 3)
    wait_all(c_wo)
    pair_wa()
    pair_wo(0, R0)
    lax.fori_loop(0, 2, layer, xb[...].astype(F32))


@jax.jit
def pallas_interleave_layers__sliding_block_cached__glu_gated_swiglu__decode_kernel(
    A_x: jax.Array,
    A_k_cache: jax.Array,
    A_v_cache: jax.Array,
    A_wq: jax.Array,
    A_wo: jax.Array,
    B_x: jax.Array,
    B_w1: jax.Array,
    B_w3: jax.Array,
    B_w2: jax.Array,
):
    del B_x
    sk = A_k_cache.shape[2]
    win = min(4096, max(256, sk // 4))
    nb = sk // 128
    nblk = win // 128

    def cache_tiles(c):
        return (c.reshape(H, nb, 128, G2, 2, 8).transpose(0, 3, 4, 1, 5, 2)
                .reshape(H, G2, 2, nb // 2, 16, 128))

    def weight_tiles(w):
        r, c = w.shape
        return w.reshape(r // 16, 2, 8, c // 128, 128).transpose(0, 1, 3, 2, 4)

    vreg = lambda n: pltpu.VMEM((-(-n // 4) * 4, 8, 128), F32)
    lhs = lambda n: pltpu.VMEM((-(-n // 4) * 4, 16, 128), BF)
    kern = lambda *refs: _kernel(*refs, blk0=nb - nblk, nblk=nblk, scale=DH ** -0.5)
    out = pl.pallas_call(
        kern,
        out_shape=jax.ShapeDtypeStruct((1, D), BF),
        in_specs=[pl.BlockSpec(memory_space=pl.ANY)] * 9,
        out_specs=pl.BlockSpec(memory_space=pltpu.VMEM),
        scratch_shapes=[
            pltpu.VMEM((1, D), BF),
            pltpu.VMEM((NP, 2, 2, G2, 2, nblk // 2, 16, 128), BF),
            pltpu.VMEM((D // 32, NP // 2, 2, 6, 16, 128), BF),
            pltpu.VMEM((6, 16, 2, KD, 16, 128), BF),
            pltpu.VMEM((H * G2 // 2, KD, 16, 128), BF),
            pltpu.VMEM((D // 16, 2, NC // 2, 16, 128), BF),
            pltpu.VMEM((D // 16, 2, NC // 2, 16, 128), BF),
            pltpu.VMEM((FF // 16, KD, 16, 128), BF),
            lhs(KD),
            vreg(1),
            vreg(3 * KD),
            lhs(16),
            vreg(3 * nblk // 8),
            vreg(nblk // 2 + (3 * NP - 3) * KD),
            pltpu.VMEM((4, 2, nblk, 128), F32),
            pltpu.VMEM((nblk * 8, 128), F32),
            pltpu.VMEM((4, 64, 128), F32),
            pltpu.VMEM((4, 8 * NR, 128), F32),
            lhs(3 * NP + 12),
            lhs(8),
            vreg(8),
            pltpu.VMEM((NP, NW, 2, 8, 128), F32),
            pltpu.SMEM((2, SC, KD, 16, 128), BF),
            pltpu.SemaphoreType.DMA((NP,)),
            pltpu.SemaphoreType.DMA((5 + len(W2_CHUNKS),)),
            pltpu.SemaphoreType.DMA((2,)),
        ],
        compiler_params=pltpu.CompilerParams(
            vmem_limit_bytes=128 * 1024 * 1024, disable_semaphore_checks=True,
            disable_bounds_checks=True),
    )(A_x.reshape(1, D), cache_tiles(A_k_cache), cache_tiles(A_v_cache),
      weight_tiles(A_wq).reshape(D // 32, NP // 2, 2, 6, 16, 128),
      weight_tiles(A_wo).reshape(12, 16, 2, KD, 16, 128),
      weight_tiles(A_wo).reshape(H * G2, KD, 16, 128),
      weight_tiles(B_w1).reshape(D // 16, 2, NC // 2, 16, 128),
      weight_tiles(B_w3).reshape(D // 16, 2, NC // 2, 16, 128),
      weight_tiles(B_w2).reshape(FF // 16, KD, 16, 128))
    return out.reshape(1, 1, D)
```

```python
import math

import jax
import jax.numpy as jnp
from jax import lax
import jax.experimental.pallas as pl
import jax.experimental.pallas.tpu as pltpu

BF = jnp.bfloat16
F32 = jnp.float32
U32 = jnp.uint32

D = 640
H = 32
DH = 192
G = DH // 8
G2 = DH // 16
NP = H // 2
FF = 1536
EPS = 1e-5
KD = D // 128
NC = FF // 128
NZ = 2 * G + 2
NR = NZ + 2
W2S = 8
W2_CHUNKS = (768 - 16 * W2S, 384, 256, 128)
NST = NP + 1
SC = 10
KVW = 2
TRG = 6

NA = 8
NW = 64
PACE_LOOP = (30.7, 36, 30)
PACE_QUAD = (33, 8, 30)
PACE_PAIR = (32.5, 16, 30)
UNPACED = 8
PM = 6
PK = 4
AEND = 4
OF = 19
CF = 8
KT13 = 6
KT14 = 20
PVB = 14
PQ1 = 8
PQH = 4
PQ2 = 16
PLG = 86
PFS = 3.75
KM = 3
FPRE = 7
FSTEP = 4
FX = 2
FLATE = (8, 10)


def _kernel(x_hbm, k_hbm, v_hbm, wq_hbm, wa_hbm, wo_hbm, w1_hbm, w3_hbm, w2_hbm,
            o_ref,
            xb, kvb, wq, wa, wo, w1, w3, w2,
            y_scr, rs_scr, qpart, pat_scr, part_a, part, p_scr, pb_scr, pb0,
            accx, olhs, plhs, vres, vx, stage,
            kvsem, wsem, ssem, *, blk0, nblk, scale):
    c2 = scale * math.log2(math.e)
    nq = nblk // 8
    SP = 4 * nq

    def kv_copies(m):
        n = nblk // 4
        return [pltpu.make_async_copy(
            src.at[pl.ds(2 * m, 2), :, t, pl.ds(blk0 // 2 + n * h, n)],
            kvb.at[m, i, :, :, t, pl.ds(n * h, n)], kvsem.at[m])
            for i, src in enumerate((k_hbm, v_hbm)) for t in range(2) for h in range(2)]

    def kv_start(m):
        for c in kv_copies(m):
            c.start()

    c_x = pltpu.make_async_copy(x_hbm, xb, wsem.at[0])
    c_wq = [pltpu.make_async_copy(wq_hbm.at[:, b], wq.at[:, b], wsem.at[1])
            for b in range(NP // 2)]
    RH = H * G2 // 2
    R0 = RH - NST * SC
    c_wo = [pltpu.make_async_copy(wa_hbm.at[pl.ds(0, 6), b], wa.at[:, b], wsem.at[2])
            for b in range(16)]
    c_wo.append(pltpu.make_async_copy(wo_hbm.at[pl.ds(RH, R0)], wo.at[pl.ds(0, R0)], wsem.at[2]))

    def to_stage(k):
        return pltpu.make_async_copy(wo_hbm.at[pl.ds(RH + R0 + SC * k, SC)], stage.at[k & 1],
                                     ssem.at[0])

    def from_stage(k):
        return pltpu.make_async_copy(stage.at[k & 1], wo.at[pl.ds(R0 + SC * k, SC)], ssem.at[1])

    def stage_step(k):
        def when(cond, f):
            if isinstance(cond, bool):
                if cond:
                    f()
            else:
                pl.when(cond)(f)

        def forward():
            to_stage(k - 1).wait()
            from_stage(k - 1).start()

        landed = not isinstance(k, int) or k >= 2
        if landed:
            from_stage(k - 2).wait()
        when(k <= NST, forward)
        when(k < NST, lambda: to_stage(k).start())
        when(k == NST, w2_in.start)
        if isinstance(k, int) and k == NST + 1:
            w2_in.wait()
            w2_out.start()
        if landed:
            pair_wo(R0 + SC * (k - 2), SC)

    c_w1 = pltpu.make_async_copy(w1_hbm, w1, wsem.at[3])
    c_w3 = pltpu.make_async_copy(w3_hbm, w3, wsem.at[4])
    w2_off = [16 * W2S + sum(W2_CHUNKS[:i]) for i in range(len(W2_CHUNKS))]
    c_w2 = [pltpu.make_async_copy(w2_hbm.at[pl.ds(o // 16, n // 16)],
                                  w2.at[pl.ds(o // 16, n // 16)], wsem.at[5 + i])
            for i, (o, n) in enumerate(zip(w2_off, W2_CHUNKS))]
    w2_slot = stage.at[NST & 1, pl.ds(0, W2S)]
    w2_in = pltpu.make_async_copy(w2_hbm.at[pl.ds(0, W2S)], w2_slot, ssem.at[0])
    w2_out = pltpu.make_async_copy(w2_slot, w2.at[pl.ds(0, W2S)], ssem.at[1])

    def wait_all(cs):
        for c in cs:
            c.wait()

    for c in c_wq[:1] + [to_stage(0), c_x] + c_wo + c_wq[1:]:
        c.start()

    def start_ffn_weights():
        for c in [c_w1, c_w3] + c_w2:
            c.start()

    kvu = kvb.bitcast(U32)
    wqu = wq.bitcast(U32)
    wau = wa.bitcast(U32)
    wou = wo.bitcast(U32)
    w1u, w3u, w2u = w1.bitcast(U32), w3.bitcast(U32), w2.bitcast(U32)
    y_u, pat_u, olhs_u = y_scr.bitcast(U32), pat_scr.bitcast(U32), olhs.bitcast(U32)
    plhs_u = plhs.bitcast(U32)

    def f32_rows(u):
        return pltpu.bitcast(u, BF).astype(F32)

    lane = lax.broadcasted_iota(jnp.int32, (8, 128), 1)
    row = lax.broadcasted_iota(jnp.int32, (8, 128), 0)
    diag_i = ((lane & 7) == row).astype(jnp.int32) * 64
    bit_i = [(lane << (3 - k)) & 64 for k in range(4)]
    uid = [0]

    def lane_sum(v):
        return jnp.broadcast_to(jnp.sum(v, axis=1, keepdims=True), (8, 128))

    def columns(v8):
        uid[0] += 1
        off = 256 * uid[0]
        dl = lane - row + off
        return [lane_sum(jnp.where(dl == off + 8 * b, v8[:, 128 * k:128 * k + 128], 0.0))
                for k in range(v8.shape[1] // 128) for b in range(16)]

    def moments(x):
        mu = jnp.mean(x, axis=-1, keepdims=True)
        xc = x - mu
        return mu, xc, 1.0 / jnp.sqrt(jnp.mean(xc * xc, axis=-1, keepdims=True) + EPS)

    def residual(x, a):
        return (x + a.astype(BF).astype(F32)).astype(BF).astype(F32)

    def tile_dot(l_u32, w_u32, rows, paced):
        w = pltpu.bitcast(w_u32.reshape(64, 128), BF)
        if paced:
            l = pltpu.bitcast(jnp.concatenate([l_u32, l_u32], axis=0), BF)[:24]
            return jnp.dot(l, w, preferred_element_type=F32)[:rows]
        l = pltpu.bitcast(l_u32, BF)[:rows]
        return jnp.dot(l, w, preferred_element_type=F32)

    def swap_halves(a, b):
        return (jnp.concatenate([a[..., :4, :], b[..., :4, :]], axis=-2),
                jnp.concatenate([a[..., 4:, :], b[..., 4:, :]], axis=-2))

    def pair_wq():
        def body(i, carry):
            for f in range(8):
                part[12 * f:12 * f + 12] = pltpu.bitcast(wqu[i, f].reshape(12, 8, 128), F32)
            for q in range(NP // 2):
                for r in range(2):
                    a, b = [pltpu.bitcast(part[48 * r + 24 * t + 3 * q:48 * r + 24 * t + 3 * q + 3], U32)
                            for t in range(2)]
                    wqu[i, q, r, 0:3], wqu[i, q, r, 3:6] = swap_halves(a, b)
            return carry
        lax.fori_loop(0, D // 32, body, 0)

    def regroup5(v):
        h = [v[:, f // 2, 4 * (f % 2):4 * (f % 2) + 4, :] for f in range(2 * KD)]
        return [jnp.concatenate([h[c], h[KD + c]], axis=1) for c in range(KD)]

    def pair_wo(r0, n):
        def body(i, carry):
            r = pl.ds(r0 + 2 * i, 2)
            for c, w in enumerate(regroup5(wou[r])):
                wou[r, c] = w
            return carry
        lax.fori_loop(0, n // 2, body, 0)

    def pair_wa():
        def body(i, carry):
            a, b = i >> 4, i & 15
            for c, w in enumerate(regroup5(wau[a, b])):
                wau[a, b, :, c] = w
            return carry
        lax.fori_loop(0, RH // 2, body, 0)

    def wo_tile(kt, n):
        if 8 * kt >= RH:
            return wou[8 * kt - RH:8 * kt - RH + 8, n]
        return wau[kt >> 2, 4 * (kt & 3):4 * (kt & 3) + 4, :, n]

    def wq_tile(m, c, k):
        c6 = 3 * m[1] + c
        return wqu[4 * k:4 * k + 4, m[0] + c6 // 6, :, 3 * (c6 & 1) + ((c6 % 6) >> 1)]

    def qproj_ops(m):
        def op(paced, c, k):
            qpart[c * KD + k] = tile_dot(
                y_u[k], wq_tile(m, c, k), 8, paced)
        return [(lambda p, c=c, k=k: op(p, c, k)) for c in range(3) for k in range(KD)]

    def oproj_ops(kt, slot, dst, d0):
        def op(paced, n):
            dst[d0 + n] = tile_dot(olhs_u[slot], wo_tile(kt, n), 8, paced)
        return [(lambda p, n=n: op(p, n)) for n in range(KD)]

    def pair_rows(m):
        def body(g2, c):
            for par in range(2):
                kvu[m, 0, par, g2, 0], kvu[m, 0, par, g2, 1] = swap_halves(
                    kvu[m, 0, par, g2, 0], kvu[m, 0, par, g2, 1])
            return c
        lax.fori_loop(0, G2, body, 0)

    def k_blocks(m, par, g0, g1, j):
        return kvu[m, 0, par, g0:g1, j & 1, j >> 1]

    jord = [8 * (i // 8) + 2 * (i % 4) + (i % 8) // 4 for i in range(nblk)]

    def qk_ops(m, po=0, pb=0):
        def op_a(paced, j):
            r = tile_dot(pat_u[po + 0], k_blocks(m, 0, 0, 8, j), 8, paced)
            part_a[j // 8, j % 8:j % 8 + 1, :] = r[j % 8:j % 8 + 1, :]

        def op_c(paced, j):
            r = tile_dot(pat_u[po + 2], k_blocks(m, 1, 4, 12, j), 8, paced)
            part[pb + 2 * nq + j // 8, j % 8:j % 8 + 1, :] = r[j % 8:j % 8 + 1, :]

        def op_b(paced, j):
            w = jnp.concatenate([k_blocks(m, 0, 8, 12, j), k_blocks(m, 1, 0, 4, j)], axis=0)
            r = tile_dot(pat_u[po + 1], w, 16, paced)
            part[pb + nq + j // 8, j % 8:j % 8 + 1, :] = r[j % 8:j % 8 + 1, :]
            part[pb + 3 * nq + j // 8, j % 8:j % 8 + 1, :] = r[8 + j % 8:8 + j % 8 + 1, :]

        return [[(lambda p, f=f, j=j: f(p, j)) for j in jord] for f in (op_a, op_b, op_c)]

    def plain(ops):
        for op in ops:
            op(False)

    steps = [(par, gb, j0) for par in range(2) for gb in range(G // NA)
             for j0 in range(0, nblk, 4) if j0 != 4 or gb == 2 - 2 * par]

    def flip(m):
        for par in range(2):
            for a in range(2):
                v = f32_rows(kvu[m, 1, par, 4 * par:4 * par + 8, :, 2 + a])
                ts = [v[:, :, 8 * b:8 * b + 8, :].reshape(128, 128).T.astype(BF) for b in range(2)]
                for b in range(2):
                    kvu[m, 1, par, 4 * par:4 * par + 8, b, 2 + a] = (
                        pltpu.bitcast(ts[b], U32).reshape(8, 8, 128))

    def pvm_ops(m, sl):
        def op(paced, par, j):
            r = tile_dot(plhs_u[2 * sl + par],
                         kvu[m, 1, par, 4 * par:4 * par + 8, j & 1, j >> 1], 8, paced)
            vres[2 * sl + par, j:j + 1, :] = r[j:j + 1, :]
        return [(lambda p, par=par, j=j: op(p, par, j))
                for j in range(4, 8) for par in range(2)]

    def units(par, gb, j0):
        return [(par, g, j0) for g in range(gb * NA, (gb + 1) * NA)]

    order = [u for s in steps for u in units(*s)]
    wide = {}
    for i, u in enumerate(order):
        if (i + 1) * NW // len(order) > i * NW // len(order):
            wide[u] = len(wide)

    def widen(m):
        for (par, g, j), e in wide.items():
            v = f32_rows(kvu[m, 1, par, g // 2, g % 2, j // 2:j // 2 + 2])
            kvu[m, 1, par, g // 2, g % 2, j // 2:j // 2 + 2] = pltpu.bitcast(v[:, :8], U32)
            vx[m, e] = v[:, 8:]

    def v_unit(m, par, g, j):
        u = kvu[m, 1, par, g // 2, g % 2, j // 2:j // 2 + 2]
        if (par, g, j) in wide:
            return jnp.concatenate([pltpu.bitcast(u, F32), vx[m, wide[(par, g, j)]]], axis=1)
        return f32_rows(u)

    def pv_ops(m, ph):
        acc = {}

        def spread(par, q, r):
            pb_scr[pl.ds(64 * q + r, 8, stride=8), :] = p_scr[ph, par, 8 * q:8 * q + 8, :]

        def psum(par):
            p = p_scr[ph, par]
            accx[ph, 8 * (2 * G + par):8 * (2 * G + par) + 8, :] = (
                (p[0:8] + p[8:16]) + (p[16:24] + p[24:32]))

        pbv = {}

        def piece(par, gb, j0, k):
            if k == 0:
                if par == 0 and j0 < 8:
                    pb = pb0[ph, 8 * j0:8 * j0 + 32, :]
                else:
                    pb = pb_scr[8 * j0:8 * j0 + 32, :]
                pbv[0] = pb.reshape(4, 8, 128)
            for _, g, _ in units(par, gb, j0)[4 * k:4 * k + 4]:
                tv = v_unit(m, par, g, j0).reshape(4, 8, 128) * pbv[0]
                tv = jnp.sum(tv, axis=0)
                acc[g] = tv if j0 == 0 else acc[g] + tv
                if j0 == nblk - 4:
                    r0 = DH * par + 8 * g
                    accx[ph, r0:r0 + 8, :] = acc[g]

        pieces = [s + (k,) for s in steps for k in range(NA // 4)]
        use = {}
        for i, (par, _, j0, k) in enumerate(pieces):
            if k == 0:
                use.setdefault((par, j0 // 8), []).append(i)
        side = {}
        for q in range(nq):
            for r in range(8):
                if q:
                    lo, hi = (use[0, q - 1][0] - 1 if q > 1 else 0), use[0, q][0] - 1
                    side.setdefault(lo + (r * (hi - lo + 1)) // 8, []).append(
                        lambda q=q, r=r: spread(0, q, r))
                lo, hi = use[0, q][-1] + 1, use[1, q][0] - 1
                side.setdefault(lo + (r * (hi - lo)) // 8, []).append(
                    lambda q=q, r=r: spread(1, q, r))
        for par in range(2):
            side.setdefault(len(pieces) // 4 + par, []).append(lambda par=par: psum(par))
        out = []
        for i, s in enumerate(pieces):
            out += [(0, f) for f in side.get(i, [])]
            out.append((2 * sum(4 if u in wide else 6 for u in units(*s[:3])[4 * s[3]:4 * s[3] + 4]),
                        (lambda s=s: piece(*s))))
        return out

    toks = []

    def fence(dst, slot, zero_i):
        for i, t in enumerate(toks):
            dst[slot + i + zero_i] = t
        toks.clear()

    def g_softmax(ph, par, pb=0, pa=0):
        s0 = part[pb + 2 * nq:pb + 3 * nq] if par else part_a[pa:pa + nq]
        s = (s0 + part[pb + (2 * par + 1) * nq:pb + (2 * par + 2) * nq]).reshape(nblk, 128)
        mx = jnp.max(jnp.max(s, axis=0, keepdims=True), axis=1, keepdims=True)
        p = jnp.exp2((s - mx) * jnp.concatenate([rs_scr[0]] * nq, axis=0))
        p_scr[ph, par] = p
        plhs[2 * ph + par, 0:8, :] = p[0:8].astype(BF)
        if par == 0:
            for r in range(8):
                pb0[ph, pl.ds(r, 8, stride=8), :] = p[0:8]
        toks.append(pltpu.bitcast(p[nblk - 8:nblk], U32))

    def recip(d):
        r = pl.reciprocal(d, approx=True)
        return r * (2.0 - d * r)

    def g_olhs(slot0, ph, tok=False):
        zz = [lane_sum(accx[ph, 8 * g:8 * g + 8, :]) for g in range(NZ)]
        inv = [jnp.broadcast_to(recip(jnp.sum(zz[2 * G + par], axis=0, keepdims=True)), (8, 128))
               for par in range(2)]
        uid[0] += 1
        bit = [b > uid[0] for b in bit_i]
        for c in range(3):
            xs = zz[16 * c:16 * c + 16]
            for k in range(4):
                xs = [jnp.where(bit[k], xs[i + 1], xs[i]) for i in range(0, len(xs), 2)]
            iv = inv[0] if c == 0 else (inv[1] if c == 2 else jnp.where(bit[3], inv[1], inv[0]))
            z = jnp.where(diag_i > uid[0], xs[0], 0.0)
            if c != 1:
                z = z + vres[2 * ph + c // 2]
            z = z * iv
            olhs[slot0 + c, 0:8, :] = z.astype(BF)
            if tok:
                toks.append(pltpu.bitcast(z, U32))

    def set_pat(c, q, po=0):
        if c == 1:
            hi = bit_i[3] > uid[0]
            pat_scr[po + c, 0:8, :] = jnp.where(hi, 0.0, q).astype(BF)
            pat_scr[po + c, 8:16, :] = jnp.where(hi, q, 0.0).astype(BF)
        else:
            pat_scr[po + c, 0:8, :] = q.astype(BF)
        if c > 0:
            toks.append(pltpu.bitcast(q, U32))

    def g_query(c):
        xs = [qpart[c * KD + k] for k in range(KD)]
        set_pat(c, ((xs[0] + xs[1]) + (xs[2] + xs[3])) + xs[4])

    def clear_acc():
        accx[2:4] = jnp.ones((2, 8 * NR, 128), F32)

    def emit(pv, seq, pace, pk=PM):
        rate, lead, tail = pace
        ntile = sum(not isinstance(e, tuple) for e in seq)
        total = sum(w for w, _ in pv) / 4
        k = done = n = 0
        for e in seq:
            if isinstance(e, tuple):
                e[0]()
                continue
            r = n // 4
            pos = lead + rate * r if r < (ntile - 1) // 4 else total - tail
            while k < len(pv) and done + pv[k][0] / 2 <= 4 * pos:
                done += pv[k][0]
                pv[k][1]()
                k += 1
            e(n < ntile - UNPACED and r % PM < pk)
            n += 1
        for _, g in pv[k:]:
            g()

    def ffn1(x):
        _, xc, rs = moments(x)
        y = jnp.broadcast_to(xc, (8, D)).astype(BF)

        def up(wu):
            cols = []
            for cp in range(NC // 2):
                ev, od = swap_halves(wu[:, 0, cp], wu[:, 1, cp])
                wu[:, 0, cp], wu[:, 1, cp] = ev, od
                cols += [jnp.dot(y, pltpu.bitcast(w.reshape(D // 2, 128), BF),
                                 preferred_element_type=F32) for w in (ev, od)]
            return jnp.concatenate(cols, axis=1) * rs

        def w2_rows(r0, n):
            nat = regroup5(w2u[r0:r0 + n])
            for c in range(KD):
                w2u[r0:r0 + n, c] = nat[c]
            return nat

        def down(o, n):
            cols = [None] * KD
            for k in range(o // 128, (o + n) // 128):
                for c, w in enumerate(w2_rows(8 * k, 8)):
                    t = jnp.dot(hh[:, 128 * k:128 * k + 128], pltpu.bitcast(w.reshape(64, 128), BF),
                                preferred_element_type=F32)[0:1]
                    cols[c] = t if cols[c] is None else cols[c] + t
            return jnp.concatenate(cols, axis=1)

        c_w1.wait()
        g = up(w1u)
        c_w3.wait()
        u = up(w3u)
        hh = (g * jax.nn.sigmoid(g) * u).astype(BF)
        hb = columns(hh[:, w2_off[-1]:].astype(F32))
        a = None
        parts = list(zip(c_w2, w2_off, W2_CHUNKS))[:-1]
        parts.insert(1, (w2_out, 0, 16 * W2S))
        for c, o, n in parts:
            c.wait()
            a = down(o, n) if a is None else a + down(o, n)
        c_w2[-1].wait()
        acc = [None] * KD
        for r in range(W2_CHUNKS[-1] // 16):
            v = f32_rows(w2u[w2_off[-1] // 16 + r])
            for f in range(2 * KD):
                tv = v[f // 2, 8 * (f % 2):8 * (f % 2) + 8] * hb[2 * r + f // KD]
                acc[f % KD] = tv if acc[f % KD] is None else acc[f % KD] + tv
        a = a + jnp.concatenate([jnp.sum(t, axis=0, keepdims=True) for t in acc], axis=1)
        return residual(x, a)

    def ffn2(x):
        mu, _, rs = moments(x)
        x8 = jnp.broadcast_to(x, (8, D))
        rowk = lax.broadcasted_iota(jnp.int32, (8, D), 0)
        y = jnp.where(rowk == 0, x8, jnp.where(rowk == 1, 1.0, 0.0)).astype(BF)
        coef = jnp.where(row == 0, 1.0, -mu)
        yb = jnp.concatenate([c - mu for c in columns(x8[:, 128 * KM:])], axis=0)
        km = [KM + ((c + 1) * FX // NC > c * FX // NC) for c in range(NC)]
        mx = {}
        out = [None] * KD
        late = []
        for c in range(NC):
            while len(mx) < min(NC, FPRE + c * FSTEP / 4):
                cc = len(mx)
                mx[cc] = [jnp.dot(y[:, :128 * km[cc]],
                                  pltpu.bitcast(wu[0:8 * km[cc], cc & 1, cc >> 1].reshape(64 * km[cc], 128), BF),
                                  preferred_element_type=F32) * coef for wu in (w1u, w3u)]
            gu = []
            for i, wu in enumerate((w1u, w3u)):
                acc = None
                for r in range(8 * km[c], 8 * KD):
                    o = 16 * (r - 8 * KM)
                    tv = f32_rows(wu[r, c & 1, c >> 1]) * yb[o:o + 16]
                    acc = tv if acc is None else acc + tv
                gu.append(jnp.sum((acc[:8] + acc[8:]) + mx[c][i], axis=0, keepdims=True) * rs)
            hg = 0.5 * gu[0]
            h = jnp.broadcast_to((hg * jnp.tanh(hg) + hg) * gu[1], (8, 128)).astype(BF)
            if c in FLATE:
                late.append((c, columns(h.astype(F32))))
                continue
            if c == NC - 1:
                ws = regroup5(w2u[8 * c:8 * c + 8])
            else:
                ws = [w2u[8 * c:8 * c + 8, n] for n in range(KD)]
            for n in range(KD):
                t = jnp.dot(h, pltpu.bitcast(ws[n].reshape(64, 128), BF),
                            preferred_element_type=F32)[0:1]
                out[n] = t if out[n] is None else out[n] + t
        if late:
            acc = [None] * KD
            for c, hb in late:
                for r in range(8):
                    for n in range(KD):
                        v = f32_rows(w2u[8 * c + r, n])
                        for t in range(2):
                            tv = v[8 * t:8 * t + 8] * hb[2 * r + t]
                            acc[n] = tv if acc[n] is None else acc[n] + tv
            out = [out[n] + jnp.sum(acc[n], axis=0, keepdims=True) for n in range(KD)]
        a = jnp.concatenate(out, axis=1)
        o_ref[...] = (x + a.astype(BF).astype(F32)).astype(BF)
        return x

    def arrive(p, last):
        def when(cond, f):
            if isinstance(cond, bool):
                if cond:
                    f()
            else:
                pl.when(cond)(f)

        cs = kv_copies(p)
        wait_all(cs[:4])
        if not last:
            stage_step(p + 3)
        wait_all(cs[4:TRG])
        if last:
            start_ffn_weights()
        wait_all(cs[TRG:])
        when(p + KVW < NP, lambda: kv_start(p + KVW))
        pair_rows(p)
        widen(p)
        flip(p)
        if last:
            stage_step(NST + 1)

    def arrivals(p0, n):
        def body(i, carry):
            arrive(p0 + i, False)
            return carry
        lax.fori_loop(0, n, body, 0)

    def layer(li, x):
        first = li == 0
        zero_i = li >> 4

        def barrier():
            @pl.when(li > 2)
            def _():
                clear_acc()

        mu, xc, rs = moments(x)
        y = jnp.broadcast_to(xc, (8, D))
        for k in range(KD):
            y_scr[k, 0:8, :] = y[:, 128 * k:128 * k + 128].astype(BF)
        rs_scr[0] = jnp.broadcast_to(rs * c2, (8, 128))
        rowd = lax.broadcasted_iota(jnp.int32, (8, D), 0)
        xo = jnp.where(rowd < 4, jnp.broadcast_to(x, (8, D)), 1.0).astype(BF)
        coef = jnp.where(row < 4, 1.0, -mu)

        def q_direct(col):
            t = jnp.dot(xo, pltpu.bitcast(wqu[:, 0, :, 3 * (col & 1) + (col >> 1)].reshape(D // 2, 128), BF), preferred_element_type=F32) * coef
            return (t + pltpu.roll(t, 4, 0)).astype(BF).astype(F32)

        def q_cols(q, slot):
            for b, col in enumerate(columns(q)):
                part[slot + b] = col

        def vpu_a(m, slot, js, pa):
            z = zero_i if m == 0 else 0
            acc = {}
            for g2 in range(8):
                qc = jnp.concatenate([part[slot + 2 * g2 + t + z] for t in range(2)], axis=0)
                for j in js:
                    tv = f32_rows(kvu[m, 0, 0, g2, j & 1, j >> 1]) * qc
                    acc[j] = tv if g2 == 0 else acc[j] + tv
            rs_ = [jnp.sum(acc[j], axis=0, keepdims=True) for j in js]
            for j, r in zip(js, rs_):
                part_a[pa + j // 8, j % 8:j % 8 + 1, :] = r
            return [pltpu.bitcast(jnp.broadcast_to(r, (8, 128)), U32) for r in rs_]

        def q_sum(c):
            xs = [qpart[c * KD + k] for k in range(KD)]
            return (((xs[0] + xs[1]) + (xs[2] + xs[3])) + xs[4]).astype(BF).astype(F32)

        q0 = [q_direct(c) for c in range(4)]
        q_cols(q0[0], SP)
        set_pat(1, q0[1], 10)
        set_pat(2, q0[2], 10)
        P0 = SP + 48

        def mark(ops, src):
            def wrap(op, v):
                def f(p):
                    op(p)
                    part[0] = v()
                return f
            return [wrap(op, v) for op, v in zip(ops, src)]

        def qp(m, lo, hi):
            return mark(qproj_ops((0, m))[lo:hi], [(lambda i=i: qpart[i]) for i in range(lo, hi)])

        st = {}

        def queries():
            g_query(1)
            g_query(2)
            st["q"] = q_sum(0)
            set_pat(0, st["q"])

        _, b0, c0 = qk_ops(0, 10, P0)
        _, b1, c1 = qk_ops(1)
        a2 = qk_ops(2)[0][PVB:]
        bc = b0 + c0

        def sprinkle(few, many):
            out = []
            for i, e in enumerate(many):
                out.append(e)
                if i % 3 == 2 and i // 3 < len(few):
                    out.append(few[i // 3])
            return out + few[len(many) // 3:]

        q2 = qproj_ops((0, 2))[KD:]
        mx = (bc[:PQ1] + qp(1, KD, 3 * KD) + qp(2, 0, KD) + [(queries,)] + bc[PQ1:]
              + [(lambda: g_softmax(0, 1, P0),)]
              + sprinkle(q2, b1) + c1 + [(lambda: g_softmax(1, 1),)]
              + [(lambda: g_query(1),), (lambda: g_query(2),)] + a2)
        vg = ([(0, SP, jord[i:i + 2], 2 * nq) for i in range(0, nblk, 2)]
              + [(1, SP + 16, jord[i:i + 2], nq) for i in range(0, nblk, 2)]
              + [(2, SP + 32, jord[i:i + 2], 0) for i in range(0, PVB, 2)])
        n = g = 0
        done = set()

        def ripe():
            if "s0" not in done and g >= nblk // 2 and n >= nblk + 3 * KD:
                done.add("s0")
                g_softmax(0, 0, P0, 2 * nq)
            if "s1" not in done and g >= nblk and n >= 3 * nblk + 5 * KD:
                done.add("s1")
                g_softmax(1, 0, 0, nq)

        for e in mx + [None]:
            while g < len(vg) and (e is None or (4 * g if g < 16 else PLG + PFS * (g - 16)) <= n):
                if g == PQH:
                    q_cols(q0[3], SP + 16)
                if g == PQ2:
                    q_cols(st["q"], SP + 32)
                toks[:] = vpu_a(*vg[g])
                if g >= 16 and e is not None:
                    fence(pat_u, 3, zero_i)
                g += 1
                ripe()
            if isinstance(e, tuple):
                e[0]()
            elif e is not None:
                e(False)
                n += 1
                ripe()
        toks.clear()

        def half(b, ph, e):
            n = 2 * b + 2 + e
            qp = qproj_ops((b, 3 + e))
            _, qb, qc = qk_ops(n)
            qa = qk_ops(n + 1)[0]
            so = 2 * (1 - ph) + e
            return ([(lambda: g_olhs(3 * (n - 2), so, True),)]
                    + qc[:CF] + qp[:KD] + [(lambda: g_query(0),)] + qc[CF:] + qb[:OF]
                    + [(lambda: fence(pat_u, 3, zero_i),)] + qb[OF:]
                    + [(lambda: g_softmax(so, 0),), (lambda: g_softmax(so, 1),)]
                    + qp[KD:] + [(lambda: g_query(1),), (lambda: g_query(2),)]
                    + pvm_ops(2 * b + e, 2 * ph + e)
                    + qa[:nblk - AEND] + [(lambda: fence(pat_u, 3, zero_i),)] + qa[nblk - AEND:])

        def body(t, carry):
            for ph in range(2):
                b = 2 * t + ph

                @pl.when(first)
                def _():
                    arrivals(2 * b + 3, 2)

                emit(pv_ops(2 * b, 2 * ph) + pv_ops(2 * b + 1, 2 * ph + 1),
                     half(b, ph, 0) + half(b, ph, 1), PACE_LOOP, PK)
            return carry

        lax.fori_loop(0, 3, body, 0)

        def big(kts):
            return [op for kt in kts for op in oproj_ops(kt, kt + 6, part, SP + KD * kt)]

        pl.when(first)(lambda: arrive(NP - 1, True))
        _, qb, qc = qk_ops(NP - 1)
        seq = (half(6, 0, 0) + [(lambda: g_olhs(3 * 13, 3, True),)] + qc + qb[:OF]
               + [(lambda: fence(pat_u, 3, zero_i),)] + qb[OF:]
               + [(lambda: g_softmax(3, 0),), (lambda: g_softmax(3, 1),)]
               + pvm_ops(13, 1) + big(range(KT13 - 1))
               + [(lambda: fence(olhs_u, 3 * NP + 4, zero_i),)] + big([KT13 - 1]))
        emit(pv_ops(12, 0) + pv_ops(13, 1), seq, PACE_QUAD)
        barrier()
        old = list(range(KT13, 36))
        k14 = old[:KT14 - 7] + list(range(36, 42)) + old[KT14 - 7:KT14 - 6]
        emit(pv_ops(14, 2), [(lambda: g_olhs(3 * 14, 0),), (lambda: g_olhs(3 * 15, 1),)]
             + pvm_ops(14, 2) + big(k14), PACE_PAIR)
        barrier()
        k15 = old[KT14 - 6:-1] + list(range(42, 45)) + old[-1:]
        emit(pv_ops(15, 3), [(lambda: g_olhs(3 * 16, 2),)] + pvm_ops(15, 3) + big(k15), PACE_PAIR)

        def epilogue(x):
            def lsum(g):
                return lane_sum(accx[3, 8 * g:8 * g + 8, :])

            den = [jnp.sum(lsum(2 * G + par), axis=0, keepdims=True) for par in range(2)]
            fac = [den[0], den[1] * recip(den[0]), recip(den[1])]
            acc = []
            for n in range(KD):
                t = part[SP + n]
                for i in range(1, 3 * NP - 3):
                    t = t + part[SP + KD * i + n]
                acc.append(t * fac[0])
            for par in range(2):
                for g2 in range(G2):
                    g = G * par + 2 * g2
                    z0, z1 = lsum(g), lsum(g + 1)
                    for n in range(KD):
                        v = f32_rows(wou[RH - G + G2 * par + g2, n])
                        acc[n] = acc[n] + (v[:8] * z0 + v[8:] * z1)
                l = vres[6 + par].astype(BF)
                acc = [acc[n] + jnp.dot(
                    l, pltpu.bitcast(wo_tile(3 * NP - 3 + 2 * par, n).reshape(64, 128), BF),
                    preferred_element_type=F32) * 1.0 for n in range(KD)]
                acc = [t * fac[par + 1] for t in acc]
            cols = [jnp.sum(t, axis=0, keepdims=True) for t in acc]
            return residual(x, jnp.concatenate(cols, axis=1))

        return lax.cond(first, lambda x: ffn1(epilogue(x)), lambda x: ffn2(epilogue(x)), x)

    for r in (y_u, pat_u, olhs_u, plhs_u):
        r[...] = jnp.zeros(r.shape, U32)
    vres[...] = jnp.zeros(vres.shape, F32)
    clear_acc()
    stage_step(1)
    stage_step(2)
    kv_start(0)
    c_x.wait()
    kv_start(1)
    wait_all(c_wq)
    pair_wq()
    arrivals(0, 3)
    wait_all(c_wo)
    pair_wa()
    pair_wo(0, R0)
    lax.fori_loop(0, 2, layer, xb[...].astype(F32))


@jax.jit
def pallas_interleave_layers__sliding_block_cached__glu_gated_swiglu__decode_kernel(
    A_x: jax.Array,
    A_k_cache: jax.Array,
    A_v_cache: jax.Array,
    A_wq: jax.Array,
    A_wo: jax.Array,
    B_x: jax.Array,
    B_w1: jax.Array,
    B_w3: jax.Array,
    B_w2: jax.Array,
):
    del B_x
    sk = A_k_cache.shape[2]
    win = min(4096, max(256, sk // 4))
    nb = sk // 128
    nblk = win // 128

    def cache_tiles(c):
        return (c.reshape(H, nb, 128, G2, 2, 8).transpose(0, 3, 4, 1, 5, 2)
                .reshape(H, G2, 2, nb // 2, 16, 128))

    def weight_tiles(w):
        r, c = w.shape
        return w.reshape(r // 16, 2, 8, c // 128, 128).transpose(0, 1, 3, 2, 4)

    vreg = lambda n: pltpu.VMEM((-(-n // 4) * 4, 8, 128), F32)
    lhs = lambda n: pltpu.VMEM((-(-n // 4) * 4, 16, 128), BF)
    kern = lambda *refs: _kernel(*refs, blk0=nb - nblk, nblk=nblk, scale=DH ** -0.5)
    out = pl.pallas_call(
        kern,
        out_shape=jax.ShapeDtypeStruct((1, D), BF),
        in_specs=[pl.BlockSpec(memory_space=pl.ANY)] * 9,
        out_specs=pl.BlockSpec(memory_space=pltpu.VMEM),
        scratch_shapes=[
            pltpu.VMEM((1, D), BF),
            pltpu.VMEM((NP, 2, 2, G2, 2, nblk // 2, 16, 128), BF),
            pltpu.VMEM((D // 32, NP // 2, 2, 6, 16, 128), BF),
            pltpu.VMEM((6, 16, 2, KD, 16, 128), BF),
            pltpu.VMEM((H * G2 // 2, KD, 16, 128), BF),
            pltpu.VMEM((D // 16, 2, NC // 2, 16, 128), BF),
            pltpu.VMEM((D // 16, 2, NC // 2, 16, 128), BF),
            pltpu.VMEM((FF // 16, KD, 16, 128), BF),
            lhs(KD),
            vreg(1),
            vreg(3 * KD),
            lhs(16),
            vreg(3 * nblk // 8),
            vreg(nblk // 2 + (3 * NP - 3) * KD),
            pltpu.VMEM((4, 2, nblk, 128), F32),
            pltpu.VMEM((nblk * 8, 128), F32),
            pltpu.VMEM((4, 64, 128), F32),
            pltpu.VMEM((4, 8 * NR, 128), F32),
            lhs(3 * NP + 12),
            lhs(8),
            vreg(8),
            pltpu.VMEM((NP, NW, 2, 8, 128), F32),
            pltpu.SMEM((2, SC, KD, 16, 128), BF),
            pltpu.SemaphoreType.DMA((NP,)),
            pltpu.SemaphoreType.DMA((5 + len(W2_CHUNKS),)),
            pltpu.SemaphoreType.DMA((2,)),
        ],
        compiler_params=pltpu.CompilerParams(
            vmem_limit_bytes=128 * 1024 * 1024, disable_semaphore_checks=True,
            disable_bounds_checks=True),
    )(A_x.reshape(1, D), cache_tiles(A_k_cache), cache_tiles(A_v_cache),
      weight_tiles(A_wq).reshape(D // 32, NP // 2, 2, 6, 16, 128),
      weight_tiles(A_wo).reshape(12, 16, 2, KD, 16, 128),
      weight_tiles(A_wo).reshape(H * G2, KD, 16, 128),
      weight_tiles(B_w1).reshape(D // 16, 2, NC // 2, 16, 128),
      weight_tiles(B_w3).reshape(D // 16, 2, NC // 2, 16, 128),
      weight_tiles(B_w2).reshape(FF // 16, KD, 16, 128))
    return out.reshape(1, 1, D)
```

```python
import math

import jax
import jax.numpy as jnp
from jax import lax
import jax.experimental.pallas as pl
import jax.experimental.pallas.tpu as pltpu

BF = jnp.bfloat16
F32 = jnp.float32
U32 = jnp.uint32

D = 640
H = 32
DH = 192
G = DH // 8
G2 = DH // 16
NP = H // 2
FF = 1536
EPS = 1e-5
KD = D // 128
NC = FF // 128
NZ = 2 * G + 2
NR = NZ + 2
W2S = 8
W2_CHUNKS = (768 - 16 * W2S, 384, 256, 128)
NST = NP + 1
SC = 10
CUT = 7
KVW = 2
TRG = 6

NA = 8
NW = 64
PACE_LOOP = (30.7, 36, 30)
PACE_QUAD = (33, 8, 30)
PACE_PAIR = (32.5, 16, 30)
UNPACED = 8
PM = 6
PK = 4
AEND = 4
OF = 19
CF = 8
KT13 = 6
KT14 = 20
PVB = 14
PQ1 = 8
PQH = 4
PQ2 = 16
PLG = 86
PFS = 3.75
KM = 3
FPRE = 7
FSTEP = 4
FX = 2
FLATE = (8, 10)


def _kernel(x_hbm, k_hbm, v_hbm, wq_hbm, wa_hbm, wo_hbm, w1_hbm, w3_hbm, w2_hbm,
            o_ref,
            xb, kvb, wq, wa, wo, w1, w3, w2,
            y_scr, rs_scr, qpart, pat_scr, part_a, part, p_scr, pb_scr, pb0,
            accx, olhs, plhs, vres, vx, stage,
            kvsem, wsem, ssem, *, blk0, nblk, scale):
    c2 = scale * math.log2(math.e)
    nq = nblk // 8
    SP = 4 * nq

    def kv_copies(m):
        return [pltpu.make_async_copy(
            src.at[pl.ds(2 * m, 2), :, t, pl.ds(blk0 // 2 + o, n)],
            kvb.at[m, i, :, :, t, pl.ds(o, n)], kvsem.at[m])
            for i, src in enumerate((k_hbm, v_hbm)) for t in range(2)
            for o, n in ((0, CUT), (CUT, nblk // 2 - CUT))]

    def kv_start(m):
        for c in kv_copies(m):
            c.start()

    c_x = pltpu.make_async_copy(x_hbm, xb, wsem.at[0])
    c_wq = [pltpu.make_async_copy(wq_hbm.at[:, b], wq.at[:, b], wsem.at[1])
            for b in range(NP // 2)]
    RH = H * G2 // 2
    R0 = RH - NST * SC
    c_wo = [pltpu.make_async_copy(wa_hbm.at[pl.ds(0, 6), b], wa.at[:, b], wsem.at[2])
            for b in range(16)]
    c_wo.append(pltpu.make_async_copy(wo_hbm.at[pl.ds(RH, R0)], wo.at[pl.ds(0, R0)], wsem.at[2]))

    def to_stage(k):
        return pltpu.make_async_copy(wo_hbm.at[pl.ds(RH + R0 + SC * k, SC)], stage.at[k & 1],
                                     ssem.at[0])

    def from_stage(k):
        return pltpu.make_async_copy(stage.at[k & 1], wo.at[pl.ds(R0 + SC * k, SC)], ssem.at[1])

    def stage_step(k):
        def when(cond, f):
            if isinstance(cond, bool):
                if cond:
                    f()
            else:
                pl.when(cond)(f)

        def forward():
            to_stage(k - 1).wait()
            from_stage(k - 1).start()

        landed = not isinstance(k, int) or k >= 2
        if landed:
            from_stage(k - 2).wait()
        when(k <= NST, forward)
        when(k < NST, lambda: to_stage(k).start())
        when(k == NST, w2_in.start)
        if isinstance(k, int) and k == NST + 1:
            w2_in.wait()
            w2_out.start()
        if landed:
            pair_wo(R0 + SC * (k - 2), SC)

    c_w1 = pltpu.make_async_copy(w1_hbm, w1, wsem.at[3])
    c_w3 = pltpu.make_async_copy(w3_hbm, w3, wsem.at[4])
    w2_off = [16 * W2S + sum(W2_CHUNKS[:i]) for i in range(len(W2_CHUNKS))]
    c_w2 = [pltpu.make_async_copy(w2_hbm.at[pl.ds(o // 16, n // 16)],
                                  w2.at[pl.ds(o // 16, n // 16)], wsem.at[5 + i])
            for i, (o, n) in enumerate(zip(w2_off, W2_CHUNKS))]
    w2_slot = stage.at[NST & 1, pl.ds(0, W2S)]
    w2_in = pltpu.make_async_copy(w2_hbm.at[pl.ds(0, W2S)], w2_slot, ssem.at[0])
    w2_out = pltpu.make_async_copy(w2_slot, w2.at[pl.ds(0, W2S)], ssem.at[1])

    def wait_all(cs):
        for c in cs:
            c.wait()

    for c in c_wq[:1] + [to_stage(0), c_x] + c_wo + c_wq[1:]:
        c.start()

    def start_ffn_weights():
        for c in [c_w1, c_w3] + c_w2:
            c.start()

    kvu = kvb.bitcast(U32)
    wqu = wq.bitcast(U32)
    wau = wa.bitcast(U32)
    wou = wo.bitcast(U32)
    w1u, w3u, w2u = w1.bitcast(U32), w3.bitcast(U32), w2.bitcast(U32)
    y_u, pat_u, olhs_u = y_scr.bitcast(U32), pat_scr.bitcast(U32), olhs.bitcast(U32)
    plhs_u = plhs.bitcast(U32)

    def f32_rows(u):
        return pltpu.bitcast(u, BF).astype(F32)

    lane = lax.broadcasted_iota(jnp.int32, (8, 128), 1)
    row = lax.broadcasted_iota(jnp.int32, (8, 128), 0)
    diag_i = ((lane & 7) == row).astype(jnp.int32) * 64
    bit_i = [(lane << (3 - k)) & 64 for k in range(4)]
    uid = [0]

    def lane_sum(v):
        return jnp.broadcast_to(jnp.sum(v, axis=1, keepdims=True), (8, 128))

    def columns(v8):
        uid[0] += 1
        off = 256 * uid[0]
        dl = lane - row + off
        return [lane_sum(jnp.where(dl == off + 8 * b, v8[:, 128 * k:128 * k + 128], 0.0))
                for k in range(v8.shape[1] // 128) for b in range(16)]

    def moments(x):
        mu = jnp.mean(x, axis=-1, keepdims=True)
        xc = x - mu
        return mu, xc, 1.0 / jnp.sqrt(jnp.mean(xc * xc, axis=-1, keepdims=True) + EPS)

    def residual(x, a):
        return (x + a.astype(BF).astype(F32)).astype(BF).astype(F32)

    def tile_dot(l_u32, w_u32, rows, paced):
        w = pltpu.bitcast(w_u32.reshape(64, 128), BF)
        if paced:
            l = pltpu.bitcast(jnp.concatenate([l_u32, l_u32], axis=0), BF)[:24]
            return jnp.dot(l, w, preferred_element_type=F32)[:rows]
        l = pltpu.bitcast(l_u32, BF)[:rows]
        return jnp.dot(l, w, preferred_element_type=F32)

    def swap_halves(a, b):
        return (jnp.concatenate([a[..., :4, :], b[..., :4, :]], axis=-2),
                jnp.concatenate([a[..., 4:, :], b[..., 4:, :]], axis=-2))

    def pair_wq():
        def body(i, carry):
            for f in range(8):
                part[12 * f:12 * f + 12] = pltpu.bitcast(wqu[i, f].reshape(12, 8, 128), F32)
            for q in range(NP // 2):
                for r in range(2):
                    a, b = [pltpu.bitcast(part[48 * r + 24 * t + 3 * q:48 * r + 24 * t + 3 * q + 3], U32)
                            for t in range(2)]
                    wqu[i, q, r, 0:3], wqu[i, q, r, 3:6] = swap_halves(a, b)
            return carry
        lax.fori_loop(0, D // 32, body, 0)

    def regroup5(v):
        h = [v[:, f // 2, 4 * (f % 2):4 * (f % 2) + 4, :] for f in range(2 * KD)]
        return [jnp.concatenate([h[c], h[KD + c]], axis=1) for c in range(KD)]

    def pair_wo(r0, n):
        def body(i, carry):
            r = pl.ds(r0 + 2 * i, 2)
            for c, w in enumerate(regroup5(wou[r])):
                wou[r, c] = w
            return carry
        lax.fori_loop(0, n // 2, body, 0)

    def pair_wa():
        def body(i, carry):
            a, b = i >> 4, i & 15
            for c, w in enumerate(regroup5(wau[a, b])):
                wau[a, b, :, c] = w
            return carry
        lax.fori_loop(0, RH // 2, body, 0)

    def wo_tile(kt, n):
        if 8 * kt >= RH:
            return wou[8 * kt - RH:8 * kt - RH + 8, n]
        return wau[kt >> 2, 4 * (kt & 3):4 * (kt & 3) + 4, :, n]

    def wq_tile(m, c, k):
        c6 = 3 * m[1] + c
        return wqu[4 * k:4 * k + 4, m[0] + c6 // 6, :, 3 * (c6 & 1) + ((c6 % 6) >> 1)]

    def qproj_ops(m):
        def op(paced, c, k):
            qpart[c * KD + k] = tile_dot(
                y_u[k], wq_tile(m, c, k), 8, paced)
        return [(lambda p, c=c, k=k: op(p, c, k)) for c in range(3) for k in range(KD)]

    def oproj_ops(kt, slot, dst, d0):
        def op(paced, n):
            dst[d0 + n] = tile_dot(olhs_u[slot], wo_tile(kt, n), 8, paced)
        return [(lambda p, n=n: op(p, n)) for n in range(KD)]

    def pair_rows(m):
        def body(g2, c):
            for par in range(2):
                kvu[m, 0, par, g2, 0], kvu[m, 0, par, g2, 1] = swap_halves(
                    kvu[m, 0, par, g2, 0], kvu[m, 0, par, g2, 1])
            return c
        lax.fori_loop(0, G2, body, 0)

    def k_blocks(m, par, g0, g1, j):
        return kvu[m, 0, par, g0:g1, j & 1, j >> 1]

    jord = [8 * (i // 8) + 2 * (i % 4) + (i % 8) // 4 for i in range(nblk)]

    def qk_ops(m, po=0, pb=0):
        def op_a(paced, j):
            r = tile_dot(pat_u[po + 0], k_blocks(m, 0, 0, 8, j), 8, paced)
            part_a[j // 8, j % 8:j % 8 + 1, :] = r[j % 8:j % 8 + 1, :]

        def op_c(paced, j):
            r = tile_dot(pat_u[po + 2], k_blocks(m, 1, 4, 12, j), 8, paced)
            part[pb + 2 * nq + j // 8, j % 8:j % 8 + 1, :] = r[j % 8:j % 8 + 1, :]

        def op_b(paced, j):
            w = jnp.concatenate([k_blocks(m, 0, 8, 12, j), k_blocks(m, 1, 0, 4, j)], axis=0)
            r = tile_dot(pat_u[po + 1], w, 16, paced)
            part[pb + nq + j // 8, j % 8:j % 8 + 1, :] = r[j % 8:j % 8 + 1, :]
            part[pb + 3 * nq + j // 8, j % 8:j % 8 + 1, :] = r[8 + j % 8:8 + j % 8 + 1, :]

        return [[(lambda p, f=f, j=j: f(p, j)) for j in jord] for f in (op_a, op_b, op_c)]

    def plain(ops):
        for op in ops:
            op(False)

    steps = [(par, gb, j0) for par in range(2) for gb in range(G // NA)
             for j0 in range(0, nblk, 4) if j0 != 4 or gb == 2 - 2 * par]

    def flip(m):
        for par in range(2):
            for a in range(2):
                v = f32_rows(kvu[m, 1, par, 4 * par:4 * par + 8, :, 2 + a])
                ts = [v[:, :, 8 * b:8 * b + 8, :].reshape(128, 128).T.astype(BF) for b in range(2)]
                for b in range(2):
                    kvu[m, 1, par, 4 * par:4 * par + 8, b, 2 + a] = (
                        pltpu.bitcast(ts[b], U32).reshape(8, 8, 128))

    def pvm_ops(m, sl):
        def op(paced, par, j):
            r = tile_dot(plhs_u[2 * sl + par],
                         kvu[m, 1, par, 4 * par:4 * par + 8, j & 1, j >> 1], 8, paced)
            vres[2 * sl + par, j:j + 1, :] = r[j:j + 1, :]
        return [(lambda p, par=par, j=j: op(p, par, j))
                for j in range(4, 8) for par in range(2)]

    def units(par, gb, j0):
        return [(par, g, j0) for g in range(gb * NA, (gb + 1) * NA)]

    order = [u for s in steps for u in units(*s)]
    wide = {}
    for i, u in enumerate(order):
        if (i + 1) * NW // len(order) > i * NW // len(order):
            wide[u] = len(wide)

    def widen(m):
        for (par, g, j), e in wide.items():
            v = f32_rows(kvu[m, 1, par, g // 2, g % 2, j // 2:j // 2 + 2])
            kvu[m, 1, par, g // 2, g % 2, j // 2:j // 2 + 2] = pltpu.bitcast(v[:, :8], U32)
            vx[m, e] = v[:, 8:]

    def v_unit(m, par, g, j):
        u = kvu[m, 1, par, g // 2, g % 2, j // 2:j // 2 + 2]
        if (par, g, j) in wide:
            return jnp.concatenate([pltpu.bitcast(u, F32), vx[m, wide[(par, g, j)]]], axis=1)
        return f32_rows(u)

    def pv_ops(m, ph):
        acc = {}

        def spread(par, q, r):
            pb_scr[pl.ds(64 * q + r, 8, stride=8), :] = p_scr[ph, par, 8 * q:8 * q + 8, :]

        def psum(par):
            p = p_scr[ph, par]
            accx[ph, 8 * (2 * G + par):8 * (2 * G + par) + 8, :] = (
                (p[0:8] + p[8:16]) + (p[16:24] + p[24:32]))

        pbv = {}

        def piece(par, gb, j0, k):
            if k == 0:
                if par == 0 and j0 < 8:
                    pb = pb0[ph, 8 * j0:8 * j0 + 32, :]
                else:
                    pb = pb_scr[8 * j0:8 * j0 + 32, :]
                pbv[0] = pb.reshape(4, 8, 128)
            for _, g, _ in units(par, gb, j0)[4 * k:4 * k + 4]:
                tv = v_unit(m, par, g, j0).reshape(4, 8, 128) * pbv[0]
                tv = jnp.sum(tv, axis=0)
                acc[g] = tv if j0 == 0 else acc[g] + tv
                if j0 == nblk - 4:
                    r0 = DH * par + 8 * g
                    accx[ph, r0:r0 + 8, :] = acc[g]

        pieces = [s + (k,) for s in steps for k in range(NA // 4)]
        use = {}
        for i, (par, _, j0, k) in enumerate(pieces):
            if k == 0:
                use.setdefault((par, j0 // 8), []).append(i)
        side = {}
        for q in range(nq):
            for r in range(8):
                if q:
                    lo, hi = (use[0, q - 1][0] - 1 if q > 1 else 0), use[0, q][0] - 1
                    side.setdefault(lo + (r * (hi - lo + 1)) // 8, []).append(
                        lambda q=q, r=r: spread(0, q, r))
                lo, hi = use[0, q][-1] + 1, use[1, q][0] - 1
                side.setdefault(lo + (r * (hi - lo)) // 8, []).append(
                    lambda q=q, r=r: spread(1, q, r))
        for par in range(2):
            side.setdefault(len(pieces) // 4 + par, []).append(lambda par=par: psum(par))
        out = []
        for i, s in enumerate(pieces):
            out += [(0, f) for f in side.get(i, [])]
            out.append((2 * sum(4 if u in wide else 6 for u in units(*s[:3])[4 * s[3]:4 * s[3] + 4]),
                        (lambda s=s: piece(*s))))
        return out

    toks = []

    def fence(dst, slot, zero_i):
        for i, t in enumerate(toks):
            dst[slot + i + zero_i] = t
        toks.clear()

    def g_softmax(ph, par, pb=0, pa=0):
        s0 = part[pb + 2 * nq:pb + 3 * nq] if par else part_a[pa:pa + nq]
        s = (s0 + part[pb + (2 * par + 1) * nq:pb + (2 * par + 2) * nq]).reshape(nblk, 128)
        mx = jnp.max(jnp.max(s, axis=0, keepdims=True), axis=1, keepdims=True)
        p = jnp.exp2((s - mx) * jnp.concatenate([rs_scr[0]] * nq, axis=0))
        p_scr[ph, par] = p
        plhs[2 * ph + par, 0:8, :] = p[0:8].astype(BF)
        if par == 0:
            for r in range(8):
                pb0[ph, pl.ds(r, 8, stride=8), :] = p[0:8]
        toks.append(pltpu.bitcast(p[nblk - 8:nblk], U32))

    def recip(d):
        r = pl.reciprocal(d, approx=True)
        return r * (2.0 - d * r)

    def g_olhs(slot0, ph, tok=False):
        zz = [lane_sum(accx[ph, 8 * g:8 * g + 8, :]) for g in range(NZ)]
        inv = [jnp.broadcast_to(recip(jnp.sum(zz[2 * G + par], axis=0, keepdims=True)), (8, 128))
               for par in range(2)]
        uid[0] += 1
        bit = [b > uid[0] for b in bit_i]
        for c in range(3):
            xs = zz[16 * c:16 * c + 16]
            for k in range(4):
                xs = [jnp.where(bit[k], xs[i + 1], xs[i]) for i in range(0, len(xs), 2)]
            iv = inv[0] if c == 0 else (inv[1] if c == 2 else jnp.where(bit[3], inv[1], inv[0]))
            z = jnp.where(diag_i > uid[0], xs[0], 0.0)
            if c != 1:
                z = z + vres[2 * ph + c // 2]
            z = z * iv
            olhs[slot0 + c, 0:8, :] = z.astype(BF)
            if tok:
                toks.append(pltpu.bitcast(z, U32))

    def set_pat(c, q, po=0):
        if c == 1:
            hi = bit_i[3] > uid[0]
            pat_scr[po + c, 0:8, :] = jnp.where(hi, 0.0, q).astype(BF)
            pat_scr[po + c, 8:16, :] = jnp.where(hi, q, 0.0).astype(BF)
        else:
            pat_scr[po + c, 0:8, :] = q.astype(BF)
        if c > 0:
            toks.append(pltpu.bitcast(q, U32))

    def g_query(c):
        xs = [qpart[c * KD + k] for k in range(KD)]
        set_pat(c, ((xs[0] + xs[1]) + (xs[2] + xs[3])) + xs[4])

    def clear_acc():
        accx[2:4] = jnp.ones((2, 8 * NR, 128), F32)

    def emit(pv, seq, pace, pk=PM):
        rate, lead, tail = pace
        ntile = sum(not isinstance(e, tuple) for e in seq)
        total = sum(w for w, _ in pv) / 4
        k = done = n = 0
        for e in seq:
            if isinstance(e, tuple):
                e[0]()
                continue
            r = n // 4
            pos = lead + rate * r if r < (ntile - 1) // 4 else total - tail
            while k < len(pv) and done + pv[k][0] / 2 <= 4 * pos:
                done += pv[k][0]
                pv[k][1]()
                k += 1
            e(n < ntile - UNPACED and r % PM < pk)
            n += 1
        for _, g in pv[k:]:
            g()

    def ffn1(x):
        _, xc, rs = moments(x)
        y = jnp.broadcast_to(xc, (8, D)).astype(BF)

        def up(wu):
            cols = []
            for cp in range(NC // 2):
                ev, od = swap_halves(wu[:, 0, cp], wu[:, 1, cp])
                wu[:, 0, cp], wu[:, 1, cp] = ev, od
                cols += [jnp.dot(y, pltpu.bitcast(w.reshape(D // 2, 128), BF),
                                 preferred_element_type=F32) for w in (ev, od)]
            return jnp.concatenate(cols, axis=1) * rs

        def w2_rows(r0, n):
            nat = regroup5(w2u[r0:r0 + n])
            for c in range(KD):
                w2u[r0:r0 + n, c] = nat[c]
            return nat

        def down(o, n):
            cols = [None] * KD
            for k in range(o // 128, (o + n) // 128):
                for c, w in enumerate(w2_rows(8 * k, 8)):
                    t = jnp.dot(hh[:, 128 * k:128 * k + 128], pltpu.bitcast(w.reshape(64, 128), BF),
                                preferred_element_type=F32)[0:1]
                    cols[c] = t if cols[c] is None else cols[c] + t
            return jnp.concatenate(cols, axis=1)

        c_w1.wait()
        g = up(w1u)
        c_w3.wait()
        u = up(w3u)
        hh = (g * jax.nn.sigmoid(g) * u).astype(BF)
        hb = columns(hh[:, w2_off[-1]:].astype(F32))
        a = None
        parts = list(zip(c_w2, w2_off, W2_CHUNKS))[:-1]
        parts.insert(1, (w2_out, 0, 16 * W2S))
        for c, o, n in parts:
            c.wait()
            a = down(o, n) if a is None else a + down(o, n)
        c_w2[-1].wait()
        acc = [None] * KD
        for r in range(W2_CHUNKS[-1] // 16):
            v = f32_rows(w2u[w2_off[-1] // 16 + r])
            for f in range(2 * KD):
                tv = v[f // 2, 8 * (f % 2):8 * (f % 2) + 8] * hb[2 * r + f // KD]
                acc[f % KD] = tv if acc[f % KD] is None else acc[f % KD] + tv
        a = a + jnp.concatenate([jnp.sum(t, axis=0, keepdims=True) for t in acc], axis=1)
        return residual(x, a)

    def ffn2(x):
        mu, _, rs = moments(x)
        x8 = jnp.broadcast_to(x, (8, D))
        rowk = lax.broadcasted_iota(jnp.int32, (8, D), 0)
        y = jnp.where(rowk == 0, x8, jnp.where(rowk == 1, 1.0, 0.0)).astype(BF)
        coef = jnp.where(row == 0, 1.0, -mu)
        yb = jnp.concatenate([c - mu for c in columns(x8[:, 128 * KM:])], axis=0)
        km = [KM + ((c + 1) * FX // NC > c * FX // NC) for c in range(NC)]
        mx = {}
        out = [None] * KD
        late = []
        for c in range(NC):
            while len(mx) < min(NC, FPRE + c * FSTEP / 4):
                cc = len(mx)
                mx[cc] = [jnp.dot(y[:, :128 * km[cc]],
                                  pltpu.bitcast(wu[0:8 * km[cc], cc & 1, cc >> 1].reshape(64 * km[cc], 128), BF),
                                  preferred_element_type=F32) * coef for wu in (w1u, w3u)]
            gu = []
            for i, wu in enumerate((w1u, w3u)):
                acc = None
                for r in range(8 * km[c], 8 * KD):
                    o = 16 * (r - 8 * KM)
                    tv = f32_rows(wu[r, c & 1, c >> 1]) * yb[o:o + 16]
                    acc = tv if acc is None else acc + tv
                gu.append(jnp.sum((acc[:8] + acc[8:]) + mx[c][i], axis=0, keepdims=True) * rs)
            hg = 0.5 * gu[0]
            h = jnp.broadcast_to((hg * jnp.tanh(hg) + hg) * gu[1], (8, 128)).astype(BF)
            if c in FLATE:
                late.append((c, columns(h.astype(F32))))
                continue
            if c == NC - 1:
                ws = regroup5(w2u[8 * c:8 * c + 8])
            else:
                ws = [w2u[8 * c:8 * c + 8, n] for n in range(KD)]
            for n in range(KD):
                t = jnp.dot(h, pltpu.bitcast(ws[n].reshape(64, 128), BF),
                            preferred_element_type=F32)[0:1]
                out[n] = t if out[n] is None else out[n] + t
        if late:
            acc = [None] * KD
            for c, hb in late:
                for r in range(8):
                    for n in range(KD):
                        v = f32_rows(w2u[8 * c + r, n])
                        for t in range(2):
                            tv = v[8 * t:8 * t + 8] * hb[2 * r + t]
                            acc[n] = tv if acc[n] is None else acc[n] + tv
            out = [out[n] + jnp.sum(acc[n], axis=0, keepdims=True) for n in range(KD)]
        a = jnp.concatenate(out, axis=1)
        o_ref[...] = (x + a.astype(BF).astype(F32)).astype(BF)
        return x

    def arrive(p, last):
        def when(cond, f):
            if isinstance(cond, bool):
                if cond:
                    f()
            else:
                pl.when(cond)(f)

        cs = kv_copies(p)
        wait_all(cs[:4])
        if not last:
            stage_step(p + 3)
        wait_all(cs[4:TRG])
        if last:
            start_ffn_weights()
        wait_all(cs[TRG:])
        when(p + KVW < NP, lambda: kv_start(p + KVW))
        pair_rows(p)
        widen(p)
        flip(p)
        if last:
            stage_step(NST + 1)

    def arrivals(p0, n):
        def body(i, carry):
            arrive(p0 + i, False)
            return carry
        lax.fori_loop(0, n, body, 0)

    def layer(li, x):
        first = li == 0
        zero_i = li >> 4

        def barrier():
            @pl.when(li > 2)
            def _():
                clear_acc()

        mu, xc, rs = moments(x)
        y = jnp.broadcast_to(xc, (8, D))
        for k in range(KD):
            y_scr[k, 0:8, :] = y[:, 128 * k:128 * k + 128].astype(BF)
        rs_scr[0] = jnp.broadcast_to(rs * c2, (8, 128))
        rowd = lax.broadcasted_iota(jnp.int32, (8, D), 0)
        xo = jnp.where(rowd < 4, jnp.broadcast_to(x, (8, D)), 1.0).astype(BF)
        coef = jnp.where(row < 4, 1.0, -mu)

        def q_direct(col):
            t = jnp.dot(xo, pltpu.bitcast(wqu[:, 0, :, 3 * (col & 1) + (col >> 1)].reshape(D // 2, 128), BF), preferred_element_type=F32) * coef
            return (t + pltpu.roll(t, 4, 0)).astype(BF).astype(F32)

        def q_cols(q, slot):
            for b, col in enumerate(columns(q)):
                part[slot + b] = col

        def vpu_a(m, slot, js, pa):
            z = zero_i if m == 0 else 0
            acc = {}
            for g2 in range(8):
                qc = jnp.concatenate([part[slot + 2 * g2 + t + z] for t in range(2)], axis=0)
                for j in js:
                    tv = f32_rows(kvu[m, 0, 0, g2, j & 1, j >> 1]) * qc
                    acc[j] = tv if g2 == 0 else acc[j] + tv
            rs_ = [jnp.sum(acc[j], axis=0, keepdims=True) for j in js]
            for j, r in zip(js, rs_):
                part_a[pa + j // 8, j % 8:j % 8 + 1, :] = r
            return [pltpu.bitcast(jnp.broadcast_to(r, (8, 128)), U32) for r in rs_]

        def q_sum(c):
            xs = [qpart[c * KD + k] for k in range(KD)]
            return (((xs[0] + xs[1]) + (xs[2] + xs[3])) + xs[4]).astype(BF).astype(F32)

        q0 = [q_direct(c) for c in range(4)]
        q_cols(q0[0], SP)
        set_pat(1, q0[1], 10)
        set_pat(2, q0[2], 10)
        P0 = SP + 48

        def mark(ops, src):
            def wrap(op, v):
                def f(p):
                    op(p)
                    part[0] = v()
                return f
            return [wrap(op, v) for op, v in zip(ops, src)]

        def qp(m, lo, hi):
            return mark(qproj_ops((0, m))[lo:hi], [(lambda i=i: qpart[i]) for i in range(lo, hi)])

        st = {}

        def queries():
            g_query(1)
            g_query(2)
            st["q"] = q_sum(0)
            set_pat(0, st["q"])

        _, b0, c0 = qk_ops(0, 10, P0)
        _, b1, c1 = qk_ops(1)
        a2 = qk_ops(2)[0][PVB:]
        bc = b0 + c0

        def sprinkle(few, many):
            out = []
            for i, e in enumerate(many):
                out.append(e)
                if i % 3 == 2 and i // 3 < len(few):
                    out.append(few[i // 3])
            return out + few[len(many) // 3:]

        q2 = qproj_ops((0, 2))[KD:]
        mx = (bc[:PQ1] + qp(1, KD, 3 * KD) + qp(2, 0, KD) + [(queries,)] + bc[PQ1:]
              + [(lambda: g_softmax(0, 1, P0),)]
              + sprinkle(q2, b1) + c1 + [(lambda: g_softmax(1, 1),)]
              + [(lambda: g_query(1),), (lambda: g_query(2),)] + a2)
        vg = ([(0, SP, jord[i:i + 2], 2 * nq) for i in range(0, nblk, 2)]
              + [(1, SP + 16, jord[i:i + 2], nq) for i in range(0, nblk, 2)]
              + [(2, SP + 32, jord[i:i + 2], 0) for i in range(0, PVB, 2)])
        n = g = 0
        done = set()

        def ripe():
            if "s0" not in done and g >= nblk // 2 and n >= nblk + 3 * KD:
                done.add("s0")
                g_softmax(0, 0, P0, 2 * nq)
            if "s1" not in done and g >= nblk and n >= 3 * nblk + 5 * KD:
                done.add("s1")
                g_softmax(1, 0, 0, nq)

        for e in mx + [None]:
            while g < len(vg) and (e is None or (4 * g if g < 16 else PLG + PFS * (g - 16)) <= n):
                if g == PQH:
                    q_cols(q0[3], SP + 16)
                if g == PQ2:
                    q_cols(st["q"], SP + 32)
                toks[:] = vpu_a(*vg[g])
                if g >= 16 and e is not None:
                    fence(pat_u, 3, zero_i)
                g += 1
                ripe()
            if isinstance(e, tuple):
                e[0]()
            elif e is not None:
                e(False)
                n += 1
                ripe()
        toks.clear()

        def half(b, ph, e):
            n = 2 * b + 2 + e
            qp = qproj_ops((b, 3 + e))
            _, qb, qc = qk_ops(n)
            qa = qk_ops(n + 1)[0]
            so = 2 * (1 - ph) + e
            return ([(lambda: g_olhs(3 * (n - 2), so, True),)]
                    + qc[:CF] + qp[:KD] + [(lambda: g_query(0),)] + qc[CF:] + qb[:OF]
                    + [(lambda: fence(pat_u, 3, zero_i),)] + qb[OF:]
                    + [(lambda: g_softmax(so, 0),), (lambda: g_softmax(so, 1),)]
                    + qp[KD:] + [(lambda: g_query(1),), (lambda: g_query(2),)]
                    + pvm_ops(2 * b + e, 2 * ph + e)
                    + qa[:nblk - AEND] + [(lambda: fence(pat_u, 3, zero_i),)] + qa[nblk - AEND:])

        def body(t, carry):
            for ph in range(2):
                b = 2 * t + ph

                @pl.when(first)
                def _():
                    arrivals(2 * b + 3, 2)

                emit(pv_ops(2 * b, 2 * ph) + pv_ops(2 * b + 1, 2 * ph + 1),
                     half(b, ph, 0) + half(b, ph, 1), PACE_LOOP, PK)
            return carry

        lax.fori_loop(0, 3, body, 0)

        def big(kts):
            return [op for kt in kts for op in oproj_ops(kt, kt + 6, part, SP + KD * kt)]

        pl.when(first)(lambda: arrive(NP - 1, True))
        _, qb, qc = qk_ops(NP - 1)
        seq = (half(6, 0, 0) + [(lambda: g_olhs(3 * 13, 3, True),)] + qc + qb[:OF]
               + [(lambda: fence(pat_u, 3, zero_i),)] + qb[OF:]
               + [(lambda: g_softmax(3, 0),), (lambda: g_softmax(3, 1),)]
               + pvm_ops(13, 1) + big(range(KT13 - 1))
               + [(lambda: fence(olhs_u, 3 * NP + 4, zero_i),)] + big([KT13 - 1]))
        emit(pv_ops(12, 0) + pv_ops(13, 1), seq, PACE_QUAD)
        barrier()
        old = list(range(KT13, 36))
        k14 = old[:KT14 - 7] + list(range(36, 42)) + old[KT14 - 7:KT14 - 6]
        emit(pv_ops(14, 2), [(lambda: g_olhs(3 * 14, 0),), (lambda: g_olhs(3 * 15, 1),)]
             + pvm_ops(14, 2) + big(k14), PACE_PAIR)
        barrier()
        k15 = old[KT14 - 6:-1] + list(range(42, 45)) + old[-1:]
        emit(pv_ops(15, 3), [(lambda: g_olhs(3 * 16, 2),)] + pvm_ops(15, 3) + big(k15), PACE_PAIR)

        def epilogue(x):
            def lsum(g):
                return lane_sum(accx[3, 8 * g:8 * g + 8, :])

            den = [jnp.sum(lsum(2 * G + par), axis=0, keepdims=True) for par in range(2)]
            fac = [den[0], den[1] * recip(den[0]), recip(den[1])]
            acc = []
            for n in range(KD):
                t = part[SP + n]
                for i in range(1, 3 * NP - 3):
                    t = t + part[SP + KD * i + n]
                acc.append(t * fac[0])
            for par in range(2):
                for g2 in range(G2):
                    g = G * par + 2 * g2
                    z0, z1 = lsum(g), lsum(g + 1)
                    for n in range(KD):
                        v = f32_rows(wou[RH - G + G2 * par + g2, n])
                        acc[n] = acc[n] + (v[:8] * z0 + v[8:] * z1)
                l = vres[6 + par].astype(BF)
                acc = [acc[n] + jnp.dot(
                    l, pltpu.bitcast(wo_tile(3 * NP - 3 + 2 * par, n).reshape(64, 128), BF),
                    preferred_element_type=F32) * 1.0 for n in range(KD)]
                acc = [t * fac[par + 1] for t in acc]
            cols = [jnp.sum(t, axis=0, keepdims=True) for t in acc]
            return residual(x, jnp.concatenate(cols, axis=1))

        return lax.cond(first, lambda x: ffn1(epilogue(x)), lambda x: ffn2(epilogue(x)), x)

    for r in (y_u, pat_u, olhs_u, plhs_u):
        r[...] = jnp.zeros(r.shape, U32)
    vres[...] = jnp.zeros(vres.shape, F32)
    clear_acc()
    stage_step(1)
    stage_step(2)
    kv_start(0)
    c_x.wait()
    kv_start(1)
    wait_all(c_wq)
    pair_wq()
    arrivals(0, 3)
    wait_all(c_wo)
    pair_wa()
    pair_wo(0, R0)
    lax.fori_loop(0, 2, layer, xb[...].astype(F32))


@jax.jit
def pallas_interleave_layers__sliding_block_cached__glu_gated_swiglu__decode_kernel(
    A_x: jax.Array,
    A_k_cache: jax.Array,
    A_v_cache: jax.Array,
    A_wq: jax.Array,
    A_wo: jax.Array,
    B_x: jax.Array,
    B_w1: jax.Array,
    B_w3: jax.Array,
    B_w2: jax.Array,
):
    del B_x
    sk = A_k_cache.shape[2]
    win = min(4096, max(256, sk // 4))
    nb = sk // 128
    nblk = win // 128

    def cache_tiles(c):
        return (c.reshape(H, nb, 128, G2, 2, 8).transpose(0, 3, 4, 1, 5, 2)
                .reshape(H, G2, 2, nb // 2, 16, 128))

    def weight_tiles(w):
        r, c = w.shape
        return w.reshape(r // 16, 2, 8, c // 128, 128).transpose(0, 1, 3, 2, 4)

    vreg = lambda n: pltpu.VMEM((-(-n // 4) * 4, 8, 128), F32)
    lhs = lambda n: pltpu.VMEM((-(-n // 4) * 4, 16, 128), BF)
    kern = lambda *refs: _kernel(*refs, blk0=nb - nblk, nblk=nblk, scale=DH ** -0.5)
    out = pl.pallas_call(
        kern,
        out_shape=jax.ShapeDtypeStruct((1, D), BF),
        in_specs=[pl.BlockSpec(memory_space=pl.ANY)] * 9,
        out_specs=pl.BlockSpec(memory_space=pltpu.VMEM),
        scratch_shapes=[
            pltpu.VMEM((1, D), BF),
            pltpu.VMEM((NP, 2, 2, G2, 2, nblk // 2, 16, 128), BF),
            pltpu.VMEM((D // 32, NP // 2, 2, 6, 16, 128), BF),
            pltpu.VMEM((6, 16, 2, KD, 16, 128), BF),
            pltpu.VMEM((H * G2 // 2, KD, 16, 128), BF),
            pltpu.VMEM((D // 16, 2, NC // 2, 16, 128), BF),
            pltpu.VMEM((D // 16, 2, NC // 2, 16, 128), BF),
            pltpu.VMEM((FF // 16, KD, 16, 128), BF),
            lhs(KD),
            vreg(1),
            vreg(3 * KD),
            lhs(16),
            vreg(3 * nblk // 8),
            vreg(nblk // 2 + (3 * NP - 3) * KD),
            pltpu.VMEM((4, 2, nblk, 128), F32),
            pltpu.VMEM((nblk * 8, 128), F32),
            pltpu.VMEM((4, 64, 128), F32),
            pltpu.VMEM((4, 8 * NR, 128), F32),
            lhs(3 * NP + 12),
            lhs(8),
            vreg(8),
            pltpu.VMEM((NP, NW, 2, 8, 128), F32),
            pltpu.SMEM((2, SC, KD, 16, 128), BF),
            pltpu.SemaphoreType.DMA((NP,)),
            pltpu.SemaphoreType.DMA((5 + len(W2_CHUNKS),)),
            pltpu.SemaphoreType.DMA((2,)),
        ],
        compiler_params=pltpu.CompilerParams(
            vmem_limit_bytes=128 * 1024 * 1024, disable_semaphore_checks=True,
            disable_bounds_checks=True),
    )(A_x.reshape(1, D), cache_tiles(A_k_cache), cache_tiles(A_v_cache),
      weight_tiles(A_wq).reshape(D // 32, NP // 2, 2, 6, 16, 128),
      weight_tiles(A_wo).reshape(12, 16, 2, KD, 16, 128),
      weight_tiles(A_wo).reshape(H * G2, KD, 16, 128),
      weight_tiles(B_w1).reshape(D // 16, 2, NC // 2, 16, 128),
      weight_tiles(B_w3).reshape(D // 16, 2, NC // 2, 16, 128),
      weight_tiles(B_w2).reshape(FF // 16, KD, 16, 128))
    return out.reshape(1, 1, D)
```

```python
import math

import jax
import jax.numpy as jnp
from jax import lax
import jax.experimental.pallas as pl
import jax.experimental.pallas.tpu as pltpu

BF = jnp.bfloat16
F32 = jnp.float32
U32 = jnp.uint32

D = 640
H = 32
DH = 192
G = DH // 8
G2 = DH // 16
NP = H // 2
FF = 1536
EPS = 1e-5
KD = D // 128
NC = FF // 128
NZ = 2 * G + 2
NR = NZ + 2
W2S = 8
W2_CHUNKS = (768 - 16 * W2S, 384, 256, 128)
NST = NP + 1
SC = 10
CUT = 7
PS = 8
KVW = 2
TRG = 6

NA = 8
NW = 64
PACE_LOOP = (30.7, 36, 30)
PACE_QUAD = (33, 8, 30)
PACE_PAIR = (32.5, 16, 30)
UNPACED = 8
PM = 6
PK = 4
AEND = 4
OF = 19
CF = 8
KT13 = 6
KT14 = 20
PVB = 14
PQ1 = 8
PQH = 4
PQ2 = 16
PLG = 86
PFS = 3.75
KM = 3
FPRE = 7
FSTEP = 4
FX = 2
FLATE = (8, 10)


def _kernel(x_hbm, k_hbm, v_hbm, wq_hbm, wa_hbm, wo_hbm, w1_hbm, w3_hbm, w2_hbm,
            o_ref,
            xb, kvb, wq, wa, wo, w1, w3, w2,
            y_scr, rs_scr, qpart, pat_scr, part_a, part, p_scr, pb_scr, pb0,
            accx, olhs, plhs, vres, vx, stage,
            kvsem, wsem, ssem, *, blk0, nblk, scale):
    c2 = scale * math.log2(math.e)
    nq = nblk // 8
    SP = 4 * nq

    def kv_copies(m):
        return [pltpu.make_async_copy(
            src.at[pl.ds(2 * m, 2), :, t, pl.ds(blk0 // 2 + o, n)],
            kvb.at[m, i, :, :, t, pl.ds(o, n)], kvsem.at[m])
            for i, src in enumerate((k_hbm, v_hbm)) for t in range(2)
            for o, n in ((0, CUT), (CUT, nblk // 2 - CUT))]

    def kv_start(m):
        for c in kv_copies(m):
            c.start()

    c_x = pltpu.make_async_copy(x_hbm, xb, wsem.at[0])
    c_wq = [pltpu.make_async_copy(wq_hbm.at[:, b], wq.at[:, b], wsem.at[1])
            for b in range(NP // 2)]
    RH = H * G2 // 2
    R0 = RH - NST * SC
    c_wo = [pltpu.make_async_copy(wa_hbm.at[pl.ds(0, 6), b], wa.at[:, b], wsem.at[2])
            for b in range(16)]
    c_wo.append(pltpu.make_async_copy(wo_hbm.at[pl.ds(RH, R0)], wo.at[pl.ds(0, R0)], wsem.at[2]))

    class Part:
        def __init__(self, src, dst, o, k, sem):
            self.copy = lambda: pltpu.make_async_copy(
                src.at[pl.ds(o, k)], dst.at[pl.ds(o, k)], sem)

        def start(self):
            self.copy().start()

        def wait(self):
            self.copy().wait()

    def halves(src, dst, n, s):
        return [Part(src, dst, 0, n - 1, ssem.at[s]), Part(src, dst, n - 1, 1, ssem.at[s + 1])]

    def slot(c):
        return stage.at[c % 3 if isinstance(c, int) else lax.rem(c, 3)]

    def fetch(c):
        return halves(wo_hbm.at[pl.ds(RH + R0 + SC * c, SC)], slot(c), SC, 0)

    def forward(c):
        return halves(slot(c), wo.at[pl.ds(R0 + SC * c, SC)], SC, 2)

    w2_in = halves(w2_hbm, slot(NST), W2S, 0)
    w2_out = halves(slot(NST), w2, W2S, 4)

    def start_all(cs):
        for c in cs:
            c.start()

    def when(cond, f):
        if isinstance(cond, bool):
            if cond:
                f()
        else:
            pl.when(cond)(f)

    def to_fetch(k):
        forward(k - 2)[0].wait()
        fetch(k - 1)[1].wait()
        when(k < NST, lambda: start_all(fetch(k)))
        when(k == NST, lambda: start_all(w2_in))

    def to_forward(k):
        when(k + 1 < NST, lambda: fetch(k + 1)[0].wait())
        when(k + 1 == NST, w2_in[0].wait)
        forward(k - 1)[1].wait()
        start_all(forward(k))
        pair_wo(R0 + SC * (k - 1), SC)

    c_w1 = pltpu.make_async_copy(w1_hbm, w1, wsem.at[3])
    c_w3 = pltpu.make_async_copy(w3_hbm, w3, wsem.at[4])
    w2_off = [16 * W2S + sum(W2_CHUNKS[:i]) for i in range(len(W2_CHUNKS))]
    c_w2 = [pltpu.make_async_copy(w2_hbm.at[pl.ds(o // 16, n // 16)],
                                  w2.at[pl.ds(o // 16, n // 16)], wsem.at[5 + i])
            for i, (o, n) in enumerate(zip(w2_off, W2_CHUNKS))]

    def wait_all(cs):
        for c in cs:
            c.wait()

    for c in c_wq[:1] + fetch(0) + [c_x] + c_wo + c_wq[1:]:
        c.start()

    def start_ffn_weights():
        for c in [c_w1, c_w3] + c_w2:
            c.start()

    kvu = kvb.bitcast(U32)
    wqu = wq.bitcast(U32)
    wau = wa.bitcast(U32)
    wou = wo.bitcast(U32)
    w1u, w3u, w2u = w1.bitcast(U32), w3.bitcast(U32), w2.bitcast(U32)
    y_u, pat_u, olhs_u = y_scr.bitcast(U32), pat_scr.bitcast(U32), olhs.bitcast(U32)
    plhs_u = plhs.bitcast(U32)

    def f32_rows(u):
        return pltpu.bitcast(u, BF).astype(F32)

    lane = lax.broadcasted_iota(jnp.int32, (8, 128), 1)
    row = lax.broadcasted_iota(jnp.int32, (8, 128), 0)
    diag_i = ((lane & 7) == row).astype(jnp.int32) * 64
    bit_i = [(lane << (3 - k)) & 64 for k in range(4)]
    uid = [0]

    def lane_sum(v):
        return jnp.broadcast_to(jnp.sum(v, axis=1, keepdims=True), (8, 128))

    def columns(v8):
        uid[0] = uid[0] % 60 + 1
        off = 256 * uid[0]
        dl = lane - row + off
        return [lane_sum(jnp.where(dl == off + 8 * b, v8[:, 128 * k:128 * k + 128], 0.0))
                for k in range(v8.shape[1] // 128) for b in range(16)]

    def moments(x):
        mu = jnp.mean(x, axis=-1, keepdims=True)
        xc = x - mu
        return mu, xc, 1.0 / jnp.sqrt(jnp.mean(xc * xc, axis=-1, keepdims=True) + EPS)

    def residual(x, a):
        return (x + a.astype(BF).astype(F32)).astype(BF).astype(F32)

    def tile_dot(l_u32, w_u32, rows, paced):
        w = pltpu.bitcast(w_u32.reshape(64, 128), BF)
        if paced:
            l = pltpu.bitcast(jnp.concatenate([l_u32, l_u32], axis=0), BF)[:24]
            return jnp.dot(l, w, preferred_element_type=F32)[:rows]
        l = pltpu.bitcast(l_u32, BF)[:rows]
        return jnp.dot(l, w, preferred_element_type=F32)

    def swap_halves(a, b):
        return (jnp.concatenate([a[..., :4, :], b[..., :4, :]], axis=-2),
                jnp.concatenate([a[..., 4:, :], b[..., 4:, :]], axis=-2))

    def pair_wq():
        def body(i, carry):
            for f in range(8):
                part[12 * f:12 * f + 12] = pltpu.bitcast(wqu[i, f].reshape(12, 8, 128), F32)
            for q in range(NP // 2):
                for r in range(2):
                    a, b = [pltpu.bitcast(part[48 * r + 24 * t + 3 * q:48 * r + 24 * t + 3 * q + 3], U32)
                            for t in range(2)]
                    wqu[i, q, r, 0:3], wqu[i, q, r, 3:6] = swap_halves(a, b)
            return carry
        lax.fori_loop(0, D // 32, body, 0)

    def regroup5(v):
        h = [v[:, f // 2, 4 * (f % 2):4 * (f % 2) + 4, :] for f in range(2 * KD)]
        return [jnp.concatenate([h[c], h[KD + c]], axis=1) for c in range(KD)]

    def pair_wo(r0, n):
        def body(i, carry):
            r = pl.ds(r0 + 2 * i, 2)
            for c, w in enumerate(regroup5(wou[r])):
                wou[r, c] = w
            return carry
        lax.fori_loop(0, n // 2, body, 0)

    def pair_wa():
        def body(i, carry):
            a, b = i >> 4, i & 15
            for c, w in enumerate(regroup5(wau[a, b])):
                wau[a, b, :, c] = w
            return carry
        lax.fori_loop(0, RH // 2, body, 0)

    def wo_tile(kt, n):
        if 8 * kt >= RH:
            return wou[8 * kt - RH:8 * kt - RH + 8, n]
        return wau[kt >> 2, 4 * (kt & 3):4 * (kt & 3) + 4, :, n]

    def wq_tile(m, c, k):
        c6 = 3 * m[1] + c
        return wqu[4 * k:4 * k + 4, m[0] + c6 // 6, :, 3 * (c6 & 1) + ((c6 % 6) >> 1)]

    def qproj_ops(m):
        def op(paced, c, k):
            qpart[c * KD + k] = tile_dot(
                y_u[k], wq_tile(m, c, k), 8, paced)
        return [(lambda p, c=c, k=k: op(p, c, k)) for c in range(3) for k in range(KD)]

    def oproj_ops(kt, slot, dst, d0):
        def op(paced, n):
            dst[d0 + n] = tile_dot(olhs_u[slot], wo_tile(kt, n), 8, paced)
        return [(lambda p, n=n: op(p, n)) for n in range(KD)]

    def pair_rows(m):
        def body(g2, c):
            for par in range(2):
                kvu[m, 0, par, g2, 0], kvu[m, 0, par, g2, 1] = swap_halves(
                    kvu[m, 0, par, g2, 0], kvu[m, 0, par, g2, 1])
            return c
        lax.fori_loop(0, G2, body, 0)

    def k_blocks(m, par, g0, g1, j):
        return kvu[m, 0, par, g0:g1, j & 1, j >> 1]

    jord = [8 * (i // 8) + 2 * (i % 4) + (i % 8) // 4 for i in range(nblk)]

    def qk_ops(m, po=0, pb=0):
        def op_a(paced, j):
            r = tile_dot(pat_u[po + 0], k_blocks(m, 0, 0, 8, j), 8, paced)
            part_a[j // 8, j % 8:j % 8 + 1, :] = r[j % 8:j % 8 + 1, :]

        def op_c(paced, j):
            r = tile_dot(pat_u[po + 2], k_blocks(m, 1, 4, 12, j), 8, paced)
            part[pb + 2 * nq + j // 8, j % 8:j % 8 + 1, :] = r[j % 8:j % 8 + 1, :]

        def op_b(paced, j):
            w = jnp.concatenate([k_blocks(m, 0, 8, 12, j), k_blocks(m, 1, 0, 4, j)], axis=0)
            r = tile_dot(pat_u[po + 1], w, 16, paced)
            part[pb + nq + j // 8, j % 8:j % 8 + 1, :] = r[j % 8:j % 8 + 1, :]
            part[pb + 3 * nq + j // 8, j % 8:j % 8 + 1, :] = r[8 + j % 8:8 + j % 8 + 1, :]

        return [[(lambda p, f=f, j=j: f(p, j)) for j in jord] for f in (op_a, op_b, op_c)]

    def plain(ops):
        for op in ops:
            op(False)

    steps = [(par, gb, j0) for par in range(2) for gb in range(G // NA)
             for j0 in range(0, nblk, 4) if j0 != 4 or gb == 2 - 2 * par]

    def flip(m):
        for par in range(2):
            for a in range(2):
                v = f32_rows(kvu[m, 1, par, 4 * par:4 * par + 8, :, 2 + a])
                ts = [v[:, :, 8 * b:8 * b + 8, :].reshape(128, 128).T.astype(BF) for b in range(2)]
                for b in range(2):
                    kvu[m, 1, par, 4 * par:4 * par + 8, b, 2 + a] = (
                        pltpu.bitcast(ts[b], U32).reshape(8, 8, 128))

    def pvm_ops(m, sl):
        def op(paced, par, j):
            r = tile_dot(plhs_u[2 * sl + par],
                         kvu[m, 1, par, 4 * par:4 * par + 8, j & 1, j >> 1], 8, paced)
            vres[2 * sl + par, j:j + 1, :] = r[j:j + 1, :]
        return [(lambda p, par=par, j=j: op(p, par, j))
                for j in range(4, 8) for par in range(2)]

    def units(par, gb, j0):
        return [(par, g, j0) for g in range(gb * NA, (gb + 1) * NA)]

    order = [u for s in steps for u in units(*s)]
    wide = {}
    for i, u in enumerate(order):
        if (i + 1) * NW // len(order) > i * NW // len(order):
            wide[u] = len(wide)

    def widen(m):
        for (par, g, j), e in wide.items():
            v = f32_rows(kvu[m, 1, par, g // 2, g % 2, j // 2:j // 2 + 2])
            kvu[m, 1, par, g // 2, g % 2, j // 2:j // 2 + 2] = pltpu.bitcast(v[:, :8], U32)
            vx[m, e] = v[:, 8:]

    def v_unit(m, par, g, j):
        u = kvu[m, 1, par, g // 2, g % 2, j // 2:j // 2 + 2]
        if (par, g, j) in wide:
            return jnp.concatenate([pltpu.bitcast(u, F32), vx[m, wide[(par, g, j)]]], axis=1)
        return f32_rows(u)

    def pv_ops(m, ph):
        acc = {}

        def spread(par, q, r):
            pb_scr[pl.ds(64 * q + r, 8, stride=8), :] = p_scr[ph, par, 8 * q:8 * q + 8, :]

        def psum(par):
            p = p_scr[ph, par]
            accx[ph, 8 * (2 * G + par):8 * (2 * G + par) + 8, :] = (
                (p[0:8] + p[8:16]) + (p[16:24] + p[24:32]))

        pbv = {}

        def piece(par, gb, j0, k):
            if k == 0:
                if par == 0 and j0 < 8:
                    pb = pb0[ph, 8 * j0:8 * j0 + 32, :]
                else:
                    pb = pb_scr[8 * j0:8 * j0 + 32, :]
                pbv[0] = pb.reshape(4, 8, 128)
            for _, g, _ in units(par, gb, j0)[4 * k:4 * k + 4]:
                tv = v_unit(m, par, g, j0).reshape(4, 8, 128) * pbv[0]
                tv = jnp.sum(tv, axis=0)
                acc[g] = tv if j0 == 0 else acc[g] + tv
                if j0 == nblk - 4:
                    r0 = DH * par + 8 * g
                    accx[ph, r0:r0 + 8, :] = acc[g]

        pieces = [s + (k,) for s in steps for k in range(NA // 4)]
        use = {}
        for i, (par, _, j0, k) in enumerate(pieces):
            if k == 0:
                use.setdefault((par, j0 // 8), []).append(i)
        side = {}
        for q in range(nq):
            for r in range(8):
                if q:
                    lo, hi = (use[0, q - 1][0] - 1 if q > 1 else 0), use[0, q][0] - 1
                    side.setdefault(lo + (r * (hi - lo + 1)) // 8, []).append(
                        lambda q=q, r=r: spread(0, q, r))
                lo, hi = use[0, q][-1] + 1, use[1, q][0] - 1
                side.setdefault(lo + (r * (hi - lo)) // 8, []).append(
                    lambda q=q, r=r: spread(1, q, r))
        for par in range(2):
            side.setdefault(len(pieces) // 4 + par, []).append(lambda par=par: psum(par))
        out = []
        for i, s in enumerate(pieces):
            out += [(0, f) for f in side.get(i, [])]
            out.append((2 * sum(4 if u in wide else 6 for u in units(*s[:3])[4 * s[3]:4 * s[3] + 4]),
                        (lambda s=s: piece(*s))))
        return out

    toks = []

    def fence(dst, slot, zero_i):
        for i, t in enumerate(toks):
            dst[slot + i + zero_i] = t
        toks.clear()

    def g_softmax(ph, par, pb=0, pa=0):
        s0 = part[pb + 2 * nq:pb + 3 * nq] if par else part_a[pa:pa + nq]
        s = (s0 + part[pb + (2 * par + 1) * nq:pb + (2 * par + 2) * nq]).reshape(nblk, 128)
        mx = jnp.max(jnp.max(s, axis=0, keepdims=True), axis=1, keepdims=True)
        p = jnp.exp2((s - mx) * jnp.concatenate([rs_scr[0]] * nq, axis=0))
        p_scr[ph, par] = p
        plhs[2 * ph + par, 0:8, :] = p[0:8].astype(BF)
        if par == 0:
            for r in range(8):
                pb0[ph, pl.ds(r, 8, stride=8), :] = p[0:8]
        toks.append(pltpu.bitcast(p[nblk - 8:nblk], U32))

    def recip(d):
        r = pl.reciprocal(d, approx=True)
        return r * (2.0 - d * r)

    def g_olhs(slot0, ph, tok=False):
        zz = [lane_sum(accx[ph, 8 * g:8 * g + 8, :]) for g in range(NZ)]
        inv = [jnp.broadcast_to(recip(jnp.sum(zz[2 * G + par], axis=0, keepdims=True)), (8, 128))
               for par in range(2)]
        uid[0] = uid[0] % 60 + 1
        bit = [b > uid[0] for b in bit_i]
        for c in range(3):
            xs = zz[16 * c:16 * c + 16]
            for k in range(4):
                xs = [jnp.where(bit[k], xs[i + 1], xs[i]) for i in range(0, len(xs), 2)]
            iv = inv[0] if c == 0 else (inv[1] if c == 2 else jnp.where(bit[3], inv[1], inv[0]))
            z = jnp.where(diag_i > uid[0], xs[0], 0.0)
            if c != 1:
                z = z + vres[2 * ph + c // 2]
            z = z * iv
            olhs[slot0 + c, 0:8, :] = z.astype(BF)
            if tok:
                toks.append(pltpu.bitcast(z, U32))

    def set_pat(c, q, po=0):
        if c == 1:
            hi = bit_i[3] > uid[0]
            pat_scr[po + c, 0:8, :] = jnp.where(hi, 0.0, q).astype(BF)
            pat_scr[po + c, 8:16, :] = jnp.where(hi, q, 0.0).astype(BF)
        else:
            pat_scr[po + c, 0:8, :] = q.astype(BF)
        if c > 0:
            toks.append(pltpu.bitcast(q, U32))

    def g_query(c):
        xs = [qpart[c * KD + k] for k in range(KD)]
        set_pat(c, ((xs[0] + xs[1]) + (xs[2] + xs[3])) + xs[4])

    def clear_acc():
        accx[2:4] = jnp.ones((2, 8 * NR, 128), F32)

    def emit(pv, seq, pace, pk=PM):
        rate, lead, tail = pace
        ntile = sum(not isinstance(e, tuple) for e in seq)
        total = sum(w for w, _ in pv) / 4
        k = done = n = 0
        for e in seq:
            if isinstance(e, tuple):
                e[0]()
                continue
            r = n // 4
            pos = lead + rate * r if r < (ntile - 1) // 4 else total - tail
            while k < len(pv) and done + pv[k][0] / 2 <= 4 * pos:
                done += pv[k][0]
                pv[k][1]()
                k += 1
            e(n < ntile - UNPACED and r % PM < pk)
            n += 1
        for _, g in pv[k:]:
            g()

    def ffn1(x):
        _, xc, rs = moments(x)
        y = jnp.broadcast_to(xc, (8, D)).astype(BF)

        def up(wu):
            cols = []
            for cp in range(NC // 2):
                ev, od = swap_halves(wu[:, 0, cp], wu[:, 1, cp])
                wu[:, 0, cp], wu[:, 1, cp] = ev, od
                cols += [jnp.dot(y, pltpu.bitcast(w.reshape(D // 2, 128), BF),
                                 preferred_element_type=F32) for w in (ev, od)]
            return jnp.concatenate(cols, axis=1) * rs

        def w2_rows(r0, n):
            nat = regroup5(w2u[r0:r0 + n])
            for c in range(KD):
                w2u[r0:r0 + n, c] = nat[c]
            return nat

        def down(o, n):
            cols = [None] * KD
            for k in range(o // 128, (o + n) // 128):
                for c, w in enumerate(w2_rows(8 * k, 8)):
                    t = jnp.dot(hh[:, 128 * k:128 * k + 128], pltpu.bitcast(w.reshape(64, 128), BF),
                                preferred_element_type=F32)[0:1]
                    cols[c] = t if cols[c] is None else cols[c] + t
            return jnp.concatenate(cols, axis=1)

        c_w1.wait()
        g = up(w1u)
        c_w3.wait()
        u = up(w3u)
        hh = (g * jax.nn.sigmoid(g) * u).astype(BF)
        hb = columns(hh[:, w2_off[-1]:].astype(F32))
        a = None
        parts = [([c], o, n) for c, o, n in zip(c_w2, w2_off, W2_CHUNKS)][:-1]
        for cs, o, n in parts[:1] + [(w2_out, 0, 16 * W2S)] + parts[1:]:
            wait_all(cs)
            a = down(o, n) if a is None else a + down(o, n)
        c_w2[-1].wait()
        acc = [None] * KD
        for r in range(W2_CHUNKS[-1] // 16):
            v = f32_rows(w2u[w2_off[-1] // 16 + r])
            for f in range(2 * KD):
                tv = v[f // 2, 8 * (f % 2):8 * (f % 2) + 8] * hb[2 * r + f // KD]
                acc[f % KD] = tv if acc[f % KD] is None else acc[f % KD] + tv
        a = a + jnp.concatenate([jnp.sum(t, axis=0, keepdims=True) for t in acc], axis=1)
        return residual(x, a)

    def ffn2(x):
        mu, _, rs = moments(x)
        x8 = jnp.broadcast_to(x, (8, D))
        rowk = lax.broadcasted_iota(jnp.int32, (8, D), 0)
        y = jnp.where(rowk == 0, x8, jnp.where(rowk == 1, 1.0, 0.0)).astype(BF)
        coef = jnp.where(row == 0, 1.0, -mu)
        yb = jnp.concatenate([c - mu for c in columns(x8[:, 128 * KM:])], axis=0)
        km = [KM + ((c + 1) * FX // NC > c * FX // NC) for c in range(NC)]
        mx = {}
        out = [None] * KD
        late = []
        for c in range(NC):
            while len(mx) < min(NC, FPRE + c * FSTEP / 4):
                cc = len(mx)
                mx[cc] = [jnp.dot(y[:, :128 * km[cc]],
                                  pltpu.bitcast(wu[0:8 * km[cc], cc & 1, cc >> 1].reshape(64 * km[cc], 128), BF),
                                  preferred_element_type=F32) * coef for wu in (w1u, w3u)]
            gu = []
            for i, wu in enumerate((w1u, w3u)):
                acc = None
                for r in range(8 * km[c], 8 * KD):
                    o = 16 * (r - 8 * KM)
                    tv = f32_rows(wu[r, c & 1, c >> 1]) * yb[o:o + 16]
                    acc = tv if acc is None else acc + tv
                gu.append(jnp.sum((acc[:8] + acc[8:]) + mx[c][i], axis=0, keepdims=True) * rs)
            hg = 0.5 * gu[0]
            h = jnp.broadcast_to((hg * jnp.tanh(hg) + hg) * gu[1], (8, 128)).astype(BF)
            if c in FLATE:
                late.append((c, columns(h.astype(F32))))
                continue
            if c == NC - 1:
                ws = regroup5(w2u[8 * c:8 * c + 8])
            else:
                ws = [w2u[8 * c:8 * c + 8, n] for n in range(KD)]
            for n in range(KD):
                t = jnp.dot(h, pltpu.bitcast(ws[n].reshape(64, 128), BF),
                            preferred_element_type=F32)[0:1]
                out[n] = t if out[n] is None else out[n] + t
        if late:
            acc = [None] * KD
            for c, hb in late:
                for r in range(8):
                    for n in range(KD):
                        v = f32_rows(w2u[8 * c + r, n])
                        for t in range(2):
                            tv = v[8 * t:8 * t + 8] * hb[2 * r + t]
                            acc[n] = tv if acc[n] is None else acc[n] + tv
            out = [out[n] + jnp.sum(acc[n], axis=0, keepdims=True) for n in range(KD)]
        a = jnp.concatenate(out, axis=1)
        o_ref[...] = (x + a.astype(BF).astype(F32)).astype(BF)
        return x

    def arrive(p, last):
        cs = kv_copies(p)
        if last:
            to_forward(NST - 1)
            wait_all(cs[:TRG])
            start_ffn_weights()
            wait_all(cs[TRG:])
        else:
            wait_all(cs[:4])
            pl.when(p <= PS)(lambda: to_fetch(p + 3))
            pl.when(p > PS)(lambda: to_forward(p + 1))
            wait_all(cs[4:])
            when(p + KVW < NP, lambda: kv_start(p + KVW))
            pl.when(p < PS)(lambda: to_forward(p + 2))
            pl.when(p > PS)(lambda: to_fetch(p + 3))
        pair_rows(p)
        widen(p)
        flip(p)

    def arrivals(p0, n):
        def body(i, carry):
            arrive(p0 + i, False)
            return carry
        lax.fori_loop(0, n, body, 0)

    def layer(li, x):
        first = li == 0
        zero_i = li >> 4

        def barrier():
            @pl.when(li > 2)
            def _():
                clear_acc()

        mu, xc, rs = moments(x)
        y = jnp.broadcast_to(xc, (8, D))
        for k in range(KD):
            y_scr[k, 0:8, :] = y[:, 128 * k:128 * k + 128].astype(BF)
        rs_scr[0] = jnp.broadcast_to(rs * c2, (8, 128))
        rowd = lax.broadcasted_iota(jnp.int32, (8, D), 0)
        xo = jnp.where(rowd < 4, jnp.broadcast_to(x, (8, D)), 1.0).astype(BF)
        coef = jnp.where(row < 4, 1.0, -mu)

        def q_direct(col):
            t = jnp.dot(xo, pltpu.bitcast(wqu[:, 0, :, 3 * (col & 1) + (col >> 1)].reshape(D // 2, 128), BF), preferred_element_type=F32) * coef
            return (t + pltpu.roll(t, 4, 0)).astype(BF).astype(F32)

        def q_cols(q, slot):
            for b, col in enumerate(columns(q)):
                part[slot + b] = col

        def vpu_a(m, slot, js, pa):
            z = zero_i if m == 0 else 0
            acc = {}
            for g2 in range(8):
                qc = jnp.concatenate([part[slot + 2 * g2 + t + z] for t in range(2)], axis=0)
                for j in js:
                    tv = f32_rows(kvu[m, 0, 0, g2, j & 1, j >> 1]) * qc
                    acc[j] = tv if g2 == 0 else acc[j] + tv
            rs_ = [jnp.sum(acc[j], axis=0, keepdims=True) for j in js]
            for j, r in zip(js, rs_):
                part_a[pa + j // 8, j % 8:j % 8 + 1, :] = r
            return [pltpu.bitcast(jnp.broadcast_to(r, (8, 128)), U32) for r in rs_]

        def q_sum(c):
            xs = [qpart[c * KD + k] for k in range(KD)]
            return (((xs[0] + xs[1]) + (xs[2] + xs[3])) + xs[4]).astype(BF).astype(F32)

        q0 = [q_direct(c) for c in range(4)]
        q_cols(q0[0], SP)
        set_pat(1, q0[1], 10)
        set_pat(2, q0[2], 10)
        P0 = SP + 48

        def mark(ops, src):
            def wrap(op, v):
                def f(p):
                    op(p)
                    part[0] = v()
                return f
            return [wrap(op, v) for op, v in zip(ops, src)]

        def qp(m, lo, hi):
            return mark(qproj_ops((0, m))[lo:hi], [(lambda i=i: qpart[i]) for i in range(lo, hi)])

        st = {}

        def queries():
            g_query(1)
            g_query(2)
            st["q"] = q_sum(0)
            set_pat(0, st["q"])

        _, b0, c0 = qk_ops(0, 10, P0)
        _, b1, c1 = qk_ops(1)
        a2 = qk_ops(2)[0][PVB:]
        bc = b0 + c0

        def sprinkle(few, many):
            out = []
            for i, e in enumerate(many):
                out.append(e)
                if i % 3 == 2 and i // 3 < len(few):
                    out.append(few[i // 3])
            return out + few[len(many) // 3:]

        q2 = qproj_ops((0, 2))[KD:]
        mx = (bc[:PQ1] + qp(1, KD, 3 * KD) + qp(2, 0, KD) + [(queries,)] + bc[PQ1:]
              + [(lambda: g_softmax(0, 1, P0),)]
              + sprinkle(q2, b1) + c1 + [(lambda: g_softmax(1, 1),)]
              + [(lambda: g_query(1),), (lambda: g_query(2),)] + a2)
        vg = ([(0, SP, jord[i:i + 2], 2 * nq) for i in range(0, nblk, 2)]
              + [(1, SP + 16, jord[i:i + 2], nq) for i in range(0, nblk, 2)]
              + [(2, SP + 32, jord[i:i + 2], 0) for i in range(0, PVB, 2)])
        n = g = 0
        done = set()

        def ripe():
            if "s0" not in done and g >= nblk // 2 and n >= nblk + 3 * KD:
                done.add("s0")
                g_softmax(0, 0, P0, 2 * nq)
            if "s1" not in done and g >= nblk and n >= 3 * nblk + 5 * KD:
                done.add("s1")
                g_softmax(1, 0, 0, nq)

        for e in mx + [None]:
            while g < len(vg) and (e is None or (4 * g if g < 16 else PLG + PFS * (g - 16)) <= n):
                if g == PQH:
                    q_cols(q0[3], SP + 16)
                if g == PQ2:
                    q_cols(st["q"], SP + 32)
                toks[:] = vpu_a(*vg[g])
                if g >= 16 and e is not None:
                    fence(pat_u, 3, zero_i)
                g += 1
                ripe()
            if isinstance(e, tuple):
                e[0]()
            elif e is not None:
                e(False)
                n += 1
                ripe()
        toks.clear()

        def half(b, ph, e):
            n = 2 * b + 2 + e
            qp = qproj_ops((b, 3 + e))
            _, qb, qc = qk_ops(n)
            qa = qk_ops(n + 1)[0]
            so = 2 * (1 - ph) + e
            return ([(lambda: g_olhs(3 * (n - 2), so, True),)]
                    + qc[:CF] + qp[:KD] + [(lambda: g_query(0),)] + qc[CF:] + qb[:OF]
                    + [(lambda: fence(pat_u, 3, zero_i),)] + qb[OF:]
                    + [(lambda: g_softmax(so, 0),), (lambda: g_softmax(so, 1),)]
                    + qp[KD:] + [(lambda: g_query(1),), (lambda: g_query(2),)]
                    + pvm_ops(2 * b + e, 2 * ph + e)
                    + qa[:nblk - AEND] + [(lambda: fence(pat_u, 3, zero_i),)] + qa[nblk - AEND:])

        def body(t, carry):
            for ph in range(2):
                b = 2 * t + ph

                @pl.when(first)
                def _():
                    arrivals(2 * b + 3, 2)

                emit(pv_ops(2 * b, 2 * ph) + pv_ops(2 * b + 1, 2 * ph + 1),
                     half(b, ph, 0) + half(b, ph, 1), PACE_LOOP, PK)
            return carry

        lax.fori_loop(0, 3, body, 0)

        def big(kts):
            return [op for kt in kts for op in oproj_ops(kt, kt + 6, part, SP + KD * kt)]

        pl.when(first)(lambda: arrive(NP - 1, True))
        _, qb, qc = qk_ops(NP - 1)
        seq = (half(6, 0, 0) + [(lambda: g_olhs(3 * 13, 3, True),)] + qc + qb[:OF]
               + [(lambda: fence(pat_u, 3, zero_i),)] + qb[OF:]
               + [(lambda: g_softmax(3, 0),), (lambda: g_softmax(3, 1),)]
               + pvm_ops(13, 1) + big(range(KT13 - 1))
               + [(lambda: fence(olhs_u, 3 * NP + 4, zero_i),)] + big([KT13 - 1]))
        emit(pv_ops(12, 0) + pv_ops(13, 1), seq, PACE_QUAD)

        @pl.when(first)
        def _():
            forward(NST - 1)[0].wait()
            w2_in[1].wait()
            start_all(w2_out)
            forward(NST - 1)[1].wait()
            pair_wo(R0 + SC * (NST - 1), SC)

        old = list(range(KT13, 36))
        k14 = old[:KT14 - 7] + list(range(36, 42)) + old[KT14 - 7:KT14 - 6]
        emit(pv_ops(14, 2), [(lambda: g_olhs(3 * 14, 0),), (lambda: g_olhs(3 * 15, 1),)]
             + pvm_ops(14, 2) + big(k14), PACE_PAIR)
        barrier()
        k15 = old[KT14 - 6:-1] + list(range(42, 45)) + old[-1:]
        emit(pv_ops(15, 3), [(lambda: g_olhs(3 * 16, 2),)] + pvm_ops(15, 3) + big(k15), PACE_PAIR)

        def epilogue(x):
            def lsum(g):
                return lane_sum(accx[3, 8 * g:8 * g + 8, :])

            den = [jnp.sum(lsum(2 * G + par), axis=0, keepdims=True) for par in range(2)]
            fac = [den[0], den[1] * recip(den[0]), recip(den[1])]
            acc = []
            for n in range(KD):
                t = part[SP + n]
                for i in range(1, 3 * NP - 3):
                    t = t + part[SP + KD * i + n]
                acc.append(t * fac[0])
            for par in range(2):
                for g2 in range(G2):
                    g = G * par + 2 * g2
                    z0, z1 = lsum(g), lsum(g + 1)
                    for n in range(KD):
                        v = f32_rows(wou[RH - G + G2 * par + g2, n])
                        acc[n] = acc[n] + (v[:8] * z0 + v[8:] * z1)
                l = vres[6 + par].astype(BF)
                acc = [acc[n] + jnp.dot(
                    l, pltpu.bitcast(wo_tile(3 * NP - 3 + 2 * par, n).reshape(64, 128), BF),
                    preferred_element_type=F32) * 1.0 for n in range(KD)]
                acc = [t * fac[par + 1] for t in acc]
            cols = [jnp.sum(t, axis=0, keepdims=True) for t in acc]
            return residual(x, jnp.concatenate(cols, axis=1))

        return lax.cond(first, lambda x: ffn1(epilogue(x)), lambda x: ffn2(epilogue(x)), x)

    for r in (y_u, pat_u, olhs_u, plhs_u):
        r[...] = jnp.zeros(r.shape, U32)
    vres[...] = jnp.zeros(vres.shape, F32)
    clear_acc()
    wait_all(fetch(0))
    start_all(fetch(1))
    fetch(1)[0].wait()
    start_all(forward(0))
    to_fetch(2)
    c_x.wait()
    kv_start(0)
    c_wo[0].wait()
    kv_start(1)
    to_forward(1)
    wait_all(c_wq)
    pair_wq()
    arrivals(0, 3)
    wait_all(c_wo[1:])
    pair_wa()
    pair_wo(0, R0)
    lax.fori_loop(0, 2, layer, xb[...].astype(F32))


@jax.jit
def pallas_interleave_layers__sliding_block_cached__glu_gated_swiglu__decode_kernel(
    A_x: jax.Array,
    A_k_cache: jax.Array,
    A_v_cache: jax.Array,
    A_wq: jax.Array,
    A_wo: jax.Array,
    B_x: jax.Array,
    B_w1: jax.Array,
    B_w3: jax.Array,
    B_w2: jax.Array,
):
    del B_x
    sk = A_k_cache.shape[2]
    win = min(4096, max(256, sk // 4))
    nb = sk // 128
    nblk = win // 128

    def cache_tiles(c):
        return (c.reshape(H, nb, 128, G2, 2, 8).transpose(0, 3, 4, 1, 5, 2)
                .reshape(H, G2, 2, nb // 2, 16, 128))

    def weight_tiles(w):
        r, c = w.shape
        return w.reshape(r // 16, 2, 8, c // 128, 128).transpose(0, 1, 3, 2, 4)

    vreg = lambda n: pltpu.VMEM((-(-n // 4) * 4, 8, 128), F32)
    lhs = lambda n: pltpu.VMEM((-(-n // 4) * 4, 16, 128), BF)
    kern = lambda *refs: _kernel(*refs, blk0=nb - nblk, nblk=nblk, scale=DH ** -0.5)
    out = pl.pallas_call(
        kern,
        out_shape=jax.ShapeDtypeStruct((1, D), BF),
        in_specs=[pl.BlockSpec(memory_space=pl.ANY)] * 9,
        out_specs=pl.BlockSpec(memory_space=pltpu.VMEM),
        scratch_shapes=[
            pltpu.VMEM((1, D), BF),
            pltpu.VMEM((NP, 2, 2, G2, 2, nblk // 2, 16, 128), BF),
            pltpu.VMEM((D // 32, NP // 2, 2, 6, 16, 128), BF),
            pltpu.VMEM((6, 16, 2, KD, 16, 128), BF),
            pltpu.VMEM((H * G2 // 2, KD, 16, 128), BF),
            pltpu.VMEM((D // 16, 2, NC // 2, 16, 128), BF),
            pltpu.VMEM((D // 16, 2, NC // 2, 16, 128), BF),
            pltpu.VMEM((FF // 16, KD, 16, 128), BF),
            lhs(KD),
            vreg(1),
            vreg(3 * KD),
            lhs(16),
            vreg(3 * nblk // 8),
            vreg(nblk // 2 + (3 * NP - 3) * KD),
            pltpu.VMEM((4, 2, nblk, 128), F32),
            pltpu.VMEM((nblk * 8, 128), F32),
            pltpu.VMEM((4, 64, 128), F32),
            pltpu.VMEM((4, 8 * NR, 128), F32),
            lhs(3 * NP + 12),
            lhs(8),
            vreg(8),
            pltpu.VMEM((NP, NW, 2, 8, 128), F32),
            pltpu.SMEM((3, SC, KD, 16, 128), BF),
            pltpu.SemaphoreType.DMA((NP,)),
            pltpu.SemaphoreType.DMA((5 + len(W2_CHUNKS),)),
            pltpu.SemaphoreType.DMA((6,)),
        ],
        compiler_params=pltpu.CompilerParams(
            vmem_limit_bytes=128 * 1024 * 1024, disable_semaphore_checks=True,
            disable_bounds_checks=True),
    )(A_x.reshape(1, D), cache_tiles(A_k_cache), cache_tiles(A_v_cache),
      weight_tiles(A_wq).reshape(D // 32, NP // 2, 2, 6, 16, 128),
      weight_tiles(A_wo).reshape(12, 16, 2, KD, 16, 128),
      weight_tiles(A_wo).reshape(H * G2, KD, 16, 128),
      weight_tiles(B_w1).reshape(D // 16, 2, NC // 2, 16, 128),
      weight_tiles(B_w3).reshape(D // 16, 2, NC // 2, 16, 128),
      weight_tiles(B_w2).reshape(FF // 16, KD, 16, 128))
    return out.reshape(1, 1, D)
```
